```python
import jax
import jax.numpy as jnp

def _softmax(x, axis=-1):
    return jax.nn.softmax(x, axis=axis)
def _gelu(x):
    return jax.nn.gelu(x, approximate=True)
def _silu(x):
    return jax.nn.silu(x)
def _sigmoid(x):
    return jax.nn.sigmoid(x)
def _layernorm(x, axis=-1, eps=1e-5):
    m = jnp.mean(x, axis=axis, keepdims=True)
    v = jnp.var(x, axis=axis, keepdims=True)
    return (x - m) / jnp.sqrt(v + eps)
def _scatter_add(tgt, idx, src, axis=0):
    return tgt.at[idx].add(src)
def _segment_sum(src, seg, n):
    return jax.ops.segment_sum(src, seg, n)
class _Rng:
    def __init__(self, key):
        self._k = key
    def _next(self):
        self._k, sub = jax.random.split(self._k)
        return sub
    def normal(self, shape):
        return jax.random.normal(self._next(), shape, dtype=jnp.bfloat16)
    def randint(self, lo, hi, shape):
        return jax.random.randint(self._next(), shape, lo, hi, dtype=jnp.int32)
    def uniform(self, shape, lo=0.0, hi=1.0):
        return jax.random.uniform(self._next(), shape, jnp.bfloat16, lo, hi)
    def permutation(self, n):
        return jax.random.permutation(self._next(), n)


kernel_name = 'interleave_layers__sliding_local_dilated__glu_gated_swiglu__prompt'

def setup_inputs():
    _rng = _Rng(jax.random.key(int.from_bytes(__import__("os").urandom(4), "little")))
    _w = (lambda a: (lambda t: t.astype(jnp.bfloat16) if jnp.issubdtype(t.dtype, jnp.floating) else t)(jnp.asarray(a)))
    def _A_setup():
        B, S, D = 1, 2048, 1024
        return {
            "x": _w((lambda *s: _rng.normal(s) * 0.05)(B, S, D)),
            "wqkv": _w((lambda *s: _rng.normal(s) * 0.05)(D, 3 * D)),
            "wo": _w((lambda *s: _rng.normal(s) * 0.05)(D, D)),
        }
    _A_in = _A_setup()

    def _B_setup():
        B, S, D, F = 1, 2048, 1024, 3584
        return {
            "x": _w((lambda *s: _rng.normal(s) * 0.05)(B, S, D)),
            "w1": _w((lambda *s: _rng.normal(s) * 0.05)(D, F) * (2.0 / D) ** 0.5),
            "w3": _w((lambda *s: _rng.normal(s) * 0.05)(D, F) * (2.0 / D) ** 0.5),
            "w2": _w((lambda *s: _rng.normal(s) * 0.05)(F, D) * (2.0 / F) ** 0.5),
        }
    _B_in = _B_setup()

    return {
        "A_x": _A_in["x"],
        "A_wqkv": _A_in["wqkv"],
        "A_wo": _A_in["wo"],
        "B_x": _B_in["x"],
        "B_w1": _B_in["w1"],
        "B_w3": _B_in["w3"],
        "B_w2": _B_in["w2"],
    }

def reference(A_x, A_wqkv, A_wo, B_x, B_w1, B_w3, B_w2):
    def _A_ref(x, wqkv, wo):
        B, S, D = x.shape
        H = 32; Dh = D // H
        W, dil = 8, 2
        qkv = (lambda x, *d: x.transpose(*d))((x @ wqkv).reshape(B, S, 3, H, Dh), 2, 0, 3, 1, 4)
        q, k, v = qkv[0], qkv[1], qkv[2]
        scale = Dh ** -0.5
        pos = jnp.arange(S)
        off = jnp.arange(W) * dil
        idx = pos[:, None] - off[None, :]
        mask = idx >= 0
        idx_c = jnp.where(mask, idx, 0).reshape(-1)
        kg = k[:, :, idx_c, :].reshape(B, H, S, W, Dh)
        vg = v[:, :, idx_c, :].reshape(B, H, S, W, Dh)
        logits = jnp.einsum("bhsd,bhswd->bhsw", q, kg) * scale
        logits = jnp.where(mask[None, None, :, :], logits, -1e9)
        attn = _softmax(logits, axis=-1)
        o = jnp.einsum("bhsw,bhswd->bhsd", attn, vg)
        return (lambda x, *d: x.transpose(*d))(o, 0, 2, 1, 3).reshape(B, S, D) @ wo

    def _B_ref(x, w1, w3, w2):
        gate = jnp.einsum("bsd,df->bsf", x, w1)
        up = jnp.einsum("bsd,df->bsf", x, w3)
        h = _silu(gate) * up
        out = jnp.einsum("bsf,fd->bsd", h, w2)
        return out

    x = A_x
    x = x + _A_ref(_layernorm(x, axis=-1), A_wqkv, A_wo)
    x = x + _B_ref(_layernorm(x, axis=-1), B_w1, B_w3, B_w2)
    x = x + _A_ref(_layernorm(x, axis=-1), A_wqkv, A_wo)
    x = x + _B_ref(_layernorm(x, axis=-1), B_w1, B_w3, B_w2)
    return x
```

```python
import functools

import jax
import jax.numpy as jnp
import jax.experimental.pallas as pl
import jax.experimental.pallas.tpu as pltpu

N_HEADS = 32
WINDOW = 8
DILATION = 2
EPS = 1e-5
LANES = 128
HALO = 16

TM = 256
FC = 512
RB = 32
LB = 32

F32 = jnp.float32
BF16 = jnp.bfloat16


def _dot(a, b):
    return jnp.dot(a, b, preferred_element_type=F32)


def _swap_bit(a, b, stride, axis):
    n = a.shape[axis]
    low = (jax.lax.broadcasted_iota(jnp.int32, a.shape, axis) & stride) == 0
    return (jnp.where(low, a, pltpu.roll(b, stride, axis)),
            jnp.where(low, pltpu.roll(a, n - stride, axis), b))


def _swap_bits(parts, strides, axis):
    parts = list(parts)
    for bit, stride in strides:
        for i in range(len(parts)):
            if not i & bit:
                parts[i], parts[i | bit] = _swap_bit(parts[i], parts[i | bit], stride, axis)
    return parts


def _kernel(x_hbm, wqkv_hbm, wo_hbm, w1_hbm, w3_hbm, w2_hbm, out_hbm,
            io_s, x_s, wqkv_s, wo_s, w1_s, w3_s, w2_s,
            q_s, k_s, v_s, xa_s, xb_s, o_s, h_s, in_sem, w_sem, out_sem):
    S, D = x_s.shape
    F = w1_s.shape[1]
    nb = S // TM
    n_items = 2 * nb
    nc = D // LANES
    scale = (D // N_HEADS) ** -0.5

    def rows(j):
        return pl.ds(pl.multiple_of(j * TM, TM), TM)

    def x_copy(j):
        return pltpu.make_async_copy(x_hbm.at[pl.ds(j * TM, TM)], io_s.at[pl.ds(j * TM, TM)], in_sem.at[j])

    def out_copy(j):
        return pltpu.make_async_copy(io_s.at[rows(j)], out_hbm.at[rows(j)], out_sem.at[j])

    def wqkv_copy(i):
        cols = pl.ds(i * D, D)
        return pltpu.make_async_copy(wqkv_hbm.at[:, cols], wqkv_s.at[:, cols], w_sem.at[i])

    wo_copy = pltpu.make_async_copy(wo_hbm, wo_s, w_sem.at[3])
    ffn_copies = [pltpu.make_async_copy(src, dst, w_sem.at[4 + i])
                  for i, (src, dst) in enumerate(((w1_hbm, w1_s), (w3_hbm, w3_s), (w2_hbm, w2_s)))]

    def permute_qkv_columns(i):
        def body(r, carry):
            rr = pl.ds(pl.multiple_of(r * 64, 64), 64)
            parts = [pltpu.bitcast(wqkv_s[rr, pl.ds(i * D + c * LANES, LANES)], jnp.uint32)
                     for c in range(nc)]
            parts = _swap_bits(parts, ((4, 16), (2, 8), (1, 4)), 1)
            for c in range(nc):
                wqkv_s[rr, pl.ds(i * D + c * LANES, LANES)] = pltpu.bitcast(parts[c], BF16)
            return carry
        jax.lax.fori_loop(0, D // 64, body, 0)

    def permute_wo_rows():
        def body(hh, carry):
            def tile(h432, d4):
                return pl.ds(pl.multiple_of(h432 * 128 + hh * 32 + d4 * 16, 16), 16)
            src = [[pltpu.bitcast(wo_s[tile(h, d4), :], jnp.uint32) for h in range(8)] for d4 in range(2)]
            src = [_swap_bits(p, ((2, 4), (1, 2)), 0) for p in src]
            for d4 in range(2):
                for h in range(8):
                    wo_s[tile((h & 3) | (d4 << 2), h >> 2), :] = pltpu.bitcast(src[d4][h], BF16)
            return carry
        jax.lax.fori_loop(0, 4, body, 0)

    def widen(j):
        x_s[pl.ds(j * TM, TM), :] = io_s[pl.ds(j * TM, TM), :].astype(F32)

    def layernorm(j, dst):
        for r in range(0, TM, LB):
            x = x_s[pl.ds(pl.multiple_of(j * TM + r, LB), LB), :]
            xc = x - jnp.mean(x, axis=-1, keepdims=True)
            var = jnp.mean(xc * xc, axis=-1, keepdims=True)
            dst[pl.ds(r, LB), :] = (xc * jax.lax.rsqrt(var + EPS)).astype(BF16)

    def qkv(j, first=False):
        xa = xa_s[...]
        for i, dst in enumerate((q_s, k_s, v_s)):
            off = 0 if i == 0 else HALO
            if i and not first:
                tails = [dst[c, pl.ds(TM, HALO), :] for c in range(nc)]
            y = _dot(xa, wqkv_s[:, pl.ds(i * D, D)])
            for c in range(nc):
                yc = y[:, c * LANES:(c + 1) * LANES]
                dst[c, pl.ds(off, TM), :] = yc
                if i:
                    head = jnp.broadcast_to(yc[0:1, :], (HALO, LANES))
                    dst[c, pl.ds(0, HALO), :] = head if first else jnp.where(j == 0, head, tails[c])

    def attention(j, r):
        lane = jax.lax.broadcasted_iota(jnp.int32, (RB, LANES), 1)
        logits = [None] * WINDOW
        for c in range(nc):
            q = q_s[c, pl.ds(r, RB), :]
            for w in range(WINDOW):
                p = q * k_s[c, pl.ds(HALO + r - DILATION * w, RB), :]
                logits[w] = p if c == 0 else logits[w] + p
        for w in range(WINDOW):
            l = logits[w]
            for s in (1, 2):
                l = l + jnp.where((lane & s) == 0, pltpu.roll(l, LANES - s, 1), pltpu.roll(l, s, 1))
            l = l * scale
            if r < DILATION * w:
                pos = j * TM + r + jax.lax.broadcasted_iota(jnp.int32, (RB, LANES), 0)
                l = jnp.where(pos >= DILATION * w, l, -1e9)
            logits[w] = l
        m = functools.reduce(jnp.maximum, logits)
        e = [jnp.exp(l - m) for l in logits]
        inv = 1.0 / functools.reduce(jnp.add, e)
        p = [x * inv for x in e]
        for c in range(nc):
            acc = None
            for w in range(WINDOW):
                t = p[w] * v_s[c, pl.ds(HALO + r - DILATION * w, RB), :]
                acc = t if acc is None else acc + t
            o_s[pl.ds(r, RB), pl.ds(c * LANES, LANES)] = acc.astype(BF16)

    def out_proj(j):
        x_s[rows(j), :] += _dot(o_s[...], wo_s[...])

    def ffn_up(f):
        cols = pl.ds(f * FC, FC)
        xb = xb_s[...]
        g = _dot(xb, w1_s[:, cols])
        u = _dot(xb, w3_s[:, cols])
        h_s[:, cols] = (g * jax.nn.sigmoid(g) * u).astype(BF16)

    def ffn_down(j):
        y = x_s[rows(j), :] + _dot(h_s[...], w2_s[...])
        x_s[rows(j), :] = y
        io_s[rows(j), :] = y.astype(BF16)

    x_copy(0).start()
    for i in range(3):
        wqkv_copy(i).start()
    for j in range(1, nb):
        x_copy(j).start()
    wo_copy.start()
    for cp in ffn_copies:
        cp.start()

    x_copy(0).wait()
    widen(0)
    layernorm(0, xa_s)
    for i in range(3):
        wqkv_copy(i).wait()
        permute_qkv_columns(i)
    for j in range(1, nb):
        x_copy(j).wait()
    wo_copy.wait()
    permute_wo_rows()
    qkv(0, first=True)
    for j in range(1, nb):
        widen(j)
    layernorm(1, xa_s)
    for r in range(0, TM, RB):
        attention(0, r)
    out_proj(0)
    qkv(1)
    layernorm(0, xb_s)
    for cp in ffn_copies:
        cp.wait()

    n_f = F // FC
    groups = list(range(0, TM, RB))

    def step(n, last):
        j0, j1, j2 = n % nb, (n + 1) % nb, (n + 2) % nb
        for f in range(n_f):
            ffn_up(f)
            for r in groups[f * len(groups) // n_f:(f + 1) * len(groups) // n_f]:
                attention(j1, r)
        if not last:
            layernorm(j2, xa_s)
        ffn_down(j0)
        out_proj(j1)
        if not last:
            qkv(j2)
        layernorm(j1, xb_s)

    def loop_body(n, carry):
        step(n, False)

        @pl.when(n >= nb)
        def _():
            out_copy(n - nb).start()
        return carry

    jax.lax.fori_loop(0, n_items - 2, loop_body, 0)

    step(n_items - 2, True)
    out_copy(nb - 2).start()
    for f in range(n_f):
        ffn_up(f)
    ffn_down(nb - 1)
    out_copy(nb - 1).start()
    for j in range(nb):
        out_copy(j).wait()


@jax.jit
def pallas_interleave_layers__sliding_local_dilated__glu_gated_swiglu__prompt_kernel(
    A_x: jax.Array,
    A_wqkv: jax.Array,
    A_wo: jax.Array,
    B_x: jax.Array,
    B_w1: jax.Array,
    B_w3: jax.Array,
    B_w2: jax.Array,
):
    del B_x
    B, S, D = A_x.shape
    F = B_w1.shape[1]
    assert B == 1 and D == N_HEADS * 32 == 8 * LANES and S % TM == 0 and S // TM >= 3 and F % FC == 0
    nb = S // TM
    nc = D // LANES
    any_spec = pl.BlockSpec(memory_space=pl.ANY)
    out = pl.pallas_call(
        _kernel,
        out_shape=jax.ShapeDtypeStruct((S, D), A_x.dtype),
        in_specs=[any_spec] * 6,
        out_specs=any_spec,
        scratch_shapes=[
            pltpu.VMEM((S, D), BF16),
            pltpu.VMEM((S, D), F32),
            pltpu.VMEM((D, 3 * D), BF16),
            pltpu.VMEM((D, D), BF16),
            pltpu.VMEM((D, F), BF16),
            pltpu.VMEM((D, F), BF16),
            pltpu.VMEM((F, D), BF16),
            pltpu.VMEM((nc, TM, LANES), F32),
            pltpu.VMEM((nc, HALO + TM, LANES), F32),
            pltpu.VMEM((nc, HALO + TM, LANES), F32),
            pltpu.VMEM((TM, D), BF16),
            pltpu.VMEM((TM, D), BF16),
            pltpu.VMEM((TM, D), BF16),
            pltpu.VMEM((TM, F), BF16),
            pltpu.SemaphoreType.DMA((nb,)),
            pltpu.SemaphoreType.DMA((7,)),
            pltpu.SemaphoreType.DMA((nb,)),
        ],
        compiler_params=pltpu.CompilerParams(vmem_limit_bytes=100 * 1024 * 1024),
    )(A_x.reshape(S, D), A_wqkv, A_wo, B_w1, B_w3, B_w2)
    return out.reshape(B, S, D)
```

```python
import functools

import jax
import jax.numpy as jnp
import jax.experimental.pallas as pl
import jax.experimental.pallas.tpu as pltpu

N_HEADS = 32
WINDOW = 8
DILATION = 2
EPS = 1e-5
LANES = 128
HALO = 16

TM = 256
FC = 256
NC = 256
RB = 16
PB = 256
RC = 64
LC = 128
LB = 32

F32 = jnp.float32
BF16 = jnp.bfloat16


def _dot(a, b):
    return jnp.dot(a, b, preferred_element_type=F32)


def _token(*vals):
    words = [pltpu.bitcast(v, jnp.uint32) for v in vals]
    regs = [w[r:r + 8, c:c + LANES] for w in words
            for r in range(0, w.shape[0], 8) for c in range(0, w.shape[1], LANES)]
    return functools.reduce(jnp.bitwise_or, regs)


def _after(x, tokens, never):
    if not tokens:
        return x
    w = pltpu.bitcast(x, jnp.uint32)
    corner = jnp.where(never, functools.reduce(jnp.bitwise_or, tokens), w[:8, :LANES])
    top = jnp.concatenate([corner, w[:8, LANES:]], axis=1)
    return pltpu.bitcast(jnp.concatenate([top, w[8:]], axis=0), BF16)


def _swap_bit(a, b, stride, axis):
    n = a.shape[axis]
    low = (jax.lax.broadcasted_iota(jnp.int32, a.shape, axis) & stride) == 0
    return (jnp.where(low, a, pltpu.roll(b, stride, axis)),
            jnp.where(low, pltpu.roll(a, n - stride, axis), b))


def _swap_bits(parts, strides, axis):
    parts = list(parts)
    for bit, stride in strides:
        for i in range(len(parts)):
            if not i & bit:
                parts[i], parts[i | bit] = _swap_bit(parts[i], parts[i | bit], stride, axis)
    return parts


def _kernel(x_hbm, wqkv_hbm, wo_hbm, w1_hbm, w3_hbm, w2_hbm, out_hbm,
            io_s, x_s, wqkv_s, wo_s, w1_s, w3_s, w2_s,
            q_s, k_s, v_s, xa_s, xb_s, o_s, h_s, in_sem, w_sem, out_sem):
    S, D = x_s.shape
    F = w3_s.shape[1]
    nb = S // TM
    n_items = 2 * nb
    nc = D // LANES
    scale = (D // N_HEADS) ** -0.5

    def rows(j):
        return pl.ds(j * TM if isinstance(j, int) else pl.multiple_of(j * TM, TM), TM)

    def x_copy(j):
        return pltpu.make_async_copy(x_hbm.at[rows(j)], io_s.at[rows(j)], in_sem.at[j])

    def out_copy(j):
        return pltpu.make_async_copy(io_s.at[rows(j)], out_hbm.at[rows(j)], out_sem.at[j])

    def wqkv_copy(i):
        cols = pl.ds(i * D, D)
        return pltpu.make_async_copy(wqkv_hbm.at[:, cols], wqkv_s.at[:, cols], w_sem.at[i])

    wo_copy = pltpu.make_async_copy(wo_hbm, wo_s, w_sem.at[3])
    w1_copy = pltpu.make_async_copy(w1_hbm, w1_s, w_sem.at[4])
    w3_copy = pltpu.make_async_copy(w3_hbm, w3_s, w_sem.at[5])
    w2_copy = pltpu.make_async_copy(w2_hbm, w2_s, w_sem.at[6])

    def permute_qkv_columns(i):
        def body(r, carry):
            rr = pl.ds(pl.multiple_of(r * PB, PB), PB)
            parts = [pltpu.bitcast(wqkv_s[rr, pl.ds(i * D + c * LANES, LANES)], jnp.uint32)
                     for c in range(nc)]
            parts = _swap_bits(parts, ((4, 16), (2, 8), (1, 4)), 1)
            for c in range(nc):
                wqkv_s[rr, pl.ds(i * D + c * LANES, LANES)] = pltpu.bitcast(parts[c], BF16)
            return carry
        jax.lax.fori_loop(0, D // PB, body, 0)

    def permute_wo_rows():
        def body(hh, carry):
            def tile(h432, d4):
                return pl.ds(pl.multiple_of(h432 * 128 + hh * 32 + d4 * 16, 16), 16)
            src = [[pltpu.bitcast(wo_s[tile(h, d4), :], jnp.uint32) for h in range(8)] for d4 in range(2)]
            src = [_swap_bits(p, ((2, 4), (1, 2)), 0) for p in src]
            for d4 in range(2):
                for h in range(8):
                    wo_s[tile((h & 3) | (d4 << 2), h >> 2), :] = pltpu.bitcast(src[d4][h], BF16)
            return carry
        jax.lax.fori_loop(0, 4, body, 0)

    def layernorm(j, dst, r, n):
        x = x_s[pl.ds(pl.multiple_of(j * TM + r, n), n), :]
        xc = x - jnp.mean(x, axis=-1, keepdims=True)
        var = jnp.mean(xc * xc, axis=-1, keepdims=True)
        y = (xc * jax.lax.rsqrt(var + EPS)).astype(BF16)
        dst[pl.ds(r, n), :] = y
        return _token(y)

    def layernorm_compact(j, dst):
        @pl.loop(0, TM // LC)
        def _(g):
            layernorm(j, dst, pl.multiple_of(g * LC, LC), LC)

    def spread(items, i, n):
        return items[i * len(items) // n:(i + 1) * len(items) // n]

    def qkv(j, side_job, never):
        tokens = []
        for i, dst in enumerate((q_s, k_s, v_s)):
            off = 0 if i == 0 else HALO
            if i:
                tails = [dst[c, pl.ds(TM, HALO), :] for c in range(nc)]
            y = _dot(_after(xa_s[...], tokens, never), wqkv_s[:, pl.ds(i * D, D)])
            for c in range(nc):
                yc = y[:, c * LANES:(c + 1) * LANES]
                dst[c, pl.ds(off, TM), :] = yc
                if i:
                    head = jnp.broadcast_to(yc[0:1, :], (HALO, LANES))
                    dst[c, pl.ds(0, HALO), :] = jnp.where(j == 0, head, tails[c])
            tokens = side_job(i)

    def attention(j, r, n, masked):
        lane = jax.lax.broadcasted_iota(jnp.int32, (n, LANES), 1)
        logits = [None] * WINDOW
        for c in range(nc):
            q = q_s[c, pl.ds(r, n), :]
            for w in range(WINDOW):
                p = q * k_s[c, pl.ds(HALO + r - DILATION * w, n), :]
                logits[w] = p if c == 0 else logits[w] + p
        for w in range(WINDOW):
            l = logits[w]
            for s in (1, 2):
                l = l + jnp.where((lane & s) == 0, pltpu.roll(l, LANES - s, 1), pltpu.roll(l, s, 1))
            l = l * scale
            if masked and w:
                pos = j * TM + r + jax.lax.broadcasted_iota(jnp.int32, (n, LANES), 0)
                l = jnp.where(pos >= DILATION * w, l, -1e9)
            logits[w] = l
        m = functools.reduce(jnp.maximum, logits)
        e = [jnp.exp(l - m) for l in logits]
        inv = 1.0 / functools.reduce(jnp.add, e)
        p = [x * inv for x in e]
        outs = []
        for c in range(nc):
            acc = None
            for w in range(WINDOW):
                t = p[w] * v_s[c, pl.ds(HALO + r - DILATION * w, n), :]
                acc = t if acc is None else acc + t
            outs.append(acc.astype(BF16))
            o_s[pl.ds(r, n), pl.ds(c * LANES, LANES)] = outs[-1]
        return _token(*outs)

    def ffn_up(side_job, never):
        tokens = []
        for f in range(F // FC):
            cols = pl.ds(f * FC, FC)
            xb = xb_s[...]
            g = _dot(_after(xb, tokens, never), w1_s[:, cols])
            tokens = side_job(2 * f)
            u = _dot(_after(xb, tokens, never), w3_s[:, cols])
            tokens = side_job(2 * f + 1)
            h_s[:, cols] = (g * jax.nn.sigmoid(g) * u).astype(BF16)

    def ffn_down(j, side_job, never):
        tokens = []
        for i in range(D // NC):
            cols = pl.ds(i * NC, NC)
            h = _after(h_s[...], tokens, never)
            tokens = side_job(i)
            y = x_s[rows(j), cols] + _dot(h, w2_s[:, cols])
            x_s[rows(j), cols] = y
            io_s[rows(j), cols] = y.astype(BF16)

    x_copy(0).start()
    wqkv_copy(0).start()
    wqkv_copy(1).start()
    wqkv_copy(0).wait()
    wqkv_copy(2).start()
    permute_qkv_columns(0)
    wqkv_copy(1).wait()
    x_copy(1).start()
    wo_copy.start()
    permute_qkv_columns(1)
    wqkv_copy(2).wait()
    w1_copy.start()
    w3_copy.start()
    permute_qkv_columns(2)

    n_f = F // FC
    last = n_items - 1

    @pl.loop(-2, n_items)
    def _(n):
        j0 = jnp.maximum(n, 0) % nb
        j1 = jnp.maximum(n + 1, 0) % nb
        j2 = (n + 2) % nb
        never = n > n_items

        def layernorm_job(j, dst, n_parts):
            def job(i):
                return [layernorm(j, dst, r, LB)
                        for r in spread(list(range(0, TM, LB)), i, n_parts) if i < n_parts]
            return job

        @pl.when(n == 0)
        def _():
            w1_copy.wait()
            w3_copy.wait()
            for j in range(3, nb):
                x_copy(j).start()

        @pl.when(n >= 0)
        def _():
            n_dots = 2 * n_f - 1

            def job(i):
                return [attention(j1, r, RB, r < HALO)
                        for r in spread(list(range(0, TM, RB)), i, n_dots) if i < n_dots]

            ffn_up(job, never)

        @pl.when(n == -1)
        def _():
            w2_copy.start()
            x_copy(2).start()

            @pl.loop(0, TM // RC)
            def _(g):
                attention(j1, pl.multiple_of(g * RC, RC), RC, True)

            wo_copy.wait()
            permute_wo_rows()

        @pl.when(n == 0)
        def _():
            w2_copy.wait()

        @pl.when(n + 2 < nb)
        def _():
            x_copy(j2).wait()
            x_s[rows(j2), :] = io_s[rows(j2), :].astype(F32)

        @pl.when(n >= 0)
        def _():
            ffn_down(j0, layernorm_job(j2, xa_s, D // NC - 1), never)

        @pl.when(n < 0)
        def _():
            layernorm_compact(j2, xa_s)

        @pl.when(n >= nb)
        def _():
            out_copy(j0).start()

        @pl.when(jnp.logical_and(n >= -1, n < last))
        def _():
            x_s[rows(j1), :] += _dot(o_s[...], wo_s[...])

        @pl.when(n < last - 1)
        def _():
            qkv(j2, layernorm_job(j1, xb_s, 2), never)

        @pl.when(n == last - 1)
        def _():
            layernorm_compact(j1, xb_s)

    for j in range(nb):
        out_copy(j).wait()


@jax.jit
def pallas_interleave_layers__sliding_local_dilated__glu_gated_swiglu__prompt_kernel(
    A_x: jax.Array,
    A_wqkv: jax.Array,
    A_wo: jax.Array,
    B_x: jax.Array,
    B_w1: jax.Array,
    B_w3: jax.Array,
    B_w2: jax.Array,
):
    del B_x
    B, S, D = A_x.shape
    F = B_w1.shape[1]
    assert B == 1 and D == N_HEADS * 32 == 8 * LANES and S % TM == 0 and S // TM >= 3 and F % FC == 0
    nb = S // TM
    nc = D // LANES
    any_spec = pl.BlockSpec(memory_space=pl.ANY)
    out = pl.pallas_call(
        _kernel,
        out_shape=jax.ShapeDtypeStruct((S, D), A_x.dtype),
        in_specs=[any_spec] * 6,
        out_specs=any_spec,
        scratch_shapes=[
            pltpu.VMEM((S, D), BF16),
            pltpu.VMEM((S, D), F32),
            pltpu.VMEM((D, 3 * D), BF16),
            pltpu.VMEM((D, D), BF16),
            pltpu.VMEM((D, F), BF16),
            pltpu.VMEM((D, F), BF16),
            pltpu.VMEM((F, D), BF16),
            pltpu.VMEM((nc, TM, LANES), F32),
            pltpu.VMEM((nc, HALO + TM, LANES), F32),
            pltpu.VMEM((nc, HALO + TM, LANES), F32),
            pltpu.VMEM((TM, D), BF16),
            pltpu.VMEM((TM, D), BF16),
            pltpu.VMEM((TM, D), BF16),
            pltpu.VMEM((TM, F), BF16),
            pltpu.SemaphoreType.DMA((nb,)),
            pltpu.SemaphoreType.DMA((7,)),
            pltpu.SemaphoreType.DMA((nb,)),
        ],
        compiler_params=pltpu.CompilerParams(vmem_limit_bytes=100 * 1024 * 1024),
    )(A_x.reshape(S, D), A_wqkv, A_wo, B_w1, B_w3, B_w2)
    return out.reshape(B, S, D)
```

```python
import functools

import jax
import jax.numpy as jnp
import jax.experimental.pallas as pl
import jax.experimental.pallas.tpu as pltpu

N_HEADS = 32
WINDOW = 8
DILATION = 2
EPS = 1e-5
LANES = 128
HALO = 16

TM = 256
FC = 256
NC = 256
RB = 16
PB = 128
RC = 64
LC = 128
LB = 32

F32 = jnp.float32
BF16 = jnp.bfloat16


def _dot(a, b):
    return jnp.dot(a, b, preferred_element_type=F32)


def _token(*vals):
    words = [pltpu.bitcast(v, jnp.uint32) for v in vals]
    regs = [w[r:r + 8, c:c + LANES] for w in words
            for r in range(0, w.shape[0], 8) for c in range(0, w.shape[1], LANES)]
    return functools.reduce(jnp.bitwise_or, regs)


def _after(x, tokens, never):
    if not tokens:
        return x
    w = pltpu.bitcast(x, jnp.uint32)
    corner = jnp.where(never, functools.reduce(jnp.bitwise_or, tokens), w[:8, :LANES])
    top = jnp.concatenate([corner, w[:8, LANES:]], axis=1)
    return pltpu.bitcast(jnp.concatenate([top, w[8:]], axis=0), BF16)


def _swap_bit(a, b, stride, axis):
    n = a.shape[axis]
    low = (jax.lax.broadcasted_iota(jnp.int32, a.shape, axis) & stride) == 0
    return (jnp.where(low, a, pltpu.roll(b, stride, axis)),
            jnp.where(low, pltpu.roll(a, n - stride, axis), b))


def _swap_bits(parts, strides, axis):
    parts = list(parts)
    for bit, stride in strides:
        for i in range(len(parts)):
            if not i & bit:
                parts[i], parts[i | bit] = _swap_bit(parts[i], parts[i | bit], stride, axis)
    return parts


def _kernel(x_hbm, wqkv_hbm, wo_hbm, w1_hbm, w3_hbm, w2_hbm, out_hbm,
            io_s, x_s, wqkv_s, wo_s, w1_s, w3_s, w2_s,
            q_s, k_s, v_s, xa_s, xb_s, o_s, h_s, in_sem, qkv_sem, w_sem, out_sem):
    S, D = x_s.shape
    F = w3_s.shape[1]
    nb = S // TM
    n_items = 2 * nb
    nc = D // LANES
    scale = (D // N_HEADS) ** -0.5

    def rows(j):
        return pl.ds(j * TM if isinstance(j, int) else pl.multiple_of(j * TM, TM), TM)

    def x_copy(j):
        return pltpu.make_async_copy(x_hbm.at[rows(j)], io_s.at[rows(j)], in_sem.at[j])

    def out_copy(j):
        return pltpu.make_async_copy(io_s.at[rows(j)], out_hbm.at[rows(j)], out_sem.at[j])

    def wqkv_copy(i):
        rr = pl.ds(i * PB if isinstance(i, int) else pl.multiple_of(i * PB, PB), PB)
        return pltpu.make_async_copy(wqkv_hbm.at[rr], wqkv_s.at[rr], qkv_sem.at[i])

    wo_copy = pltpu.make_async_copy(wo_hbm, wo_s, w_sem.at[0])
    w1_copy = pltpu.make_async_copy(w1_hbm, w1_s, w_sem.at[1])
    w3_copy = pltpu.make_async_copy(w3_hbm, w3_s, w_sem.at[2])
    w2_copy = pltpu.make_async_copy(w2_hbm, w2_s, w_sem.at[3])

    def permute_qkv_columns(r):
        rr = pl.ds(pl.multiple_of(r * PB, PB), PB)
        for i in range(3):
            parts = [pltpu.bitcast(wqkv_s[rr, pl.ds(i * D + c * LANES, LANES)], jnp.uint32)
                     for c in range(nc)]
            parts = _swap_bits(parts, ((4, 16), (2, 8), (1, 4)), 1)
            for c in range(nc):
                wqkv_s[rr, pl.ds(i * D + c * LANES, LANES)] = pltpu.bitcast(parts[c], BF16)

    def permute_wo_rows():
        def body(hh, carry):
            def tile(h432, d4):
                return pl.ds(pl.multiple_of(h432 * 128 + hh * 32 + d4 * 16, 16), 16)
            src = [[pltpu.bitcast(wo_s[tile(h, d4), :], jnp.uint32) for h in range(8)] for d4 in range(2)]
            src = [_swap_bits(p, ((2, 4), (1, 2)), 0) for p in src]
            for d4 in range(2):
                for h in range(8):
                    wo_s[tile((h & 3) | (d4 << 2), h >> 2), :] = pltpu.bitcast(src[d4][h], BF16)
            return carry
        jax.lax.fori_loop(0, 4, body, 0)

    def residual(rr, fresh):
        if fresh is None:
            return x_s[rr, :]
        return jnp.where(fresh, io_s[rr, :].astype(F32), x_s[rr, :])

    def layernorm(j, fresh, dst, r, n):
        x = residual(pl.ds(pl.multiple_of(j * TM + r, n), n), fresh)
        xc = x - jnp.mean(x, axis=-1, keepdims=True)
        var = jnp.mean(xc * xc, axis=-1, keepdims=True)
        y = (xc * jax.lax.rsqrt(var + EPS)).astype(BF16)
        dst[pl.ds(r, n), :] = y
        return _token(y)

    def layernorm_compact(j, fresh, dst):
        @pl.loop(0, TM // LC)
        def _(g):
            layernorm(j, fresh, dst, pl.multiple_of(g * LC, LC), LC)

    def spread(items, i, n):
        return items[i * len(items) // n:(i + 1) * len(items) // n]

    def qkv(j, side_job, never):
        tokens = []
        for i, dst in enumerate((q_s, k_s, v_s)):
            off = 0 if i == 0 else HALO
            if i:
                tails = [dst[c, pl.ds(TM, HALO), :] for c in range(nc)]
            y = _dot(_after(xa_s[...], tokens, never), wqkv_s[:, pl.ds(i * D, D)])
            for c in range(nc):
                yc = y[:, c * LANES:(c + 1) * LANES]
                dst[c, pl.ds(off, TM), :] = yc
                if i:
                    head = jnp.broadcast_to(yc[0:1, :], (HALO, LANES))
                    dst[c, pl.ds(0, HALO), :] = jnp.where(j == 0, head, tails[c])
            tokens = side_job(i)

    def attention(j, r, n, masked):
        lane = jax.lax.broadcasted_iota(jnp.int32, (n, LANES), 1)
        logits = [None] * WINDOW
        for c in range(nc):
            q = q_s[c, pl.ds(r, n), :]
            for w in range(WINDOW):
                p = q * k_s[c, pl.ds(HALO + r - DILATION * w, n), :]
                logits[w] = p if c == 0 else logits[w] + p
        for w in range(WINDOW):
            l = logits[w]
            for s in (1, 2):
                l = l + jnp.where((lane & s) == 0, pltpu.roll(l, LANES - s, 1), pltpu.roll(l, s, 1))
            l = l * scale
            if masked and w:
                pos = j * TM + r + jax.lax.broadcasted_iota(jnp.int32, (n, LANES), 0)
                l = jnp.where(pos >= DILATION * w, l, -1e9)
            logits[w] = l
        m = functools.reduce(jnp.maximum, logits)
        e = [jnp.exp(l - m) for l in logits]
        inv = 1.0 / functools.reduce(jnp.add, e)
        p = [x * inv for x in e]
        outs = []
        for c in range(nc):
            acc = None
            for w in range(WINDOW):
                t = p[w] * v_s[c, pl.ds(HALO + r - DILATION * w, n), :]
                acc = t if acc is None else acc + t
            outs.append(acc.astype(BF16))
            o_s[pl.ds(r, n), pl.ds(c * LANES, LANES)] = outs[-1]
        return _token(*outs)

    def ffn_up(side_job, never):
        tokens = []
        for f in range(F // FC):
            cols = pl.ds(f * FC, FC)
            xb = xb_s[...]
            g = _dot(_after(xb, tokens, never), w1_s[:, cols])
            tokens = side_job(2 * f)
            u = _dot(_after(xb, tokens, never), w3_s[:, cols])
            tokens = side_job(2 * f + 1)
            half = 0.5 * g
            h_s[:, cols] = ((half + half * jnp.tanh(half)) * u).astype(BF16)

    def ffn_down(j, side_job, never):
        tokens = []
        for i in range(D // NC):
            cols = pl.ds(i * NC, NC)
            h = _after(h_s[...], tokens, never)
            tokens = side_job(i)
            y = x_s[rows(j), cols] + _dot(h, w2_s[:, cols])
            x_s[rows(j), cols] = y
            io_s[rows(j), cols] = y.astype(BF16)

    x_copy(0).start()

    @pl.loop(0, D // PB)
    def _(r):
        wqkv_copy(r).start()

    n_f = F // FC
    last = n_items - 1

    @pl.loop(-2, n_items)
    def _(n):
        j0 = jnp.maximum(n, 0) % nb
        j1 = jnp.maximum(n + 1, 0) % nb
        j2 = (n + 2) % nb
        never = n > n_items

        def layernorm_job(j, fresh, dst, n_parts):
            def job(i):
                return [layernorm(j, fresh, dst, r, LB)
                        for r in spread(list(range(0, TM, LB)), i, n_parts) if i < n_parts]
            return job

        @pl.when(n == 0)
        def _():
            w1_copy.wait()
            w3_copy.wait()
            x_copy(2).start()
            w2_copy.start()

        @pl.when(n >= 0)
        def _():
            n_dots = 2 * n_f - 1

            def job(i):
                return [attention(j1, r, RB, r < HALO)
                        for r in spread(list(range(0, TM, RB)), i, n_dots) if i < n_dots]

            ffn_up(job, never)

        @pl.when(n == -1)
        def _():
            @pl.loop(0, TM // RC)
            def _(g):
                attention(j1, pl.multiple_of(g * RC, RC), RC, True)

            wo_copy.wait()
            permute_wo_rows()

        @pl.when(n == 0)
        def _():
            w2_copy.wait()
            for j in range(3, nb):
                x_copy(j).start()

        @pl.when(n + 2 < nb)
        def _():
            x_copy(j2).wait()

        @pl.when(n >= 0)
        def _():
            ffn_down(j0, layernorm_job(j2, n + 2 < nb, xa_s, D // NC - 1), never)

        @pl.when(n < 0)
        def _():
            layernorm_compact(j2, n + 2 < nb, xa_s)

        @pl.when(n == -2)
        def _():
            @pl.loop(0, D // PB)
            def _(r):
                wqkv_copy(r).wait()

                @pl.when(r == D // PB - 2)
                def _():
                    x_copy(1).start()
                    wo_copy.start()
                    w1_copy.start()
                    w3_copy.start()

                permute_qkv_columns(r)

        @pl.when(n >= nb)
        def _():
            out_copy(j0).start()

        @pl.when(jnp.logical_and(n >= -1, n < last))
        def _():
            x_s[rows(j1), :] = residual(rows(j1), n + 1 < nb) + _dot(o_s[...], wo_s[...])

        @pl.when(n < last - 1)
        def _():
            qkv(j2, layernorm_job(j1, None, xb_s, 2), never)

        @pl.when(n == last - 1)
        def _():
            layernorm_compact(j1, None, xb_s)

    for j in range(nb):
        out_copy(j).wait()


@jax.jit
def pallas_interleave_layers__sliding_local_dilated__glu_gated_swiglu__prompt_kernel(
    A_x: jax.Array,
    A_wqkv: jax.Array,
    A_wo: jax.Array,
    B_x: jax.Array,
    B_w1: jax.Array,
    B_w3: jax.Array,
    B_w2: jax.Array,
):
    del B_x
    B, S, D = A_x.shape
    F = B_w1.shape[1]
    assert B == 1 and D == N_HEADS * 32 == 8 * LANES and S % TM == 0 and S // TM >= 3 and F % FC == 0
    nb = S // TM
    nc = D // LANES
    any_spec = pl.BlockSpec(memory_space=pl.ANY)
    out = pl.pallas_call(
        _kernel,
        out_shape=jax.ShapeDtypeStruct((S, D), A_x.dtype),
        in_specs=[any_spec] * 6,
        out_specs=any_spec,
        scratch_shapes=[
            pltpu.VMEM((S, D), BF16),
            pltpu.VMEM((S, D), F32),
            pltpu.VMEM((D, 3 * D), BF16),
            pltpu.VMEM((D, D), BF16),
            pltpu.VMEM((D, F), BF16),
            pltpu.VMEM((D, F), BF16),
            pltpu.VMEM((F, D), BF16),
            pltpu.VMEM((nc, TM, LANES), F32),
            pltpu.VMEM((nc, HALO + TM, LANES), F32),
            pltpu.VMEM((nc, HALO + TM, LANES), F32),
            pltpu.VMEM((TM, D), BF16),
            pltpu.VMEM((TM, D), BF16),
            pltpu.VMEM((TM, D), BF16),
            pltpu.VMEM((TM, F), BF16),
            pltpu.SemaphoreType.DMA((nb,)),
            pltpu.SemaphoreType.DMA((D // PB,)),
            pltpu.SemaphoreType.DMA((4,)),
            pltpu.SemaphoreType.DMA((nb,)),
        ],
        compiler_params=pltpu.CompilerParams(vmem_limit_bytes=100 * 1024 * 1024),
    )(A_x.reshape(S, D), A_wqkv, A_wo, B_w1, B_w3, B_w2)
    return out.reshape(B, S, D)
```

```python
import functools

import jax
import jax.numpy as jnp
import jax.experimental.pallas as pl
import jax.experimental.pallas.tpu as pltpu

N_HEADS = 32
WINDOW = 8
DILATION = 2
EPS = 1e-5
LANES = 128
HALO = 16

TM = 256
FC = 256
NC = 256
SPLIT = [2]
RB = 32
PB = 128
RC = 64
LC = 128
LB = 32

F32 = jnp.float32
BF16 = jnp.bfloat16


def _dot(a, b):
    return jnp.dot(a, b, preferred_element_type=F32)


def _token(*vals):
    words = [pltpu.bitcast(v, jnp.uint32) for v in vals]
    regs = [w[r:r + 8, c:c + LANES] for w in words
            for r in range(0, w.shape[0], 8) for c in range(0, w.shape[1], LANES)]
    return functools.reduce(jnp.bitwise_or, regs)


def _after(x, tokens, never):
    if not tokens:
        return x
    w = pltpu.bitcast(x, jnp.uint32)
    corner = jnp.where(never, functools.reduce(jnp.bitwise_or, tokens), w[:8, :LANES])
    top = jnp.concatenate([corner, w[:8, LANES:]], axis=1)
    return pltpu.bitcast(jnp.concatenate([top, w[8:]], axis=0), BF16)


def _swap_bit(a, b, stride, axis):
    n = a.shape[axis]
    low = (jax.lax.broadcasted_iota(jnp.int32, a.shape, axis) & stride) == 0
    return (jnp.where(low, a, pltpu.roll(b, stride, axis)),
            jnp.where(low, pltpu.roll(a, n - stride, axis), b))


def _swap_bits(parts, strides, axis):
    parts = list(parts)
    for bit, stride in strides:
        for i in range(len(parts)):
            if not i & bit:
                parts[i], parts[i | bit] = _swap_bit(parts[i], parts[i | bit], stride, axis)
    return parts


def _kernel(x_hbm, wqkv_hbm, wo_hbm, w1_hbm, w3_hbm, w2_hbm, out_hbm,
            io_s, x_s, wqkv_s, wo_s, w1_s, w3_s, w2_s,
            qkv_s, xa_s, xb_s, o_s, h_s, in_sem, qkv_sem, w_sem, out_sem):
    S, D = x_s.shape
    F = w3_s.shape[1]
    nb = S // TM
    n_items = 2 * nb
    nc = D // LANES
    scale = (D // N_HEADS) ** -0.5

    def rows(j):
        return pl.ds(j * TM if isinstance(j, int) else pl.multiple_of(j * TM, TM), TM)

    def x_copy(j):
        return pltpu.make_async_copy(x_hbm.at[rows(j)], io_s.at[rows(j)], in_sem.at[j])

    def out_copy(j):
        return pltpu.make_async_copy(io_s.at[rows(j)], out_hbm.at[rows(j)], out_sem.at[j])

    def wqkv_copy(i):
        rr = pl.ds(i * PB if isinstance(i, int) else pl.multiple_of(i * PB, PB), PB)
        return pltpu.make_async_copy(wqkv_hbm.at[rr], wqkv_s.at[rr], qkv_sem.at[i])

    wo_copy = pltpu.make_async_copy(wo_hbm, wo_s, w_sem.at[0])
    w1_copy = pltpu.make_async_copy(w1_hbm, w1_s, w_sem.at[1])
    w3_copy = pltpu.make_async_copy(w3_hbm, w3_s, w_sem.at[2])
    w2_copy = pltpu.make_async_copy(w2_hbm, w2_s, w_sem.at[3])

    def permute_and_project(r):
        rr = pl.ds(pl.multiple_of(r * PB, PB), PB)
        xa = xa_s[:, rr]
        for i in range(3):
            parts = [pltpu.bitcast(wqkv_s[rr, pl.ds(i * D + c * LANES, LANES)], jnp.uint32)
                     for c in range(nc)]
            parts = _swap_bits(parts, ((4, 16), (2, 8), (1, 4)), 1)
            w = pltpu.bitcast(jnp.concatenate(parts, axis=1), BF16)
            wqkv_s[rr, pl.ds(i * D, D)] = w
            y = _dot(xa, w)
            for c in range(nc):
                qkv_s[i * nc + c, pl.ds(HALO, TM), :] += y[:, c * LANES:(c + 1) * LANES]

    def permute_wo_rows():
        def body(hh, carry):
            def tile(h432, d4):
                return pl.ds(pl.multiple_of(h432 * 128 + hh * 32 + d4 * 16, 16), 16)
            src = [[pltpu.bitcast(wo_s[tile(h, d4), :], jnp.uint32) for h in range(8)] for d4 in range(2)]
            src = [_swap_bits(p, ((2, 4), (1, 2)), 0) for p in src]
            for d4 in range(2):
                for h in range(8):
                    wo_s[tile((h & 3) | (d4 << 2), h >> 2), :] = pltpu.bitcast(src[d4][h], BF16)
            return carry
        jax.lax.fori_loop(0, 4, body, 0)

    def residual(rr, fresh):
        if fresh is None:
            return x_s[rr, :]
        return jnp.where(fresh, io_s[rr, :].astype(F32), x_s[rr, :])

    def layernorm(j, fresh, dst, r, n):
        x = residual(pl.ds(pl.multiple_of(j * TM + r, n), n), fresh)
        xc = x - jnp.mean(x, axis=-1, keepdims=True)
        var = jnp.mean(xc * xc, axis=-1, keepdims=True)
        y = (xc * jax.lax.rsqrt(var + EPS)).astype(BF16)
        dst[pl.ds(r, n), :] = y
        return _token(y)

    def layernorm_compact(j, fresh, dst):
        @pl.loop(0, TM // LC)
        def _(g):
            layernorm(j, fresh, dst, pl.multiple_of(g * LC, LC), LC)

    def spread(items, i, n):
        return items[i * len(items) // n:(i + 1) * len(items) // n]

    def first_token(t):
        return jnp.broadcast_to(qkv_s[t, pl.ds(HALO, 1), :], (HALO, LANES))

    def project(j, side_job, never):
        tokens = []
        for i in range(3):
            tails = [qkv_s[i * nc + c, pl.ds(TM, HALO), :] for c in range(nc if i else 0)]
            y = _dot(_after(xa_s[...], tokens, never), wqkv_s[:, pl.ds(i * D, D)])
            tokens = side_job(i)
            for c in range(nc):
                yc = y[:, c * LANES:(c + 1) * LANES]
                qkv_s[i * nc + c, pl.ds(HALO, TM), :] = yc
                if i:
                    head = jnp.broadcast_to(yc[0:1, :], (HALO, LANES))
                    qkv_s[i * nc + c, pl.ds(0, HALO), :] = jnp.where(j == 0, head, tails[c])

    def attention(j, r, n, masked):
        lane = jax.lax.broadcasted_iota(jnp.int32, (n, LANES), 1)
        logits = [None] * WINDOW
        for c in range(nc):
            q = qkv_s[c, pl.ds(HALO + r, n), :]
            for w in range(WINDOW):
                p = q * qkv_s[nc + c, pl.ds(HALO + r - DILATION * w, n), :]
                logits[w] = p if c == 0 else logits[w] + p
        for s in (1, 2):
            logits = [l + jnp.where((lane & s) == 0, pltpu.roll(l, LANES - s, 1), pltpu.roll(l, s, 1))
                      for l in logits]
            if s in SPLIT:
                yield _token(*logits)
        logits = [l * scale for l in logits]
        if masked:
            pos = j * TM + r + jax.lax.broadcasted_iota(jnp.int32, (n, LANES), 0)
            logits = [jnp.where(pos >= DILATION * w, l, -1e9) if w else l for w, l in enumerate(logits)]
        m = functools.reduce(jnp.maximum, logits)
        e = [jnp.exp(l - m) for l in logits]
        inv = 1.0 / functools.reduce(jnp.add, e)
        p = [x * inv for x in e]
        outs = []
        for c in range(nc):
            acc = None
            for w in range(WINDOW):
                t = p[w] * qkv_s[2 * nc + c, pl.ds(HALO + r - DILATION * w, n), :]
                acc = t if acc is None else acc + t
            outs.append(acc.astype(BF16))
            o_s[pl.ds(r, n), pl.ds(c * LANES, LANES)] = outs[-1]
        yield _token(*outs)

    def ffn_up(side_job, never):
        tokens = []
        for f in range(F // FC):
            cols = pl.ds(f * FC, FC)
            xb = xb_s[...]
            g = _dot(_after(xb, tokens, never), w1_s[:, cols])
            tokens = side_job(2 * f)
            u = _dot(_after(xb, tokens, never), w3_s[:, cols])
            tokens = side_job(2 * f + 1)
            half = 0.5 * g
            h_s[:, cols] = ((half + half * jnp.tanh(half)) * u).astype(BF16)

    def ffn_down(j, side_job, never):
        tokens = []
        for i in range(D // NC):
            cols = pl.ds(i * NC, NC)
            h = _after(h_s[...], tokens, never)
            tokens = side_job(i)
            y = x_s[rows(j), cols] + _dot(h, w2_s[:, cols])
            x_s[rows(j), cols] = y
            io_s[rows(j), cols] = y.astype(BF16)

    copies = ([x_copy(0)] + [wqkv_copy(r) for r in range(D // PB)]
              + [x_copy(1), wo_copy, w1_copy, w3_copy, x_copy(2), w2_copy]
              + [x_copy(j) for j in range(3, nb)])

    @pl.loop(0, len(copies))
    def _(i):
        for k, copy in enumerate(copies):
            pl.when(i == k)(copy.start)

    n_f = F // FC
    last = n_items - 1

    @pl.loop(-2, n_items)
    def _(n):
        j0 = jnp.maximum(n, 0) % nb
        j1 = jnp.maximum(n + 1, 0) % nb
        j2 = (n + 2) % nb
        never = n > n_items

        def layernorm_job(j, fresh, dst, n_parts):
            def job(i):
                return [layernorm(j, fresh, dst, r, LB)
                        for r in spread(list(range(0, TM, LB)), i, n_parts) if i < n_parts]
            return job

        @pl.when(n == 0)
        def _():
            w1_copy.wait()
            w3_copy.wait()

        @pl.when(n >= 0)
        def _():
            n_dots = 2 * n_f - 1

            groups = [attention(j1, r, RB, r < HALO) for r in range(0, TM, RB)]
            steps = [g for g in groups for _ in range(len(SPLIT) + 1)]

            def job(i):
                return [next(g) for g in spread(steps, i, n_dots) if i < n_dots]

            ffn_up(job, never)

        @pl.when(n == -1)
        def _():
            @pl.loop(0, TM // RC)
            def _(g):
                list(attention(j1, pl.multiple_of(g * RC, RC), RC, True))

            wo_copy.wait()
            permute_wo_rows()

        @pl.when(n == 0)
        def _():
            w2_copy.wait()

        @pl.when(n + 2 < nb)
        def _():
            x_copy(j2).wait()

        @pl.when(n >= 0)
        def _():
            ffn_down(j0, layernorm_job(j2, n + 2 < nb, xa_s, D // NC - 1), never)

        @pl.when(n < 0)
        def _():
            layernorm_compact(j2, n + 2 < nb, xa_s)

        @pl.when(n == -2)
        def _():
            qkv_s[...] = jnp.zeros(qkv_s.shape, F32)

            @pl.loop(0, D // PB)
            def _(r):
                wqkv_copy(r).wait()
                permute_and_project(r)

            for t in range(nc, 3 * nc):
                qkv_s[t, pl.ds(0, HALO), :] = first_token(t)

        @pl.when(n >= nb)
        def _():
            out_copy(j0).start()

        @pl.when(jnp.logical_and(n >= -1, n < last - 1))
        def _():
            x_s[rows(j1), :] = residual(rows(j1), n + 1 < nb) + _dot(o_s[...], wo_s[...])
            project(j2, layernorm_job(j1, None, xb_s, 2), never)

        @pl.when(n == last - 1)
        def _():
            @pl.loop(0, D // NC)
            def _(i):
                cols = pl.ds(pl.multiple_of(i * NC, NC), NC)
                x_s[rows(j1), cols] += _dot(o_s[...], wo_s[:, cols])

            layernorm_compact(j1, None, xb_s)

    for j in range(nb):
        out_copy(j).wait()


@jax.jit
def pallas_interleave_layers__sliding_local_dilated__glu_gated_swiglu__prompt_kernel(
    A_x: jax.Array,
    A_wqkv: jax.Array,
    A_wo: jax.Array,
    B_x: jax.Array,
    B_w1: jax.Array,
    B_w3: jax.Array,
    B_w2: jax.Array,
):
    del B_x
    B, S, D = A_x.shape
    F = B_w1.shape[1]
    assert B == 1 and D == N_HEADS * 32 == 8 * LANES and S % TM == 0 and S // TM >= 3 and F % FC == 0
    nb = S // TM
    nc = D // LANES
    any_spec = pl.BlockSpec(memory_space=pl.ANY)
    out = pl.pallas_call(
        _kernel,
        out_shape=jax.ShapeDtypeStruct((S, D), A_x.dtype),
        in_specs=[any_spec] * 6,
        out_specs=any_spec,
        scratch_shapes=[
            pltpu.VMEM((S, D), BF16),
            pltpu.VMEM((S, D), F32),
            pltpu.VMEM((D, 3 * D), BF16),
            pltpu.VMEM((D, D), BF16),
            pltpu.VMEM((D, F), BF16),
            pltpu.VMEM((D, F), BF16),
            pltpu.VMEM((F, D), BF16),
            pltpu.VMEM((3 * nc, HALO + TM, LANES), F32),
            pltpu.VMEM((TM, D), BF16),
            pltpu.VMEM((TM, D), BF16),
            pltpu.VMEM((TM, D), BF16),
            pltpu.VMEM((TM, F), BF16),
            pltpu.SemaphoreType.DMA((nb,)),
            pltpu.SemaphoreType.DMA((D // PB,)),
            pltpu.SemaphoreType.DMA((4,)),
            pltpu.SemaphoreType.DMA((nb,)),
        ],
        compiler_params=pltpu.CompilerParams(vmem_limit_bytes=100 * 1024 * 1024),
    )(A_x.reshape(S, D), A_wqkv, A_wo, B_w1, B_w3, B_w2)
    return out.reshape(B, S, D)
```

```python
import functools

import jax
import jax.numpy as jnp
import jax.experimental.pallas as pl
import jax.experimental.pallas.tpu as pltpu

N_HEADS = 32
WINDOW = 8
DILATION = 2
EPS = 1e-5
LANES = 128
HALO = 16

TM = 256
FC = 256
NC = 256
NA2 = 0
LN1 = 1
NS2 = 3
SPLIT = '2'
RB = 32
PB = 128
RC = 64
LC = 128
LB = 32

F32 = jnp.float32
BF16 = jnp.bfloat16


def _dot(a, b):
    return jnp.dot(a, b, preferred_element_type=F32)


def _token(*vals):
    words = [pltpu.bitcast(v, jnp.uint32) for v in vals]
    regs = [w[r:r + 8, c:c + LANES] for w in words
            for r in range(0, w.shape[0], 8) for c in range(0, w.shape[1], LANES)]
    return functools.reduce(jnp.bitwise_or, regs)


def _after(x, tokens, never):
    if not tokens:
        return x
    w = pltpu.bitcast(x, jnp.uint32)
    corner = jnp.where(never, functools.reduce(jnp.bitwise_or, tokens), w[:8, :LANES])
    top = jnp.concatenate([corner, w[:8, LANES:]], axis=1)
    return pltpu.bitcast(jnp.concatenate([top, w[8:]], axis=0), BF16)


def _swap_bit(a, b, stride, axis):
    n = a.shape[axis]
    low = (jax.lax.broadcasted_iota(jnp.int32, a.shape, axis) & stride) == 0
    return (jnp.where(low, a, pltpu.roll(b, stride, axis)),
            jnp.where(low, pltpu.roll(a, n - stride, axis), b))


def _swap_bits(parts, strides, axis):
    parts = list(parts)
    for bit, stride in strides:
        for i in range(len(parts)):
            if not i & bit:
                parts[i], parts[i | bit] = _swap_bit(parts[i], parts[i | bit], stride, axis)
    return parts


def _kernel(x_hbm, wqkv_hbm, wo_hbm, w1_hbm, w3_hbm, w2_hbm, out_hbm,
            io_s, x_s, wqkv_s, wo_s, w1_s, w3_s, w2_s,
            qkv_s, xa_s, xb_s, o_s, h_s, in_sem, qkv_sem, w_sem, out_sem):
    S, D = x_s.shape
    F = w3_s.shape[1]
    nb = S // TM
    n_items = 2 * nb
    nc = D // LANES
    scale = (D // N_HEADS) ** -0.5

    def rows(j):
        return pl.ds(j * TM if isinstance(j, int) else pl.multiple_of(j * TM, TM), TM)

    def x_copy(j):
        return pltpu.make_async_copy(x_hbm.at[rows(j)], io_s.at[rows(j)], in_sem.at[j])

    def out_copy(j):
        return pltpu.make_async_copy(io_s.at[rows(j)], out_hbm.at[rows(j)], out_sem.at[j])

    def wqkv_copy(i):
        rr = pl.ds(i * PB if isinstance(i, int) else pl.multiple_of(i * PB, PB), PB)
        return pltpu.make_async_copy(wqkv_hbm.at[rr], wqkv_s.at[rr], qkv_sem.at[i])

    wo_copy = pltpu.make_async_copy(wo_hbm, wo_s, w_sem.at[0])
    w1_copy = pltpu.make_async_copy(w1_hbm, w1_s, w_sem.at[1])
    w3_copy = pltpu.make_async_copy(w3_hbm, w3_s, w_sem.at[2])
    w2_copy = pltpu.make_async_copy(w2_hbm, w2_s, w_sem.at[3])

    def permute_and_project(r):
        rr = pl.ds(pl.multiple_of(r * PB, PB), PB)
        xa = xa_s[:, rr]
        for i in range(3):
            parts = [pltpu.bitcast(wqkv_s[rr, pl.ds(i * D + c * LANES, LANES)], jnp.uint32)
                     for c in range(nc)]
            parts = _swap_bits(parts, ((4, 16), (2, 8), (1, 4)), 1)
            w = pltpu.bitcast(jnp.concatenate(parts, axis=1), BF16)
            wqkv_s[rr, pl.ds(i * D, D)] = w
            y = _dot(xa, w)
            for c in range(nc):
                qkv_s[i * nc + c, pl.ds(HALO, TM), :] += y[:, c * LANES:(c + 1) * LANES]

    def permute_wo_rows():
        def body(hh, carry):
            def tile(h432, d4):
                return pl.ds(pl.multiple_of(h432 * 128 + hh * 32 + d4 * 16, 16), 16)
            src = [[pltpu.bitcast(wo_s[tile(h, d4), :], jnp.uint32) for h in range(8)] for d4 in range(2)]
            src = [_swap_bits(p, ((2, 4), (1, 2)), 0) for p in src]
            for d4 in range(2):
                for h in range(8):
                    wo_s[tile((h & 3) | (d4 << 2), h >> 2), :] = pltpu.bitcast(src[d4][h], BF16)
            return carry
        jax.lax.fori_loop(0, 4, body, 0)

    def residual(rr, fresh):
        if fresh is None:
            return x_s[rr, :]
        return jnp.where(fresh, io_s[rr, :].astype(F32), x_s[rr, :])

    def layernorm(j, fresh, dst, r, n):
        x = residual(pl.ds(pl.multiple_of(j * TM + r, n), n), fresh)
        xc = x - jnp.mean(x, axis=-1, keepdims=True)
        var = jnp.mean(xc * xc, axis=-1, keepdims=True)
        y = (xc * jax.lax.rsqrt(var + EPS)).astype(BF16)
        dst[pl.ds(r, n), :] = y
        return _token(y)

    def layernorm_compact(j, fresh, dst):
        @pl.loop(0, TM // LC)
        def _(g):
            layernorm(j, fresh, dst, pl.multiple_of(g * LC, LC), LC)

    def spread(items, i, n):
        return items[i * len(items) // n:(i + 1) * len(items) // n]

    def first_token(t):
        return jnp.broadcast_to(qkv_s[t, pl.ds(HALO, 1), :], (HALO, LANES))

    def project(j, side_job, never):
        tokens = []
        for i in range(3):
            tails = [qkv_s[i * nc + c, pl.ds(TM, HALO), :] for c in range(nc if i else 0)]
            y = _dot(_after(xa_s[...], tokens, never), wqkv_s[:, pl.ds(i * D, D)])
            tokens = side_job(i)
            for c in range(nc):
                yc = y[:, c * LANES:(c + 1) * LANES]
                qkv_s[i * nc + c, pl.ds(HALO, TM), :] = yc
                if i:
                    head = jnp.broadcast_to(yc[0:1, :], (HALO, LANES))
                    qkv_s[i * nc + c, pl.ds(0, HALO), :] = jnp.where(j == 0, head, tails[c])

    def attention(j, r, n, masked):
        lane = jax.lax.broadcasted_iota(jnp.int32, (n, LANES), 1)
        logits = [None] * WINDOW
        for c in range(nc):
            q = qkv_s[c, pl.ds(HALO + r, n), :]
            for w in range(WINDOW):
                p = q * qkv_s[nc + c, pl.ds(HALO + r - DILATION * w, n), :]
                logits[w] = p if c == 0 else logits[w] + p
            if (c == 3 and "a" in SPLIT) or (c == 7 and "q" in SPLIT):
                yield _token(*logits)
        for s in (1, 2):
            logits = [l + jnp.where((lane & s) == 0, pltpu.roll(l, LANES - s, 1), pltpu.roll(l, s, 1))
                      for l in logits]
            if str(s) in SPLIT:
                yield _token(*logits)
        logits = [l * scale for l in logits]
        if masked:
            pos = j * TM + r + jax.lax.broadcasted_iota(jnp.int32, (n, LANES), 0)
            logits = [jnp.where(pos >= DILATION * w, l, -1e9) if w else l for w, l in enumerate(logits)]
        m = functools.reduce(jnp.maximum, logits)
        e = [jnp.exp(l - m) for l in logits]
        inv = 1.0 / functools.reduce(jnp.add, e)
        p = [x * inv for x in e]
        if "s" in SPLIT:
            yield _token(*p)
        outs = []
        for c in range(nc):
            if c == 4 and "v" in SPLIT:
                yield _token(*outs)
                outs = []
            acc = None
            for w in range(WINDOW):
                t = p[w] * qkv_s[2 * nc + c, pl.ds(HALO + r - DILATION * w, n), :]
                acc = t if acc is None else acc + t
            outs.append(acc.astype(BF16))
            o_s[pl.ds(r, n), pl.ds(c * LANES, LANES)] = outs[-1]
        yield _token(*outs)

    def ffn_up(side_job, never):
        tokens = []
        for f in range(F // FC):
            cols = pl.ds(f * FC, FC)
            xb = xb_s[...]
            g = _dot(_after(xb, tokens, never), w1_s[:, cols])
            tokens = side_job(2 * f)
            u = _dot(_after(xb, tokens, never), w3_s[:, cols])
            tokens = side_job(2 * f + 1)
            half = 0.5 * g
            h_s[:, cols] = ((half + half * jnp.tanh(half)) * u).astype(BF16)

    def ffn_down(j, side_job, never):
        tokens = []
        for i in range(D // NC):
            cols = pl.ds(i * NC, NC)
            h = _after(h_s[...], tokens, never)
            tokens = side_job(i)
            y = x_s[rows(j), cols] + _dot(h, w2_s[:, cols])
            x_s[rows(j), cols] = y
            io_s[rows(j), cols] = y.astype(BF16)

    copies = ([x_copy(0)] + [wqkv_copy(r) for r in range(D // PB)]
              + [x_copy(1), wo_copy, w1_copy, w3_copy, x_copy(2), w2_copy]
              + [x_copy(j) for j in range(3, nb)])

    @pl.loop(0, len(copies))
    def _(i):
        for k, copy in enumerate(copies):
            pl.when(i == k)(copy.start)

    n_f = F // FC
    last = n_items - 1

    @pl.loop(-2, n_items)
    def _(n):
        j0 = jnp.maximum(n, 0) % nb
        j1 = jnp.maximum(n + 1, 0) % nb
        j2 = (n + 2) % nb
        never = n > n_items

        def attention_steps(g0, g1):
            groups = [attention(j1, g * RB, RB, g * RB < HALO) for g in range(g0, g1)]
            return [functools.partial(next, g) for g in groups for _ in range(len(SPLIT) + 1)]

        def layernorm_steps(j, fresh, dst):
            return [functools.partial(layernorm, j, fresh, dst, r, LB) for r in range(0, TM, LB)]

        def side_job(steps, n_slots):
            return lambda i: [step() for step in spread(steps, i, n_slots) if i < n_slots]

        @pl.when(n == 0)
        def _():
            w1_copy.wait()
            w3_copy.wait()

        @pl.when(n >= 0)
        def _():
            steps = attention_steps(0, TM // RB - NA2)
            if LN1:
                steps += layernorm_steps(j2, n + 2 < nb, xa_s)
            ffn_up(side_job(steps, 2 * n_f - 1), never)

        @pl.when(n == -1)
        def _():
            @pl.loop(0, TM // RC)
            def _(g):
                list(attention(j1, pl.multiple_of(g * RC, RC), RC, True))

            wo_copy.wait()
            permute_wo_rows()

        @pl.when(n == 0)
        def _():
            w2_copy.wait()

        @pl.when(n + 2 < nb)
        def _():
            x_copy(j2).wait()

        @pl.when(n >= 0)
        def _():
            steps = attention_steps(TM // RB - NA2, TM // RB)
            if not LN1:
                steps += layernorm_steps(j2, n + 2 < nb, xa_s)
            ffn_down(j0, side_job(steps, NS2), never)

        @pl.when(n < 0)
        def _():
            layernorm_compact(j2, n + 2 < nb, xa_s)

        @pl.when(n == -2)
        def _():
            qkv_s[...] = jnp.zeros(qkv_s.shape, F32)

            @pl.loop(0, D // PB)
            def _(r):
                wqkv_copy(r).wait()
                permute_and_project(r)

            for t in range(nc, 3 * nc):
                qkv_s[t, pl.ds(0, HALO), :] = first_token(t)

        @pl.when(n >= nb)
        def _():
            out_copy(j0).start()

        @pl.when(jnp.logical_and(n >= -1, n < last - 1))
        def _():
            x_s[rows(j1), :] = residual(rows(j1), n + 1 < nb) + _dot(o_s[...], wo_s[...])
            project(j2, side_job(layernorm_steps(j1, None, xb_s), 2), never)

        @pl.when(n == last - 1)
        def _():
            @pl.loop(0, D // NC)
            def _(i):
                cols = pl.ds(pl.multiple_of(i * NC, NC), NC)
                x_s[rows(j1), cols] += _dot(o_s[...], wo_s[:, cols])

            layernorm_compact(j1, None, xb_s)

    for j in range(nb):
        out_copy(j).wait()


@jax.jit
def pallas_interleave_layers__sliding_local_dilated__glu_gated_swiglu__prompt_kernel(
    A_x: jax.Array,
    A_wqkv: jax.Array,
    A_wo: jax.Array,
    B_x: jax.Array,
    B_w1: jax.Array,
    B_w3: jax.Array,
    B_w2: jax.Array,
):
    del B_x
    B, S, D = A_x.shape
    F = B_w1.shape[1]
    assert B == 1 and D == N_HEADS * 32 == 8 * LANES and S % TM == 0 and S // TM >= 3 and F % FC == 0
    nb = S // TM
    nc = D // LANES
    any_spec = pl.BlockSpec(memory_space=pl.ANY)
    out = pl.pallas_call(
        _kernel,
        out_shape=jax.ShapeDtypeStruct((S, D), A_x.dtype),
        in_specs=[any_spec] * 6,
        out_specs=any_spec,
        scratch_shapes=[
            pltpu.VMEM((S, D), BF16),
            pltpu.VMEM((S, D), F32),
            pltpu.VMEM((D, 3 * D), BF16),
            pltpu.VMEM((D, D), BF16),
            pltpu.VMEM((D, F), BF16),
            pltpu.VMEM((D, F), BF16),
            pltpu.VMEM((F, D), BF16),
            pltpu.VMEM((3 * nc, HALO + TM, LANES), F32),
            pltpu.VMEM((TM, D), BF16),
            pltpu.VMEM((TM, D), BF16),
            pltpu.VMEM((TM, D), BF16),
            pltpu.VMEM((TM, F), BF16),
            pltpu.SemaphoreType.DMA((nb,)),
            pltpu.SemaphoreType.DMA((D // PB,)),
            pltpu.SemaphoreType.DMA((4,)),
            pltpu.SemaphoreType.DMA((nb,)),
        ],
        compiler_params=pltpu.CompilerParams(vmem_limit_bytes=100 * 1024 * 1024),
    )(A_x.reshape(S, D), A_wqkv, A_wo, B_w1, B_w3, B_w2)
    return out.reshape(B, S, D)
```

```python
import functools

import jax
import jax.numpy as jnp
import jax.experimental.pallas as pl
import jax.experimental.pallas.tpu as pltpu

N_HEADS = 32
WINDOW = 8
DILATION = 2
EPS = 1e-5
LANES = 128
HALO = 16

TM = 256
FC = 256
NC = 256
FH = 11
NA2 = 0
NE1 = 1
NS4 = 2
LN1 = 0
NS2 = 3
SPLIT = '2'
RB = 32
PB = 128
RC = 128
LC = 256
LB = 32

F32 = jnp.float32
BF16 = jnp.bfloat16


def _dot(a, b):
    return jnp.dot(a, b, preferred_element_type=F32)


def _token(*vals):
    words = [pltpu.bitcast(v, jnp.uint32) for v in vals]
    regs = [w[r:r + 8, c:c + LANES] for w in words
            for r in range(0, w.shape[0], 8) for c in range(0, w.shape[1], LANES)]
    return functools.reduce(jnp.bitwise_or, regs)


def _after(x, tokens, never):
    if not tokens:
        return x
    w = pltpu.bitcast(x, jnp.uint32)
    corner = jnp.where(never, functools.reduce(jnp.bitwise_or, tokens), w[:8, :LANES])
    top = jnp.concatenate([corner, w[:8, LANES:]], axis=1) if w.shape[1] > LANES else corner
    return pltpu.bitcast(jnp.concatenate([top, w[8:]], axis=0), BF16)


def _swap_bit(a, b, stride, axis):
    n = a.shape[axis]
    low = (jax.lax.broadcasted_iota(jnp.int32, a.shape, axis) & stride) == 0
    return (jnp.where(low, a, pltpu.roll(b, stride, axis)),
            jnp.where(low, pltpu.roll(a, n - stride, axis), b))


def _swap_bits(parts, strides, axis):
    parts = list(parts)
    for bit, stride in strides:
        for i in range(len(parts)):
            if not i & bit:
                parts[i], parts[i | bit] = _swap_bit(parts[i], parts[i | bit], stride, axis)
    return parts


def _kernel(x_hbm, wqkv_hbm, wo_hbm, w1_hbm, w3_hbm, w2_hbm, out_hbm,
            io_s, x_s, wqkv_raw, wo_raw, wqkv_s, wo_s, w1_s, w3_s, w2_s,
            qkv_s, xa_s, xb_s, o_s, h_s, in_sem, qkv_sem, w_sem, out_sem):
    S, D = x_s.shape
    F = w3_s.shape[1]
    nb = S // TM
    n_items = 2 * nb
    nc = D // LANES
    scale = (D // N_HEADS) ** -0.5

    def rows(j):
        return pl.ds(j * TM if isinstance(j, int) else pl.multiple_of(j * TM, TM), TM)

    def x_copy(j):
        return pltpu.make_async_copy(x_hbm.at[rows(j)], io_s.at[rows(j)], in_sem.at[j])

    def out_copy(j):
        return pltpu.make_async_copy(io_s.at[rows(j)], out_hbm.at[rows(j)], out_sem.at[j])

    def wqkv_copy(i):
        rr = pl.ds(i * PB if isinstance(i, int) else pl.multiple_of(i * PB, PB), PB)
        return pltpu.make_async_copy(wqkv_hbm.at[rr], wqkv_raw.at[rr], qkv_sem.at[i])

    wo_copy = pltpu.make_async_copy(wo_hbm, wo_raw, w_sem.at[0])
    head, tail = pl.ds(0, FH * FC), pl.ds(FH * FC, F - FH * FC)
    ffn_head = [pltpu.make_async_copy(w1_hbm.at[:, head], w1_s.at[:, head], w_sem.at[1]),
                pltpu.make_async_copy(w3_hbm.at[:, head], w3_s.at[:, head], w_sem.at[2])]
    ffn_tail = [pltpu.make_async_copy(w1_hbm.at[:, tail], w1_s.at[:, tail], w_sem.at[3]),
                pltpu.make_async_copy(w3_hbm.at[:, tail], w3_s.at[:, tail], w_sem.at[4]),
                pltpu.make_async_copy(w2_hbm, w2_s, w_sem.at[5])]

    def chunk(r):
        return pl.ds(r * PB if isinstance(r, int) else pl.multiple_of(r * PB, PB), PB)

    def permute_qkv_columns(r):
        for i in range(3):
            cols = [pl.ds(i * D + c * LANES, LANES) for c in range(nc)]
            parts = [pltpu.bitcast(wqkv_raw[chunk(r), cc], jnp.uint32) for cc in cols]
            for cc, part in zip(cols, _swap_bits(parts, ((4, 16), (2, 8), (1, 4)), 1)):
                wqkv_s[chunk(r), cc] = pltpu.bitcast(part, BF16)

    def project_partial(r):
        y = _dot(xa_s[:, chunk(r)], wqkv_s[chunk(r), :])
        for t in range(3 * nc):
            qkv_s[t, pl.ds(HALO, TM), :] += y[:, t * LANES:(t + 1) * LANES]

    def permute_wo_rows():
        def body(hh, carry):
            def tile(h432, d4):
                return pl.ds(pl.multiple_of(h432 * 128 + hh * 32 + d4 * 16, 16), 16)
            src = [[pltpu.bitcast(wo_raw[tile(h, d4), :], jnp.uint32) for h in range(8)] for d4 in range(2)]
            src = [_swap_bits(p, ((2, 4), (1, 2)), 0) for p in src]
            for d4 in range(2):
                for h in range(8):
                    wo_s[tile((h & 3) | (d4 << 2), h >> 2), :] = pltpu.bitcast(src[d4][h], BF16)
            return carry
        jax.lax.fori_loop(0, 4, body, 0)

    def residual(rr, fresh):
        if fresh is None:
            return x_s[rr, :]
        return jnp.where(fresh, io_s[rr, :].astype(F32), x_s[rr, :])

    def layernorm(j, fresh, dst, r, n):
        x = residual(pl.ds(pl.multiple_of(j * TM + r, n), n), fresh)
        xc = x - jnp.mean(x, axis=-1, keepdims=True)
        var = jnp.mean(xc * xc, axis=-1, keepdims=True)
        y = (xc * jax.lax.rsqrt(var + EPS)).astype(BF16)
        dst[pl.ds(r, n), :] = y
        return _token(y)

    def layernorm_compact(j, fresh, dst):
        @pl.loop(0, TM // LC)
        def _(g):
            layernorm(j, fresh, dst, pl.multiple_of(g * LC, LC), LC)

    def spread(items, i, n):
        return items[i * len(items) // n:(i + 1) * len(items) // n]

    def first_token(t):
        return jnp.broadcast_to(qkv_s[t, pl.ds(HALO, 1), :], (HALO, LANES))

    def project(j, side_job, never):
        tokens = []
        for i in range(3):
            tails = [qkv_s[i * nc + c, pl.ds(TM, HALO), :] for c in range(nc if i else 0)]
            y = _dot(_after(xa_s[...], tokens, never), wqkv_s[:, pl.ds(i * D, D)])
            tokens = side_job(i)
            for c in range(nc):
                yc = y[:, c * LANES:(c + 1) * LANES]
                qkv_s[i * nc + c, pl.ds(HALO, TM), :] = yc
                if i:
                    head = jnp.broadcast_to(yc[0:1, :], (HALO, LANES))
                    qkv_s[i * nc + c, pl.ds(0, HALO), :] = jnp.where(j == 0, head, tails[c])

    def attention(j, r, n, masked):
        lane = jax.lax.broadcasted_iota(jnp.int32, (n, LANES), 1)
        logits = [None] * WINDOW
        for c in range(nc):
            q = qkv_s[c, pl.ds(HALO + r, n), :]
            for w in range(WINDOW):
                p = q * qkv_s[nc + c, pl.ds(HALO + r - DILATION * w, n), :]
                logits[w] = p if c == 0 else logits[w] + p
            if (c == 3 and "a" in SPLIT) or (c == 7 and "q" in SPLIT):
                yield _token(*logits)
        for s in (1, 2):
            logits = [l + jnp.where((lane & s) == 0, pltpu.roll(l, LANES - s, 1), pltpu.roll(l, s, 1))
                      for l in logits]
            if str(s) in SPLIT:
                yield _token(*logits)
        logits = [l * scale for l in logits]
        if masked:
            pos = j * TM + r + jax.lax.broadcasted_iota(jnp.int32, (n, LANES), 0)
            logits = [jnp.where(pos >= DILATION * w, l, -1e9) if w else l for w, l in enumerate(logits)]
        m = functools.reduce(jnp.maximum, logits)
        e = [jnp.exp(l - m) for l in logits]
        inv = 1.0 / functools.reduce(jnp.add, e)
        p = [x * inv for x in e]
        if "s" in SPLIT:
            yield _token(*p)
        outs = []
        for c in range(nc):
            if c == 4 and "v" in SPLIT:
                yield _token(*outs)
                outs = []
            acc = None
            for w in range(WINDOW):
                t = p[w] * qkv_s[2 * nc + c, pl.ds(HALO + r - DILATION * w, n), :]
                acc = t if acc is None else acc + t
            outs.append(acc.astype(BF16))
            o_s[pl.ds(r, n), pl.ds(c * LANES, LANES)] = outs[-1]
        yield _token(*outs)

    def ffn_up(f0, f1, side_job, never):
        tokens = []
        for f in range(f0, f1):
            cols = pl.ds(f * FC, FC)
            xb = xb_s[...]
            g = _dot(_after(xb, tokens, never), w1_s[:, cols])
            tokens = side_job(2 * (f - f0))
            u = _dot(_after(xb, tokens, never), w3_s[:, cols])
            tokens = side_job(2 * (f - f0) + 1)
            half = 0.5 * g
            h_s[:, cols] = ((half + half * jnp.tanh(half)) * u).astype(BF16)
        return tokens

    def ffn_down(j, tokens, side_job, never):
        for i in range(D // NC):
            cols = pl.ds(i * NC, NC)
            h = _after(h_s[...], tokens, never)
            tokens = side_job(i)
            y = x_s[rows(j), cols] + _dot(h, w2_s[:, cols])
            x_s[rows(j), cols] = y
            io_s[rows(j), cols] = y.astype(BF16)

    copies = ([x_copy(0)] + [wqkv_copy(r) for r in range(D // PB)]
              + [x_copy(1), wo_copy, x_copy(2), ] + ffn_head + ffn_tail
              + [x_copy(j) for j in range(3, nb)])

    @pl.loop(0, len(copies))
    def _(i):
        for k, copy in enumerate(copies):
            pl.when(i == k)(copy.start)

    n_f = F // FC
    last = n_items - 1

    @pl.loop(-2, n_items)
    def _(n):
        j0 = jnp.maximum(n, 0) % nb
        j1 = jnp.maximum(n + 1, 0) % nb
        j2 = (n + 2) % nb
        never = n > n_items

        def attention_steps(g0, g1):
            groups = [attention(j1, g * RB, RB, g * RB < HALO) for g in range(g0, g1)]
            return [functools.partial(next, g) for g in groups for _ in range(len(SPLIT) + 1)]

        def layernorm_steps(j, fresh, dst):
            return [functools.partial(layernorm, j, fresh, dst, r, LB) for r in range(0, TM, LB)]

        def side_job(steps, n_slots):
            return lambda i: [step() for step in spread(steps, i, n_slots) if i < n_slots]

        @pl.when(n + 2 < nb)
        def _():
            x_copy(j2).wait()

        @pl.when(n == 0)
        def _():
            for copy in ffn_head:
                copy.wait()

        @pl.when(n >= 0)
        def _():
            steps = attention_steps(0, TM // RB - NA2)
            ln = layernorm_steps(j2, n + 2 < nb, xa_s)
            if LN1 == 1:
                job = side_job(steps + ln, 2 * FH - NE1)
            elif LN1 == 2:
                job = side_job(ln + steps, 2 * FH - NE1)
            elif LN1 == 3:
                ja, jb = side_job(steps, 2 * FH - NE1), side_job(ln, 2 * FH - NE1)
                job = lambda i: ja(i) + jb(i)
            else:
                job = side_job(steps, 2 * FH - NE1)
            ffn_up(0, FH, job, never)

        @pl.when(n == -1)
        def _():
            @pl.loop(0, TM // RC)
            def _(g):
                list(attention(j1, pl.multiple_of(g * RC, RC), RC, True))

            wo_copy.wait()
            permute_wo_rows()

        @pl.when(n == 0)
        def _():
            for copy in ffn_tail:
                copy.wait()

        @pl.when(n >= 0)
        def _():
            steps = attention_steps(TM // RB - NA2, TM // RB)
            if not LN1:
                steps += layernorm_steps(j2, n + 2 < nb, xa_s)
            n_up = 2 * (n_f - FH)
            job = side_job(steps, n_up + NS2)
            tokens = ffn_up(FH, n_f, job, never)
            ffn_down(j0, tokens, lambda i: job(n_up + i), never)

        @pl.when(n < 0)
        def _():
            layernorm_compact(j2, n + 2 < nb, xa_s)

        @pl.when(n == -2)
        def _():
            qkv_s[...] = jnp.zeros(qkv_s.shape, F32)

            n_chunks = D // PB

            @pl.loop(0, n_chunks + 1)
            def _(r):
                @pl.when(r < n_chunks)
                def _():
                    wqkv_copy(r).wait()

                @pl.when(r == 0)
                def _():
                    permute_qkv_columns(0)

                @pl.when(r > 0)
                def _():
                    project_partial(r - 1)
                    permute_qkv_columns(jnp.minimum(r, n_chunks - 1))

            for t in range(nc, 3 * nc):
                qkv_s[t, pl.ds(0, HALO), :] = first_token(t)

        @pl.when(n >= nb)
        def _():
            out_copy(j0).start()

        @pl.when(jnp.logical_and(n >= -1, n < last - 1))
        def _():
            x_s[rows(j1), :] = residual(rows(j1), n + 1 < nb) + _dot(o_s[...], wo_s[...])
            project(j2, side_job(layernorm_steps(j1, None, xb_s), NS4), never)

        @pl.when(n == last - 1)
        def _():
            @pl.loop(0, D // NC)
            def _(i):
                cols = pl.ds(pl.multiple_of(i * NC, NC), NC)
                x_s[rows(j1), cols] += _dot(o_s[...], wo_s[:, cols])

            layernorm_compact(j1, None, xb_s)

    for j in range(nb):
        out_copy(j).wait()


@jax.jit
def pallas_interleave_layers__sliding_local_dilated__glu_gated_swiglu__prompt_kernel(
    A_x: jax.Array,
    A_wqkv: jax.Array,
    A_wo: jax.Array,
    B_x: jax.Array,
    B_w1: jax.Array,
    B_w3: jax.Array,
    B_w2: jax.Array,
):
    del B_x
    B, S, D = A_x.shape
    F = B_w1.shape[1]
    assert B == 1 and D == N_HEADS * 32 == 8 * LANES and S % TM == 0 and S // TM >= 3 and F % FC == 0
    nb = S // TM
    nc = D // LANES
    any_spec = pl.BlockSpec(memory_space=pl.ANY)
    out = pl.pallas_call(
        _kernel,
        out_shape=jax.ShapeDtypeStruct((S, D), A_x.dtype),
        in_specs=[any_spec] * 6,
        out_specs=any_spec,
        scratch_shapes=[
            pltpu.VMEM((S, D), BF16),
            pltpu.VMEM((S, D), F32),
            pltpu.VMEM((D, 3 * D), BF16),
            pltpu.VMEM((D, D), BF16),
            pltpu.VMEM((D, 3 * D), BF16),
            pltpu.VMEM((D, D), BF16),
            pltpu.VMEM((D, F), BF16),
            pltpu.VMEM((D, F), BF16),
            pltpu.VMEM((F, D), BF16),
            pltpu.VMEM((3 * nc, HALO + TM, LANES), F32),
            pltpu.VMEM((TM, D), BF16),
            pltpu.VMEM((TM, D), BF16),
            pltpu.VMEM((TM, D), BF16),
            pltpu.VMEM((TM, F), BF16),
            pltpu.SemaphoreType.DMA((nb,)),
            pltpu.SemaphoreType.DMA((D // PB,)),
            pltpu.SemaphoreType.DMA((6,)),
            pltpu.SemaphoreType.DMA((nb,)),
        ],
        compiler_params=pltpu.CompilerParams(vmem_limit_bytes=100 * 1024 * 1024),
    )(A_x.reshape(S, D), A_wqkv, A_wo, B_w1, B_w3, B_w2)
    return out.reshape(B, S, D)
```

```python
import functools

import jax
import jax.numpy as jnp
import jax.experimental.pallas as pl
import jax.experimental.pallas.tpu as pltpu

N_HEADS = 32
WINDOW = 8
DILATION = 2
EPS = 1e-5
LANES = 128
HALO = 16

TM = 256
FC = 256
NC = 256
FH = 11
NA2 = 0
NE1 = 1
NS4 = 3
LN1 = 0
NS2 = 3
RB = 16
PB = 128
RC = 128
LC = 256
LB = 32

F32 = jnp.float32
BF16 = jnp.bfloat16


def _dot(a, b):
    return jnp.dot(a, b, preferred_element_type=F32)


def _token(*vals):
    words = [pltpu.bitcast(v, jnp.uint32) for v in vals]
    regs = [w[r:r + 8, c:c + LANES] for w in words
            for r in range(0, w.shape[0], 8) for c in range(0, w.shape[1], LANES)]
    return functools.reduce(jnp.bitwise_or, regs)


def _after(x, tokens, never):
    if not tokens:
        return x
    w = pltpu.bitcast(x, jnp.uint32)
    corner = jnp.where(never, functools.reduce(jnp.bitwise_or, tokens), w[:8, :LANES])
    top = jnp.concatenate([corner, w[:8, LANES:]], axis=1) if w.shape[1] > LANES else corner
    return pltpu.bitcast(jnp.concatenate([top, w[8:]], axis=0), BF16)


def _swap_bit(a, b, stride, axis):
    n = a.shape[axis]
    low = (jax.lax.broadcasted_iota(jnp.int32, a.shape, axis) & stride) == 0
    return (jnp.where(low, a, pltpu.roll(b, stride, axis)),
            jnp.where(low, pltpu.roll(a, n - stride, axis), b))


def _swap_bits(parts, strides, axis):
    parts = list(parts)
    for bit, stride in strides:
        for i in range(len(parts)):
            if not i & bit:
                parts[i], parts[i | bit] = _swap_bit(parts[i], parts[i | bit], stride, axis)
    return parts


def _kernel(x_hbm, wqkv_hbm, wo_hbm, w1_hbm, w3_hbm, w2_hbm, out_hbm,
            io_s, x_s, wqkv_raw, wo_raw, wqkv_s, wo_s, w1_s, w3_s, w2_s,
            qkv_s, xa_s, xb_s, o_s, h_s, in_sem, qkv_sem, w_sem, out_sem):
    S, D = x_s.shape
    F = w3_s.shape[1]
    nb = S // TM
    n_items = 2 * nb
    nc = D // LANES
    scale = (D // N_HEADS) ** -0.5

    def rows(j):
        return pl.ds(j * TM if isinstance(j, int) else pl.multiple_of(j * TM, TM), TM)

    def x_copy(j):
        return pltpu.make_async_copy(x_hbm.at[rows(j)], io_s.at[rows(j)], in_sem.at[j])

    def out_copy(j):
        return pltpu.make_async_copy(io_s.at[rows(j)], out_hbm.at[rows(j)], out_sem.at[j])

    def wqkv_copy(i):
        rr = pl.ds(i * PB if isinstance(i, int) else pl.multiple_of(i * PB, PB), PB)
        return pltpu.make_async_copy(wqkv_hbm.at[rr], wqkv_raw.at[rr], qkv_sem.at[i])

    wo_copy = pltpu.make_async_copy(wo_hbm, wo_raw, w_sem.at[0])
    head, tail = pl.ds(0, FH * FC), pl.ds(FH * FC, F - FH * FC)
    ffn_head = [pltpu.make_async_copy(w1_hbm.at[:, head], w1_s.at[:, head], w_sem.at[1]),
                pltpu.make_async_copy(w3_hbm.at[:, head], w3_s.at[:, head], w_sem.at[2])]
    ffn_tail = [pltpu.make_async_copy(w1_hbm.at[:, tail], w1_s.at[:, tail], w_sem.at[3]),
                pltpu.make_async_copy(w3_hbm.at[:, tail], w3_s.at[:, tail], w_sem.at[4]),
                pltpu.make_async_copy(w2_hbm, w2_s, w_sem.at[5])]

    def chunk(r):
        return pl.ds(r * PB if isinstance(r, int) else pl.multiple_of(r * PB, PB), PB)

    def permute_qkv_columns(r):
        for i in range(3):
            cols = [pl.ds(i * D + c * LANES, LANES) for c in range(nc)]
            parts = [pltpu.bitcast(wqkv_raw[chunk(r), cc], jnp.uint32) for cc in cols]
            for cc, part in zip(cols, _swap_bits(parts, ((4, 16), (2, 8), (1, 4)), 1)):
                wqkv_s[chunk(r), cc] = pltpu.bitcast(part, BF16)

    def project_partial(r):
        y = _dot(xa_s[:, chunk(r)], wqkv_s[chunk(r), :])
        for t in range(3 * nc):
            qkv_s[t, pl.ds(HALO, TM), :] += y[:, t * LANES:(t + 1) * LANES]

    def permute_wo_rows():
        def body(hh, carry):
            def tile(h432, d4):
                return pl.ds(pl.multiple_of(h432 * 128 + hh * 32 + d4 * 16, 16), 16)
            src = [[pltpu.bitcast(wo_raw[tile(h, d4), :], jnp.uint32) for h in range(8)] for d4 in range(2)]
            src = [_swap_bits(p, ((2, 4), (1, 2)), 0) for p in src]
            for d4 in range(2):
                for h in range(8):
                    wo_s[tile((h & 3) | (d4 << 2), h >> 2), :] = pltpu.bitcast(src[d4][h], BF16)
            return carry
        jax.lax.fori_loop(0, 4, body, 0)

    def residual(rr, fresh):
        if fresh is None:
            return x_s[rr, :]
        return jnp.where(fresh, io_s[rr, :].astype(F32), x_s[rr, :])

    def layernorm(j, fresh, dst, r, n):
        x = residual(pl.ds(pl.multiple_of(j * TM + r, n), n), fresh)
        xc = x - jnp.mean(x, axis=-1, keepdims=True)
        var = jnp.mean(xc * xc, axis=-1, keepdims=True)
        y = (xc * jax.lax.rsqrt(var + EPS)).astype(BF16)
        dst[pl.ds(r, n), :] = y
        return _token(y)

    def layernorm_compact(j, fresh, dst):
        @pl.loop(0, TM // LC)
        def _(g):
            layernorm(j, fresh, dst, pl.multiple_of(g * LC, LC), LC)

    def spread(items, i, n):
        return items[i * len(items) // n:(i + 1) * len(items) // n]

    def first_token(t):
        return jnp.broadcast_to(qkv_s[t, pl.ds(HALO, 1), :], (HALO, LANES))

    def project(j, side_job, never):
        tokens = []
        for i in range(3):
            tails = [qkv_s[i * nc + c, pl.ds(TM, HALO), :] for c in range(nc if i else 0)]
            y = _dot(_after(xa_s[...], tokens, never), wqkv_s[:, pl.ds(i * D, D)])
            tokens = side_job(i)
            for c in range(nc):
                yc = y[:, c * LANES:(c + 1) * LANES]
                qkv_s[i * nc + c, pl.ds(HALO, TM), :] = yc
                if i:
                    head = jnp.broadcast_to(yc[0:1, :], (HALO, LANES))
                    qkv_s[i * nc + c, pl.ds(0, HALO), :] = jnp.where(j == 0, head, tails[c])

    def attention(j, r, n, masked):
        lane = jax.lax.broadcasted_iota(jnp.int32, (n, LANES), 1)
        logits = [None] * WINDOW
        for c in range(nc):
            q = qkv_s[c, pl.ds(HALO + r, n), :]
            for w in range(WINDOW):
                p = q * qkv_s[nc + c, pl.ds(HALO + r - DILATION * w, n), :]
                logits[w] = p if c == 0 else logits[w] + p
        for s in (1, 2):
            logits = [l + jnp.where((lane & s) == 0, pltpu.roll(l, LANES - s, 1), pltpu.roll(l, s, 1))
                      for l in logits]
        logits = [l * scale for l in logits]
        if masked:
            pos = j * TM + r + jax.lax.broadcasted_iota(jnp.int32, (n, LANES), 0)
            logits = [jnp.where(pos >= DILATION * w, l, -1e9) if w else l for w, l in enumerate(logits)]
        m = functools.reduce(jnp.maximum, logits)
        e = [jnp.exp(l - m) for l in logits]
        inv = 1.0 / functools.reduce(jnp.add, e)
        p = [x * inv for x in e]
        outs = []
        for c in range(nc):
            terms = [p[w] * qkv_s[2 * nc + c, pl.ds(HALO + r - DILATION * w, n), :] for w in range(WINDOW)]
            outs.append(functools.reduce(jnp.add, terms))
        o = jnp.concatenate(outs, axis=1).astype(BF16)
        o_s[pl.ds(r, n), :] = o
        return _token(o)

    def ffn_up(f0, f1, side_job, never):
        tokens = []
        for f in range(f0, f1):
            cols = pl.ds(f * FC, FC)
            xb = xb_s[...]
            g = _dot(_after(xb, tokens, never), w1_s[:, cols])
            tokens = side_job(2 * (f - f0))
            u = _dot(_after(xb, tokens, never), w3_s[:, cols])
            tokens = side_job(2 * (f - f0) + 1)
            half = 0.5 * g
            h_s[:, cols] = ((half + half * jnp.tanh(half)) * u).astype(BF16)
        return tokens

    def ffn_down(j, tokens, side_job, never):
        for i in range(D // NC):
            cols = pl.ds(i * NC, NC)
            h = _after(h_s[...], tokens, never)
            tokens = side_job(i)
            y = x_s[rows(j), cols] + _dot(h, w2_s[:, cols])
            x_s[rows(j), cols] = y
            io_s[rows(j), cols] = y.astype(BF16)

    copies = ([x_copy(0)] + [wqkv_copy(r) for r in range(D // PB)]
              + [x_copy(1), wo_copy, x_copy(2), ] + ffn_head + ffn_tail
              + [x_copy(j) for j in range(3, nb)])

    @pl.loop(0, len(copies))
    def _(i):
        for k, copy in enumerate(copies):
            pl.when(i == k)(copy.start)

    n_f = F // FC
    last = n_items - 1

    @pl.loop(-2, n_items)
    def _(n):
        j0 = jnp.maximum(n, 0) % nb
        j1 = jnp.maximum(n + 1, 0) % nb
        j2 = (n + 2) % nb
        never = n > n_items

        def attention_steps(g0, g1):
            return [functools.partial(attention, j1, g * RB, RB, g * RB < HALO) for g in range(g0, g1)]

        def layernorm_steps(j, fresh, dst):
            return [functools.partial(layernorm, j, fresh, dst, r, LB) for r in range(0, TM, LB)]

        def side_job(steps, n_slots):
            return lambda i: [step() for step in spread(steps, i, n_slots) if i < n_slots]

        @pl.when(n + 2 < nb)
        def _():
            x_copy(j2).wait()

        @pl.when(n == 0)
        def _():
            for copy in ffn_head:
                copy.wait()

        @pl.when(n >= 0)
        def _():
            steps = attention_steps(0, TM // RB - NA2)
            ln = layernorm_steps(j2, n + 2 < nb, xa_s)
            if LN1 == 1:
                job = side_job(steps + ln, 2 * FH - NE1)
            elif LN1 == 2:
                job = side_job(ln + steps, 2 * FH - NE1)
            elif LN1 == 3:
                ja, jb = side_job(steps, 2 * FH - NE1), side_job(ln, 2 * FH - NE1)
                job = lambda i: ja(i) + jb(i)
            else:
                job = side_job(steps, 2 * FH - NE1)
            ffn_up(0, FH, job, never)

        @pl.when(n == -1)
        def _():
            @pl.loop(0, TM // RC)
            def _(g):
                attention(j1, pl.multiple_of(g * RC, RC), RC, True)

            wo_copy.wait()
            permute_wo_rows()

        @pl.when(n == 0)
        def _():
            for copy in ffn_tail:
                copy.wait()

        @pl.when(n >= 0)
        def _():
            steps = attention_steps(TM // RB - NA2, TM // RB)
            if not LN1:
                steps += layernorm_steps(j2, n + 2 < nb, xa_s)
            n_up = 2 * (n_f - FH)
            job = side_job(steps, n_up + NS2)
            tokens = ffn_up(FH, n_f, job, never)
            ffn_down(j0, tokens, lambda i: job(n_up + i), never)

        @pl.when(n < 0)
        def _():
            layernorm_compact(j2, n + 2 < nb, xa_s)

        @pl.when(n == -2)
        def _():
            qkv_s[...] = jnp.zeros(qkv_s.shape, F32)

            n_chunks = D // PB

            @pl.loop(0, n_chunks + 1)
            def _(r):
                @pl.when(r < n_chunks)
                def _():
                    wqkv_copy(r).wait()

                @pl.when(r == 0)
                def _():
                    permute_qkv_columns(0)

                @pl.when(r > 0)
                def _():
                    project_partial(r - 1)
                    permute_qkv_columns(jnp.minimum(r, n_chunks - 1))

            for t in range(nc, 3 * nc):
                qkv_s[t, pl.ds(0, HALO), :] = first_token(t)

        @pl.when(n >= nb)
        def _():
            out_copy(j0).start()

        @pl.when(jnp.logical_and(n >= -1, n < last - 1))
        def _():
            x_s[rows(j1), :] = residual(rows(j1), n + 1 < nb) + _dot(o_s[...], wo_s[...])
            project(j2, side_job(layernorm_steps(j1, None, xb_s), NS4), never)

        @pl.when(n == last - 1)
        def _():
            @pl.loop(0, D // NC)
            def _(i):
                cols = pl.ds(pl.multiple_of(i * NC, NC), NC)
                x_s[rows(j1), cols] += _dot(o_s[...], wo_s[:, cols])

            layernorm_compact(j1, None, xb_s)

    for j in range(nb):
        out_copy(j).wait()


@jax.jit
def pallas_interleave_layers__sliding_local_dilated__glu_gated_swiglu__prompt_kernel(
    A_x: jax.Array,
    A_wqkv: jax.Array,
    A_wo: jax.Array,
    B_x: jax.Array,
    B_w1: jax.Array,
    B_w3: jax.Array,
    B_w2: jax.Array,
):
    del B_x
    B, S, D = A_x.shape
    F = B_w1.shape[1]
    assert B == 1 and D == N_HEADS * 32 == 8 * LANES and S % TM == 0 and S // TM >= 3 and F % FC == 0
    nb = S // TM
    nc = D // LANES
    any_spec = pl.BlockSpec(memory_space=pl.ANY)
    out = pl.pallas_call(
        _kernel,
        out_shape=jax.ShapeDtypeStruct((S, D), A_x.dtype),
        in_specs=[any_spec] * 6,
        out_specs=any_spec,
        scratch_shapes=[
            pltpu.VMEM((S, D), BF16),
            pltpu.VMEM((S, D), F32),
            pltpu.VMEM((D, 3 * D), BF16),
            pltpu.VMEM((D, D), BF16),
            pltpu.VMEM((D, 3 * D), BF16),
            pltpu.VMEM((D, D), BF16),
            pltpu.VMEM((D, F), BF16),
            pltpu.VMEM((D, F), BF16),
            pltpu.VMEM((F, D), BF16),
            pltpu.VMEM((3 * nc, HALO + TM, LANES), F32),
            pltpu.VMEM((TM, D), BF16),
            pltpu.VMEM((TM, D), BF16),
            pltpu.VMEM((TM, D), BF16),
            pltpu.VMEM((TM, F), BF16),
            pltpu.SemaphoreType.DMA((nb,)),
            pltpu.SemaphoreType.DMA((D // PB,)),
            pltpu.SemaphoreType.DMA((6,)),
            pltpu.SemaphoreType.DMA((nb,)),
        ],
        compiler_params=pltpu.CompilerParams(vmem_limit_bytes=100 * 1024 * 1024),
    )(A_x.reshape(S, D), A_wqkv, A_wo, B_w1, B_w3, B_w2)
    return out.reshape(B, S, D)
```

```python
import functools

import jax
import jax.numpy as jnp
import jax.experimental.pallas as pl
import jax.experimental.pallas.tpu as pltpu

N_HEADS = 32
WINDOW = 8
DILATION = 2
EPS = 1e-5
LANES = 128
HALO = 16

TM = 256
FC = 256
NC = 256
NE1 = 1
NS4 = 3
NS2 = 1
RB = 16
PB = 128
RC = 128
LB = 32

F32 = jnp.float32
BF16 = jnp.bfloat16


def _dot(a, b):
    return jnp.dot(a, b, preferred_element_type=F32)


def _token(*vals):
    words = [pltpu.bitcast(v, jnp.uint32) for v in vals]
    regs = [w[r:r + 8, c:c + LANES] for w in words
            for r in range(0, w.shape[0], 8) for c in range(0, w.shape[1], LANES)]
    return functools.reduce(jnp.bitwise_or, regs)


def _after(x, tokens, never):
    if not tokens:
        return x
    w = pltpu.bitcast(x, jnp.uint32)
    corner = jnp.where(never, functools.reduce(jnp.bitwise_or, tokens), w[:8, :LANES])
    top = jnp.concatenate([corner, w[:8, LANES:]], axis=1) if w.shape[1] > LANES else corner
    return pltpu.bitcast(jnp.concatenate([top, w[8:]], axis=0), BF16)


def _swap_bit(a, b, stride, axis):
    n = a.shape[axis]
    low = (jax.lax.broadcasted_iota(jnp.int32, a.shape, axis) & stride) == 0
    return (jnp.where(low, a, pltpu.roll(b, stride, axis)),
            jnp.where(low, pltpu.roll(a, n - stride, axis), b))


def _swap_bits(parts, strides, axis):
    parts = list(parts)
    for bit, stride in strides:
        for i in range(len(parts)):
            if not i & bit:
                parts[i], parts[i | bit] = _swap_bit(parts[i], parts[i | bit], stride, axis)
    return parts


def _left_operands(a11, a12, a21, a22):
    return (a11 + a22, a21 + a22, a11, a22, a11 + a12, a21 - a11, a12 - a22)


def _right_operands(b11, b12, b21, b22):
    return (b11 + b22, b11, b12 - b22, b21 - b11, b22, b11 + b12, b21 + b22)


_FEEDS = (((0, 1), (3, 1)), ((2, 1), (3, -1)), ((1, 1), (3, 1)), ((0, 1), (2, 1)),
          ((0, -1), (1, 1)), ((3, 1),), ((0, 1),))


def _block_product(product, start=(None,) * 4):
    c = list(start)
    for i, feeds in enumerate(_FEEDS):
        m = product(i)
        for k, sign in feeds:
            c[k] = m if c[k] is None else (c[k] + m if sign > 0 else c[k] - m)
    return c


def _kernel(x_hbm, wqkv_hbm, wo_hbm, w1_hbm, w3_hbm, w2_hbm, out_hbm,
            io_s, x_s, wqkv_raw, wo_raw, wqkv_s, wo_s, w1_raw, w3_raw, w2_raw, up_s, down_s,
            qkv_s, xa_s, xb_s, o_s, h_s, in_sem, qkv_sem, w_sem, up_sem, out_sem):
    S, D = x_s.shape
    F = w3_raw.shape[1]
    TH, DH, FH = TM // 2, D // 2, F // 2
    nb = S // TM
    n_items = 2 * nb
    nc = D // LANES
    scale = (D // N_HEADS) ** -0.5

    def rows(j):
        return pl.ds(j * TM if isinstance(j, int) else pl.multiple_of(j * TM, TM), TM)

    def x_copy(j):
        return pltpu.make_async_copy(x_hbm.at[rows(j)], io_s.at[rows(j)], in_sem.at[j])

    def out_copy(j):
        return pltpu.make_async_copy(io_s.at[rows(j)], out_hbm.at[rows(j)], out_sem.at[j])

    def wqkv_copy(i):
        rr = pl.ds(i * PB if isinstance(i, int) else pl.multiple_of(i * PB, PB), PB)
        return pltpu.make_async_copy(wqkv_hbm.at[rr], wqkv_raw.at[rr], qkv_sem.at[i])

    wo_copy = pltpu.make_async_copy(wo_hbm, wo_raw, w_sem.at[0])
    w2_copy = pltpu.make_async_copy(w2_hbm, w2_raw, w_sem.at[1])

    def up_copies(r):
        return [pltpu.make_async_copy(src.at[chunk(r + h * (DH // PB))], dst.at[chunk(r + h * (DH // PB))],
                                      up_sem.at[4 * r + 2 * m + h])
                for m, (src, dst) in enumerate(((w1_hbm, w1_raw), (w3_hbm, w3_raw))) for h in range(2)]

    def chunk(r):
        return pl.ds(r * PB if isinstance(r, int) else pl.multiple_of(r * PB, PB), PB)

    def permute_qkv_columns(r):
        for i in range(3):
            cols = [pl.ds(i * D + c * LANES, LANES) for c in range(nc)]
            parts = [pltpu.bitcast(wqkv_raw[chunk(r), cc], jnp.uint32) for cc in cols]
            for cc, part in zip(cols, _swap_bits(parts, ((4, 16), (2, 8), (1, 4)), 1)):
                wqkv_s[chunk(r), cc] = pltpu.bitcast(part, BF16)

    def project_partial(r):
        y = _dot(xa_s[:, chunk(r)], wqkv_s[chunk(r), :])
        for t in range(3 * nc):
            qkv_s[t, pl.ds(HALO, TM), :] += y[:, t * LANES:(t + 1) * LANES]

    def combine_up(r):
        top, bottom = chunk(r), chunk(r + DH // PB)

        @pl.loop(0, FH // FC)
        def _(f):
            left = pl.ds(pl.multiple_of(f * FC, FC), FC)
            right = pl.ds(pl.multiple_of(FH + f * FC, FC), FC)
            for m, w in enumerate((w1_raw, w3_raw)):
                blocks = [w[rr, cc].astype(F32) for rr in (top, bottom) for cc in (left, right)]
                for i, b in enumerate(_right_operands(*blocks)):
                    up_s[i, top, pl.ds(pl.multiple_of((2 * f + m) * FC, FC), FC)] = b.astype(BF16)

    def combine_down():
        @pl.loop(0, FH // PB)
        def _(r):
            top, bottom = chunk(r), chunk(r + FH // PB)
            blocks = [w2_raw[rr, cc].astype(F32) for rr in (top, bottom) for cc in (pl.ds(0, DH), pl.ds(DH, DH))]
            for i, b in enumerate(_right_operands(*blocks)):
                down_s[i, top, :] = b.astype(BF16)

    def permute_wo_rows():
        def body(hh, carry):
            def tile(h432, d4):
                return pl.ds(pl.multiple_of(h432 * 128 + hh * 32 + d4 * 16, 16), 16)
            src = [[pltpu.bitcast(wo_raw[tile(h, d4), :], jnp.uint32) for h in range(8)] for d4 in range(2)]
            src = [_swap_bits(p, ((2, 4), (1, 2)), 0) for p in src]
            for d4 in range(2):
                for h in range(8):
                    wo_s[tile((h & 3) | (d4 << 2), h >> 2), :] = pltpu.bitcast(src[d4][h], BF16)
            return carry
        jax.lax.fori_loop(0, 4, body, 0)

    def residual(rr, fresh):
        if fresh is None:
            return x_s[rr, :]
        return jnp.where(fresh, io_s[rr, :].astype(F32), x_s[rr, :])

    def normed(j, fresh, r, n):
        x = residual(pl.ds(pl.multiple_of(j * TM + r, n), n), fresh)
        xc = x - jnp.mean(x, axis=-1, keepdims=True)
        var = jnp.mean(xc * xc, axis=-1, keepdims=True)
        return xc * jax.lax.rsqrt(var + EPS)

    def norm_for_attention(j, fresh, r, n):
        y = normed(j, fresh, r, n).astype(BF16)
        xa_s[pl.ds(r, n), :] = y
        return _token(y)

    def norm_for_ffn(j, r, n):
        top, bottom = normed(j, None, r, n), normed(j, None, TH + r, n)
        ops = [a.astype(BF16) for a in _left_operands(top[:, :DH], top[:, DH:], bottom[:, :DH], bottom[:, DH:])]
        for i, a in enumerate(ops):
            xb_s[i, pl.ds(r, n), :] = a
        return _token(*ops)

    def spread(items, i, n):
        return items[i * len(items) // n:(i + 1) * len(items) // n]

    def first_token(t):
        return jnp.broadcast_to(qkv_s[t, pl.ds(HALO, 1), :], (HALO, LANES))

    def project(j, side_job, never):
        tokens = []
        for i in range(3):
            tails = [qkv_s[i * nc + c, pl.ds(TM, HALO), :] for c in range(nc if i else 0)]
            y = _dot(_after(xa_s[...], tokens, never), wqkv_s[:, pl.ds(i * D, D)])
            tokens = side_job(i)
            for c in range(nc):
                yc = y[:, c * LANES:(c + 1) * LANES]
                qkv_s[i * nc + c, pl.ds(HALO, TM), :] = yc
                if i:
                    head = jnp.broadcast_to(yc[0:1, :], (HALO, LANES))
                    qkv_s[i * nc + c, pl.ds(0, HALO), :] = jnp.where(j == 0, head, tails[c])

    def attention(j, r, n, masked):
        lane = jax.lax.broadcasted_iota(jnp.int32, (n, LANES), 1)
        logits = [None] * WINDOW
        for c in range(nc):
            q = qkv_s[c, pl.ds(HALO + r, n), :]
            for w in range(WINDOW):
                p = q * qkv_s[nc + c, pl.ds(HALO + r - DILATION * w, n), :]
                logits[w] = p if c == 0 else logits[w] + p
        for s in (1, 2):
            logits = [l + jnp.where((lane & s) == 0, pltpu.roll(l, LANES - s, 1), pltpu.roll(l, s, 1))
                      for l in logits]
        logits = [l * scale for l in logits]
        if masked:
            pos = j * TM + r + jax.lax.broadcasted_iota(jnp.int32, (n, LANES), 0)
            logits = [jnp.where(pos >= DILATION * w, l, -1e9) if w else l for w, l in enumerate(logits)]
        m = functools.reduce(jnp.maximum, logits)
        e = [jnp.exp(l - m) for l in logits]
        inv = 1.0 / functools.reduce(jnp.add, e)
        p = [x * inv for x in e]
        outs = []
        for c in range(nc):
            terms = [p[w] * qkv_s[2 * nc + c, pl.ds(HALO + r - DILATION * w, n), :] for w in range(WINDOW)]
            outs.append(functools.reduce(jnp.add, terms))
        o = jnp.concatenate(outs, axis=1).astype(BF16)
        o_s[pl.ds(r, n), :] = o
        return _token(o)

    def ffn_up(side_job, never):
        tokens = []
        for f in range(FH // FC):
            def product(i):
                nonlocal tokens
                m = _dot(_after(xb_s[i], tokens, never), up_s[i, :, pl.ds(2 * f * FC, 2 * FC)])
                tokens = side_job(7 * f + i)
                return m

            hidden = []
            for gu in _block_product(product):
                half = 0.5 * gu[:, :FC]
                hidden.append((half + half * jnp.tanh(half)) * gu[:, FC:])
            for i, a in enumerate(_left_operands(*hidden)):
                h_s[i, :, pl.ds(f * FC, FC)] = a.astype(BF16)

    def ffn_down(j, side_job, never):
        tokens = []
        for p in range(DH // NC):
            def product(i):
                nonlocal tokens
                m = _dot(_after(h_s[i], tokens, never), down_s[i, :, pl.ds(p * NC, NC)])
                tokens = side_job(7 * p + i)
                return m

            where = [(pl.ds(pl.multiple_of(j * TM + r0, TH), TH), pl.ds(c0 + p * NC, NC))
                     for r0 in (0, TH) for c0 in (0, DH)]
            for at, y in zip(where, _block_product(product)):
                y = x_s[at] + y
                x_s[at] = y
                io_s[at] = y.astype(BF16)

    copies = ([x_copy(0)] + [wqkv_copy(r) for r in range(D // PB)]
              + [x_copy(1), wo_copy, x_copy(2)]
              + [c for r in range(DH // PB) for c in up_copies(r)] + [w2_copy]
              + [x_copy(j) for j in range(3, nb)])

    @pl.loop(0, len(copies))
    def _(i):
        for k, copy in enumerate(copies):
            pl.when(i == k)(copy.start)

    last = n_items - 1

    @pl.loop(-2, n_items)
    def _(n):
        j0 = jnp.maximum(n, 0) % nb
        j1 = jnp.maximum(n + 1, 0) % nb
        j2 = (n + 2) % nb
        never = n > n_items

        def side_job(steps, n_slots):
            return lambda i: [step() for step in spread(steps, i, n_slots) if i < n_slots]

        @pl.when(n + 2 < nb)
        def _():
            x_copy(j2).wait()

        @pl.when(n == 0)
        def _():
            @pl.loop(0, DH // PB)
            def _(r):
                for copy in up_copies(r):
                    copy.wait()
                combine_up(r)

        @pl.when(n >= 0)
        def _():
            steps = [functools.partial(attention, j1, r, RB, r < HALO) for r in range(0, TM, RB)]
            ffn_up(side_job(steps, 7 * (FH // FC) - NE1), never)

        @pl.when(n == -1)
        def _():
            @pl.loop(0, TM // RC)
            def _(g):
                attention(j1, pl.multiple_of(g * RC, RC), RC, True)

            wo_copy.wait()
            permute_wo_rows()

        @pl.when(n == 0)
        def _():
            w2_copy.wait()
            combine_down()

        @pl.when(n >= 0)
        def _():
            steps = [functools.partial(norm_for_attention, j2, n + 2 < nb, r, LB) for r in range(0, TM, LB)]
            ffn_down(j0, side_job(steps, 7 * (DH // NC) - NS2), never)

        @pl.when(n < 0)
        def _():
            norm_for_attention(j2, n + 2 < nb, 0, TM)

        @pl.when(n == -2)
        def _():
            qkv_s[...] = jnp.zeros(qkv_s.shape, F32)

            n_chunks = D // PB

            @pl.loop(0, n_chunks + 1)
            def _(r):
                @pl.when(r < n_chunks)
                def _():
                    wqkv_copy(r).wait()

                @pl.when(r == 0)
                def _():
                    permute_qkv_columns(0)

                @pl.when(r > 0)
                def _():
                    project_partial(r - 1)
                    permute_qkv_columns(jnp.minimum(r, n_chunks - 1))

            for t in range(nc, 3 * nc):
                qkv_s[t, pl.ds(0, HALO), :] = first_token(t)

        @pl.when(n >= nb)
        def _():
            out_copy(j0).start()

        @pl.when(jnp.logical_and(n >= -1, n < last - 1))
        def _():
            x_s[rows(j1), :] = residual(rows(j1), n + 1 < nb) + _dot(o_s[...], wo_s[...])
            project(j2, side_job([functools.partial(norm_for_ffn, j1, r, LB // 2) for r in range(0, TH, LB // 2)], NS4), never)

        @pl.when(n == last - 1)
        def _():
            @pl.loop(0, D // NC)
            def _(i):
                cols = pl.ds(pl.multiple_of(i * NC, NC), NC)
                x_s[rows(j1), cols] += _dot(o_s[...], wo_s[:, cols])

            norm_for_ffn(j1, 0, TH)

    for j in range(nb):
        out_copy(j).wait()


@jax.jit
def pallas_interleave_layers__sliding_local_dilated__glu_gated_swiglu__prompt_kernel(
    A_x: jax.Array,
    A_wqkv: jax.Array,
    A_wo: jax.Array,
    B_x: jax.Array,
    B_w1: jax.Array,
    B_w3: jax.Array,
    B_w2: jax.Array,
):
    del B_x
    B, S, D = A_x.shape
    F = B_w1.shape[1]
    assert B == 1 and D == N_HEADS * 32 == 8 * LANES and S % TM == 0 and S // TM >= 3 and F % (2 * FC) == 0
    nb = S // TM
    nc = D // LANES
    any_spec = pl.BlockSpec(memory_space=pl.ANY)
    out = pl.pallas_call(
        _kernel,
        out_shape=jax.ShapeDtypeStruct((S, D), A_x.dtype),
        in_specs=[any_spec] * 6,
        out_specs=any_spec,
        scratch_shapes=[
            pltpu.VMEM((S, D), BF16),
            pltpu.VMEM((S, D), F32),
            pltpu.VMEM((D, 3 * D), BF16),
            pltpu.VMEM((D, D), BF16),
            pltpu.VMEM((D, 3 * D), BF16),
            pltpu.VMEM((D, D), BF16),
            pltpu.VMEM((D, F), BF16),
            pltpu.VMEM((D, F), BF16),
            pltpu.VMEM((F, D), BF16),
            pltpu.VMEM((7, D // 2, F), BF16),
            pltpu.VMEM((7, F // 2, D // 2), BF16),
            pltpu.VMEM((3 * nc, HALO + TM, LANES), F32),
            pltpu.VMEM((TM, D), BF16),
            pltpu.VMEM((7, TM // 2, D // 2), BF16),
            pltpu.VMEM((TM, D), BF16),
            pltpu.VMEM((7, TM // 2, F // 2), BF16),
            pltpu.SemaphoreType.DMA((nb,)),
            pltpu.SemaphoreType.DMA((D // PB,)),
            pltpu.SemaphoreType.DMA((2,)),
            pltpu.SemaphoreType.DMA((2 * D // PB,)),
            pltpu.SemaphoreType.DMA((nb,)),
        ],
        compiler_params=pltpu.CompilerParams(vmem_limit_bytes=120 * 1024 * 1024),
    )(A_x.reshape(S, D), A_wqkv, A_wo, B_w1, B_w3, B_w2)
    return out.reshape(B, S, D)
```

```python
import functools

import jax
import jax.numpy as jnp
import jax.experimental.pallas as pl
import jax.experimental.pallas.tpu as pltpu

N_HEADS = 32
WINDOW = 8
DILATION = 2
EPS = 1e-5
LANES = 128
HALO = 16

TM = 256
FC = 256
NC = 256
NE1 = 1
NS4 = 3
NS2 = 1
RB = 16
PB = 128
CW = 256
CB = 32
RC = 128
LB = 32

F32 = jnp.float32
BF16 = jnp.bfloat16
U32 = jnp.uint32


def _dot(a, b):
    return jnp.dot(a, b, preferred_element_type=F32)


def _pack(x):
    return pltpu.bitcast(x.astype(BF16), U32)


def _unpack(words):
    return pltpu.bitcast(words, BF16)


def _word_rows(r, n):
    return pl.ds(r // 2 if isinstance(r, int) else pl.multiple_of(r // 2, n // 2), n // 2)


def _token(*words):
    regs = [w[r:r + 8, c:c + LANES] for w in words
            for r in range(0, w.shape[0], 8) for c in range(0, w.shape[1], LANES)]
    return functools.reduce(jnp.bitwise_or, regs)


def _after(words, tokens, never):
    if tokens:
        corner = jnp.where(never, functools.reduce(jnp.bitwise_or, tokens), words[:8, :LANES])
        top = jnp.concatenate([corner, words[:8, LANES:]], axis=1)
        words = jnp.concatenate([top, words[8:]], axis=0)
    return _unpack(words)


def _swap_bit(a, b, stride, axis):
    n = a.shape[axis]
    low = (jax.lax.broadcasted_iota(jnp.int32, a.shape, axis) & stride) == 0
    return (jnp.where(low, a, pltpu.roll(b, stride, axis)),
            jnp.where(low, pltpu.roll(a, n - stride, axis), b))


def _swap_bits(parts, strides, axis):
    parts = list(parts)
    for bit, stride in strides:
        for i in range(len(parts)):
            if not i & bit:
                parts[i], parts[i | bit] = _swap_bit(parts[i], parts[i | bit], stride, axis)
    return parts


def _left_operands(a11, a12, a21, a22):
    return (a11 + a22, a21 + a22, a11, a22, a11 + a12, a21 - a11, a12 - a22)


def _right_operands(b11, b12, b21, b22):
    return (b11 + b22, b11, b12 - b22, b21 - b11, b22, b11 + b12, b21 + b22)


_FEEDS = (((0, 1), (3, 1)), ((2, 1), (3, -1)), ((1, 1), (3, 1)), ((0, 1), (2, 1)),
          ((0, -1), (1, 1)), ((3, 1),), ((0, 1),))


def _block_product(product, start=(None,) * 4):
    c = list(start)
    for i, feeds in enumerate(_FEEDS):
        m = product(i)
        for k, sign in feeds:
            c[k] = m if c[k] is None else (c[k] + m if sign > 0 else c[k] - m)
    return c


def _kernel(x_hbm, wqkv_hbm, wo_hbm, w1_hbm, w3_hbm, w2_hbm, out_hbm,
            io_s, x_s, wqkv_raw, wo_raw, wqkv_s, wo_s, w1_raw, w3_raw, w2_raw, up_s, down_s,
            qkv_s, xa_s, xb_s, o_s, h_s, in_sem, qkv_sem, w_sem, up_sem, out_sem):
    S, D = x_s.shape
    F = w3_raw.shape[1]
    TH, DH, FH = TM // 2, D // 2, F // 2
    nb = S // TM
    n_items = 2 * nb
    nc = D // LANES
    scale = (D // N_HEADS) ** -0.5

    def rows(j):
        return pl.ds(j * TM if isinstance(j, int) else pl.multiple_of(j * TM, TM), TM)

    def x_copy(j):
        return pltpu.make_async_copy(x_hbm.at[rows(j)], io_s.at[rows(j)], in_sem.at[j])

    def out_copy(j):
        return pltpu.make_async_copy(io_s.at[rows(j)], out_hbm.at[rows(j)], out_sem.at[j])

    def wqkv_copy(i):
        rr = pl.ds(i * PB if isinstance(i, int) else pl.multiple_of(i * PB, PB), PB)
        return pltpu.make_async_copy(wqkv_hbm.at[rr], wqkv_raw.at[rr], qkv_sem.at[i])

    wo_copy = pltpu.make_async_copy(wo_hbm, wo_raw, w_sem.at[0])
    w2_copy = pltpu.make_async_copy(w2_hbm, w2_raw, w_sem.at[1])

    def up_copies(r):
        return [pltpu.make_async_copy(src.at[chunk(r + h * (DH // PB))], dst.at[chunk(r + h * (DH // PB))],
                                      up_sem.at[4 * r + 2 * m + h])
                for m, (src, dst) in enumerate(((w1_hbm, w1_raw), (w3_hbm, w3_raw))) for h in range(2)]

    def chunk(r):
        return pl.ds(r * PB if isinstance(r, int) else pl.multiple_of(r * PB, PB), PB)

    def permute_qkv_columns(r):
        for i in range(3):
            cols = [pl.ds(i * D + c * LANES, LANES) for c in range(nc)]
            parts = [pltpu.bitcast(wqkv_raw[chunk(r), cc], U32) for cc in cols]
            for cc, part in zip(cols, _swap_bits(parts, ((4, 16), (2, 8), (1, 4)), 1)):
                wqkv_s[_word_rows(r * PB, PB), cc] = part

    def project_partial(r):
        y = _dot(_unpack(xa_s[:, chunk(r)]), _unpack(wqkv_s[_word_rows(r * PB, PB), :]))
        for t in range(3 * nc):
            qkv_s[t, pl.ds(HALO, TM), :] += y[:, t * LANES:(t + 1) * LANES]

    def combine(src, r, half_rows, c, half_cols, dst, c_dst, width):
        for r0 in range(0, PB, CB):
            for c0 in range(0, width, CW):
                def cols(col):
                    return pl.ds(pl.multiple_of(col + c0, CW), CW)
                blocks = [src[pl.ds(pl.multiple_of(r * PB + dr + r0, CB), CB), cols(c + dc)]
                          for dr in (0, half_rows) for dc in (0, half_cols)]
                words = [pltpu.bitcast(b, U32) for b in blocks]
                halves = [_right_operands(*[
                    pltpu.unpack_elementwise(w, index=k, packed_dtype=BF16, unpacked_dtype=F32) for w in words])
                    for k in range(2)]
                for i, pair in enumerate(zip(*halves)):
                    packed = pltpu.pack_elementwise(list(pair), packed_dtype=BF16)
                    dst[i, _word_rows(r * PB + r0, CB), cols(c_dst)] = packed.astype(U32)

    def combine_up(r):
        @pl.loop(0, FH // FC)
        def _(f):
            for m, w in enumerate((w1_raw, w3_raw)):
                combine(w, r, DH, f * FC, FH, up_s, (2 * f + m) * FC, FC)

    def combine_down():
        @pl.loop(0, FH // PB)
        def _(r):
            combine(w2_raw, r, FH, r * 0, DH, down_s, r * 0, DH)

    def permute_wo_rows():
        def body(hh, carry):
            def tile(h432, d4):
                return pl.ds(pl.multiple_of(h432 * 128 + hh * 32 + d4 * 16, 16), 16)
            src = [[pltpu.bitcast(wo_raw[tile(h, d4), :], U32) for h in range(8)] for d4 in range(2)]
            src = [_swap_bits(p, ((2, 4), (1, 2)), 0) for p in src]
            for d4 in range(2):
                for h in range(8):
                    wo_s[_word_rows(((h & 3) | (d4 << 2)) * 128 + hh * 32 + (h >> 2) * 16, 16), :] = src[d4][h]
            return carry
        jax.lax.fori_loop(0, 4, body, 0)

    def residual(rr, fresh):
        if fresh is None:
            return x_s[rr, :]
        return jnp.where(fresh, io_s[rr, :].astype(F32), x_s[rr, :])

    def normed(j, fresh, r, n):
        x = residual(pl.ds(pl.multiple_of(j * TM + r, n), n), fresh)
        xc = x - jnp.mean(x, axis=-1, keepdims=True)
        var = jnp.mean(xc * xc, axis=-1, keepdims=True)
        return xc * jax.lax.rsqrt(var + EPS)

    def norm_for_attention(j, fresh, r, n):
        y = _pack(normed(j, fresh, r, n))
        xa_s[_word_rows(r, n), :] = y
        return _token(y)

    def norm_for_ffn(j, r, n):
        top, bottom = normed(j, None, r, n), normed(j, None, TH + r, n)
        ops = [_pack(a) for a in _left_operands(top[:, :DH], top[:, DH:], bottom[:, :DH], bottom[:, DH:])]
        for i, a in enumerate(ops):
            xb_s[i, _word_rows(r, n), :] = a
        return _token(*ops)

    def spread(items, i, n):
        return items[i * len(items) // n:(i + 1) * len(items) // n]

    def first_token(t):
        return jnp.broadcast_to(qkv_s[t, pl.ds(HALO, 1), :], (HALO, LANES))

    def project(j, side_job, never):
        tokens = []
        for i in range(3):
            tails = [qkv_s[i * nc + c, pl.ds(TM, HALO), :] for c in range(nc if i else 0)]
            y = _dot(_after(xa_s[...], tokens, never), _unpack(wqkv_s[:, pl.ds(i * D, D)]))
            tokens = side_job(i)
            for c in range(nc):
                yc = y[:, c * LANES:(c + 1) * LANES]
                qkv_s[i * nc + c, pl.ds(HALO, TM), :] = yc
                if i:
                    head = jnp.broadcast_to(yc[0:1, :], (HALO, LANES))
                    qkv_s[i * nc + c, pl.ds(0, HALO), :] = jnp.where(j == 0, head, tails[c])

    def attention(j, r, n, masked):
        lane = jax.lax.broadcasted_iota(jnp.int32, (n, LANES), 1)
        logits = [None] * WINDOW
        for c in range(nc):
            q = qkv_s[c, pl.ds(HALO + r, n), :]
            for w in range(WINDOW):
                p = q * qkv_s[nc + c, pl.ds(HALO + r - DILATION * w, n), :]
                logits[w] = p if c == 0 else logits[w] + p
        for s in (1, 2):
            logits = [l + jnp.where((lane & s) == 0, pltpu.roll(l, LANES - s, 1), pltpu.roll(l, s, 1))
                      for l in logits]
        logits = [l * scale for l in logits]
        if masked:
            pos = j * TM + r + jax.lax.broadcasted_iota(jnp.int32, (n, LANES), 0)
            logits = [jnp.where(pos >= DILATION * w, l, -1e9) if w else l for w, l in enumerate(logits)]
        m = functools.reduce(jnp.maximum, logits)
        e = [jnp.exp(l - m) for l in logits]
        inv = 1.0 / functools.reduce(jnp.add, e)
        p = [x * inv for x in e]
        outs = []
        for c in range(nc):
            terms = [p[w] * qkv_s[2 * nc + c, pl.ds(HALO + r - DILATION * w, n), :] for w in range(WINDOW)]
            outs.append(functools.reduce(jnp.add, terms))
        o = _pack(jnp.concatenate(outs, axis=1))
        o_s[_word_rows(r, n), :] = o
        return _token(o)

    def ffn_up(side_job, never):
        tokens = []
        for f in range(FH // FC):
            def product(i):
                nonlocal tokens
                m = _dot(_after(xb_s[i], tokens, never), _unpack(up_s[i, :, pl.ds(2 * f * FC, 2 * FC)]))
                tokens = side_job(7 * f + i)
                return m

            hidden = []
            for gu in _block_product(product):
                half = 0.5 * gu[:, :FC]
                hidden.append((half + half * jnp.tanh(half)) * gu[:, FC:])
            for i, a in enumerate(_left_operands(*hidden)):
                h_s[i, :, pl.ds(f * FC, FC)] = _pack(a)

    def ffn_down(j, side_job, never):
        tokens = []
        for p in range(DH // NC):
            def product(i):
                nonlocal tokens
                m = _dot(_after(h_s[i], tokens, never), _unpack(down_s[i, :, pl.ds(p * NC, NC)]))
                tokens = side_job(7 * p + i)
                return m

            where = [(pl.ds(pl.multiple_of(j * TM + r0, TH), TH), pl.ds(c0 + p * NC, NC))
                     for r0 in (0, TH) for c0 in (0, DH)]
            for at, y in zip(where, _block_product(product)):
                y = x_s[at] + y
                x_s[at] = y
                io_s[at] = y.astype(BF16)

    def start_in_order(n, copies):
        @pl.loop(0, n)
        def _(i):
            for copy in copies(i):
                copy.start()

    x_copy(0).start()
    start_in_order(D // PB, lambda r: [wqkv_copy(r)])

    last = n_items - 1

    @pl.loop(-2, n_items)
    def _(n):
        j0 = jnp.maximum(n, 0) % nb
        j1 = jnp.maximum(n + 1, 0) % nb
        j2 = (n + 2) % nb
        never = n > n_items

        def side_job(steps, n_slots):
            return lambda i: [step() for step in spread(steps, i, n_slots) if i < n_slots]

        @pl.when(n + 2 < nb)
        def _():
            x_copy(j2).wait()

        @pl.when(n == 0)
        def _():
            @pl.loop(0, DH // PB)
            def _(r):
                for copy in up_copies(r):
                    copy.wait()
                combine_up(r)

        @pl.when(n >= 0)
        def _():
            steps = [functools.partial(attention, j1, r, RB, r < HALO) for r in range(0, TM, RB)]
            ffn_up(side_job(steps, 7 * (FH // FC) - NE1), never)

        @pl.when(n == -1)
        def _():
            @pl.loop(0, TM // RC)
            def _(g):
                attention(j1, pl.multiple_of(g * RC, RC), RC, True)

            wo_copy.wait()
            permute_wo_rows()

        @pl.when(n == 0)
        def _():
            w2_copy.wait()
            combine_down()

        @pl.when(n >= 0)
        def _():
            steps = [functools.partial(norm_for_attention, j2, n + 2 < nb, r, LB) for r in range(0, TM, LB)]
            ffn_down(j0, side_job(steps, 7 * (DH // NC) - NS2), never)

        @pl.when(n < 0)
        def _():
            norm_for_attention(j2, n + 2 < nb, 0, TM)

        @pl.when(n == -2)
        def _():
            x_copy(1).start()
            wo_copy.start()
            x_copy(2).start()
            start_in_order(DH // PB, up_copies)
            w2_copy.start()
            start_in_order(nb - 3, lambda j: [x_copy(j + 3)])
            qkv_s[...] = jnp.zeros(qkv_s.shape, F32)

            n_chunks = D // PB

            @pl.loop(0, n_chunks + 1)
            def _(r):
                @pl.when(r < n_chunks)
                def _():
                    wqkv_copy(r).wait()

                @pl.when(r == 0)
                def _():
                    permute_qkv_columns(0)

                @pl.when(r > 0)
                def _():
                    project_partial(r - 1)
                    permute_qkv_columns(jnp.minimum(r, n_chunks - 1))

            for t in range(nc, 3 * nc):
                qkv_s[t, pl.ds(0, HALO), :] = first_token(t)

        @pl.when(n >= nb)
        def _():
            out_copy(j0).start()

        @pl.when(jnp.logical_and(n >= -1, n < last - 1))
        def _():
            x_s[rows(j1), :] = residual(rows(j1), n + 1 < nb) + _dot(_unpack(o_s[...]), _unpack(wo_s[...]))
            project(j2, side_job([functools.partial(norm_for_ffn, j1, r, LB // 2) for r in range(0, TH, LB // 2)], NS4), never)

        @pl.when(n == last - 1)
        def _():
            @pl.loop(0, D // NC)
            def _(i):
                cols = pl.ds(pl.multiple_of(i * NC, NC), NC)
                x_s[rows(j1), cols] += _dot(_unpack(o_s[...]), _unpack(wo_s[:, cols]))

            norm_for_ffn(j1, 0, TH)

    for j in range(nb):
        out_copy(j).wait()


@jax.jit
def pallas_interleave_layers__sliding_local_dilated__glu_gated_swiglu__prompt_kernel(
    A_x: jax.Array,
    A_wqkv: jax.Array,
    A_wo: jax.Array,
    B_x: jax.Array,
    B_w1: jax.Array,
    B_w3: jax.Array,
    B_w2: jax.Array,
):
    del B_x
    B, S, D = A_x.shape
    F = B_w1.shape[1]
    assert B == 1 and D == N_HEADS * 32 == 8 * LANES and S % TM == 0 and S // TM >= 3 and F % (2 * FC) == 0
    nb = S // TM
    nc = D // LANES
    any_spec = pl.BlockSpec(memory_space=pl.ANY)
    out = pl.pallas_call(
        _kernel,
        out_shape=jax.ShapeDtypeStruct((S, D), A_x.dtype),
        in_specs=[any_spec] * 6,
        out_specs=any_spec,
        scratch_shapes=[
            pltpu.VMEM((S, D), BF16),
            pltpu.VMEM((S, D), F32),
            pltpu.VMEM((D, 3 * D), BF16),
            pltpu.VMEM((D, D), BF16),
            pltpu.VMEM((D // 2, 3 * D), U32),
            pltpu.VMEM((D // 2, D), U32),
            pltpu.VMEM((D, F), BF16),
            pltpu.VMEM((D, F), BF16),
            pltpu.VMEM((F, D), BF16),
            pltpu.VMEM((7, D // 4, F), U32),
            pltpu.VMEM((7, F // 4, D // 2), U32),
            pltpu.VMEM((3 * nc, HALO + TM, LANES), F32),
            pltpu.VMEM((TM // 2, D), U32),
            pltpu.VMEM((7, TM // 4, D // 2), U32),
            pltpu.VMEM((TM // 2, D), U32),
            pltpu.VMEM((7, TM // 4, F // 2), U32),
            pltpu.SemaphoreType.DMA((nb,)),
            pltpu.SemaphoreType.DMA((D // PB,)),
            pltpu.SemaphoreType.DMA((2,)),
            pltpu.SemaphoreType.DMA((2 * D // PB,)),
            pltpu.SemaphoreType.DMA((nb,)),
        ],
        compiler_params=pltpu.CompilerParams(vmem_limit_bytes=120 * 1024 * 1024),
    )(A_x.reshape(S, D), A_wqkv, A_wo, B_w1, B_w3, B_w2)
    return out.reshape(B, S, D)
```

```python
import functools

import jax
import jax.numpy as jnp
import jax.experimental.pallas as pl
import jax.experimental.pallas.tpu as pltpu

N_HEADS = 32
WINDOW = 8
DILATION = 2
EPS = 1e-5
LANES = 128
HALO = 16

TM = 256
FC = 256
NC = 256
NE1 = 1
NS4 = 3
NS2 = 1
RB = 16
PB = 128
CW = 256
CB = 32
RC = 128
LB = 32

F32 = jnp.float32
BF16 = jnp.bfloat16
U32 = jnp.uint32


def _dot(a, b):
    return jnp.dot(a, b, preferred_element_type=F32)


def _unpack(words):
    return pltpu.bitcast(words, BF16)


def _word_rows(r, n):
    return pl.ds(r // 2 if isinstance(r, int) else pl.multiple_of(r // 2, n // 2), n // 2)


def _token(*vals):
    regs = [pltpu.bitcast(v[r:r + 8, c:c + LANES], U32) for v in vals
            for r in range(0, v.shape[0], 8) for c in range(0, v.shape[1], LANES)]
    return functools.reduce(jnp.bitwise_or, regs)


def _after(x, tokens, never):
    if not tokens:
        return x
    words = pltpu.bitcast(x, U32)
    corner = jnp.where(never, functools.reduce(jnp.bitwise_or, tokens), words[:8, :LANES])
    top = jnp.concatenate([corner, words[:8, LANES:]], axis=1)
    return _unpack(jnp.concatenate([top, words[8:]], axis=0))


def _swap_bit(a, b, stride, axis):
    n = a.shape[axis]
    low = (jax.lax.broadcasted_iota(jnp.int32, a.shape, axis) & stride) == 0
    return (jnp.where(low, a, pltpu.roll(b, stride, axis)),
            jnp.where(low, pltpu.roll(a, n - stride, axis), b))


def _swap_bits(parts, strides, axis):
    parts = list(parts)
    for bit, stride in strides:
        for i in range(len(parts)):
            if not i & bit:
                parts[i], parts[i | bit] = _swap_bit(parts[i], parts[i | bit], stride, axis)
    return parts


def _left_operands(a11, a12, a21, a22):
    return (a11 + a22, a21 + a22, a11, a22, a11 + a12, a21 - a11, a12 - a22)


def _right_operands(b11, b12, b21, b22):
    return (b11 + b22, b11, b12 - b22, b21 - b11, b22, b11 + b12, b21 + b22)


_FEEDS = (((0, 1), (3, 1)), ((2, 1), (3, -1)), ((1, 1), (3, 1)), ((0, 1), (2, 1)),
          ((0, -1), (1, 1)), ((3, 1),), ((0, 1),))


def _block_product(product, start=(None,) * 4):
    c = list(start)
    for i, feeds in enumerate(_FEEDS):
        m = product(i)
        for k, sign in feeds:
            c[k] = m if c[k] is None else (c[k] + m if sign > 0 else c[k] - m)
    return c


def _kernel(x_hbm, wqkv_hbm, wo_hbm, w1_hbm, w3_hbm, w2_hbm, out_hbm,
            io_s, x_s, wqkv_raw, wo_raw, wqkv_s, wo_s, w1_raw, w3_raw, w2_raw, up_s, down_s,
            qkv_s, xa_s, xb_s, o_s, h_s, in_sem, qkv_sem, w_sem, up_sem, out_sem):
    S, D = x_s.shape
    F = w3_raw.shape[1]
    TH, DH, FH = TM // 2, D // 2, F // 2
    nb = S // TM
    n_items = 2 * nb
    nc = D // LANES
    scale = (D // N_HEADS) ** -0.5

    def rows(j):
        return pl.ds(j * TM if isinstance(j, int) else pl.multiple_of(j * TM, TM), TM)

    def x_copy(j):
        return pltpu.make_async_copy(x_hbm.at[rows(j)], io_s.at[rows(j)], in_sem.at[j])

    def out_copy(j):
        return pltpu.make_async_copy(io_s.at[rows(j)], out_hbm.at[rows(j)], out_sem.at[j])

    def wqkv_copy(i):
        rr = pl.ds(i * PB if isinstance(i, int) else pl.multiple_of(i * PB, PB), PB)
        return pltpu.make_async_copy(wqkv_hbm.at[rr], wqkv_raw.at[rr], qkv_sem.at[i])

    wo_copy = pltpu.make_async_copy(wo_hbm, wo_raw, w_sem.at[0])
    w2_copy = pltpu.make_async_copy(w2_hbm, w2_raw, w_sem.at[1])

    def up_copies(r):
        return [pltpu.make_async_copy(src.at[chunk(r + h * (DH // PB))], dst.at[chunk(r + h * (DH // PB))],
                                      up_sem.at[4 * r + 2 * m + h])
                for m, (src, dst) in enumerate(((w1_hbm, w1_raw), (w3_hbm, w3_raw))) for h in range(2)]

    def chunk(r):
        return pl.ds(r * PB if isinstance(r, int) else pl.multiple_of(r * PB, PB), PB)

    def permute_qkv_columns(r):
        for i in range(3):
            cols = [pl.ds(i * D + c * LANES, LANES) for c in range(nc)]
            parts = [pltpu.bitcast(wqkv_raw[chunk(r), cc], U32) for cc in cols]
            for cc, part in zip(cols, _swap_bits(parts, ((4, 16), (2, 8), (1, 4)), 1)):
                wqkv_s[_word_rows(r * PB, PB), cc] = part

    def project_partial(r):
        y = _dot(xa_s[:, chunk(r)], _unpack(wqkv_s[_word_rows(r * PB, PB), :]))
        for t in range(3 * nc):
            qkv_s[t, pl.ds(HALO, TM), :] += y[:, t * LANES:(t + 1) * LANES]

    def combine(src, r, half_rows, c, half_cols, dst, c_dst, width):
        for r0 in range(0, PB, CB):
            for c0 in range(0, width, CW):
                def cols(col):
                    return pl.ds(pl.multiple_of(col + c0, CW), CW)
                blocks = [src[pl.ds(pl.multiple_of(r * PB + dr + r0, CB), CB), cols(c + dc)]
                          for dr in (0, half_rows) for dc in (0, half_cols)]
                words = [pltpu.bitcast(b, U32) for b in blocks]
                halves = [_right_operands(*[
                    pltpu.unpack_elementwise(w, index=k, packed_dtype=BF16, unpacked_dtype=F32) for w in words])
                    for k in range(2)]
                for i, pair in enumerate(zip(*halves)):
                    packed = pltpu.pack_elementwise(list(pair), packed_dtype=BF16)
                    dst[i, _word_rows(r * PB + r0, CB), cols(c_dst)] = packed.astype(U32)

    def combine_up(r):
        @pl.loop(0, FH // FC)
        def _(f):
            for m, w in enumerate((w1_raw, w3_raw)):
                combine(w, r, DH, f * FC, FH, up_s, (2 * f + m) * FC, FC)

    def combine_down():
        @pl.loop(0, FH // PB)
        def _(r):
            combine(w2_raw, r, FH, r * 0, DH, down_s, r * 0, DH)

    def permute_wo_rows():
        def body(hh, carry):
            def tile(h432, d4):
                return pl.ds(pl.multiple_of(h432 * 128 + hh * 32 + d4 * 16, 16), 16)
            src = [[pltpu.bitcast(wo_raw[tile(h, d4), :], U32) for h in range(8)] for d4 in range(2)]
            src = [_swap_bits(p, ((2, 4), (1, 2)), 0) for p in src]
            for d4 in range(2):
                for h in range(8):
                    wo_s[_word_rows(((h & 3) | (d4 << 2)) * 128 + hh * 32 + (h >> 2) * 16, 16), :] = src[d4][h]
            return carry
        jax.lax.fori_loop(0, 4, body, 0)

    def residual(rr, fresh):
        if fresh is None:
            return x_s[rr, :]
        return jnp.where(fresh, io_s[rr, :].astype(F32), x_s[rr, :])

    def normed(j, fresh, r, n):
        x = residual(pl.ds(pl.multiple_of(j * TM + r, n), n), fresh)
        xc = x - jnp.mean(x, axis=-1, keepdims=True)
        var = jnp.mean(xc * xc, axis=-1, keepdims=True)
        return xc * jax.lax.rsqrt(var + EPS)

    def norm_for_attention(j, fresh, r, n):
        y = normed(j, fresh, r, n)
        xa_s[pl.ds(r, n), :] = y.astype(BF16)
        return _token(y)

    def norm_for_ffn(j, r, n):
        top, bottom = normed(j, None, r, n), normed(j, None, TH + r, n)
        ops = _left_operands(top[:, :DH], top[:, DH:], bottom[:, :DH], bottom[:, DH:])
        for i, a in enumerate(ops):
            xb_s[i, pl.ds(r, n), :] = a.astype(BF16)
        return _token(ops[0], ops[1], ops[4])

    def spread(items, i, n):
        return items[i * len(items) // n:(i + 1) * len(items) // n]

    def first_token(t):
        return jnp.broadcast_to(qkv_s[t, pl.ds(HALO, 1), :], (HALO, LANES))

    def project(j, side_job, never):
        tokens = []
        for i in range(3):
            tails = [qkv_s[i * nc + c, pl.ds(TM, HALO), :] for c in range(nc if i else 0)]
            y = _dot(_after(xa_s[...], tokens, never), _unpack(wqkv_s[:, pl.ds(i * D, D)]))
            tokens = side_job(i)
            for c in range(nc):
                yc = y[:, c * LANES:(c + 1) * LANES]
                qkv_s[i * nc + c, pl.ds(HALO, TM), :] = yc
                if i:
                    head = jnp.broadcast_to(yc[0:1, :], (HALO, LANES))
                    qkv_s[i * nc + c, pl.ds(0, HALO), :] = jnp.where(j == 0, head, tails[c])

    def attention(j, r, n, masked):
        lane = jax.lax.broadcasted_iota(jnp.int32, (n, LANES), 1)
        logits = [None] * WINDOW
        for c in range(nc):
            q = qkv_s[c, pl.ds(HALO + r, n), :]
            for w in range(WINDOW):
                p = q * qkv_s[nc + c, pl.ds(HALO + r - DILATION * w, n), :]
                logits[w] = p if c == 0 else logits[w] + p
        for s in (1, 2):
            logits = [l + jnp.where((lane & s) == 0, pltpu.roll(l, LANES - s, 1), pltpu.roll(l, s, 1))
                      for l in logits]
        logits = [l * scale for l in logits]
        if masked:
            pos = j * TM + r + jax.lax.broadcasted_iota(jnp.int32, (n, LANES), 0)
            logits = [jnp.where(pos >= DILATION * w, l, -1e9) if w else l for w, l in enumerate(logits)]
        m = functools.reduce(jnp.maximum, logits)
        e = [jnp.exp(l - m) for l in logits]
        inv = 1.0 / functools.reduce(jnp.add, e)
        p = [x * inv for x in e]
        outs = []
        for c in range(nc):
            terms = [p[w] * qkv_s[2 * nc + c, pl.ds(HALO + r - DILATION * w, n), :] for w in range(WINDOW)]
            outs.append(functools.reduce(jnp.add, terms))
        o = jnp.concatenate(outs, axis=1)
        o_s[pl.ds(r, n), :] = o.astype(BF16)
        return _token(o)

    def ffn_up(side_job, never):
        tokens = []
        for f in range(FH // FC):
            def product(i):
                nonlocal tokens
                m = _dot(_after(xb_s[i], tokens, never), _unpack(up_s[i, :, pl.ds(2 * f * FC, 2 * FC)]))
                tokens = side_job(7 * f + i)
                return m

            hidden = []
            for gu in _block_product(product):
                half = 0.5 * gu[:, :FC]
                hidden.append((half + half * jnp.tanh(half)) * gu[:, FC:])
            for i, a in enumerate(_left_operands(*hidden)):
                h_s[i, :, pl.ds(f * FC, FC)] = a.astype(BF16)

    def ffn_down(j, side_job, never):
        tokens = []
        for p in range(DH // NC):
            def product(i):
                nonlocal tokens
                m = _dot(_after(h_s[i], tokens, never), _unpack(down_s[i, :, pl.ds(p * NC, NC)]))
                tokens = side_job(7 * p + i)
                return m

            where = [(pl.ds(pl.multiple_of(j * TM + r0, TH), TH), pl.ds(c0 + p * NC, NC))
                     for r0 in (0, TH) for c0 in (0, DH)]
            for at, y in zip(where, _block_product(product)):
                y = x_s[at] + y
                x_s[at] = y
                io_s[at] = y.astype(BF16)

    def start_in_order(n, copies):
        @pl.loop(0, n)
        def _(i):
            for copy in copies(i):
                copy.start()

    x_copy(0).start()
    start_in_order(D // PB, lambda r: [wqkv_copy(r)])

    last = n_items - 1

    @pl.loop(-2, n_items)
    def _(n):
        j0 = jnp.maximum(n, 0) % nb
        j1 = jnp.maximum(n + 1, 0) % nb
        j2 = (n + 2) % nb
        never = n > n_items

        def side_job(steps, n_slots):
            return lambda i: [step() for step in spread(steps, i, n_slots) if i < n_slots]

        @pl.when(n + 2 < nb)
        def _():
            x_copy(j2).wait()

        @pl.when(n == 0)
        def _():
            @pl.loop(0, DH // PB)
            def _(r):
                for copy in up_copies(r):
                    copy.wait()
                combine_up(r)

        @pl.when(n >= 0)
        def _():
            steps = [functools.partial(attention, j1, r, RB, r < HALO) for r in range(0, TM, RB)]
            ffn_up(side_job(steps, 7 * (FH // FC) - NE1), never)

        @pl.when(n == -1)
        def _():
            @pl.loop(0, TM // RC)
            def _(g):
                attention(j1, pl.multiple_of(g * RC, RC), RC, True)

            wo_copy.wait()
            permute_wo_rows()

        @pl.when(n == 0)
        def _():
            w2_copy.wait()
            combine_down()

        @pl.when(n >= 0)
        def _():
            steps = [functools.partial(norm_for_attention, j2, n + 2 < nb, r, LB) for r in range(0, TM, LB)]
            ffn_down(j0, side_job(steps, 7 * (DH // NC) - NS2), never)

        @pl.when(n < 0)
        def _():
            norm_for_attention(j2, n + 2 < nb, 0, TM)

        @pl.when(n == -2)
        def _():
            x_copy(1).start()
            wo_copy.start()
            x_copy(2).start()
            start_in_order(DH // PB, up_copies)
            w2_copy.start()
            start_in_order(nb - 3, lambda j: [x_copy(j + 3)])
            qkv_s[...] = jnp.zeros(qkv_s.shape, F32)

            n_chunks = D // PB

            @pl.loop(0, n_chunks + 1)
            def _(r):
                @pl.when(r < n_chunks)
                def _():
                    wqkv_copy(r).wait()

                @pl.when(r == 0)
                def _():
                    permute_qkv_columns(0)

                @pl.when(r > 0)
                def _():
                    project_partial(r - 1)
                    permute_qkv_columns(jnp.minimum(r, n_chunks - 1))

            for t in range(nc, 3 * nc):
                qkv_s[t, pl.ds(0, HALO), :] = first_token(t)

        @pl.when(n >= nb)
        def _():
            out_copy(j0).start()

        @pl.when(jnp.logical_and(n >= -1, n < last - 1))
        def _():
            x_s[rows(j1), :] = residual(rows(j1), n + 1 < nb) + _dot(o_s[...], _unpack(wo_s[...]))
            project(j2, side_job([functools.partial(norm_for_ffn, j1, r, LB // 2) for r in range(0, TH, LB // 2)], NS4), never)

        @pl.when(n == last - 1)
        def _():
            @pl.loop(0, D // NC)
            def _(i):
                cols = pl.ds(pl.multiple_of(i * NC, NC), NC)
                x_s[rows(j1), cols] += _dot(o_s[...], _unpack(wo_s[:, cols]))

            norm_for_ffn(j1, 0, TH)

    for j in range(nb):
        out_copy(j).wait()


@jax.jit
def pallas_interleave_layers__sliding_local_dilated__glu_gated_swiglu__prompt_kernel(
    A_x: jax.Array,
    A_wqkv: jax.Array,
    A_wo: jax.Array,
    B_x: jax.Array,
    B_w1: jax.Array,
    B_w3: jax.Array,
    B_w2: jax.Array,
):
    del B_x
    B, S, D = A_x.shape
    F = B_w1.shape[1]
    assert B == 1 and D == N_HEADS * 32 == 8 * LANES and S % TM == 0 and S // TM >= 3 and F % (2 * FC) == 0
    nb = S // TM
    nc = D // LANES
    any_spec = pl.BlockSpec(memory_space=pl.ANY)
    out = pl.pallas_call(
        _kernel,
        out_shape=jax.ShapeDtypeStruct((S, D), A_x.dtype),
        in_specs=[any_spec] * 6,
        out_specs=any_spec,
        scratch_shapes=[
            pltpu.VMEM((S, D), BF16),
            pltpu.VMEM((S, D), F32),
            pltpu.VMEM((D, 3 * D), BF16),
            pltpu.VMEM((D, D), BF16),
            pltpu.VMEM((D // 2, 3 * D), U32),
            pltpu.VMEM((D // 2, D), U32),
            pltpu.VMEM((D, F), BF16),
            pltpu.VMEM((D, F), BF16),
            pltpu.VMEM((F, D), BF16),
            pltpu.VMEM((7, D // 4, F), U32),
            pltpu.VMEM((7, F // 4, D // 2), U32),
            pltpu.VMEM((3 * nc, HALO + TM, LANES), F32),
            pltpu.VMEM((TM, D), BF16),
            pltpu.VMEM((7, TM // 2, D // 2), BF16),
            pltpu.VMEM((TM, D), BF16),
            pltpu.VMEM((7, TM // 2, F // 2), BF16),
            pltpu.SemaphoreType.DMA((nb,)),
            pltpu.SemaphoreType.DMA((D // PB,)),
            pltpu.SemaphoreType.DMA((2,)),
            pltpu.SemaphoreType.DMA((2 * D // PB,)),
            pltpu.SemaphoreType.DMA((nb,)),
        ],
        compiler_params=pltpu.CompilerParams(vmem_limit_bytes=120 * 1024 * 1024),
    )(A_x.reshape(S, D), A_wqkv, A_wo, B_w1, B_w3, B_w2)
    return out.reshape(B, S, D)
```

```python
import functools

import jax
import jax.numpy as jnp
import jax.experimental.pallas as pl
import jax.experimental.pallas.tpu as pltpu

N_HEADS = 32
WINDOW = 8
DILATION = 2
EPS = 1e-5
LANES = 128
HALO = 16

TM = 256
FC = 256
NC = 256
NE1 = 1
NS4 = 20
NS2 = 1
RB = 16
PB = 128
CW = 256
CB = 32
RC = 128
LB = 16

F32 = jnp.float32
BF16 = jnp.bfloat16
U32 = jnp.uint32


def _dot(a, b):
    return jnp.dot(a, b, preferred_element_type=F32)


def _unpack(words):
    return pltpu.bitcast(words, BF16)


def _word_rows(r, n):
    return pl.ds(r // 2 if isinstance(r, int) else pl.multiple_of(r // 2, n // 2), n // 2)


def _token(*vals):
    regs = [pltpu.bitcast(v[r:r + 8, c:c + LANES], U32) for v in vals
            for r in range(0, v.shape[0], 8) for c in range(0, v.shape[1], LANES)]
    return functools.reduce(jnp.bitwise_or, regs)


def _after(x, tokens, never):
    if not tokens:
        return x
    words = pltpu.bitcast(x, U32)
    corner = jnp.where(never, functools.reduce(jnp.bitwise_or, tokens), words[:8, :LANES])
    top = jnp.concatenate([corner, words[:8, LANES:]], axis=1)
    return _unpack(jnp.concatenate([top, words[8:]], axis=0))


def _swap_bit(a, b, stride, axis):
    n = a.shape[axis]
    low = (jax.lax.broadcasted_iota(jnp.int32, a.shape, axis) & stride) == 0
    return (jnp.where(low, a, pltpu.roll(b, stride, axis)),
            jnp.where(low, pltpu.roll(a, n - stride, axis), b))


def _swap_bits(parts, strides, axis):
    parts = list(parts)
    for bit, stride in strides:
        for i in range(len(parts)):
            if not i & bit:
                parts[i], parts[i | bit] = _swap_bit(parts[i], parts[i | bit], stride, axis)
    return parts


def _left_operands(a11, a12, a21, a22):
    return (a11 + a22, a21 + a22, a11, a22, a11 + a12, a21 - a11, a12 - a22)


def _right_operands(b11, b12, b21, b22):
    return (b11 + b22, b11, b12 - b22, b21 - b11, b22, b11 + b12, b21 + b22)


_FEEDS = (((0, 1), (3, 1)), ((2, 1), (3, -1)), ((1, 1), (3, 1)), ((0, 1), (2, 1)),
          ((0, -1), (1, 1)), ((3, 1),), ((0, 1),))


def _block_product(product):
    c = [None] * 4
    for i, feeds in enumerate(_FEEDS):
        m = product(i)
        for k, sign in feeds:
            c[k] = m if c[k] is None else (c[k] + m if sign > 0 else c[k] - m)
    return c


def _kernel(x_hbm, wqkv_hbm, wo_hbm, w1_hbm, w3_hbm, w2_hbm, out_hbm,
            io_s, x_s, wqkv_raw, wo_raw, wqkv_s, wo_s, w1_raw, w3_raw, w2_raw, up_s, down_s, in_s, out_s,
            qkv_s, xp_s, xa_s, xb_s, o_s, oa_s, h_s, in_sem, qkv_sem, w_sem, up_sem, out_sem):
    S, D = x_s.shape
    F = w3_raw.shape[1]
    TH, DH, FH = TM // 2, D // 2, F // 2
    nb = S // TM
    n_items = 2 * nb
    nc = D // LANES
    scale = (D // N_HEADS) ** -0.5

    def rows(j):
        return pl.ds(j * TM if isinstance(j, int) else pl.multiple_of(j * TM, TM), TM)

    def x_copy(j):
        return pltpu.make_async_copy(x_hbm.at[rows(j)], io_s.at[rows(j)], in_sem.at[j])

    def out_copy(j):
        return pltpu.make_async_copy(io_s.at[rows(j)], out_hbm.at[rows(j)], out_sem.at[j])

    def wqkv_copy(i):
        rr = pl.ds(i * PB if isinstance(i, int) else pl.multiple_of(i * PB, PB), PB)
        return pltpu.make_async_copy(wqkv_hbm.at[rr], wqkv_raw.at[rr], qkv_sem.at[i])

    wo_copy = pltpu.make_async_copy(wo_hbm, wo_raw, w_sem.at[0])
    w2_copy = pltpu.make_async_copy(w2_hbm, w2_raw, w_sem.at[1])

    def up_copies(r):
        return [pltpu.make_async_copy(src.at[chunk(r + h * (DH // PB))], dst.at[chunk(r + h * (DH // PB))],
                                      up_sem.at[4 * r + 2 * m + h])
                for m, (src, dst) in enumerate(((w1_hbm, w1_raw), (w3_hbm, w3_raw))) for h in range(2)]

    def chunk(r):
        return pl.ds(r * PB if isinstance(r, int) else pl.multiple_of(r * PB, PB), PB)

    def permute_qkv_columns(r):
        for i in range(3):
            cols = [pl.ds(i * D + c * LANES, LANES) for c in range(nc)]
            parts = [pltpu.bitcast(wqkv_raw[chunk(r), cc], U32) for cc in cols]
            for cc, part in zip(cols, _swap_bits(parts, ((4, 16), (2, 8), (1, 4)), 1)):
                wqkv_s[_word_rows(r * PB, PB), cc] = part

    def project_partial(r):
        y = _dot(xp_s[:, chunk(r)], _unpack(wqkv_s[_word_rows(r * PB, PB), :]))
        for t in range(3 * nc):
            qkv_s[t, pl.ds(HALO, TM), :] += y[:, t * LANES:(t + 1) * LANES]

    def combine(src, r, c, dst, c_dst, width):
        words = src.dtype == U32
        half_rows, half_cols = src.shape[0] // (1 if words else 2), src.shape[1] // 2
        for r0 in range(0, PB, CB):
            for c0 in range(0, width, CW):
                def load(dr, dc):
                    row, cols = r * PB + dr + r0, pl.ds(pl.multiple_of(c + dc + c0, CW), CW)
                    if words:
                        return src[_word_rows(row, CB), cols]
                    return pltpu.bitcast(src[pl.ds(pl.multiple_of(row, CB), CB), cols], U32)
                blocks = [load(dr, dc) for dr in (0, half_rows) for dc in (0, half_cols)]
                halves = [_right_operands(*[
                    pltpu.unpack_elementwise(w, index=k, packed_dtype=BF16, unpacked_dtype=F32)
                    for w in blocks]) for k in range(2)]
                for i, pair in enumerate(zip(*halves)):
                    packed = pltpu.pack_elementwise(list(pair), packed_dtype=BF16).astype(U32)
                    dst[i, _word_rows(r * PB + r0, CB), pl.ds(pl.multiple_of(c_dst + c0, CW), CW)] = packed

    def combine_up(r):
        @pl.loop(0, FH // FC)
        def _(f):
            for m, w in enumerate((w1_raw, w3_raw)):
                combine(w, r, f * FC, up_s, (2 * f + m) * FC, FC)

    def combine_all(src, dst):
        n_cols = dst.shape[2] // DH

        @pl.loop(0, dst.shape[1] * 2 // PB * n_cols)
        def _(i):
            c = i % n_cols * DH
            combine(src, i // n_cols, c, dst, c, DH)

    def permute_wo_rows():
        def body(hh, carry):
            def tile(h432, d4):
                return pl.ds(pl.multiple_of(h432 * 128 + hh * 32 + d4 * 16, 16), 16)
            src = [[pltpu.bitcast(wo_raw[tile(h, d4), :], U32) for h in range(8)] for d4 in range(2)]
            src = [_swap_bits(p, ((2, 4), (1, 2)), 0) for p in src]
            for d4 in range(2):
                for h in range(8):
                    wo_s[_word_rows(((h & 3) | (d4 << 2)) * 128 + hh * 32 + (h >> 2) * 16, 16), :] = src[d4][h]
            return carry
        jax.lax.fori_loop(0, 4, body, 0)

    def residual(rr, fresh):
        if fresh is None:
            return x_s[rr, :]
        return jnp.where(fresh, io_s[rr, :].astype(F32), x_s[rr, :])

    def normed(j, fresh, r, n):
        x = residual(pl.ds(pl.multiple_of(j * TM + r, n), n), fresh)
        xc = x - jnp.mean(x, axis=-1, keepdims=True)
        var = jnp.mean(xc * xc, axis=-1, keepdims=True)
        return xc * jax.lax.rsqrt(var + EPS)

    def store_left_operands(dst, r, top, bottom):
        ops = _left_operands(top[:, :DH], top[:, DH:], bottom[:, :DH], bottom[:, DH:])
        for i, a in enumerate(ops):
            dst[i, pl.ds(r, top.shape[0]), :] = a.astype(BF16)
        return _token(ops[0], ops[1], ops[4])

    def norm(j, fresh, dst, r, n, plain=None):
        top, bottom = normed(j, fresh, r, n), normed(j, fresh, TH + r, n)
        if plain is not None:
            plain[pl.ds(r, n), :] = top.astype(BF16)
            plain[pl.ds(TH + r, n), :] = bottom.astype(BF16)
        return store_left_operands(dst, r, top, bottom)

    def attention_operands(r, n):
        return store_left_operands(oa_s, r, o_s[pl.ds(r, n), :], o_s[pl.ds(TH + r, n), :])

    def matmul(left, right, width, side_job, never, finish):
        tokens = []
        for p in range(right.shape[2] // width):
            def product(i):
                nonlocal tokens
                m = _dot(_after(left[i], tokens, never), _unpack(right[i, :, pl.ds(p * width, width)]))
                tokens = side_job(7 * p + i)
                return m
            finish(p, _block_product(product))

    def spread(items, i, n):
        return items[i * len(items) // n:(i + 1) * len(items) // n]

    def first_token(t):
        return jnp.broadcast_to(qkv_s[t, pl.ds(HALO, 1), :], (HALO, LANES))

    def project(j, side_job, never):
        per = DH // LANES
        tiles = [[half * 3 * nc // 2 + p * per + c for c in range(per)] for p in range(3) for half in range(2)]
        tails = {t: qkv_s[t, pl.ds(TM, HALO), :] for t in range(nc, 3 * nc)}

        def finish(p, blocks):
            for k, y in enumerate(blocks):
                for c, t in enumerate(tiles[2 * p + k % 2]):
                    yc = y[:, c * LANES:(c + 1) * LANES]
                    qkv_s[t, pl.ds(HALO + k // 2 * TH, TH), :] = yc
                    if t in tails and k < 2:
                        head = jnp.broadcast_to(yc[0:1, :], (HALO, LANES))
                        qkv_s[t, pl.ds(0, HALO), :] = jnp.where(j == 0, head, tails[t])
        matmul(xa_s, in_s, DH, side_job, never, finish)

    def block_slices(j, c, width):
        return [(pl.ds(pl.multiple_of(j * TM + r0, TH), TH), pl.ds(c0 + c, width))
                for r0 in (0, TH) for c0 in (0, DH)]

    def out_project(j, fresh, never):
        def finish(p, blocks):
            for at, y in zip(block_slices(j, 0, DH), blocks):
                x_s[at] = jnp.where(fresh, io_s[at].astype(F32), x_s[at]) + y
        matmul(oa_s, out_s, DH, lambda i: [], never, finish)

    def attention(j, r, n, masked):
        lane = jax.lax.broadcasted_iota(jnp.int32, (n, LANES), 1)
        logits = [None] * WINDOW
        for c in range(nc):
            q = qkv_s[c, pl.ds(HALO + r, n), :]
            for w in range(WINDOW):
                p = q * qkv_s[nc + c, pl.ds(HALO + r - DILATION * w, n), :]
                logits[w] = p if c == 0 else logits[w] + p
        for s in (1, 2):
            logits = [l + jnp.where((lane & s) == 0, pltpu.roll(l, LANES - s, 1), pltpu.roll(l, s, 1))
                      for l in logits]
        logits = [l * scale for l in logits]
        if masked:
            pos = j * TM + r + jax.lax.broadcasted_iota(jnp.int32, (n, LANES), 0)
            logits = [jnp.where(pos >= DILATION * w, l, -1e9) if w else l for w, l in enumerate(logits)]
        m = functools.reduce(jnp.maximum, logits)
        e = [jnp.exp(l - m) for l in logits]
        inv = 1.0 / functools.reduce(jnp.add, e)
        p = [x * inv for x in e]
        outs = []
        for c in range(nc):
            terms = [p[w] * qkv_s[2 * nc + c, pl.ds(HALO + r - DILATION * w, n), :] for w in range(WINDOW)]
            outs.append(functools.reduce(jnp.add, terms))
            o_s[pl.ds(r, n), pl.ds(c * LANES, LANES)] = outs[-1]
        return _token(*outs)

    def ffn_up(side_job, never):
        def finish(f, blocks):
            hidden = []
            for gu in blocks:
                half = 0.5 * gu[:, :FC]
                hidden.append((half + half * jnp.tanh(half)) * gu[:, FC:])
            for i, a in enumerate(_left_operands(*hidden)):
                h_s[i, :, pl.ds(f * FC, FC)] = a.astype(BF16)
        matmul(xb_s, up_s, 2 * FC, side_job, never, finish)

    def ffn_down(j, side_job, never):
        def finish(p, blocks):
            for at, y in zip(block_slices(j, p * NC, NC), blocks):
                y = x_s[at] + y
                x_s[at] = y
                io_s[at] = y.astype(BF16)
        matmul(h_s, down_s, NC, side_job, never, finish)

    def start_in_order(n, copies):
        @pl.loop(0, n)
        def _(i):
            for copy in copies(i):
                copy.start()

    x_copy(0).start()
    start_in_order(D // PB, lambda r: [wqkv_copy(r)])

    last = n_items - 1

    @pl.loop(-2, n_items)
    def _(n):
        j0 = jnp.maximum(n, 0) % nb
        j1 = jnp.maximum(n + 1, 0) % nb
        j2 = (n + 2) % nb
        never = n > n_items

        def side_job(steps, n_slots):
            return lambda i: [step() for step in spread(steps, i, n_slots) if i < n_slots]

        @pl.when(n + 2 < nb)
        def _():
            x_copy(j2).wait()

        @pl.when(n == 0)
        def _():
            @pl.loop(0, DH // PB)
            def _(r):
                for copy in up_copies(r):
                    copy.wait()
                combine_up(r)

        @pl.when(n >= 0)
        def _():
            steps = [functools.partial(attention, j1, r, RB, r < HALO) for r in range(0, TM, RB)]
            ffn_up(side_job(steps, 7 * (FH // FC) - NE1), never)

        @pl.when(n == -1)
        def _():
            @pl.loop(0, TM // RC)
            def _(g):
                attention(j1, pl.multiple_of(g * RC, RC), RC, True)

            wo_copy.wait()
            permute_wo_rows()
            combine_all(wo_s, out_s)
            combine_all(wqkv_s, in_s)
            attention_operands(0, TH)

        @pl.when(n == 0)
        def _():
            w2_copy.wait()
            combine_all(w2_raw, down_s)

        @pl.when(n >= 0)
        def _():
            steps = [functools.partial(attention_operands, r, LB) for r in range(0, TH, LB)]
            steps += [functools.partial(norm, j2, n + 2 < nb, xa_s, r, LB) for r in range(0, TH, LB)]
            ffn_down(j0, side_job(steps, 7 * (DH // NC) - NS2), never)

        @pl.when(n < 0)
        def _():
            norm(j2, n + 2 < nb, xa_s, 0, TH, plain=xp_s)

        @pl.when(n == -2)
        def _():
            x_copy(1).start()
            wo_copy.start()
            x_copy(2).start()
            start_in_order(DH // PB, up_copies)
            w2_copy.start()
            start_in_order(nb - 3, lambda j: [x_copy(j + 3)])
            qkv_s[...] = jnp.zeros(qkv_s.shape, F32)

            n_chunks = D // PB

            @pl.loop(0, n_chunks + 1)
            def _(r):
                @pl.when(r < n_chunks)
                def _():
                    wqkv_copy(r).wait()

                @pl.when(r == 0)
                def _():
                    permute_qkv_columns(0)

                @pl.when(r > 0)
                def _():
                    project_partial(r - 1)
                    permute_qkv_columns(jnp.minimum(r, n_chunks - 1))

            for t in range(nc, 3 * nc):
                qkv_s[t, pl.ds(0, HALO), :] = first_token(t)

        @pl.when(n >= nb)
        def _():
            out_copy(j0).start()

        @pl.when(jnp.logical_and(n >= -1, n < last - 1))
        def _():
            out_project(j1, n + 1 < nb, never)
            project(j2, side_job([functools.partial(norm, j1, None, xb_s, r, LB) for r in range(0, TH, LB)], NS4), never)

        @pl.when(n == last - 1)
        def _():
            @pl.loop(0, D // NC)
            def _(i):
                cols = pl.ds(pl.multiple_of(i * NC, NC), NC)
                x_s[rows(j1), cols] += _dot(o_s[...].astype(BF16), _unpack(wo_s[:, cols]))

            norm(j1, None, xb_s, 0, TH)

    for j in range(nb):
        out_copy(j).wait()


@jax.jit
def pallas_interleave_layers__sliding_local_dilated__glu_gated_swiglu__prompt_kernel(
    A_x: jax.Array,
    A_wqkv: jax.Array,
    A_wo: jax.Array,
    B_x: jax.Array,
    B_w1: jax.Array,
    B_w3: jax.Array,
    B_w2: jax.Array,
):
    del B_x
    B, S, D = A_x.shape
    F = B_w1.shape[1]
    assert B == 1 and D == N_HEADS * 32 == 8 * LANES and S % TM == 0 and S // TM >= 3 and F % (2 * FC) == 0
    nb = S // TM
    nc = D // LANES
    any_spec = pl.BlockSpec(memory_space=pl.ANY)
    out = pl.pallas_call(
        _kernel,
        out_shape=jax.ShapeDtypeStruct((S, D), A_x.dtype),
        in_specs=[any_spec] * 6,
        out_specs=any_spec,
        scratch_shapes=[
            pltpu.VMEM((S, D), BF16),
            pltpu.VMEM((S, D), F32),
            pltpu.VMEM((D, 3 * D), BF16),
            pltpu.VMEM((D, D), BF16),
            pltpu.VMEM((D // 2, 3 * D), U32),
            pltpu.VMEM((D // 2, D), U32),
            pltpu.VMEM((D, F), BF16),
            pltpu.VMEM((D, F), BF16),
            pltpu.VMEM((F, D), BF16),
            pltpu.VMEM((7, D // 4, F), U32),
            pltpu.VMEM((7, F // 4, D // 2), U32),
            pltpu.VMEM((7, D // 4, 3 * D // 2), U32),
            pltpu.VMEM((7, D // 4, D // 2), U32),
            pltpu.VMEM((3 * nc, HALO + TM, LANES), F32),
            pltpu.VMEM((TM, D), BF16),
            pltpu.VMEM((7, TM // 2, D // 2), BF16),
            pltpu.VMEM((7, TM // 2, D // 2), BF16),
            pltpu.VMEM((TM, D), F32),
            pltpu.VMEM((7, TM // 2, D // 2), BF16),
            pltpu.VMEM((7, TM // 2, F // 2), BF16),
            pltpu.SemaphoreType.DMA((nb,)),
            pltpu.SemaphoreType.DMA((D // PB,)),
            pltpu.SemaphoreType.DMA((2,)),
            pltpu.SemaphoreType.DMA((2 * D // PB,)),
            pltpu.SemaphoreType.DMA((nb,)),
        ],
        compiler_params=pltpu.CompilerParams(vmem_limit_bytes=120 * 1024 * 1024),
    )(A_x.reshape(S, D), A_wqkv, A_wo, B_w1, B_w3, B_w2)
    return out.reshape(B, S, D)
```

```python
import functools

import jax
import jax.numpy as jnp
import jax.experimental.pallas as pl
import jax.experimental.pallas.tpu as pltpu

N_HEADS = 32
WINDOW = 8
DILATION = 2
EPS = 1e-5
LANES = 128
HALO = 16

TM = 256
UP_CHUNKS = tuple((t, 1) for t in range(7))
UB = 64
NC = 256
NE1 = 1
NS4 = 20
NS2 = 1
RB = 16
PB = 128
CW = 256
CB = 32
RC = 128
LB = 16

F32 = jnp.float32
BF16 = jnp.bfloat16
U32 = jnp.uint32


def _dot(a, b):
    return jnp.dot(a, b, preferred_element_type=F32)


def _unpack(words):
    return pltpu.bitcast(words, BF16)


def _word_rows(r, n):
    return pl.ds(r // 2 if isinstance(r, int) else pl.multiple_of(r // 2, n // 2), n // 2)


def _token(*vals):
    regs = [pltpu.bitcast(v[r:r + 8, c:c + LANES], U32) for v in vals
            for r in range(0, v.shape[0], 8) for c in range(0, v.shape[1], LANES)]
    return functools.reduce(jnp.bitwise_or, regs)


def _after(x, tokens, never):
    if not tokens:
        return x
    words = pltpu.bitcast(x, U32)
    corner = jnp.where(never, functools.reduce(jnp.bitwise_or, tokens), words[:8, :LANES])
    top = jnp.concatenate([corner, words[:8, LANES:]], axis=1)
    return _unpack(jnp.concatenate([top, words[8:]], axis=0))


def _swap_bit(a, b, stride, axis):
    n = a.shape[axis]
    low = (jax.lax.broadcasted_iota(jnp.int32, a.shape, axis) & stride) == 0
    return (jnp.where(low, a, pltpu.roll(b, stride, axis)),
            jnp.where(low, pltpu.roll(a, n - stride, axis), b))


def _swap_bits(parts, strides, axis):
    parts = list(parts)
    for bit, stride in strides:
        for i in range(len(parts)):
            if not i & bit:
                parts[i], parts[i | bit] = _swap_bit(parts[i], parts[i | bit], stride, axis)
    return parts


def _left_operands(a11, a12, a21, a22):
    return (a11 + a22, a21 + a22, a11, a22, a11 + a12, a21 - a11, a12 - a22)


def _right_operands(b11, b12, b21, b22):
    return (b11 + b22, b11, b12 - b22, b21 - b11, b22, b11 + b12, b21 + b22)


_FEEDS = (((0, 1), (3, 1)), ((2, 1), (3, -1)), ((1, 1), (3, 1)), ((0, 1), (2, 1)),
          ((0, -1), (1, 1)), ((3, 1),), ((0, 1),))


def _block_product(product):
    c = [None] * 4
    for i, feeds in enumerate(_FEEDS):
        m = product(i)
        for k, sign in feeds:
            c[k] = m if c[k] is None else (c[k] + m if sign > 0 else c[k] - m)
    return c


def _twice(operands, grid):
    outer = [operands(*[grid[2 * a + u][2 * b + v] for a in range(2) for b in range(2)])
             for u in range(2) for v in range(2)]
    return [op for quarters in zip(*outer) for op in operands(*quarters)]


def _kernel(x_hbm, wqkv_hbm, wo_hbm, w1_hbm, w3_hbm, w2_hbm, out_hbm,
            io_s, x_s, wqkv_raw, wo_raw, wqkv_s, wo_s, w1_raw, w3_raw, up_s, down_s, in_s, out_s,
            qkv_s, xp_s, xa_s, xb_s, o_s, oa_s, h_s, in_sem, qkv_sem, w_sem, up_sem, out_sem):
    S, D = x_s.shape
    F = w3_raw.shape[1]
    TH, DH, FH = TM // 2, D // 2, F // 2
    TQ, DQ, FQ = TM // 4, D // 4, F // 4
    nb = S // TM
    n_items = 2 * nb
    nc = D // LANES
    scale = (D // N_HEADS) ** -0.5

    def rows(j):
        return pl.ds(j * TM if isinstance(j, int) else pl.multiple_of(j * TM, TM), TM)

    def x_copy(j):
        return pltpu.make_async_copy(x_hbm.at[rows(j)], io_s.at[rows(j)], in_sem.at[j])

    def out_copy(j):
        return pltpu.make_async_copy(io_s.at[rows(j)], out_hbm.at[rows(j)], out_sem.at[j])

    def wqkv_copy(i):
        rr = pl.ds(i * PB if isinstance(i, int) else pl.multiple_of(i * PB, PB), PB)
        return pltpu.make_async_copy(wqkv_hbm.at[rr], wqkv_raw.at[rr], qkv_sem.at[i])

    wo_copy = pltpu.make_async_copy(wo_hbm, wo_raw, w_sem.at[0])
    w2_pieces = [(r0, min(D, FH - r0)) for r0 in range(0, FH, D)]
    w2_copies = [pltpu.make_async_copy(w2_hbm.at[pl.ds(h * FH + r0, n)], dst.at[pl.ds(0, n), pl.ds(r0, D)],
                                       w_sem.at[1 + 2 * k + h])
                 for k, (r0, n) in enumerate(w2_pieces) for h, dst in enumerate((w1_raw, w3_raw))]

    def up_copies(r):
        at = [pl.ds(pl.multiple_of(a * DQ + r * UB, UB), UB) for a in range(4)]
        return [pltpu.make_async_copy(src.at[at[a]], dst.at[at[a]], up_sem.at[8 * r + 4 * m + a])
                for m, (src, dst) in enumerate(((w1_hbm, w1_raw), (w3_hbm, w3_raw))) for a in range(4)]

    def chunk(r):
        return pl.ds(r * PB if isinstance(r, int) else pl.multiple_of(r * PB, PB), PB)

    def permute_qkv_columns(r):
        for i in range(3):
            cols = [pl.ds(i * D + c * LANES, LANES) for c in range(nc)]
            parts = [pltpu.bitcast(wqkv_raw[chunk(r), cc], U32) for cc in cols]
            for cc, part in zip(cols, _swap_bits(parts, ((4, 16), (2, 8), (1, 4)), 1)):
                wqkv_s[_word_rows(r * PB, PB), cc] = part

    def project_partial(r):
        y = _dot(xp_s[:, chunk(r)], _unpack(wqkv_s[_word_rows(r * PB, PB), :]))
        for t in range(3 * nc):
            qkv_s[t, pl.ds(HALO, TM), :] += y[:, t * LANES:(t + 1) * LANES]

    def combine(operands, blocks, store):
        halves = [operands(jax.tree.map(
            lambda w: pltpu.unpack_elementwise(w, index=k, packed_dtype=BF16, unpacked_dtype=F32), blocks))
            for k in range(2)]
        for i, pair in enumerate(zip(*halves)):
            store(i, pltpu.pack_elementwise(list(pair), packed_dtype=BF16).astype(U32))

    def combine_up(r):
        @pl.loop(0, FQ // LANES)
        def _(t):
            for m, w in enumerate((w1_raw, w3_raw)):
                for r0 in range(0, UB, 16):
                    row = r * UB + r0
                    grid = [[pltpu.bitcast(w[pl.ds(pl.multiple_of(a * DQ + row, 16), 16),
                                             pl.ds(pl.multiple_of(b * FQ + t * LANES, LANES), LANES)], U32)
                             for b in range(4)] for a in range(4)]

                    def store(i, words):
                        up_s[i, _word_rows(row, 16), pl.ds(pl.multiple_of((2 * t + m) * LANES, LANES), LANES)] = words
                    combine(functools.partial(_twice, _right_operands), grid, store)

    def combine_down():
        for r0, n in w2_pieces:
            @pl.loop(0, n // CB)
            def _(g):
                for c in range(0, DH, CW):
                    blocks = [pltpu.bitcast(w[pl.ds(pl.multiple_of(g * CB, CB), CB), pl.ds(r0 + dc + c, CW)], U32)
                              for w in (w1_raw, w3_raw) for dc in (0, DH)]

                    def store(i, words):
                        down_s[i, _word_rows(r0 + g * CB, CB), pl.ds(c, CW)] = words
                    combine(lambda b: _right_operands(*b), blocks, store)

    def combine_all(src, dst):
        half_rows, half_cols = src.shape[0], src.shape[1] // 2

        @pl.loop(0, half_rows // CB)
        def _(g):
            for c in range(0, half_cols, CW):
                blocks = [src[_word_rows(g * CB + dr, CB), pl.ds(dc + c, CW)]
                          for dr in (0, half_rows) for dc in (0, half_cols)]

                def store(i, words):
                    dst[i, _word_rows(g * CB, CB), pl.ds(c, CW)] = words
                combine(lambda b: _right_operands(*b), blocks, store)

    def permute_wo_rows():
        def body(hh, carry):
            def tile(h432, d4):
                return pl.ds(pl.multiple_of(h432 * 128 + hh * 32 + d4 * 16, 16), 16)
            src = [[pltpu.bitcast(wo_raw[tile(h, d4), :], U32) for h in range(8)] for d4 in range(2)]
            src = [_swap_bits(p, ((2, 4), (1, 2)), 0) for p in src]
            for d4 in range(2):
                for h in range(8):
                    wo_s[_word_rows(((h & 3) | (d4 << 2)) * 128 + hh * 32 + (h >> 2) * 16, 16), :] = src[d4][h]
            return carry
        jax.lax.fori_loop(0, 4, body, 0)

    def residual(rr, fresh):
        if fresh is None:
            return x_s[rr, :]
        return jnp.where(fresh, io_s[rr, :].astype(F32), x_s[rr, :])

    def normed(j, fresh, r, n):
        x = residual(pl.ds(pl.multiple_of(j * TM + r, n), n), fresh)
        xc = x - jnp.mean(x, axis=-1, keepdims=True)
        var = jnp.mean(xc * xc, axis=-1, keepdims=True)
        return xc * jax.lax.rsqrt(var + EPS)

    def store_left_operands(dst, r, top, bottom):
        ops = _left_operands(top[:, :DH], top[:, DH:], bottom[:, :DH], bottom[:, DH:])
        for i, a in enumerate(ops):
            dst[i, pl.ds(r, top.shape[0]), :] = a.astype(BF16)
        return _token(ops[0], ops[1], ops[4])

    def norm(j, fresh, dst, r, n, plain=None):
        top, bottom = normed(j, fresh, r, n), normed(j, fresh, TH + r, n)
        if plain is not None:
            plain[pl.ds(r, n), :] = top.astype(BF16)
            plain[pl.ds(TH + r, n), :] = bottom.astype(BF16)
        return store_left_operands(dst, r, top, bottom)

    def norm_for_ffn(j, r, n):
        quarters = [normed(j, None, a * TQ + r, n) for a in range(4)]
        ops = _twice(_left_operands, [[y[:, b * DQ:(b + 1) * DQ] for b in range(4)] for y in quarters])
        for i, a in enumerate(ops):
            xb_s[i, pl.ds(r, n), :] = a.astype(BF16)
        return _token(*quarters)

    def attention_operands(r, n):
        return store_left_operands(oa_s, r, o_s[pl.ds(r, n), :], o_s[pl.ds(TH + r, n), :])

    def matmul(left, right, width, side_job, never, finish):
        tokens = []
        for p in range(right.shape[2] // width):
            def product(i):
                nonlocal tokens
                m = _dot(_after(left[i], tokens, never), _unpack(right[i, :, pl.ds(p * width, width)]))
                tokens = side_job(7 * p + i)
                return m
            finish(p, _block_product(product))

    def spread(items, i, n):
        return items[i * len(items) // n:(i + 1) * len(items) // n]

    def first_token(t):
        return jnp.broadcast_to(qkv_s[t, pl.ds(HALO, 1), :], (HALO, LANES))

    def project(j, side_job, never):
        per = DH // LANES
        tiles = [[half * 3 * nc // 2 + p * per + c for c in range(per)] for p in range(3) for half in range(2)]
        tails = {t: qkv_s[t, pl.ds(TM, HALO), :] for t in range(nc, 3 * nc)}

        def finish(p, blocks):
            for k, y in enumerate(blocks):
                for c, t in enumerate(tiles[2 * p + k % 2]):
                    yc = y[:, c * LANES:(c + 1) * LANES]
                    qkv_s[t, pl.ds(HALO + k // 2 * TH, TH), :] = yc
                    if t in tails and k < 2:
                        head = jnp.broadcast_to(yc[0:1, :], (HALO, LANES))
                        qkv_s[t, pl.ds(0, HALO), :] = jnp.where(j == 0, head, tails[t])
        matmul(xa_s, in_s, DH, side_job, never, finish)

    def block_slices(j, c, width):
        return [(pl.ds(pl.multiple_of(j * TM + r0, TH), TH), pl.ds(c0 + c, width))
                for r0 in (0, TH) for c0 in (0, DH)]

    def out_project(j, fresh, never):
        def finish(p, blocks):
            for at, y in zip(block_slices(j, 0, DH), blocks):
                x_s[at] = jnp.where(fresh, io_s[at].astype(F32), x_s[at]) + y
        matmul(oa_s, out_s, DH, lambda i: [], never, finish)

    def attention(j, r, n, masked):
        lane = jax.lax.broadcasted_iota(jnp.int32, (n, LANES), 1)
        logits = [None] * WINDOW
        for c in range(nc):
            q = qkv_s[c, pl.ds(HALO + r, n), :]
            for w in range(WINDOW):
                p = q * qkv_s[nc + c, pl.ds(HALO + r - DILATION * w, n), :]
                logits[w] = p if c == 0 else logits[w] + p
        for s in (1, 2):
            logits = [l + jnp.where((lane & s) == 0, pltpu.roll(l, LANES - s, 1), pltpu.roll(l, s, 1))
                      for l in logits]
        logits = [l * scale for l in logits]
        if masked:
            pos = j * TM + r + jax.lax.broadcasted_iota(jnp.int32, (n, LANES), 0)
            logits = [jnp.where(pos >= DILATION * w, l, -1e9) if w else l for w, l in enumerate(logits)]
        m = functools.reduce(jnp.maximum, logits)
        e = [jnp.exp(l - m) for l in logits]
        inv = 1.0 / functools.reduce(jnp.add, e)
        p = [x * inv for x in e]
        outs = []
        for c in range(nc):
            terms = [p[w] * qkv_s[2 * nc + c, pl.ds(HALO + r - DILATION * w, n), :] for w in range(WINDOW)]
            outs.append(functools.reduce(jnp.add, terms))
            o_s[pl.ds(r, n), pl.ds(c * LANES, LANES)] = outs[-1]
        return _token(*outs)

    def ffn_up(side_job, never):
        tokens = []
        for p, (t0, nt) in enumerate(UP_CHUNKS):
            def outer(i):
                def inner(k):
                    right = up_s[7 * i + k, :, pl.ds(2 * t0 * LANES, 2 * nt * LANES)]
                    return _dot(_after(xb_s[7 * i + k], tokens if k == 0 else [], never), _unpack(right))
                nonlocal tokens
                m = jnp.concatenate(_block_product(inner), axis=0)
                tokens = side_job(7 * p + i)
                return m

            blocks = _block_product(outer)
            for k in range(4):
                for t in range(nt):
                    hidden = []
                    for gu in blocks:
                        g, u = (gu[k * TQ:(k + 1) * TQ, (2 * t + m) * LANES:(2 * t + m + 1) * LANES] for m in range(2))
                        half = 0.5 * g
                        hidden.append((half + half * jnp.tanh(half)) * u)
                    for i, a in enumerate(_left_operands(*hidden)):
                        h_s[i, pl.ds(k // 2 * TQ, TQ), pl.ds(k % 2 * FQ + (t0 + t) * LANES, LANES)] = a.astype(BF16)

    def ffn_down(j, side_job, never):
        def finish(p, blocks):
            for at, y in zip(block_slices(j, p * NC, NC), blocks):
                y = x_s[at] + y
                x_s[at] = y
                io_s[at] = y.astype(BF16)
        matmul(h_s, down_s, NC, side_job, never, finish)

    def start_in_order(n, copies):
        @pl.loop(0, n)
        def _(i):
            for copy in copies(i):
                copy.start()

    x_copy(0).start()
    start_in_order(D // PB, lambda r: [wqkv_copy(r)])

    last = n_items - 1

    @pl.loop(-2, n_items)
    def _(n):
        j0 = jnp.maximum(n, 0) % nb
        j1 = jnp.maximum(n + 1, 0) % nb
        j2 = (n + 2) % nb
        never = n > n_items

        def side_job(steps, n_slots):
            return lambda i: [step() for step in spread(steps, i, n_slots) if i < n_slots]

        @pl.when(n + 2 < nb)
        def _():
            x_copy(j2).wait()

        @pl.when(n == 0)
        def _():
            @pl.loop(0, DQ // UB)
            def _(r):
                for copy in up_copies(r):
                    copy.wait()
                combine_up(r)

            for copy in w2_copies:
                copy.start()

        @pl.when(n >= 0)
        def _():
            steps = [functools.partial(attention, j1, r, RB, r < HALO) for r in range(0, TM, RB)]
            ffn_up(side_job(steps, 7 * len(UP_CHUNKS) - NE1), never)

        @pl.when(n == -1)
        def _():
            @pl.loop(0, TM // RC)
            def _(g):
                attention(j1, pl.multiple_of(g * RC, RC), RC, True)

            wo_copy.wait()
            permute_wo_rows()
            combine_all(wo_s, out_s)
            combine_all(wqkv_s, in_s)
            attention_operands(0, TH)

        @pl.when(n == 0)
        def _():
            for copy in w2_copies:
                copy.wait()
            combine_down()

        @pl.when(n >= 0)
        def _():
            steps = [functools.partial(attention_operands, r, LB) for r in range(0, TH, LB)]
            steps += [functools.partial(norm, j2, n + 2 < nb, xa_s, r, LB) for r in range(0, TH, LB)]
            ffn_down(j0, side_job(steps, 7 * (DH // NC) - NS2), never)

        @pl.when(n < 0)
        def _():
            norm(j2, n + 2 < nb, xa_s, 0, TH, plain=xp_s)

        @pl.when(n == -2)
        def _():
            x_copy(1).start()
            wo_copy.start()
            x_copy(2).start()
            start_in_order(DQ // UB, up_copies)
            start_in_order(nb - 3, lambda j: [x_copy(j + 3)])
            qkv_s[...] = jnp.zeros(qkv_s.shape, F32)

            n_chunks = D // PB

            @pl.loop(0, n_chunks + 1)
            def _(r):
                @pl.when(r < n_chunks)
                def _():
                    wqkv_copy(r).wait()

                @pl.when(r == 0)
                def _():
                    permute_qkv_columns(0)

                @pl.when(r > 0)
                def _():
                    project_partial(r - 1)
                    permute_qkv_columns(jnp.minimum(r, n_chunks - 1))

            for t in range(nc, 3 * nc):
                qkv_s[t, pl.ds(0, HALO), :] = first_token(t)

        @pl.when(n >= nb)
        def _():
            out_copy(j0).start()

        @pl.when(jnp.logical_and(n >= -1, n < last - 1))
        def _():
            out_project(j1, n + 1 < nb, never)
            project(j2, side_job([functools.partial(norm_for_ffn, j1, r, LB) for r in range(0, TQ, LB)], NS4), never)

        @pl.when(n == last - 1)
        def _():
            @pl.loop(0, D // NC)
            def _(i):
                cols = pl.ds(pl.multiple_of(i * NC, NC), NC)
                x_s[rows(j1), cols] += _dot(o_s[...].astype(BF16), _unpack(wo_s[:, cols]))


            @pl.loop(0, TQ // LB)
            def _(g):
                norm_for_ffn(j1, pl.multiple_of(g * LB, LB), LB)

    for j in range(nb):
        out_copy(j).wait()


@jax.jit
def pallas_interleave_layers__sliding_local_dilated__glu_gated_swiglu__prompt_kernel(
    A_x: jax.Array,
    A_wqkv: jax.Array,
    A_wo: jax.Array,
    B_x: jax.Array,
    B_w1: jax.Array,
    B_w3: jax.Array,
    B_w2: jax.Array,
):
    del B_x
    B, S, D = A_x.shape
    F = B_w1.shape[1]
    assert B == 1 and D == N_HEADS * 32 == 8 * LANES and S % TM == 0 and S // TM >= 3 and F == 4 * LANES * sum(n for _, n in UP_CHUNKS)
    nb = S // TM
    nc = D // LANES
    any_spec = pl.BlockSpec(memory_space=pl.ANY)
    out = pl.pallas_call(
        _kernel,
        out_shape=jax.ShapeDtypeStruct((S, D), A_x.dtype),
        in_specs=[any_spec] * 6,
        out_specs=any_spec,
        scratch_shapes=[
            pltpu.VMEM((S, D), BF16),
            pltpu.VMEM((S, D), F32),
            pltpu.VMEM((D, 3 * D), BF16),
            pltpu.VMEM((D, D), BF16),
            pltpu.VMEM((D // 2, 3 * D), U32),
            pltpu.VMEM((D // 2, D), U32),
            pltpu.VMEM((D, F), BF16),
            pltpu.VMEM((D, F), BF16),
            pltpu.VMEM((49, D // 8, F // 2), U32),
            pltpu.VMEM((7, F // 4, D // 2), U32),
            pltpu.VMEM((7, D // 4, 3 * D // 2), U32),
            pltpu.VMEM((7, D // 4, D // 2), U32),
            pltpu.VMEM((3 * nc, HALO + TM, LANES), F32),
            pltpu.VMEM((TM, D), BF16),
            pltpu.VMEM((7, TM // 2, D // 2), BF16),
            pltpu.VMEM((49, TM // 4, D // 4), BF16),
            pltpu.VMEM((TM, D), F32),
            pltpu.VMEM((7, TM // 2, D // 2), BF16),
            pltpu.VMEM((7, TM // 2, F // 2), BF16),
            pltpu.SemaphoreType.DMA((nb,)),
            pltpu.SemaphoreType.DMA((D // PB,)),
            pltpu.SemaphoreType.DMA((5,)),
            pltpu.SemaphoreType.DMA((2 * D // UB,)),
            pltpu.SemaphoreType.DMA((nb,)),
        ],
        compiler_params=pltpu.CompilerParams(vmem_limit_bytes=127 * 1024 * 1024),
    )(A_x.reshape(S, D), A_wqkv, A_wo, B_w1, B_w3, B_w2)
    return out.reshape(B, S, D)
```

```python
import functools

import jax
import jax.numpy as jnp
import jax.experimental.pallas as pl
import jax.experimental.pallas.tpu as pltpu

N_HEADS = 32
WINDOW = 8
DILATION = 2
EPS = 1e-5
LANES = 128
HALO = 16

TM = 256
UP_CHUNKS = tuple((t, 1) for t in range(7))
UB = 64
NC = 256
NE1 = 1
NS4 = 20
NS2 = 1
RB = 16
PB = 128
CW = 256
CB = 32
RC = 128
LB = 16

F32 = jnp.float32
BF16 = jnp.bfloat16
U32 = jnp.uint32


def _dot(a, b):
    return jnp.dot(a, b, preferred_element_type=F32)


def _unpack(words):
    return pltpu.bitcast(words, BF16)


def _word_rows(r, n):
    return pl.ds(r // 2 if isinstance(r, int) else pl.multiple_of(r // 2, n // 2), n // 2)


def _token(*vals):
    regs = [pltpu.bitcast(v[r:r + 8, c:c + LANES], U32) for v in vals
            for r in range(0, v.shape[0], 8) for c in range(0, v.shape[1], LANES)]
    return functools.reduce(jnp.bitwise_or, regs)


def _after(x, tokens, never):
    if not tokens:
        return x
    words = pltpu.bitcast(x, U32)
    corner = jnp.where(never, functools.reduce(jnp.bitwise_or, tokens), words[:8, :LANES])
    top = jnp.concatenate([corner, words[:8, LANES:]], axis=1)
    return _unpack(jnp.concatenate([top, words[8:]], axis=0))


def _swap_bit(a, b, stride, axis):
    n = a.shape[axis]
    low = (jax.lax.broadcasted_iota(jnp.int32, a.shape, axis) & stride) == 0
    return (jnp.where(low, a, pltpu.roll(b, stride, axis)),
            jnp.where(low, pltpu.roll(a, n - stride, axis), b))


def _swap_bits(parts, strides, axis):
    parts = list(parts)
    for bit, stride in strides:
        for i in range(len(parts)):
            if not i & bit:
                parts[i], parts[i | bit] = _swap_bit(parts[i], parts[i | bit], stride, axis)
    return parts


def _left_operands(a11, a12, a21, a22):
    return (a11 + a22, a21 + a22, a11, a22, a11 + a12, a21 - a11, a12 - a22)


def _right_operands(b11, b12, b21, b22):
    return (b11 + b22, b11, b12 - b22, b21 - b11, b22, b11 + b12, b21 + b22)


_FEEDS = (((0, 1), (3, 1)), ((2, 1), (3, -1)), ((1, 1), (3, 1)), ((0, 1), (2, 1)),
          ((0, -1), (1, 1)), ((3, 1),), ((0, 1),))


def _block_product(product):
    c = [None] * 4
    for i, feeds in enumerate(_FEEDS):
        m = product(i)
        for k, sign in feeds:
            c[k] = m if c[k] is None else (c[k] + m if sign > 0 else c[k] - m)
    return c


def _twice(operands, grid):
    outer = [operands(*[grid[2 * a + u][2 * b + v] for a in range(2) for b in range(2)])
             for u in range(2) for v in range(2)]
    return [op for quarters in zip(*outer) for op in operands(*quarters)]


def _kernel(x_hbm, wqkv_hbm, wo_hbm, w1_hbm, w3_hbm, w2_hbm, out_hbm,
            io_s, x_s, wqkv_raw, wo_raw, wqkv_s, wo_s, w1_raw, w3_raw, up_s, down_s, in_s, out_s,
            qkv_s, xp_s, xa_s, xb_s, o_s, oa_s, h_s, in_sem, qkv_sem, w_sem, up_sem, out_sem):
    S, D = x_s.shape
    F = w3_raw.shape[1]
    TH, DH, FH = TM // 2, D // 2, F // 2
    TQ, DQ, FQ = TM // 4, D // 4, F // 4
    nb = S // TM
    n_items = 2 * nb
    nc = D // LANES
    scale = (D // N_HEADS) ** -0.5

    def rows(j):
        return pl.ds(j * TM if isinstance(j, int) else pl.multiple_of(j * TM, TM), TM)

    def x_copy(j):
        return pltpu.make_async_copy(x_hbm.at[rows(j)], io_s.at[rows(j)], in_sem.at[j])

    def out_copy(j):
        return pltpu.make_async_copy(io_s.at[rows(j)], out_hbm.at[rows(j)], out_sem.at[j])

    def wqkv_copy(i):
        rr = pl.ds(i * PB if isinstance(i, int) else pl.multiple_of(i * PB, PB), PB)
        return pltpu.make_async_copy(wqkv_hbm.at[rr], wqkv_raw.at[rr], qkv_sem.at[i])

    wo_copy = pltpu.make_async_copy(wo_hbm, wo_raw, w_sem.at[0])
    w2_pieces = [(r0, min(D, FH - r0)) for r0 in range(0, FH, D)]
    w2_copies = [pltpu.make_async_copy(w2_hbm.at[pl.ds(h * FH + r0, n)], dst.at[pl.ds(0, n), pl.ds(r0, D)],
                                       w_sem.at[1 + 2 * k + h])
                 for k, (r0, n) in enumerate(w2_pieces) for h, dst in enumerate((w1_raw, w3_raw))]

    def up_copies(r):
        at = [pl.ds(pl.multiple_of(a * DQ + r * UB, UB), UB) for a in range(4)]
        return [pltpu.make_async_copy(src.at[at[a]], dst.at[at[a]], up_sem.at[8 * r + 4 * m + a])
                for m, (src, dst) in enumerate(((w1_hbm, w1_raw), (w3_hbm, w3_raw))) for a in range(4)]

    def chunk(r):
        return pl.ds(r * PB if isinstance(r, int) else pl.multiple_of(r * PB, PB), PB)

    def permute_qkv_columns(r):
        for i in range(3):
            cols = [pl.ds(i * D + c * LANES, LANES) for c in range(nc)]
            parts = [pltpu.bitcast(wqkv_raw[chunk(r), cc], U32) for cc in cols]
            for cc, part in zip(cols, _swap_bits(parts, ((4, 16), (2, 8), (1, 4)), 1)):
                wqkv_s[_word_rows(r * PB, PB), cc] = part

    def project_partial(r):
        y = _dot(xp_s[:, chunk(r)], _unpack(wqkv_s[_word_rows(r * PB, PB), :]))
        for t in range(3 * nc):
            qkv_s[t, pl.ds(HALO, TM), :] += y[:, t * LANES:(t + 1) * LANES]

    def combine(operands, blocks, store):
        halves = [operands(jax.tree.map(
            lambda w: pltpu.unpack_elementwise(w, index=k, packed_dtype=BF16, unpacked_dtype=F32), blocks))
            for k in range(2)]
        for i, pair in enumerate(zip(*halves)):
            store(i, pltpu.pack_elementwise(list(pair), packed_dtype=BF16).astype(U32))

    def combine_up(r):
        @pl.loop(0, FQ // LANES)
        def _(t):
            dst = up_s.at[:, _word_rows(r * UB, UB), pl.ds(pl.multiple_of(2 * t * LANES, LANES), 2 * LANES)]
            for m, w in enumerate((w1_raw, w3_raw)):
                src = w.at[pl.ds(pl.multiple_of(r * UB, UB), 3 * DQ + UB),
                           pl.ds(pl.multiple_of(t * LANES, LANES), 3 * FQ + LANES)]
                for r0 in range(0, UB, 16):
                    grid = [[pltpu.bitcast(src[pl.ds(a * DQ + r0, 16), pl.ds(b * FQ, LANES)], U32)
                             for b in range(4)] for a in range(4)]

                    def store(i, words):
                        dst[i, _word_rows(r0, 16), pl.ds(m * LANES, LANES)] = words
                    combine(functools.partial(_twice, _right_operands), grid, store)

    def combine_down():
        for r0, n in w2_pieces:
            @pl.loop(0, n // CB)
            def _(g):
                for c in range(0, DH, CW):
                    blocks = [pltpu.bitcast(w[pl.ds(pl.multiple_of(g * CB, CB), CB), pl.ds(r0 + dc + c, CW)], U32)
                              for w in (w1_raw, w3_raw) for dc in (0, DH)]

                    def store(i, words):
                        down_s[i, _word_rows(r0 + g * CB, CB), pl.ds(c, CW)] = words
                    combine(lambda b: _right_operands(*b), blocks, store)

    def combine_all(src, dst):
        half_rows, half_cols = src.shape[0], src.shape[1] // 2

        @pl.loop(0, half_rows // CB)
        def _(g):
            for c in range(0, half_cols, CW):
                blocks = [src[_word_rows(g * CB + dr, CB), pl.ds(dc + c, CW)]
                          for dr in (0, half_rows) for dc in (0, half_cols)]

                def store(i, words):
                    dst[i, _word_rows(g * CB, CB), pl.ds(c, CW)] = words
                combine(lambda b: _right_operands(*b), blocks, store)

    def permute_wo_rows():
        def body(hh, carry):
            def tile(h432, d4):
                return pl.ds(pl.multiple_of(h432 * 128 + hh * 32 + d4 * 16, 16), 16)
            src = [[pltpu.bitcast(wo_raw[tile(h, d4), :], U32) for h in range(8)] for d4 in range(2)]
            src = [_swap_bits(p, ((2, 4), (1, 2)), 0) for p in src]
            for d4 in range(2):
                for h in range(8):
                    wo_s[_word_rows(((h & 3) | (d4 << 2)) * 128 + hh * 32 + (h >> 2) * 16, 16), :] = src[d4][h]
            return carry
        jax.lax.fori_loop(0, 4, body, 0)

    def residual(rr, fresh):
        if fresh is None:
            return x_s[rr, :]
        return jnp.where(fresh, io_s[rr, :].astype(F32), x_s[rr, :])

    def normed(j, fresh, r, n):
        x = residual(pl.ds(pl.multiple_of(j * TM + r, n), n), fresh)
        xc = x - jnp.mean(x, axis=-1, keepdims=True)
        var = jnp.mean(xc * xc, axis=-1, keepdims=True)
        return xc * jax.lax.rsqrt(var + EPS)

    def store_left_operands(dst, r, top, bottom):
        ops = _left_operands(top[:, :DH], top[:, DH:], bottom[:, :DH], bottom[:, DH:])
        for i, a in enumerate(ops):
            dst[i, pl.ds(r, top.shape[0]), :] = a.astype(BF16)
        return _token(ops[0], ops[1], ops[4])

    def norm(j, fresh, dst, r, n, plain=None):
        top, bottom = normed(j, fresh, r, n), normed(j, fresh, TH + r, n)
        if plain is not None:
            plain[pl.ds(r, n), :] = top.astype(BF16)
            plain[pl.ds(TH + r, n), :] = bottom.astype(BF16)
        return store_left_operands(dst, r, top, bottom)

    def norm_for_ffn(j, r, n):
        quarters = [normed(j, None, a * TQ + r, n) for a in range(4)]
        ops = _twice(_left_operands, [[y[:, b * DQ:(b + 1) * DQ] for b in range(4)] for y in quarters])
        for i, a in enumerate(ops):
            xb_s[i, pl.ds(r, n), :] = a.astype(BF16)
        return _token(*quarters)

    def attention_operands(r, n):
        return store_left_operands(oa_s, r, o_s[pl.ds(r, n), :], o_s[pl.ds(TH + r, n), :])

    def matmul(left, right, width, side_job, never, finish):
        tokens = []
        for p in range(right.shape[2] // width):
            def product(i):
                nonlocal tokens
                m = _dot(_after(left[i], tokens, never), _unpack(right[i, :, pl.ds(p * width, width)]))
                tokens = side_job(7 * p + i)
                return m
            finish(p, _block_product(product))

    def spread(items, i, n):
        return items[i * len(items) // n:(i + 1) * len(items) // n]

    def first_token(t):
        return jnp.broadcast_to(qkv_s[t, pl.ds(HALO, 1), :], (HALO, LANES))

    def project(j, side_job, never):
        per = DH // LANES
        tiles = [[half * 3 * nc // 2 + p * per + c for c in range(per)] for p in range(3) for half in range(2)]
        tails = {t: qkv_s[t, pl.ds(TM, HALO), :] for t in range(nc, 3 * nc)}

        def finish(p, blocks):
            for k, y in enumerate(blocks):
                for c, t in enumerate(tiles[2 * p + k % 2]):
                    yc = y[:, c * LANES:(c + 1) * LANES]
                    qkv_s[t, pl.ds(HALO + k // 2 * TH, TH), :] = yc
                    if t in tails and k < 2:
                        head = jnp.broadcast_to(yc[0:1, :], (HALO, LANES))
                        qkv_s[t, pl.ds(0, HALO), :] = jnp.where(j == 0, head, tails[t])
        matmul(xa_s, in_s, DH, side_job, never, finish)

    def block_slices(j, c, width):
        return [(pl.ds(pl.multiple_of(j * TM + r0, TH), TH), pl.ds(c0 + c, width))
                for r0 in (0, TH) for c0 in (0, DH)]

    def out_project(j, fresh, never):
        def finish(p, blocks):
            for at, y in zip(block_slices(j, 0, DH), blocks):
                x_s[at] = jnp.where(fresh, io_s[at].astype(F32), x_s[at]) + y
        matmul(oa_s, out_s, DH, lambda i: [], never, finish)

    def attention(j, r, n, masked):
        lane = jax.lax.broadcasted_iota(jnp.int32, (n, LANES), 1)
        logits = [None] * WINDOW
        for c in range(nc):
            q = qkv_s[c, pl.ds(HALO + r, n), :]
            for w in range(WINDOW):
                p = q * qkv_s[nc + c, pl.ds(HALO + r - DILATION * w, n), :]
                logits[w] = p if c == 0 else logits[w] + p
        for s in (1, 2):
            logits = [l + jnp.where((lane & s) == 0, pltpu.roll(l, LANES - s, 1), pltpu.roll(l, s, 1))
                      for l in logits]
        logits = [l * scale for l in logits]
        if masked:
            pos = j * TM + r + jax.lax.broadcasted_iota(jnp.int32, (n, LANES), 0)
            logits = [jnp.where(pos >= DILATION * w, l, -1e9) if w else l for w, l in enumerate(logits)]
        m = functools.reduce(jnp.maximum, logits)
        e = [jnp.exp(l - m) for l in logits]
        inv = 1.0 / functools.reduce(jnp.add, e)
        p = [x * inv for x in e]
        outs = []
        for c in range(nc):
            terms = [p[w] * qkv_s[2 * nc + c, pl.ds(HALO + r - DILATION * w, n), :] for w in range(WINDOW)]
            outs.append(functools.reduce(jnp.add, terms))
            o_s[pl.ds(r, n), pl.ds(c * LANES, LANES)] = outs[-1]
        return _token(*outs)

    def ffn_up(side_job, never):
        tokens = []
        for p, (t0, nt) in enumerate(UP_CHUNKS):
            def outer(i):
                def inner(k):
                    right = up_s[7 * i + k, :, pl.ds(2 * t0 * LANES, 2 * nt * LANES)]
                    return _dot(_after(xb_s[7 * i + k], tokens if k == 0 else [], never), _unpack(right))
                nonlocal tokens
                m = jnp.concatenate(_block_product(inner), axis=0)
                tokens = side_job(7 * p + i)
                return m

            blocks = _block_product(outer)
            for k in range(4):
                for t in range(nt):
                    hidden = []
                    for gu in blocks:
                        g, u = (gu[k * TQ:(k + 1) * TQ, (2 * t + m) * LANES:(2 * t + m + 1) * LANES] for m in range(2))
                        half = 0.5 * g
                        hidden.append((half + half * jnp.tanh(half)) * u)
                    for i, a in enumerate(_left_operands(*hidden)):
                        h_s[i, pl.ds(k // 2 * TQ, TQ), pl.ds(k % 2 * FQ + (t0 + t) * LANES, LANES)] = a.astype(BF16)

    def ffn_down(j, side_job, never):
        def finish(p, blocks):
            for at, y in zip(block_slices(j, p * NC, NC), blocks):
                y = x_s[at] + y
                x_s[at] = y
                io_s[at] = y.astype(BF16)
        matmul(h_s, down_s, NC, side_job, never, finish)

    def start_in_order(n, copies):
        @pl.loop(0, n)
        def _(i):
            for copy in copies(i):
                copy.start()

    x_copy(0).start()
    start_in_order(D // PB, lambda r: [wqkv_copy(r)])

    last = n_items - 1

    @pl.loop(-2, n_items)
    def _(n):
        j0 = jnp.maximum(n, 0) % nb
        j1 = jnp.maximum(n + 1, 0) % nb
        j2 = (n + 2) % nb
        never = n > n_items

        def side_job(steps, n_slots):
            return lambda i: [step() for step in spread(steps, i, n_slots) if i < n_slots]

        @pl.when(n + 2 < nb)
        def _():
            x_copy(j2).wait()

        @pl.when(n == 0)
        def _():
            @pl.loop(0, DQ // UB)
            def _(r):
                for copy in up_copies(r):
                    copy.wait()
                combine_up(r)

            for copy in w2_copies:
                copy.start()

        @pl.when(n >= 0)
        def _():
            steps = [functools.partial(attention, j1, r, RB, r < HALO) for r in range(0, TM, RB)]
            ffn_up(side_job(steps, 7 * len(UP_CHUNKS) - NE1), never)

        @pl.when(n == -1)
        def _():
            @pl.loop(0, TM // RC)
            def _(g):
                attention(j1, pl.multiple_of(g * RC, RC), RC, True)

            wo_copy.wait()
            permute_wo_rows()
            combine_all(wo_s, out_s)
            combine_all(wqkv_s, in_s)
            attention_operands(0, TH)

        @pl.when(n == 0)
        def _():
            for copy in w2_copies:
                copy.wait()
            combine_down()

        @pl.when(n >= 0)
        def _():
            steps = [functools.partial(attention_operands, r, LB) for r in range(0, TH, LB)]
            steps += [functools.partial(norm, j2, n + 2 < nb, xa_s, r, LB) for r in range(0, TH, LB)]
            ffn_down(j0, side_job(steps, 7 * (DH // NC) - NS2), never)

        @pl.when(n < 0)
        def _():
            norm(j2, n + 2 < nb, xa_s, 0, TH, plain=xp_s)

        @pl.when(n == -2)
        def _():
            x_copy(1).start()
            wo_copy.start()
            x_copy(2).start()
            start_in_order(DQ // UB, up_copies)
            start_in_order(nb - 3, lambda j: [x_copy(j + 3)])
            qkv_s[...] = jnp.zeros(qkv_s.shape, F32)

            n_chunks = D // PB

            @pl.loop(0, n_chunks + 1)
            def _(r):
                @pl.when(r < n_chunks)
                def _():
                    wqkv_copy(r).wait()

                @pl.when(r == 0)
                def _():
                    permute_qkv_columns(0)

                @pl.when(r > 0)
                def _():
                    project_partial(r - 1)
                    permute_qkv_columns(jnp.minimum(r, n_chunks - 1))

            for t in range(nc, 3 * nc):
                qkv_s[t, pl.ds(0, HALO), :] = first_token(t)

        @pl.when(n >= nb)
        def _():
            out_copy(j0).start()

        @pl.when(jnp.logical_and(n >= -1, n < last - 1))
        def _():
            out_project(j1, n + 1 < nb, never)
            project(j2, side_job([functools.partial(norm_for_ffn, j1, r, LB) for r in range(0, TQ, LB)], NS4), never)

        @pl.when(n == last - 1)
        def _():
            @pl.loop(0, D // NC)
            def _(i):
                cols = pl.ds(pl.multiple_of(i * NC, NC), NC)
                x_s[rows(j1), cols] += _dot(o_s[...].astype(BF16), _unpack(wo_s[:, cols]))


            @pl.loop(0, TQ // LB)
            def _(g):
                norm_for_ffn(j1, pl.multiple_of(g * LB, LB), LB)

    for j in range(nb):
        out_copy(j).wait()


@jax.jit
def pallas_interleave_layers__sliding_local_dilated__glu_gated_swiglu__prompt_kernel(
    A_x: jax.Array,
    A_wqkv: jax.Array,
    A_wo: jax.Array,
    B_x: jax.Array,
    B_w1: jax.Array,
    B_w3: jax.Array,
    B_w2: jax.Array,
):
    del B_x
    B, S, D = A_x.shape
    F = B_w1.shape[1]
    assert B == 1 and D == N_HEADS * 32 == 8 * LANES and S % TM == 0 and S // TM >= 3 and F == 4 * LANES * sum(n for _, n in UP_CHUNKS)
    nb = S // TM
    nc = D // LANES
    any_spec = pl.BlockSpec(memory_space=pl.ANY)
    out = pl.pallas_call(
        _kernel,
        out_shape=jax.ShapeDtypeStruct((S, D), A_x.dtype),
        in_specs=[any_spec] * 6,
        out_specs=any_spec,
        scratch_shapes=[
            pltpu.VMEM((S, D), BF16),
            pltpu.VMEM((S, D), F32),
            pltpu.VMEM((D, 3 * D), BF16),
            pltpu.VMEM((D, D), BF16),
            pltpu.VMEM((D // 2, 3 * D), U32),
            pltpu.VMEM((D // 2, D), U32),
            pltpu.VMEM((D, F), BF16),
            pltpu.VMEM((D, F), BF16),
            pltpu.VMEM((49, D // 8, F // 2), U32),
            pltpu.VMEM((7, F // 4, D // 2), U32),
            pltpu.VMEM((7, D // 4, 3 * D // 2), U32),
            pltpu.VMEM((7, D // 4, D // 2), U32),
            pltpu.VMEM((3 * nc, HALO + TM, LANES), F32),
            pltpu.VMEM((TM, D), BF16),
            pltpu.VMEM((7, TM // 2, D // 2), BF16),
            pltpu.VMEM((49, TM // 4, D // 4), BF16),
            pltpu.VMEM((TM, D), F32),
            pltpu.VMEM((7, TM // 2, D // 2), BF16),
            pltpu.VMEM((7, TM // 2, F // 2), BF16),
            pltpu.SemaphoreType.DMA((nb,)),
            pltpu.SemaphoreType.DMA((D // PB,)),
            pltpu.SemaphoreType.DMA((5,)),
            pltpu.SemaphoreType.DMA((2 * D // UB,)),
            pltpu.SemaphoreType.DMA((nb,)),
        ],
        compiler_params=pltpu.CompilerParams(vmem_limit_bytes=127 * 1024 * 1024),
    )(A_x.reshape(S, D), A_wqkv, A_wo, B_w1, B_w3, B_w2)
    return out.reshape(B, S, D)
```

```python
import functools

import jax
import jax.numpy as jnp
import jax.experimental.pallas as pl
import jax.experimental.pallas.tpu as pltpu

N_HEADS = 32
WINDOW = 8
DILATION = 2
EPS = 1e-5
LANES = 128
HALO = 16

TM = 256
UB = 64
NC = 256
NS4 = 20
NA2 = 0
NE1 = 7
NS2 = 14
RB = 16
PB = 128
CW = 256
CB = 16
RC = 128
LB = 16

F32 = jnp.float32
BF16 = jnp.bfloat16
U32 = jnp.uint32


def _dot(a, b):
    return jnp.dot(a, b, preferred_element_type=F32)


def _unpack(words):
    return pltpu.bitcast(words, BF16)


def _word_rows(r, n):
    return pl.ds(r // 2 if isinstance(r, int) else pl.multiple_of(r // 2, n // 2), n // 2)


def _token(*vals):
    regs = [pltpu.bitcast(v[r:r + 8, c:c + LANES], U32) for v in vals
            for r in range(0, v.shape[0], 8) for c in range(0, v.shape[1], LANES)]
    return functools.reduce(jnp.bitwise_or, regs)


def _after(x, tokens, never):
    if not tokens:
        return x
    words = pltpu.bitcast(x, U32)
    corner = jnp.where(never, functools.reduce(jnp.bitwise_or, tokens), words[:8, :LANES])
    top = jnp.concatenate([corner, words[:8, LANES:]], axis=1)
    return _unpack(jnp.concatenate([top, words[8:]], axis=0))


def _swap_bit(a, b, stride, axis):
    n = a.shape[axis]
    low = (jax.lax.broadcasted_iota(jnp.int32, a.shape, axis) & stride) == 0
    return (jnp.where(low, a, pltpu.roll(b, stride, axis)),
            jnp.where(low, pltpu.roll(a, n - stride, axis), b))


def _swap_bits(parts, strides, axis):
    parts = list(parts)
    for bit, stride in strides:
        for i in range(len(parts)):
            if not i & bit:
                parts[i], parts[i | bit] = _swap_bit(parts[i], parts[i | bit], stride, axis)
    return parts


def _left_operands(a11, a12, a21, a22):
    return (a11 + a22, a21 + a22, a11, a22, a11 + a12, a21 - a11, a12 - a22)


def _right_operands(b11, b12, b21, b22):
    return (b11 + b22, b11, b12 - b22, b21 - b11, b22, b11 + b12, b21 + b22)


_FEEDS = (((0, 1), (3, 1)), ((2, 1), (3, -1)), ((1, 1), (3, 1)), ((0, 1), (2, 1)),
          ((0, -1), (1, 1)), ((3, 1),), ((0, 1),))


def _block_product(product):
    c = [None] * 4
    for i, feeds in enumerate(_FEEDS):
        m = product(i)
        for k, sign in feeds:
            c[k] = m if c[k] is None else (c[k] + m if sign > 0 else c[k] - m)
    return c


def _twice(operands, grid):
    outer = [operands(*[grid[2 * a + u][2 * b + v] for a in range(2) for b in range(2)])
             for u in range(2) for v in range(2)]
    return [op for quarters in zip(*outer) for op in operands(*quarters)]


def _kernel(x_hbm, wqkv_hbm, wo_hbm, w1_hbm, w3_hbm, w2_hbm, out_hbm,
            io_s, x_s, wqkv_raw, wo_raw, wqkv_s, wo_s, w1_raw, w3_raw, up_s, down_s, in_s, out_s,
            qkv_s, xp_s, xa_s, o_s, oa_s, in_sem, qkv_sem, w_sem, up_sem, out_sem):
    S, D = x_s.shape
    F = w3_raw.shape[1]
    TH, DH, FH = TM // 2, D // 2, F // 2
    TQ, DQ, FQ = TM // 4, D // 4, F // 4
    nb = S // TM
    n_items = 2 * nb
    nc = D // LANES
    scale = (D // N_HEADS) ** -0.5

    def slots(ref, n_rows, n_cols):
        return [ref.at[pl.ds(r, n_rows), pl.ds(c, n_cols)]
                for r in range(0, ref.shape[0] - n_rows + 1, n_rows)
                for c in range(0, ref.shape[1] - n_cols + 1, n_cols)]

    wo_slots = slots(wo_raw, TQ, DQ)
    xb_ops = wo_slots[4:4 + 49]
    h_ops = (slots(wqkv_raw, TQ, FQ) + slots(wo_raw, TQ, FQ)[:1])[:49]
    down_ops = slots(wqkv_s, FQ // 2, DQ) + slots(down_s, FQ // 2, DQ)
    assert len(xb_ops) == len(h_ops) == len(down_ops) == 49

    def rows(j):
        return pl.ds(j * TM if isinstance(j, int) else pl.multiple_of(j * TM, TM), TM)

    def x_copy(j):
        return pltpu.make_async_copy(x_hbm.at[rows(j)], io_s.at[rows(j)], in_sem.at[j])

    def out_copy(j):
        return pltpu.make_async_copy(io_s.at[rows(j)], out_hbm.at[rows(j)], out_sem.at[j])

    def wqkv_copy(i):
        rr = pl.ds(i * PB if isinstance(i, int) else pl.multiple_of(i * PB, PB), PB)
        return pltpu.make_async_copy(wqkv_hbm.at[rr], wqkv_raw.at[rr], qkv_sem.at[i])

    wo_copy = pltpu.make_async_copy(wo_hbm, wo_raw, w_sem.at[0])
    w2_quarters = [w.at[pl.ds(0, FQ), pl.ds(c, D)] for w in (w1_raw, w3_raw) for c in (0, D)]
    w2_copies = [pltpu.make_async_copy(w2_hbm.at[pl.ds(a * FQ, FQ)], dst, w_sem.at[1 + a])
                 for a, dst in enumerate(w2_quarters)]

    def up_copies(r):
        at = [pl.ds(pl.multiple_of(a * DQ + r * UB, UB), UB) for a in range(4)]
        return [pltpu.make_async_copy(src.at[at[a]], dst.at[at[a]], up_sem.at[8 * r + 4 * m + a])
                for m, (src, dst) in enumerate(((w1_hbm, w1_raw), (w3_hbm, w3_raw))) for a in range(4)]

    def chunk(r):
        return pl.ds(r * PB if isinstance(r, int) else pl.multiple_of(r * PB, PB), PB)

    def permute_qkv_columns(r):
        for i in range(3):
            cols = [pl.ds(i * D + c * LANES, LANES) for c in range(nc)]
            parts = [pltpu.bitcast(wqkv_raw[chunk(r), cc], U32) for cc in cols]
            for cc, part in zip(cols, _swap_bits(parts, ((4, 16), (2, 8), (1, 4)), 1)):
                wqkv_s[_word_rows(r * PB, PB), cc] = part

    def project_partial(r):
        y = _dot(xp_s[:, chunk(r)], _unpack(wqkv_s[_word_rows(r * PB, PB), :]))
        for t in range(3 * nc):
            qkv_s[t, pl.ds(HALO, TM), :] += y[:, t * LANES:(t + 1) * LANES]

    def combine(operands, blocks, store):
        halves = [operands(jax.tree.map(
            lambda w: pltpu.unpack_elementwise(w, index=k, packed_dtype=BF16, unpacked_dtype=F32), blocks))
            for k in range(2)]
        for i, pair in enumerate(zip(*halves)):
            store(i, pltpu.pack_elementwise(list(pair), packed_dtype=BF16).astype(U32))

    def combine_up(r):
        @pl.loop(0, FQ // LANES)
        def _(t):
            dst = up_s.at[:, _word_rows(r * UB, UB), pl.ds(pl.multiple_of(2 * t * LANES, LANES), 2 * LANES)]
            for m, w in enumerate((w1_raw, w3_raw)):
                src = w.at[pl.ds(pl.multiple_of(r * UB, UB), 3 * DQ + UB),
                           pl.ds(pl.multiple_of(t * LANES, LANES), 3 * FQ + LANES)]
                for r0 in range(0, UB, 16):
                    grid = [[pltpu.bitcast(src[pl.ds(a * DQ + r0, 16), pl.ds(b * FQ, LANES)], U32)
                             for b in range(4)] for a in range(4)]

                    def store(i, words):
                        dst[i, _word_rows(r0, 16), pl.ds(m * LANES, LANES)] = words
                    combine(functools.partial(_twice, _right_operands), grid, store)

    def combine_down():
        @pl.loop(0, FQ // CB)
        def _(g):
            for c in range(0, DQ, LANES):
                grid = [[pltpu.bitcast(w[pl.ds(pl.multiple_of(g * CB, CB), CB), pl.ds(b * DQ + c, LANES)], U32)
                         for b in range(4)] for w in w2_quarters]

                def store(i, words):
                    down_ops[i][_word_rows(g * CB, CB), pl.ds(c, LANES)] = words
                combine(functools.partial(_twice, _right_operands), grid, store)

    def combine_all(src, dst):
        half_rows, half_cols = src.shape[0], src.shape[1] // 2

        @pl.loop(0, half_rows // CB)
        def _(g):
            for c in range(0, half_cols, CW):
                blocks = [src[_word_rows(g * CB + dr, CB), pl.ds(dc + c, CW)]
                          for dr in (0, half_rows) for dc in (0, half_cols)]

                def store(i, words):
                    dst[i, _word_rows(g * CB, CB), pl.ds(c, CW)] = words
                combine(lambda b: _right_operands(*b), blocks, store)

    def permute_wo_rows():
        def body(hh, carry):
            def tile(h432, d4):
                return pl.ds(pl.multiple_of(h432 * 128 + hh * 32 + d4 * 16, 16), 16)
            src = [[pltpu.bitcast(wo_raw[tile(h, d4), :], U32) for h in range(8)] for d4 in range(2)]
            src = [_swap_bits(p, ((2, 4), (1, 2)), 0) for p in src]
            for d4 in range(2):
                for h in range(8):
                    wo_s[_word_rows(((h & 3) | (d4 << 2)) * 128 + hh * 32 + (h >> 2) * 16, 16), :] = src[d4][h]
            return carry
        jax.lax.fori_loop(0, 4, body, 0)

    def residual(rr, fresh):
        if fresh is None:
            return x_s[rr, :]
        return jnp.where(fresh, io_s[rr, :].astype(F32), x_s[rr, :])

    def normed(j, fresh, r, n):
        x = residual(pl.ds(pl.multiple_of(j * TM + r, n), n), fresh)
        xc = x - jnp.mean(x, axis=-1, keepdims=True)
        var = jnp.mean(xc * xc, axis=-1, keepdims=True)
        return xc * jax.lax.rsqrt(var + EPS)

    def store_left_operands(dst, r, top, bottom):
        ops = _left_operands(top[:, :DH], top[:, DH:], bottom[:, :DH], bottom[:, DH:])
        for i, a in enumerate(ops):
            dst[i, pl.ds(r, top.shape[0]), :] = a.astype(BF16)
        return _token(ops[0], ops[1], ops[4])

    def norm(j, fresh, dst, r, n, plain=None):
        top, bottom = normed(j, fresh, r, n), normed(j, fresh, TH + r, n)
        if plain is not None:
            plain[pl.ds(r, n), :] = top.astype(BF16)
            plain[pl.ds(TH + r, n), :] = bottom.astype(BF16)
        return store_left_operands(dst, r, top, bottom)

    def norm_for_ffn(j, r, n):
        quarters = [normed(j, None, a * TQ + r, n) for a in range(4)]
        ops = _twice(_left_operands, [[y[:, b * DQ:(b + 1) * DQ] for b in range(4)] for y in quarters])
        for i, a in enumerate(ops):
            xb_ops[i][pl.ds(r, n), :] = a.astype(BF16)
        return _token(*quarters)

    def attention_operands(r, n):
        return store_left_operands(oa_s, r, o_s[pl.ds(r, n), :], o_s[pl.ds(TH + r, n), :])

    def matmul(left, right, width, side_job, never, finish):
        tokens = []
        for p in range(right.shape[2] // width):
            def product(i):
                nonlocal tokens
                m = _dot(_after(left[i], tokens, never), _unpack(right[i, :, pl.ds(p * width, width)]))
                tokens = side_job(7 * p + i)
                return m
            finish(p, _block_product(product))

    def spread(items, i, n):
        return items[i * len(items) // n:(i + 1) * len(items) // n]

    def first_token(t):
        return jnp.broadcast_to(qkv_s[t, pl.ds(HALO, 1), :], (HALO, LANES))

    def project(j, side_job, never):
        per = DH // LANES
        tiles = [[half * 3 * nc // 2 + p * per + c for c in range(per)] for p in range(3) for half in range(2)]
        tails = {t: qkv_s[t, pl.ds(TM, HALO), :] for t in range(nc, 3 * nc)}

        def finish(p, blocks):
            for k, y in enumerate(blocks):
                for c, t in enumerate(tiles[2 * p + k % 2]):
                    yc = y[:, c * LANES:(c + 1) * LANES]
                    qkv_s[t, pl.ds(HALO + k // 2 * TH, TH), :] = yc
                    if t in tails and k < 2:
                        head = jnp.broadcast_to(yc[0:1, :], (HALO, LANES))
                        qkv_s[t, pl.ds(0, HALO), :] = jnp.where(j == 0, head, tails[t])
        matmul(xa_s, in_s, DH, side_job, never, finish)

    def out_project(j, fresh, never):
        def finish(p, blocks):
            for k, y in enumerate(blocks):
                at = (pl.ds(pl.multiple_of(j * TM + k // 2 * TH, TH), TH), pl.ds(k % 2 * DH, DH))
                x_s[at] = jnp.where(fresh, io_s[at].astype(F32), x_s[at]) + y
        matmul(oa_s, out_s, DH, lambda i: [], never, finish)

    def attention(j, r, n, masked):
        lane = jax.lax.broadcasted_iota(jnp.int32, (n, LANES), 1)
        logits = [None] * WINDOW
        for c in range(nc):
            q = qkv_s[c, pl.ds(HALO + r, n), :]
            for w in range(WINDOW):
                p = q * qkv_s[nc + c, pl.ds(HALO + r - DILATION * w, n), :]
                logits[w] = p if c == 0 else logits[w] + p
        for s in (1, 2):
            logits = [l + jnp.where((lane & s) == 0, pltpu.roll(l, LANES - s, 1), pltpu.roll(l, s, 1))
                      for l in logits]
        logits = [l * scale for l in logits]
        if masked:
            pos = j * TM + r + jax.lax.broadcasted_iota(jnp.int32, (n, LANES), 0)
            logits = [jnp.where(pos >= DILATION * w, l, -1e9) if w else l for w, l in enumerate(logits)]
        m = functools.reduce(jnp.maximum, logits)
        e = [jnp.exp(l - m) for l in logits]
        inv = 1.0 / functools.reduce(jnp.add, e)
        p = [x * inv for x in e]
        outs = []
        for c in range(nc):
            terms = [p[w] * qkv_s[2 * nc + c, pl.ds(HALO + r - DILATION * w, n), :] for w in range(WINDOW)]
            outs.append(functools.reduce(jnp.add, terms))
            o_s[pl.ds(r, n), pl.ds(c * LANES, LANES)] = outs[-1]
        return _token(*outs)

    def matmul_twice(left, right, side_job, never, tokens):
        def outer(i):
            def inner(k):
                nonlocal tokens
                m = _dot(_after(left(7 * i + k), tokens, never), _unpack(right(7 * i + k)))
                tokens = side_job(7 * i + k)
                return m
            return jnp.concatenate(_block_product(inner), axis=0)

        c = _block_product(outer)
        return [[c[a // 2 * 2 + b // 2][(a % 2 * 2 + b % 2) * TQ:][:TQ] for b in range(4)]
                for a in range(4)], tokens

    def ffn_up(side_job, never):
        tokens = []
        for t in range(FQ // LANES):
            grid, tokens = matmul_twice(lambda i: xb_ops[i][...],
                                        lambda i: up_s[i, :, pl.ds(2 * t * LANES, 2 * LANES)],
                                        lambda i: side_job(49 * t + i), never, tokens)

            def swiglu(gu):
                half = 0.5 * gu[:, :LANES]
                return (half + half * jnp.tanh(half)) * gu[:, LANES:]
            for i, a in enumerate(_twice(_left_operands, jax.tree.map(swiglu, grid))):
                h_ops[i][:, pl.ds(t * LANES, LANES)] = a.astype(BF16)

    def ffn_down(j, side_job, never):
        grid, _ = matmul_twice(lambda i: h_ops[i][...], lambda i: down_ops[i][...], side_job, never, [])
        for a in range(4):
            for b in range(4):
                at = (pl.ds(pl.multiple_of(j * TM + a * TQ, TQ), TQ), pl.ds(b * DQ, DQ))
                y = x_s[at] + grid[a][b]
                x_s[at] = y
                io_s[at] = y.astype(BF16)

    def start_in_order(n, copies):
        @pl.loop(0, n)
        def _(i):
            for copy in copies(i):
                copy.start()

    x_copy(0).start()
    start_in_order(D // PB, lambda r: [wqkv_copy(r)])

    last = n_items - 1

    @pl.loop(-2, n_items)
    def _(n):
        j0 = jnp.maximum(n, 0) % nb
        j1 = jnp.maximum(n + 1, 0) % nb
        j2 = (n + 2) % nb
        never = n > n_items

        att = [functools.partial(attention, j1, r, RB, r < HALO) for r in range(0, TM, RB)]

        def side_job(steps, n_slots):
            return lambda i: [step() for step in spread(steps, i, n_slots) if i < n_slots]

        @pl.when(n + 2 < nb)
        def _():
            x_copy(j2).wait()

        @pl.when(n == 0)
        def _():
            @pl.loop(0, DQ // UB)
            def _(r):
                for copy in up_copies(r):
                    copy.wait()
                combine_up(r)

            for copy in w2_copies:
                copy.start()

        @pl.when(n >= 0)
        def _():
            ffn_up(side_job(att[:len(att) - NA2], 49 * (FQ // LANES) - NE1), never)

        @pl.when(n == -1)
        def _():
            @pl.loop(0, TM // RC)
            def _(g):
                attention(j1, pl.multiple_of(g * RC, RC), RC, True)

            wo_copy.wait()
            permute_wo_rows()
            combine_all(wo_s, out_s)
            combine_all(wqkv_s, in_s)
            attention_operands(0, TH)

        @pl.when(n == 0)
        def _():
            for copy in w2_copies:
                copy.wait()
            combine_down()

        @pl.when(n >= 0)
        def _():
            steps = att[len(att) - NA2:]
            steps += [functools.partial(norm, j2, n + 2 < nb, xa_s, r, LB) for r in range(0, TH, LB)]
            steps += [functools.partial(attention_operands, r, LB) for r in range(0, TH, LB)]
            ffn_down(j0, side_job(steps, 49 - NS2), never)

        @pl.when(n < 0)
        def _():
            norm(j2, n + 2 < nb, xa_s, 0, TH, plain=xp_s)

        @pl.when(n == -2)
        def _():
            x_copy(1).start()
            wo_copy.start()
            x_copy(2).start()
            start_in_order(DQ // UB, up_copies)
            start_in_order(nb - 3, lambda j: [x_copy(j + 3)])
            qkv_s[...] = jnp.zeros(qkv_s.shape, F32)

            n_chunks = D // PB

            @pl.loop(0, n_chunks + 1)
            def _(r):
                @pl.when(r < n_chunks)
                def _():
                    wqkv_copy(r).wait()

                @pl.when(r == 0)
                def _():
                    permute_qkv_columns(0)

                @pl.when(r > 0)
                def _():
                    project_partial(r - 1)
                    permute_qkv_columns(jnp.minimum(r, n_chunks - 1))

            for t in range(nc, 3 * nc):
                qkv_s[t, pl.ds(0, HALO), :] = first_token(t)

        @pl.when(n >= nb)
        def _():
            out_copy(j0).start()

        @pl.when(jnp.logical_and(n >= -1, n < last - 1))
        def _():
            out_project(j1, n + 1 < nb, never)
            project(j2, side_job([functools.partial(norm_for_ffn, j1, r, LB) for r in range(0, TQ, LB)], NS4), never)

        @pl.when(n == last - 1)
        def _():
            @pl.loop(0, D // NC)
            def _(i):
                cols = pl.ds(pl.multiple_of(i * NC, NC), NC)
                x_s[rows(j1), cols] += _dot(o_s[...].astype(BF16), _unpack(wo_s[:, cols]))


            @pl.loop(0, TQ // LB)
            def _(g):
                norm_for_ffn(j1, pl.multiple_of(g * LB, LB), LB)

    for j in range(nb):
        out_copy(j).wait()


@jax.jit
def pallas_interleave_layers__sliding_local_dilated__glu_gated_swiglu__prompt_kernel(
    A_x: jax.Array,
    A_wqkv: jax.Array,
    A_wo: jax.Array,
    B_x: jax.Array,
    B_w1: jax.Array,
    B_w3: jax.Array,
    B_w2: jax.Array,
):
    del B_x
    B, S, D = A_x.shape
    F = B_w1.shape[1]
    assert B == 1 and D == N_HEADS * 32 == 8 * LANES and S % TM == 0 and S // TM >= 3 and F == 28 * LANES
    nb = S // TM
    nc = D // LANES
    any_spec = pl.BlockSpec(memory_space=pl.ANY)
    out = pl.pallas_call(
        _kernel,
        out_shape=jax.ShapeDtypeStruct((S, D), A_x.dtype),
        in_specs=[any_spec] * 6,
        out_specs=any_spec,
        scratch_shapes=[
            pltpu.VMEM((S, D), BF16),
            pltpu.VMEM((S, D), F32),
            pltpu.VMEM((D, 3 * D), BF16),
            pltpu.VMEM((D, D), BF16),
            pltpu.VMEM((D // 2, 3 * D), U32),
            pltpu.VMEM((D // 2, D), U32),
            pltpu.VMEM((D, F), BF16),
            pltpu.VMEM((D, F), BF16),
            pltpu.VMEM((49, D // 8, F // 2), U32),
            pltpu.VMEM((F // 8, (49 - 12) * D // 4), U32),
            pltpu.VMEM((7, D // 4, 3 * D // 2), U32),
            pltpu.VMEM((7, D // 4, D // 2), U32),
            pltpu.VMEM((3 * nc, HALO + TM, LANES), F32),
            pltpu.VMEM((TM, D), BF16),
            pltpu.VMEM((7, TM // 2, D // 2), BF16),
            pltpu.VMEM((TM, D), F32),
            pltpu.VMEM((7, TM // 2, D // 2), BF16),
            pltpu.SemaphoreType.DMA((nb,)),
            pltpu.SemaphoreType.DMA((D // PB,)),
            pltpu.SemaphoreType.DMA((5,)),
            pltpu.SemaphoreType.DMA((2 * D // UB,)),
            pltpu.SemaphoreType.DMA((nb,)),
        ],
        compiler_params=pltpu.CompilerParams(vmem_limit_bytes=127 * 1024 * 1024),
    )(A_x.reshape(S, D), A_wqkv, A_wo, B_w1, B_w3, B_w2)
    return out.reshape(B, S, D)
```

```python
import functools

import jax
import jax.numpy as jnp
import jax.experimental.pallas as pl
import jax.experimental.pallas.tpu as pltpu

N_HEADS = 32
WINDOW = 8
DILATION = 2
EPS = 1e-5
LANES = 128
HALO = 16

TM = 256
UB = 64
NC = 256
NS4 = 20
AT0 = (6, 20, 34, 48)
AT1 = (13, 34)
NS2 = 14
RB = 16
PB = 128
CW = 256
CB = 16
RC = 128
LB = 16

F32 = jnp.float32
BF16 = jnp.bfloat16
U32 = jnp.uint32


def _dot(a, b):
    return jnp.dot(a, b, preferred_element_type=F32)


def _unpack(words):
    return pltpu.bitcast(words, BF16)


def _word_rows(r, n):
    return pl.ds(r // 2 if isinstance(r, int) else pl.multiple_of(r // 2, n // 2), n // 2)


def _token(*vals):
    regs = [pltpu.bitcast(v[r:r + 8, c:c + LANES], U32) for v in vals
            for r in range(0, v.shape[0], 8) for c in range(0, v.shape[1], LANES)]
    return functools.reduce(jnp.bitwise_or, regs)


def _after(x, tokens, never):
    if not tokens:
        return x
    words = pltpu.bitcast(x, U32)
    corner = jnp.where(never, functools.reduce(jnp.bitwise_or, tokens), words[:8, :LANES])
    top = jnp.concatenate([corner, words[:8, LANES:]], axis=1)
    return _unpack(jnp.concatenate([top, words[8:]], axis=0))


def _swap_bit(a, b, stride, axis):
    n = a.shape[axis]
    low = (jax.lax.broadcasted_iota(jnp.int32, a.shape, axis) & stride) == 0
    return (jnp.where(low, a, pltpu.roll(b, stride, axis)),
            jnp.where(low, pltpu.roll(a, n - stride, axis), b))


def _swap_bits(parts, strides, axis):
    parts = list(parts)
    for bit, stride in strides:
        for i in range(len(parts)):
            if not i & bit:
                parts[i], parts[i | bit] = _swap_bit(parts[i], parts[i | bit], stride, axis)
    return parts


def _left_operands(a11, a12, a21, a22):
    return (a11 + a22, a21 + a22, a11, a22, a11 + a12, a21 - a11, a12 - a22)


def _right_operands(b11, b12, b21, b22):
    return (b11 + b22, b11, b12 - b22, b21 - b11, b22, b11 + b12, b21 + b22)


_FEEDS = (((0, 1), (3, 1)), ((2, 1), (3, -1)), ((1, 1), (3, 1)), ((0, 1), (2, 1)),
          ((0, -1), (1, 1)), ((3, 1),), ((0, 1),))


def _block_product(product):
    c = [None] * 4
    for i, feeds in enumerate(_FEEDS):
        m = product(i)
        for k, sign in feeds:
            c[k] = m if c[k] is None else (c[k] + m if sign > 0 else c[k] - m)
    return c


def _twice(operands, grid):
    outer = [operands(*[grid[2 * a + u][2 * b + v] for a in range(2) for b in range(2)])
             for u in range(2) for v in range(2)]
    return [op for quarters in zip(*outer) for op in operands(*quarters)]


def _kernel(x_hbm, wqkv_hbm, wo_hbm, w1_hbm, w3_hbm, w2_hbm, out_hbm,
            io_s, x_s, wqkv_raw, wo_raw, wqkv_s, wo_s, w1_raw, w3_raw, up_s, down_s, in_s, out_s,
            qkv_s, xp_s, xa_s, o_s, oa_s, in_sem, qkv_sem, w_sem, up_sem, out_sem):
    S, D = x_s.shape
    F = w3_raw.shape[1]
    TH, DH, FH = TM // 2, D // 2, F // 2
    TQ, DQ, FQ = TM // 4, D // 4, F // 4
    nb = S // TM
    n_items = 2 * nb
    nc = D // LANES
    scale = (D // N_HEADS) ** -0.5

    def slots(ref, n_rows, n_cols):
        return [ref.at[pl.ds(r, n_rows), pl.ds(c, n_cols)]
                for r in range(0, ref.shape[0] - n_rows + 1, n_rows)
                for c in range(0, ref.shape[1] - n_cols + 1, n_cols)]

    wo_slots = slots(wo_raw, TQ, DQ)
    xb_ops = wo_slots[4:4 + 49]
    h_ops = (slots(wqkv_raw, TQ, FQ) + slots(wo_raw, TQ, FQ)[:1])[:49]
    down_ops = slots(wqkv_s, FQ // 2, DQ) + slots(down_s, FQ // 2, DQ)
    assert len(xb_ops) == len(h_ops) == len(down_ops) == 49

    def rows(j):
        return pl.ds(j * TM if isinstance(j, int) else pl.multiple_of(j * TM, TM), TM)

    def x_copy(j):
        return pltpu.make_async_copy(x_hbm.at[rows(j)], io_s.at[rows(j)], in_sem.at[j])

    def out_copy(j):
        return pltpu.make_async_copy(io_s.at[rows(j)], out_hbm.at[rows(j)], out_sem.at[j])

    def wqkv_copy(i):
        rr = pl.ds(i * PB if isinstance(i, int) else pl.multiple_of(i * PB, PB), PB)
        return pltpu.make_async_copy(wqkv_hbm.at[rr], wqkv_raw.at[rr], qkv_sem.at[i])

    wo_copy = pltpu.make_async_copy(wo_hbm, wo_raw, w_sem.at[0])
    w2_quarters = [w.at[pl.ds(0, FQ), pl.ds(c, D)] for w in (w1_raw, w3_raw) for c in (0, D)]
    w2_copies = [pltpu.make_async_copy(w2_hbm.at[pl.ds(a * FQ, FQ)], dst, w_sem.at[1 + a])
                 for a, dst in enumerate(w2_quarters)]

    def up_copies(r):
        at = [pl.ds(pl.multiple_of(a * DQ + r * UB, UB), UB) for a in range(4)]
        return [pltpu.make_async_copy(src.at[at[a]], dst.at[at[a]], up_sem.at[8 * r + 4 * m + a])
                for m, (src, dst) in enumerate(((w1_hbm, w1_raw), (w3_hbm, w3_raw))) for a in range(4)]

    def chunk(r):
        return pl.ds(r * PB if isinstance(r, int) else pl.multiple_of(r * PB, PB), PB)

    def permute_qkv_columns(r):
        for i in range(3):
            cols = [pl.ds(i * D + c * LANES, LANES) for c in range(nc)]
            parts = [pltpu.bitcast(wqkv_raw[chunk(r), cc], U32) for cc in cols]
            for cc, part in zip(cols, _swap_bits(parts, ((4, 16), (2, 8), (1, 4)), 1)):
                wqkv_s[_word_rows(r * PB, PB), cc] = part

    def project_partial(r):
        y = _dot(xp_s[:, chunk(r)], _unpack(wqkv_s[_word_rows(r * PB, PB), :]))
        for t in range(3 * nc):
            qkv_s[t, pl.ds(HALO, TM), :] += y[:, t * LANES:(t + 1) * LANES]

    def combine(operands, blocks, store):
        halves = [operands(jax.tree.map(
            lambda w: pltpu.unpack_elementwise(w, index=k, packed_dtype=BF16, unpacked_dtype=F32), blocks))
            for k in range(2)]
        for i, pair in enumerate(zip(*halves)):
            store(i, pltpu.pack_elementwise(list(pair), packed_dtype=BF16).astype(U32))

    def combine_up(r):
        @pl.loop(0, FQ // LANES)
        def _(t):
            dst = up_s.at[:, _word_rows(r * UB, UB), pl.ds(pl.multiple_of(2 * t * LANES, LANES), 2 * LANES)]
            for m, w in enumerate((w1_raw, w3_raw)):
                src = w.at[pl.ds(pl.multiple_of(r * UB, UB), 3 * DQ + UB),
                           pl.ds(pl.multiple_of(t * LANES, LANES), 3 * FQ + LANES)]
                for r0 in range(0, UB, 16):
                    grid = [[pltpu.bitcast(src[pl.ds(a * DQ + r0, 16), pl.ds(b * FQ, LANES)], U32)
                             for b in range(4)] for a in range(4)]

                    def store(i, words):
                        dst[i, _word_rows(r0, 16), pl.ds(m * LANES, LANES)] = words
                    combine(functools.partial(_twice, _right_operands), grid, store)

    def combine_down():
        @pl.loop(0, FQ // CB)
        def _(g):
            for c in range(0, DQ, LANES):
                grid = [[pltpu.bitcast(w[pl.ds(pl.multiple_of(g * CB, CB), CB), pl.ds(b * DQ + c, LANES)], U32)
                         for b in range(4)] for w in w2_quarters]

                def store(i, words):
                    down_ops[i][_word_rows(g * CB, CB), pl.ds(c, LANES)] = words
                combine(functools.partial(_twice, _right_operands), grid, store)

    def combine_all(src, dst):
        half_rows, half_cols = src.shape[0], src.shape[1] // 2

        @pl.loop(0, half_rows // CB)
        def _(g):
            for c in range(0, half_cols, CW):
                blocks = [src[_word_rows(g * CB + dr, CB), pl.ds(dc + c, CW)]
                          for dr in (0, half_rows) for dc in (0, half_cols)]

                def store(i, words):
                    dst[i, _word_rows(g * CB, CB), pl.ds(c, CW)] = words
                combine(lambda b: _right_operands(*b), blocks, store)

    def permute_wo_rows():
        def body(hh, carry):
            def tile(h432, d4):
                return pl.ds(pl.multiple_of(h432 * 128 + hh * 32 + d4 * 16, 16), 16)
            src = [[pltpu.bitcast(wo_raw[tile(h, d4), :], U32) for h in range(8)] for d4 in range(2)]
            src = [_swap_bits(p, ((2, 4), (1, 2)), 0) for p in src]
            for d4 in range(2):
                for h in range(8):
                    wo_s[_word_rows(((h & 3) | (d4 << 2)) * 128 + hh * 32 + (h >> 2) * 16, 16), :] = src[d4][h]
            return carry
        jax.lax.fori_loop(0, 4, body, 0)

    def residual(rr, fresh):
        if fresh is None:
            return x_s[rr, :]
        return jnp.where(fresh, io_s[rr, :].astype(F32), x_s[rr, :])

    def normed(j, fresh, r, n):
        x = residual(pl.ds(pl.multiple_of(j * TM + r, n), n), fresh)
        xc = x - jnp.mean(x, axis=-1, keepdims=True)
        var = jnp.mean(xc * xc, axis=-1, keepdims=True)
        return xc * jax.lax.rsqrt(var + EPS)

    def store_left_operands(dst, r, top, bottom):
        ops = _left_operands(top[:, :DH], top[:, DH:], bottom[:, :DH], bottom[:, DH:])
        for i, a in enumerate(ops):
            dst[i, pl.ds(r, top.shape[0]), :] = a.astype(BF16)
        return _token(ops[0], ops[1], ops[4])

    def norm(j, fresh, dst, r, n, plain=None):
        top, bottom = normed(j, fresh, r, n), normed(j, fresh, TH + r, n)
        if plain is not None:
            plain[pl.ds(r, n), :] = top.astype(BF16)
            plain[pl.ds(TH + r, n), :] = bottom.astype(BF16)
        return store_left_operands(dst, r, top, bottom)

    def norm_for_ffn(j, r, n):
        quarters = [normed(j, None, a * TQ + r, n) for a in range(4)]
        ops = _twice(_left_operands, [[y[:, b * DQ:(b + 1) * DQ] for b in range(4)] for y in quarters])
        for i, a in enumerate(ops):
            xb_ops[i][pl.ds(r, n), :] = a.astype(BF16)
        return _token(*quarters)

    def attention_operands(r, n):
        return store_left_operands(oa_s, r, o_s[pl.ds(r, n), :], o_s[pl.ds(TH + r, n), :])

    def matmul(left, right, width, side_job, never, finish):
        tokens = []
        for p in range(right.shape[2] // width):
            def product(i):
                nonlocal tokens
                m = _dot(_after(left[i], tokens, never), _unpack(right[i, :, pl.ds(p * width, width)]))
                tokens = side_job(7 * p + i)
                return m
            finish(p, _block_product(product))

    def spread(items, i, n):
        return items[i * len(items) // n:(i + 1) * len(items) // n]

    def first_token(t):
        return jnp.broadcast_to(qkv_s[t, pl.ds(HALO, 1), :], (HALO, LANES))

    def project(j, side_job, never):
        per = DH // LANES
        tiles = [[half * 3 * nc // 2 + p * per + c for c in range(per)] for p in range(3) for half in range(2)]
        tails = {t: qkv_s[t, pl.ds(TM, HALO), :] for t in range(nc, 3 * nc)}

        def finish(p, blocks):
            for k, y in enumerate(blocks):
                for c, t in enumerate(tiles[2 * p + k % 2]):
                    yc = y[:, c * LANES:(c + 1) * LANES]
                    qkv_s[t, pl.ds(HALO + k // 2 * TH, TH), :] = yc
                    if t in tails and k < 2:
                        head = jnp.broadcast_to(yc[0:1, :], (HALO, LANES))
                        qkv_s[t, pl.ds(0, HALO), :] = jnp.where(j == 0, head, tails[t])
        matmul(xa_s, in_s, DH, side_job, never, finish)

    def out_project(j, fresh, never):
        def finish(p, blocks):
            for k, y in enumerate(blocks):
                at = (pl.ds(pl.multiple_of(j * TM + k // 2 * TH, TH), TH), pl.ds(k % 2 * DH, DH))
                x_s[at] = jnp.where(fresh, io_s[at].astype(F32), x_s[at]) + y
        matmul(oa_s, out_s, DH, lambda i: [], never, finish)

    def attention(j, r, n, masked):
        lane = jax.lax.broadcasted_iota(jnp.int32, (n, LANES), 1)
        logits = [None] * WINDOW
        for c in range(nc):
            q = qkv_s[c, pl.ds(HALO + r, n), :]
            for w in range(WINDOW):
                p = q * qkv_s[nc + c, pl.ds(HALO + r - DILATION * w, n), :]
                logits[w] = p if c == 0 else logits[w] + p
        for s in (1, 2):
            logits = [l + jnp.where((lane & s) == 0, pltpu.roll(l, LANES - s, 1), pltpu.roll(l, s, 1))
                      for l in logits]
        logits = [l * scale for l in logits]
        if masked:
            pos = j * TM + r + jax.lax.broadcasted_iota(jnp.int32, (n, LANES), 0)
            logits = [jnp.where(pos >= DILATION * w, l, -1e9) if w else l for w, l in enumerate(logits)]
        m = functools.reduce(jnp.maximum, logits)
        e = [jnp.exp(l - m) for l in logits]
        inv = 1.0 / functools.reduce(jnp.add, e)
        p = [x * inv for x in e]
        outs = []
        for c in range(nc):
            terms = [p[w] * qkv_s[2 * nc + c, pl.ds(HALO + r - DILATION * w, n), :] for w in range(WINDOW)]
            outs.append(functools.reduce(jnp.add, terms))
            o_s[pl.ds(r, n), pl.ds(c * LANES, LANES)] = outs[-1]
        return _token(*outs)

    def matmul_twice(left, right, side_job, never, tokens):
        def outer(i):
            def inner(k):
                nonlocal tokens
                m = _dot(_after(left(7 * i + k), tokens, never), _unpack(right(7 * i + k)))
                tokens = side_job(7 * i + k)
                return m
            return jnp.concatenate(_block_product(inner), axis=0)

        c = _block_product(outer)
        return [[c[a // 2 * 2 + b // 2][(a % 2 * 2 + b % 2) * TQ:][:TQ] for b in range(4)]
                for a in range(4)], tokens

    def ffn_up(side_job, never):
        tokens = []
        for t in range(FQ // LANES):
            grid, tokens = matmul_twice(lambda i: xb_ops[i][...],
                                        lambda i: up_s[i, :, pl.ds(2 * t * LANES, 2 * LANES)],
                                        lambda i: side_job(49 * t + i), never, tokens)

            def swiglu(gu):
                half = 0.5 * gu[:, :LANES]
                return (half + half * jnp.tanh(half)) * gu[:, LANES:]
            for i, a in enumerate(_twice(_left_operands, jax.tree.map(swiglu, grid))):
                h_ops[i][:, pl.ds(t * LANES, LANES)] = a.astype(BF16)

    def ffn_down(j, side_job, never):
        grid, _ = matmul_twice(lambda i: h_ops[i][...], lambda i: down_ops[i][...], side_job, never, [])
        for a in range(4):
            for b in range(4):
                at = (pl.ds(pl.multiple_of(j * TM + a * TQ, TQ), TQ), pl.ds(b * DQ, DQ))
                y = x_s[at] + grid[a][b]
                x_s[at] = y
                io_s[at] = y.astype(BF16)

    def start_in_order(n, copies):
        @pl.loop(0, n)
        def _(i):
            for copy in copies(i):
                copy.start()

    x_copy(0).start()
    start_in_order(D // PB, lambda r: [wqkv_copy(r)])

    last = n_items - 1

    @pl.loop(-2, n_items)
    def _(n):
        j0 = jnp.maximum(n, 0) % nb
        j1 = jnp.maximum(n + 1, 0) % nb
        j2 = (n + 2) % nb
        never = n > n_items

        att = [functools.partial(attention, j1, r, RB, r < HALO) for r in range(0, TM, RB)]

        def side_job(steps, n_slots):
            return lambda i: [step() for step in spread(steps, i, n_slots) if i < n_slots]

        @pl.when(n + 2 < nb)
        def _():
            x_copy(j2).wait()

        @pl.when(n == 0)
        def _():
            @pl.loop(0, DQ // UB)
            def _(r):
                for copy in up_copies(r):
                    copy.wait()
                combine_up(r)

            for copy in w2_copies:
                copy.start()

        @pl.when(n >= 0)
        def _():
            due = dict(zip(list(AT0) + [49 * t + i for t in range(1, FQ // LANES) for i in AT1], att, strict=True))
            ffn_up(lambda i: [due[i]()] if i in due else [], never)

        @pl.when(n == -1)
        def _():
            @pl.loop(0, TM // RC)
            def _(g):
                attention(j1, pl.multiple_of(g * RC, RC), RC, True)

            wo_copy.wait()
            permute_wo_rows()
            combine_all(wo_s, out_s)
            combine_all(wqkv_s, in_s)
            attention_operands(0, TH)

        @pl.when(n == 0)
        def _():
            for copy in w2_copies:
                copy.wait()
            combine_down()

        @pl.when(n >= 0)
        def _():
            steps = [functools.partial(norm, j2, n + 2 < nb, xa_s, r, LB) for r in range(0, TH, LB)]
            steps += [functools.partial(attention_operands, r, LB) for r in range(0, TH, LB)]
            ffn_down(j0, side_job(steps, 49 - NS2), never)

        @pl.when(n < 0)
        def _():
            norm(j2, n + 2 < nb, xa_s, 0, TH, plain=xp_s)

        @pl.when(n == -2)
        def _():
            x_copy(1).start()
            wo_copy.start()
            x_copy(2).start()
            start_in_order(DQ // UB, up_copies)
            start_in_order(nb - 3, lambda j: [x_copy(j + 3)])
            qkv_s[...] = jnp.zeros(qkv_s.shape, F32)

            n_chunks = D // PB

            @pl.loop(0, n_chunks + 1)
            def _(r):
                @pl.when(r < n_chunks)
                def _():
                    wqkv_copy(r).wait()

                @pl.when(r == 0)
                def _():
                    permute_qkv_columns(0)

                @pl.when(r > 0)
                def _():
                    project_partial(r - 1)
                    permute_qkv_columns(jnp.minimum(r, n_chunks - 1))

            for t in range(nc, 3 * nc):
                qkv_s[t, pl.ds(0, HALO), :] = first_token(t)

        @pl.when(n >= nb)
        def _():
            out_copy(j0).start()

        @pl.when(jnp.logical_and(n >= -1, n < last - 1))
        def _():
            out_project(j1, n + 1 < nb, never)
            project(j2, side_job([functools.partial(norm_for_ffn, j1, r, LB) for r in range(0, TQ, LB)], NS4), never)

        @pl.when(n == last - 1)
        def _():
            @pl.loop(0, D // NC)
            def _(i):
                cols = pl.ds(pl.multiple_of(i * NC, NC), NC)
                x_s[rows(j1), cols] += _dot(o_s[...].astype(BF16), _unpack(wo_s[:, cols]))


            @pl.loop(0, TQ // LB)
            def _(g):
                norm_for_ffn(j1, pl.multiple_of(g * LB, LB), LB)

    for j in range(nb):
        out_copy(j).wait()


@jax.jit
def pallas_interleave_layers__sliding_local_dilated__glu_gated_swiglu__prompt_kernel(
    A_x: jax.Array,
    A_wqkv: jax.Array,
    A_wo: jax.Array,
    B_x: jax.Array,
    B_w1: jax.Array,
    B_w3: jax.Array,
    B_w2: jax.Array,
):
    del B_x
    B, S, D = A_x.shape
    F = B_w1.shape[1]
    assert B == 1 and D == N_HEADS * 32 == 8 * LANES and S % TM == 0 and S // TM >= 3 and F == 28 * LANES
    nb = S // TM
    nc = D // LANES
    any_spec = pl.BlockSpec(memory_space=pl.ANY)
    out = pl.pallas_call(
        _kernel,
        out_shape=jax.ShapeDtypeStruct((S, D), A_x.dtype),
        in_specs=[any_spec] * 6,
        out_specs=any_spec,
        scratch_shapes=[
            pltpu.VMEM((S, D), BF16),
            pltpu.VMEM((S, D), F32),
            pltpu.VMEM((D, 3 * D), BF16),
            pltpu.VMEM((D, D), BF16),
            pltpu.VMEM((D // 2, 3 * D), U32),
            pltpu.VMEM((D // 2, D), U32),
            pltpu.VMEM((D, F), BF16),
            pltpu.VMEM((D, F), BF16),
            pltpu.VMEM((49, D // 8, F // 2), U32),
            pltpu.VMEM((F // 8, (49 - 12) * D // 4), U32),
            pltpu.VMEM((7, D // 4, 3 * D // 2), U32),
            pltpu.VMEM((7, D // 4, D // 2), U32),
            pltpu.VMEM((3 * nc, HALO + TM, LANES), F32),
            pltpu.VMEM((TM, D), BF16),
            pltpu.VMEM((7, TM // 2, D // 2), BF16),
            pltpu.VMEM((TM, D), F32),
            pltpu.VMEM((7, TM // 2, D // 2), BF16),
            pltpu.SemaphoreType.DMA((nb,)),
            pltpu.SemaphoreType.DMA((D // PB,)),
            pltpu.SemaphoreType.DMA((5,)),
            pltpu.SemaphoreType.DMA((2 * D // UB,)),
            pltpu.SemaphoreType.DMA((nb,)),
        ],
        compiler_params=pltpu.CompilerParams(vmem_limit_bytes=127 * 1024 * 1024),
    )(A_x.reshape(S, D), A_wqkv, A_wo, B_w1, B_w3, B_w2)
    return out.reshape(B, S, D)
```

```python
import functools

import jax
import jax.numpy as jnp
import jax.experimental.pallas as pl
import jax.experimental.pallas.tpu as pltpu

N_HEADS = 32
WINDOW = 8
DILATION = 2
EPS = 1e-5
LANES = 128
HALO = 16

TM = 256
UB = 128
NC = 256
NS4 = 20
AT0 = (6, 13, 27, 41)
AT1 = (13, 34)
NS2 = 14
RB = 16
PB = 128
CW = 256
CB = 16
RC = 128
LB = 16

F32 = jnp.float32
BF16 = jnp.bfloat16
U32 = jnp.uint32


def _dot(a, b):
    return jnp.dot(a, b, preferred_element_type=F32)


def _unpack(words):
    return pltpu.bitcast(words, BF16)


def _word_rows(r, n):
    return pl.ds(r // 2 if isinstance(r, int) else pl.multiple_of(r // 2, n // 2), n // 2)


def _token(*vals):
    regs = [pltpu.bitcast(v[r:r + 8, c:c + LANES], U32) for v in vals
            for r in range(0, v.shape[0], 8) for c in range(0, v.shape[1], LANES)]
    return functools.reduce(jnp.bitwise_or, regs)


def _after(x, tokens, never):
    if not tokens:
        return x
    words = pltpu.bitcast(x, U32)
    corner = jnp.where(never, functools.reduce(jnp.bitwise_or, tokens), words[:8, :LANES])
    top = jnp.concatenate([corner, words[:8, LANES:]], axis=1)
    return _unpack(jnp.concatenate([top, words[8:]], axis=0))


def _swap_bit(a, b, stride, axis):
    n = a.shape[axis]
    low = (jax.lax.broadcasted_iota(jnp.int32, a.shape, axis) & stride) == 0
    return (jnp.where(low, a, pltpu.roll(b, stride, axis)),
            jnp.where(low, pltpu.roll(a, n - stride, axis), b))


def _swap_bits(parts, strides, axis):
    parts = list(parts)
    for bit, stride in strides:
        for i in range(len(parts)):
            if not i & bit:
                parts[i], parts[i | bit] = _swap_bit(parts[i], parts[i | bit], stride, axis)
    return parts


def _left_operands(a11, a12, a21, a22):
    return (a11 + a22, a21 + a22, a11, a22, a11 + a12, a21 - a11, a12 - a22)


def _right_operands(b11, b12, b21, b22):
    return (b11 + b22, b11, b12 - b22, b21 - b11, b22, b11 + b12, b21 + b22)


_FEEDS = (((0, 1), (3, 1)), ((2, 1), (3, -1)), ((1, 1), (3, 1)), ((0, 1), (2, 1)),
          ((0, -1), (1, 1)), ((3, 1),), ((0, 1),))


def _block_product(product):
    c = [None] * 4
    for i, feeds in enumerate(_FEEDS):
        m = product(i)
        for k, sign in feeds:
            c[k] = m if c[k] is None else (c[k] + m if sign > 0 else c[k] - m)
    return c


def _twice(operands, grid):
    outer = [operands(*[grid[2 * a + u][2 * b + v] for a in range(2) for b in range(2)])
             for u in range(2) for v in range(2)]
    return [op for quarters in zip(*outer) for op in operands(*quarters)]


def _kernel(x_hbm, wqkv_hbm, wo_hbm, w1_hbm, w3_hbm, w2_hbm, out_hbm,
            io_s, x_s, wqkv_raw, wo_raw, wqkv_s, wo_s, w1_raw, w3_raw, up_s, down_s, in_s, out_s,
            qkv_s, xp_s, xa_s, o_s, oa_s, in_sem, qkv_sem, w_sem, up_sem, out_sem):
    S, D = x_s.shape
    F = w3_raw.shape[1]
    TH, DH, FH = TM // 2, D // 2, F // 2
    TQ, DQ, FQ = TM // 4, D // 4, F // 4
    nb = S // TM
    n_items = 2 * nb
    nc = D // LANES
    scale = (D // N_HEADS) ** -0.5

    def slots(ref, n_rows, n_cols):
        return [ref.at[pl.ds(r, n_rows), pl.ds(c, n_cols)]
                for r in range(0, ref.shape[0] - n_rows + 1, n_rows)
                for c in range(0, ref.shape[1] - n_cols + 1, n_cols)]

    n_tiles = FQ // LANES
    xb_ops = slots(wo_raw, TQ, DQ)[:49]
    h_pairs = slots(wqkv_raw, TQ, 2 * LANES)
    down_ops = slots(wqkv_s, FQ // 2, DQ) + slots(down_s, FQ // 2, DQ)
    assert len(xb_ops) == len(down_ops) == 49 and len(h_pairs) >= 25 * n_tiles

    def rows(j):
        return pl.ds(j * TM if isinstance(j, int) else pl.multiple_of(j * TM, TM), TM)

    def x_copy(j):
        return pltpu.make_async_copy(x_hbm.at[rows(j)], io_s.at[rows(j)], in_sem.at[j])

    def out_copy(j):
        return pltpu.make_async_copy(io_s.at[rows(j)], out_hbm.at[rows(j)], out_sem.at[j])

    def wqkv_copy(i):
        rr = pl.ds(i * PB if isinstance(i, int) else pl.multiple_of(i * PB, PB), PB)
        return pltpu.make_async_copy(wqkv_hbm.at[rr], wqkv_raw.at[rr], qkv_sem.at[i])

    wo_copy = pltpu.make_async_copy(wo_hbm, wo_raw, w_sem.at[0])
    w2_quarters = [w.at[pl.ds(0, FQ), pl.ds(c, D)] for w in (w1_raw, w3_raw) for c in (0, D)]
    w2_copies = [pltpu.make_async_copy(w2_hbm.at[pl.ds(a * FQ, FQ)], dst, w_sem.at[1 + a])
                 for a, dst in enumerate(w2_quarters)]

    def up_copies(r):
        at = [pl.ds(pl.multiple_of(a * DQ + r * UB, UB), UB) for a in range(4)]
        return [pltpu.make_async_copy(src.at[at[a]], dst.at[at[a]], up_sem.at[8 * r + 4 * m + a])
                for m, (src, dst) in enumerate(((w1_hbm, w1_raw), (w3_hbm, w3_raw))) for a in range(4)]

    def chunk(r):
        return pl.ds(r * PB if isinstance(r, int) else pl.multiple_of(r * PB, PB), PB)

    def permute_qkv_columns(r):
        for i in range(3):
            cols = [pl.ds(i * D + c * LANES, LANES) for c in range(nc)]
            parts = [pltpu.bitcast(wqkv_raw[chunk(r), cc], U32) for cc in cols]
            for cc, part in zip(cols, _swap_bits(parts, ((4, 16), (2, 8), (1, 4)), 1)):
                wqkv_s[_word_rows(r * PB, PB), cc] = part

    def project_partial(r):
        y = _dot(xp_s[:, chunk(r)], _unpack(wqkv_s[_word_rows(r * PB, PB), :]))
        for t in range(3 * nc):
            qkv_s[t, pl.ds(HALO, TM), :] += y[:, t * LANES:(t + 1) * LANES]

    def combine(operands, blocks, store):
        halves = [operands(jax.tree.map(
            lambda w: pltpu.unpack_elementwise(w, index=k, packed_dtype=BF16, unpacked_dtype=F32), blocks))
            for k in range(2)]
        for i, pair in enumerate(zip(*halves)):
            store(i, pltpu.pack_elementwise(list(pair), packed_dtype=BF16).astype(U32))

    def combine_up(r):
        @pl.loop(0, n_tiles)
        def _(t):
            dst = up_s.at[:, _word_rows(r * UB, UB), pl.ds(pl.multiple_of(2 * t * LANES, LANES), 2 * LANES)]
            for m, w in enumerate((w1_raw, w3_raw)):
                src = w.at[pl.ds(pl.multiple_of(r * UB, UB), 3 * DQ + UB),
                           pl.ds(pl.multiple_of(t * LANES, LANES), 3 * FQ + LANES)]
                for r0 in range(0, UB, 16):
                    grid = [[pltpu.bitcast(src[pl.ds(a * DQ + r0, 16), pl.ds(b * FQ, LANES)], U32)
                             for b in range(4)] for a in range(4)]

                    def store(i, words):
                        dst[i, _word_rows(r0, 16), pl.ds(m * LANES, LANES)] = words
                    combine(functools.partial(_twice, _right_operands), grid, store)

    def combine_down():
        @pl.loop(0, FQ // CB)
        def _(g):
            for c in range(0, DQ, LANES):
                grid = [[pltpu.bitcast(w[pl.ds(pl.multiple_of(g * CB, CB), CB), pl.ds(b * DQ + c, LANES)], U32)
                         for b in range(4)] for w in w2_quarters]

                def store(i, words):
                    down_ops[i][_word_rows(g * CB, CB), pl.ds(c, LANES)] = words
                combine(functools.partial(_twice, _right_operands), grid, store)

    def combine_all(src, dst):
        half_rows, half_cols = src.shape[0], src.shape[1] // 2

        @pl.loop(0, half_rows // CB)
        def _(g):
            for c in range(0, half_cols, CW):
                blocks = [src[_word_rows(g * CB + dr, CB), pl.ds(dc + c, CW)]
                          for dr in (0, half_rows) for dc in (0, half_cols)]

                def store(i, words):
                    dst[i, _word_rows(g * CB, CB), pl.ds(c, CW)] = words
                combine(lambda b: _right_operands(*b), blocks, store)

    def permute_wo_rows():
        def body(hh, carry):
            def tile(h432, d4):
                return pl.ds(pl.multiple_of(h432 * 128 + hh * 32 + d4 * 16, 16), 16)
            src = [[pltpu.bitcast(wo_raw[tile(h, d4), :], U32) for h in range(8)] for d4 in range(2)]
            src = [_swap_bits(p, ((2, 4), (1, 2)), 0) for p in src]
            for d4 in range(2):
                for h in range(8):
                    wo_s[_word_rows(((h & 3) | (d4 << 2)) * 128 + hh * 32 + (h >> 2) * 16, 16), :] = src[d4][h]
            return carry
        jax.lax.fori_loop(0, 4, body, 0)

    def residual(rr, fresh):
        if fresh is None:
            return x_s[rr, :]
        return jnp.where(fresh, io_s[rr, :].astype(F32), x_s[rr, :])

    def normed(j, fresh, r, n):
        x = residual(pl.ds(pl.multiple_of(j * TM + r, n), n), fresh)
        xc = x - jnp.mean(x, axis=-1, keepdims=True)
        var = jnp.mean(xc * xc, axis=-1, keepdims=True)
        return xc * jax.lax.rsqrt(var + EPS)

    def store_left_operands(dst, r, top, bottom):
        ops = _left_operands(top[:, :DH], top[:, DH:], bottom[:, :DH], bottom[:, DH:])
        for i, a in enumerate(ops):
            dst[i, pl.ds(r, top.shape[0]), :] = a.astype(BF16)
        return _token(ops[0], ops[1], ops[4])

    def norm(j, fresh, dst, r, n, plain=None):
        top, bottom = normed(j, fresh, r, n), normed(j, fresh, TH + r, n)
        if plain is not None:
            plain[pl.ds(r, n), :] = top.astype(BF16)
            plain[pl.ds(TH + r, n), :] = bottom.astype(BF16)
        return store_left_operands(dst, r, top, bottom)

    def norm_for_ffn(j, r, n):
        quarters = [normed(j, None, a * TQ + r, n) for a in range(4)]
        ops = _twice(_left_operands, [[y[:, b * DQ:(b + 1) * DQ] for b in range(4)] for y in quarters])
        for i, a in enumerate(ops):
            xb_ops[i][pl.ds(r, n), :] = a.astype(BF16)
        return _token(*quarters)

    def attention_operands(r, n):
        return store_left_operands(oa_s, r, o_s[pl.ds(r, n), :], o_s[pl.ds(TH + r, n), :])

    def matmul(left, right, width, side_job, never, finish):
        tokens = []
        for p in range(right.shape[2] // width):
            def product(i):
                nonlocal tokens
                m = _dot(_after(left[i], tokens, never), _unpack(right[i, :, pl.ds(p * width, width)]))
                tokens = side_job(7 * p + i)
                return m
            finish(p, _block_product(product))

    def spread(items, i, n):
        return items[i * len(items) // n:(i + 1) * len(items) // n]

    def first_token(t):
        return jnp.broadcast_to(qkv_s[t, pl.ds(HALO, 1), :], (HALO, LANES))

    def project(j, side_job, never):
        per = DH // LANES
        tiles = [[half * 3 * nc // 2 + p * per + c for c in range(per)] for p in range(3) for half in range(2)]
        tails = {t: qkv_s[t, pl.ds(TM, HALO), :] for t in range(nc, 3 * nc)}

        def finish(p, blocks):
            for k, y in enumerate(blocks):
                for c, t in enumerate(tiles[2 * p + k % 2]):
                    yc = y[:, c * LANES:(c + 1) * LANES]
                    qkv_s[t, pl.ds(HALO + k // 2 * TH, TH), :] = yc
                    if t in tails and k < 2:
                        head = jnp.broadcast_to(yc[0:1, :], (HALO, LANES))
                        qkv_s[t, pl.ds(0, HALO), :] = jnp.where(j == 0, head, tails[t])
        matmul(xa_s, in_s, DH, side_job, never, finish)

    def out_project(j, fresh, never):
        def finish(p, blocks):
            for k, y in enumerate(blocks):
                at = (pl.ds(pl.multiple_of(j * TM + k // 2 * TH, TH), TH), pl.ds(k % 2 * DH, DH))
                x_s[at] = jnp.where(fresh, io_s[at].astype(F32), x_s[at]) + y
        matmul(oa_s, out_s, DH, lambda i: [], never, finish)

    def attention(j, r, n, masked):
        lane = jax.lax.broadcasted_iota(jnp.int32, (n, LANES), 1)
        logits = [None] * WINDOW
        for c in range(nc):
            q = qkv_s[c, pl.ds(HALO + r, n), :]
            for w in range(WINDOW):
                p = q * qkv_s[nc + c, pl.ds(HALO + r - DILATION * w, n), :]
                logits[w] = p if c == 0 else logits[w] + p
        for s in (1, 2):
            logits = [l + jnp.where((lane & s) == 0, pltpu.roll(l, LANES - s, 1), pltpu.roll(l, s, 1))
                      for l in logits]
        logits = [l * scale for l in logits]
        if masked:
            pos = j * TM + r + jax.lax.broadcasted_iota(jnp.int32, (n, LANES), 0)
            logits = [jnp.where(pos >= DILATION * w, l, -1e9) if w else l for w, l in enumerate(logits)]
        m = functools.reduce(jnp.maximum, logits)
        e = [jnp.exp(l - m) for l in logits]
        inv = 1.0 / functools.reduce(jnp.add, e)
        p = [x * inv for x in e]
        outs = []
        for c in range(nc):
            terms = [p[w] * qkv_s[2 * nc + c, pl.ds(HALO + r - DILATION * w, n), :] for w in range(WINDOW)]
            outs.append(functools.reduce(jnp.add, terms))
            o_s[pl.ds(r, n), pl.ds(c * LANES, LANES)] = outs[-1]
        return _token(*outs)

    def matmul_twice(left, right, side_job, never, tokens):
        def outer(i):
            def inner(k):
                nonlocal tokens
                m = _dot(_after(left(7 * i + k), tokens, never), _unpack(right(7 * i + k)))
                tokens = side_job(7 * i + k)
                return m
            return jnp.concatenate(_block_product(inner), axis=0)

        c = _block_product(outer)
        return [[c[a // 2 * 2 + b // 2][(a % 2 * 2 + b % 2) * TQ:][:TQ] for b in range(4)]
                for a in range(4)], tokens

    def ffn_up(side_job, never):
        tokens = []
        for t in range(n_tiles):
            grid, tokens = matmul_twice(lambda i: xb_ops[i][...],
                                        lambda i: up_s[i, :, pl.ds(2 * t * LANES, 2 * LANES)],
                                        lambda i: side_job(49 * t + i), never, tokens)

            def swiglu(gu):
                half = 0.5 * gu[:, :LANES]
                return (half + half * jnp.tanh(half)) * gu[:, LANES:]
            ops = _twice(_left_operands, jax.tree.map(swiglu, grid))
            for i in range(0, 49, 2):
                pair = jnp.concatenate(ops[i:i + 2], axis=1)
                h_pairs[i // 2 * n_tiles + t][:, pl.ds(0, pair.shape[1])] = pair.astype(BF16)

    def ffn_down(j, side_job, never):
        def hidden(i):
            return jnp.concatenate([h_pairs[i // 2 * n_tiles + t][:, pl.ds(i % 2 * LANES, LANES)]
                                    for t in range(n_tiles)], axis=1)

        grid, _ = matmul_twice(hidden, lambda i: down_ops[i][...], side_job, never, [])
        for a in range(4):
            for b in range(4):
                at = (pl.ds(pl.multiple_of(j * TM + a * TQ, TQ), TQ), pl.ds(b * DQ, DQ))
                y = x_s[at] + grid[a][b]
                x_s[at] = y
                io_s[at] = y.astype(BF16)

    def start_in_order(n, copies):
        @pl.loop(0, n)
        def _(i):
            for copy in copies(i):
                copy.start()

    x_copy(0).start()
    start_in_order(D // PB, lambda r: [wqkv_copy(r)])

    last = n_items - 1

    @pl.loop(-2, n_items)
    def _(n):
        j0 = jnp.maximum(n, 0) % nb
        j1 = jnp.maximum(n + 1, 0) % nb
        j2 = (n + 2) % nb
        never = n > n_items

        att = [functools.partial(attention, j1, r, RB, r < HALO) for r in range(0, TM, RB)]

        def side_job(steps, n_slots):
            return lambda i: [step() for step in spread(steps, i, n_slots) if i < n_slots]

        @pl.when(n + 2 < nb)
        def _():
            x_copy(j2).wait()

        @pl.when(n == 0)
        def _():
            @pl.loop(0, DQ // UB)
            def _(r):
                for copy in up_copies(r):
                    copy.wait()
                combine_up(r)

            for copy in w2_copies:
                copy.start()

        @pl.when(n >= 0)
        def _():
            due = dict(zip(list(AT0) + [49 * t + i for t in range(1, n_tiles) for i in AT1], att, strict=True))
            ffn_up(lambda i: [due[i]()] if i in due else [], never)

        @pl.when(n == -1)
        def _():
            @pl.loop(0, TM // RC)
            def _(g):
                attention(j1, pl.multiple_of(g * RC, RC), RC, True)

            wo_copy.wait()
            permute_wo_rows()
            combine_all(wo_s, out_s)
            combine_all(wqkv_s, in_s)
            attention_operands(0, TH)

        @pl.when(n == 0)
        def _():
            for copy in w2_copies:
                copy.wait()
            combine_down()

        @pl.when(n >= 0)
        def _():
            steps = [functools.partial(norm, j2, n + 2 < nb, xa_s, r, LB) for r in range(0, TH, LB)]
            steps += [functools.partial(attention_operands, r, LB) for r in range(0, TH, LB)]
            ffn_down(j0, side_job(steps, 49 - NS2), never)

        @pl.when(n < 0)
        def _():
            norm(j2, n + 2 < nb, xa_s, 0, TH, plain=xp_s)

        @pl.when(n == -2)
        def _():
            x_copy(1).start()
            wo_copy.start()
            x_copy(2).start()
            start_in_order(DQ // UB, up_copies)
            start_in_order(nb - 3, lambda j: [x_copy(j + 3)])
            qkv_s[...] = jnp.zeros(qkv_s.shape, F32)

            n_chunks = D // PB

            @pl.loop(0, n_chunks + 1)
            def _(r):
                @pl.when(r < n_chunks)
                def _():
                    wqkv_copy(r).wait()

                @pl.when(r == 0)
                def _():
                    permute_qkv_columns(0)

                @pl.when(r > 0)
                def _():
                    project_partial(r - 1)
                    permute_qkv_columns(jnp.minimum(r, n_chunks - 1))

            for t in range(nc, 3 * nc):
                qkv_s[t, pl.ds(0, HALO), :] = first_token(t)

        @pl.when(n >= nb)
        def _():
            out_copy(j0).start()

        @pl.when(jnp.logical_and(n >= -1, n < last - 1))
        def _():
            out_project(j1, n + 1 < nb, never)
            project(j2, side_job([functools.partial(norm_for_ffn, j1, r, LB) for r in range(0, TQ, LB)], NS4), never)

        @pl.when(n == last - 1)
        def _():
            @pl.loop(0, D // NC)
            def _(i):
                cols = pl.ds(pl.multiple_of(i * NC, NC), NC)
                x_s[rows(j1), cols] += _dot(o_s[...].astype(BF16), _unpack(wo_s[:, cols]))


            @pl.loop(0, TQ // LB)
            def _(g):
                norm_for_ffn(j1, pl.multiple_of(g * LB, LB), LB)

    for j in range(nb):
        out_copy(j).wait()


@jax.jit
def pallas_interleave_layers__sliding_local_dilated__glu_gated_swiglu__prompt_kernel(
    A_x: jax.Array,
    A_wqkv: jax.Array,
    A_wo: jax.Array,
    B_x: jax.Array,
    B_w1: jax.Array,
    B_w3: jax.Array,
    B_w2: jax.Array,
):
    del B_x
    B, S, D = A_x.shape
    F = B_w1.shape[1]
    assert B == 1 and D == N_HEADS * 32 == 8 * LANES and S % TM == 0 and S // TM >= 3 and F == 28 * LANES
    nb = S // TM
    nc = D // LANES
    any_spec = pl.BlockSpec(memory_space=pl.ANY)
    out = pl.pallas_call(
        _kernel,
        out_shape=jax.ShapeDtypeStruct((S, D), A_x.dtype),
        in_specs=[any_spec] * 6,
        out_specs=any_spec,
        scratch_shapes=[
            pltpu.VMEM((S, D), BF16),
            pltpu.VMEM((S, D), F32),
            pltpu.VMEM((D, 3 * D), BF16),
            pltpu.VMEM((D, D), BF16),
            pltpu.VMEM((D // 2, 3 * D), U32),
            pltpu.VMEM((D // 2, D), U32),
            pltpu.VMEM((D, F), BF16),
            pltpu.VMEM((D, F), BF16),
            pltpu.VMEM((49, D // 8, F // 2), U32),
            pltpu.VMEM((F // 8, (49 - 12) * D // 4), U32),
            pltpu.VMEM((7, D // 4, 3 * D // 2), U32),
            pltpu.VMEM((7, D // 4, D // 2), U32),
            pltpu.VMEM((3 * nc, HALO + TM, LANES), F32),
            pltpu.VMEM((TM, D), BF16),
            pltpu.VMEM((7, TM // 2, D // 2), BF16),
            pltpu.VMEM((TM, D), F32),
            pltpu.VMEM((7, TM // 2, D // 2), BF16),
            pltpu.SemaphoreType.DMA((nb,)),
            pltpu.SemaphoreType.DMA((D // PB,)),
            pltpu.SemaphoreType.DMA((5,)),
            pltpu.SemaphoreType.DMA((2 * D // UB,)),
            pltpu.SemaphoreType.DMA((nb,)),
        ],
        compiler_params=pltpu.CompilerParams(vmem_limit_bytes=127 * 1024 * 1024),
    )(A_x.reshape(S, D), A_wqkv, A_wo, B_w1, B_w3, B_w2)
    return out.reshape(B, S, D)
```

```python
import functools

import jax
import jax.numpy as jnp
import jax.experimental.pallas as pl
import jax.experimental.pallas.tpu as pltpu

N_HEADS = 32
WINDOW = 8
DILATION = 2
EPS = 1e-5
LANES = 128
HALO = 16

TM = 256
RB = 16
RC = 128
LB = 16
PB = 128
UB = 128
CB = 16
CW = 256
NC = 256
DUE_FIRST = (6, 13, 27, 41)
DUE_LATER = (13, 34)

F32 = jnp.float32
BF16 = jnp.bfloat16
U32 = jnp.uint32


def _dot(a, b):
    return jnp.dot(a, b, preferred_element_type=F32)


def _unpack(words):
    return pltpu.bitcast(words, BF16)


def _word_rows(r, n):
    return pl.ds(r // 2 if isinstance(r, int) else pl.multiple_of(r // 2, n // 2), n // 2)


def _token(*vals):
    regs = [pltpu.bitcast(v[r:r + 8, c:c + LANES], U32) for v in vals
            for r in range(0, v.shape[0], 8) for c in range(0, v.shape[1], LANES)]
    return functools.reduce(jnp.bitwise_or, regs)


def _after(x, tokens, never):
    if not tokens:
        return x
    words = pltpu.bitcast(x, U32)
    corner = jnp.where(never, functools.reduce(jnp.bitwise_or, tokens), words[:8, :LANES])
    top = jnp.concatenate([corner, words[:8, LANES:]], axis=1)
    return _unpack(jnp.concatenate([top, words[8:]], axis=0))


def _swap_bit(a, b, stride, axis):
    n = a.shape[axis]
    low = (jax.lax.broadcasted_iota(jnp.int32, a.shape, axis) & stride) == 0
    return (jnp.where(low, a, pltpu.roll(b, stride, axis)),
            jnp.where(low, pltpu.roll(a, n - stride, axis), b))


def _swap_bits(parts, strides, axis):
    parts = list(parts)
    for bit, stride in strides:
        for i in range(len(parts)):
            if not i & bit:
                parts[i], parts[i | bit] = _swap_bit(parts[i], parts[i | bit], stride, axis)
    return parts


def _left_operands(a11, a12, a21, a22):
    return (a11 + a22, a21 + a22, a11, a22, a11 + a12, a21 - a11, a12 - a22)


def _right_operands(b11, b12, b21, b22):
    return (b11 + b22, b11, b12 - b22, b21 - b11, b22, b11 + b12, b21 + b22)


_FEEDS = (((0, 1), (3, 1)), ((2, 1), (3, -1)), ((1, 1), (3, 1)), ((0, 1), (2, 1)),
          ((0, -1), (1, 1)), ((3, 1),), ((0, 1),))


def _block_product(product):
    c = [None] * 4
    for i, feeds in enumerate(_FEEDS):
        m = product(i)
        for k, sign in feeds:
            c[k] = m if c[k] is None else (c[k] + m if sign > 0 else c[k] - m)
    return c


def _twice(operands, grid):
    outer = [operands(*[grid[2 * a + u][2 * b + v] for a in range(2) for b in range(2)])
             for u in range(2) for v in range(2)]
    return [op for quarters in zip(*outer) for op in operands(*quarters)]


def _kernel(x_hbm, wqkv_hbm, wo_hbm, w1_hbm, w3_hbm, w2_hbm, out_hbm,
            io_s, x_s, wqkv_raw, wo_raw, wqkv_s, wo_s, w1_raw, w3_raw, up_s, down_s, in_s, out_s,
            qkv_s, xp_s, xa_s, o_s, oa_s, in_sem, qkv_sem, w_sem, up_sem, out_sem):
    S, D = x_s.shape
    F = w3_raw.shape[1]
    TH, DH, FH = TM // 2, D // 2, F // 2
    TQ, DQ, FQ = TM // 4, D // 4, F // 4
    nb = S // TM
    n_items = 2 * nb
    nc = D // LANES
    scale = (D // N_HEADS) ** -0.5

    def slots(ref, n_rows, n_cols):
        return [ref.at[pl.ds(r, n_rows), pl.ds(c, n_cols)]
                for r in range(0, ref.shape[0] - n_rows + 1, n_rows)
                for c in range(0, ref.shape[1] - n_cols + 1, n_cols)]

    n_tiles = FQ // LANES
    xb_ops = slots(wo_raw, TQ, DQ)[:49]
    h_pairs = slots(wqkv_raw, TQ, 2 * LANES)
    down_ops = slots(wqkv_s, FQ // 2, DQ) + slots(down_s, FQ // 2, DQ)
    assert len(xb_ops) == len(down_ops) == 49 and len(h_pairs) >= 25 * n_tiles

    def rows(j):
        return pl.ds(j * TM if isinstance(j, int) else pl.multiple_of(j * TM, TM), TM)

    def x_copy(j):
        return pltpu.make_async_copy(x_hbm.at[rows(j)], io_s.at[rows(j)], in_sem.at[j])

    def out_copy(j):
        return pltpu.make_async_copy(io_s.at[rows(j)], out_hbm.at[rows(j)], out_sem.at[j])

    def wqkv_copy(i):
        rr = pl.ds(i * PB if isinstance(i, int) else pl.multiple_of(i * PB, PB), PB)
        return pltpu.make_async_copy(wqkv_hbm.at[rr], wqkv_raw.at[rr], qkv_sem.at[i])

    wo_copy = pltpu.make_async_copy(wo_hbm, wo_raw, w_sem.at[0])
    w2_quarters = [w.at[pl.ds(0, FQ), pl.ds(c, D)] for w in (w1_raw, w3_raw) for c in (0, D)]
    w2_copies = [pltpu.make_async_copy(w2_hbm.at[pl.ds(a * FQ, FQ)], dst, w_sem.at[1 + a])
                 for a, dst in enumerate(w2_quarters)]

    def up_copies(r):
        at = [pl.ds(pl.multiple_of(a * DQ + r * UB, UB), UB) for a in range(4)]
        return [pltpu.make_async_copy(src.at[at[a]], dst.at[at[a]], up_sem.at[8 * r + 4 * m + a])
                for m, (src, dst) in enumerate(((w1_hbm, w1_raw), (w3_hbm, w3_raw))) for a in range(4)]

    def chunk(r):
        return pl.ds(r * PB if isinstance(r, int) else pl.multiple_of(r * PB, PB), PB)

    def permute_qkv_columns(r):
        for i in range(3):
            cols = [pl.ds(i * D + c * LANES, LANES) for c in range(nc)]
            parts = [pltpu.bitcast(wqkv_raw[chunk(r), cc], U32) for cc in cols]
            for cc, part in zip(cols, _swap_bits(parts, ((4, 16), (2, 8), (1, 4)), 1)):
                wqkv_s[_word_rows(r * PB, PB), cc] = part

    def project_partial(r):
        y = _dot(xp_s[:, chunk(r)], _unpack(wqkv_s[_word_rows(r * PB, PB), :]))
        for t in range(3 * nc):
            qkv_s[t, pl.ds(HALO, TM), :] += y[:, t * LANES:(t + 1) * LANES]

    def combine(operands, blocks, store):
        halves = [operands(jax.tree.map(
            lambda w: pltpu.unpack_elementwise(w, index=k, packed_dtype=BF16, unpacked_dtype=F32), blocks))
            for k in range(2)]
        for i, pair in enumerate(zip(*halves)):
            store(i, pltpu.pack_elementwise(list(pair), packed_dtype=BF16).astype(U32))

    def combine_up(r):
        @pl.loop(0, n_tiles)
        def _(t):
            dst = up_s.at[:, _word_rows(r * UB, UB), pl.ds(pl.multiple_of(2 * t * LANES, LANES), 2 * LANES)]
            for m, w in enumerate((w1_raw, w3_raw)):
                src = w.at[pl.ds(pl.multiple_of(r * UB, UB), 3 * DQ + UB),
                           pl.ds(pl.multiple_of(t * LANES, LANES), 3 * FQ + LANES)]
                for r0 in range(0, UB, 16):
                    grid = [[pltpu.bitcast(src[pl.ds(a * DQ + r0, 16), pl.ds(b * FQ, LANES)], U32)
                             for b in range(4)] for a in range(4)]

                    def store(i, words):
                        dst[i, _word_rows(r0, 16), pl.ds(m * LANES, LANES)] = words
                    combine(functools.partial(_twice, _right_operands), grid, store)

    def combine_down():
        @pl.loop(0, FQ // CB)
        def _(g):
            for c in range(0, DQ, LANES):
                grid = [[pltpu.bitcast(w[pl.ds(pl.multiple_of(g * CB, CB), CB), pl.ds(b * DQ + c, LANES)], U32)
                         for b in range(4)] for w in w2_quarters]

                def store(i, words):
                    down_ops[i][_word_rows(g * CB, CB), pl.ds(c, LANES)] = words
                combine(functools.partial(_twice, _right_operands), grid, store)

    def combine_all(src, dst):
        half_rows, half_cols = src.shape[0], src.shape[1] // 2

        @pl.loop(0, half_rows // CB)
        def _(g):
            for c in range(0, half_cols, CW):
                blocks = [src[_word_rows(g * CB + dr, CB), pl.ds(dc + c, CW)]
                          for dr in (0, half_rows) for dc in (0, half_cols)]

                def store(i, words):
                    dst[i, _word_rows(g * CB, CB), pl.ds(c, CW)] = words
                combine(lambda b: _right_operands(*b), blocks, store)

    def permute_wo_rows():
        def body(hh, carry):
            def tile(h432, d4):
                return pl.ds(pl.multiple_of(h432 * 128 + hh * 32 + d4 * 16, 16), 16)
            src = [[pltpu.bitcast(wo_raw[tile(h, d4), :], U32) for h in range(8)] for d4 in range(2)]
            src = [_swap_bits(p, ((2, 4), (1, 2)), 0) for p in src]
            for d4 in range(2):
                for h in range(8):
                    wo_s[_word_rows(((h & 3) | (d4 << 2)) * 128 + hh * 32 + (h >> 2) * 16, 16), :] = src[d4][h]
            return carry
        jax.lax.fori_loop(0, 4, body, 0)

    def residual(rr, fresh):
        if fresh is None:
            return x_s[rr, :]
        return jnp.where(fresh, io_s[rr, :].astype(F32), x_s[rr, :])

    def normed(j, fresh, r, n):
        x = residual(pl.ds(pl.multiple_of(j * TM + r, n), n), fresh)
        xc = x - jnp.mean(x, axis=-1, keepdims=True)
        var = jnp.mean(xc * xc, axis=-1, keepdims=True)
        return xc * jax.lax.rsqrt(var + EPS)

    def store_left_operands(dst, r, top, bottom):
        ops = _left_operands(top[:, :DH], top[:, DH:], bottom[:, :DH], bottom[:, DH:])
        for i, a in enumerate(ops):
            dst[i, pl.ds(r, top.shape[0]), :] = a.astype(BF16)
        return _token(ops[0], ops[1], ops[4])

    def norm(j, fresh, dst, r, n, plain=None):
        top, bottom = normed(j, fresh, r, n), normed(j, fresh, TH + r, n)
        if plain is not None:
            plain[pl.ds(r, n), :] = top.astype(BF16)
            plain[pl.ds(TH + r, n), :] = bottom.astype(BF16)
        return store_left_operands(dst, r, top, bottom)

    def norm_for_ffn(j, r, n):
        quarters = [normed(j, None, a * TQ + r, n) for a in range(4)]
        ops = _twice(_left_operands, [[y[:, b * DQ:(b + 1) * DQ] for b in range(4)] for y in quarters])
        for i, a in enumerate(ops):
            xb_ops[i][pl.ds(r, n), :] = a.astype(BF16)
        return _token(*quarters)

    def attention_operands(r, n):
        return store_left_operands(oa_s, r, o_s[pl.ds(r, n), :], o_s[pl.ds(TH + r, n), :])

    def matmul(left, right, width, side_job, never, finish):
        tokens = []
        for p in range(right.shape[2] // width):
            def product(i):
                nonlocal tokens
                m = _dot(_after(left[i], tokens, never), _unpack(right[i, :, pl.ds(p * width, width)]))
                tokens = side_job(7 * p + i)
                return m
            finish(p, _block_product(product))

    def spread(items, i, n):
        return items[i * len(items) // n:(i + 1) * len(items) // n]

    def first_token(t):
        return jnp.broadcast_to(qkv_s[t, pl.ds(HALO, 1), :], (HALO, LANES))

    def project(j, side_job, never):
        per = DH // LANES
        tiles = [[half * 3 * nc // 2 + p * per + c for c in range(per)] for p in range(3) for half in range(2)]
        tails = {t: qkv_s[t, pl.ds(TM, HALO), :] for t in range(nc, 3 * nc)}

        def finish(p, blocks):
            for k, y in enumerate(blocks):
                for c, t in enumerate(tiles[2 * p + k % 2]):
                    yc = y[:, c * LANES:(c + 1) * LANES]
                    qkv_s[t, pl.ds(HALO + k // 2 * TH, TH), :] = yc
                    if t in tails and k < 2:
                        head = jnp.broadcast_to(yc[0:1, :], (HALO, LANES))
                        qkv_s[t, pl.ds(0, HALO), :] = jnp.where(j == 0, head, tails[t])
        matmul(xa_s, in_s, DH, side_job, never, finish)

    def out_project(j, fresh, never):
        def finish(p, blocks):
            for k, y in enumerate(blocks):
                at = (pl.ds(pl.multiple_of(j * TM + k // 2 * TH, TH), TH), pl.ds(k % 2 * DH, DH))
                x_s[at] = jnp.where(fresh, io_s[at].astype(F32), x_s[at]) + y
        matmul(oa_s, out_s, DH, lambda i: [], never, finish)

    def attention(j, r, n, masked):
        lane = jax.lax.broadcasted_iota(jnp.int32, (n, LANES), 1)
        logits = [None] * WINDOW
        for c in range(nc):
            q = qkv_s[c, pl.ds(HALO + r, n), :]
            for w in range(WINDOW):
                p = q * qkv_s[nc + c, pl.ds(HALO + r - DILATION * w, n), :]
                logits[w] = p if c == 0 else logits[w] + p
        for s in (1, 2):
            logits = [l + jnp.where((lane & s) == 0, pltpu.roll(l, LANES - s, 1), pltpu.roll(l, s, 1))
                      for l in logits]
        logits = [l * scale for l in logits]
        if masked:
            pos = j * TM + r + jax.lax.broadcasted_iota(jnp.int32, (n, LANES), 0)
            logits = [jnp.where(pos >= DILATION * w, l, -1e9) if w else l for w, l in enumerate(logits)]
        m = functools.reduce(jnp.maximum, logits)
        e = [jnp.exp(l - m) for l in logits]
        inv = 1.0 / functools.reduce(jnp.add, e)
        p = [x * inv for x in e]
        outs = []
        for c in range(nc):
            terms = [p[w] * qkv_s[2 * nc + c, pl.ds(HALO + r - DILATION * w, n), :] for w in range(WINDOW)]
            outs.append(functools.reduce(jnp.add, terms))
            o_s[pl.ds(r, n), pl.ds(c * LANES, LANES)] = outs[-1]
        return _token(*outs)

    def matmul_twice(left, right, side_job, never, tokens):
        def outer(i):
            def inner(k):
                nonlocal tokens
                m = _dot(_after(left(7 * i + k), tokens, never), _unpack(right(7 * i + k)))
                tokens = side_job(7 * i + k)
                return m
            return jnp.concatenate(_block_product(inner), axis=0)

        c = _block_product(outer)
        return [[c[a // 2 * 2 + b // 2][(a % 2 * 2 + b % 2) * TQ:][:TQ] for b in range(4)]
                for a in range(4)], tokens

    def ffn_up(side_job, never):
        tokens = []
        for t in range(n_tiles):
            grid, tokens = matmul_twice(lambda i: xb_ops[i][...],
                                        lambda i: up_s[i, :, pl.ds(2 * t * LANES, 2 * LANES)],
                                        lambda i: side_job(49 * t + i), never, tokens)

            def swiglu(gu):
                half = 0.5 * gu[:, :LANES]
                return (half + half * jnp.tanh(half)) * gu[:, LANES:]
            ops = _twice(_left_operands, jax.tree.map(swiglu, grid))
            for i in range(0, 49, 2):
                pair = jnp.concatenate(ops[i:i + 2], axis=1)
                h_pairs[i // 2 * n_tiles + t][:, pl.ds(0, pair.shape[1])] = pair.astype(BF16)

    def ffn_down(j, side_job, never):
        def hidden(i):
            return jnp.concatenate([h_pairs[i // 2 * n_tiles + t][:, pl.ds(i % 2 * LANES, LANES)]
                                    for t in range(n_tiles)], axis=1)

        grid, _ = matmul_twice(hidden, lambda i: down_ops[i][...], side_job, never, [])
        for a in range(4):
            for b in range(4):
                at = (pl.ds(pl.multiple_of(j * TM + a * TQ, TQ), TQ), pl.ds(b * DQ, DQ))
                y = x_s[at] + grid[a][b]
                x_s[at] = y
                io_s[at] = y.astype(BF16)

    def start_in_order(n, copies):
        @pl.loop(0, n)
        def _(i):
            for copy in copies(i):
                copy.start()

    x_copy(0).start()
    start_in_order(D // PB, lambda r: [wqkv_copy(r)])

    last = n_items - 1

    @pl.loop(-2, n_items)
    def _(n):
        j0 = jnp.maximum(n, 0) % nb
        j1 = jnp.maximum(n + 1, 0) % nb
        j2 = (n + 2) % nb
        never = n > n_items

        att = [functools.partial(attention, j1, r, RB, r < HALO) for r in range(0, TM, RB)]

        def side_job(steps, n_slots):
            return lambda i: [step() for step in spread(steps, i, n_slots) if i < n_slots]

        @pl.when(n + 2 < nb)
        def _():
            x_copy(j2).wait()

        @pl.when(n == 0)
        def _():
            @pl.loop(0, DQ // UB)
            def _(r):
                for copy in up_copies(r):
                    copy.wait()
                combine_up(r)

            for copy in w2_copies:
                copy.start()

        @pl.when(n >= 0)
        def _():
            due = dict(zip(list(DUE_FIRST) + [49 * t + i for t in range(1, n_tiles) for i in DUE_LATER],
                           att, strict=True))
            ffn_up(lambda i: [due[i]()] if i in due else [], never)

        @pl.when(n == -1)
        def _():
            @pl.loop(0, TM // RC)
            def _(g):
                attention(j1, pl.multiple_of(g * RC, RC), RC, True)

            wo_copy.wait()
            permute_wo_rows()
            combine_all(wo_s, out_s)
            combine_all(wqkv_s, in_s)
            attention_operands(0, TH)

        @pl.when(n == 0)
        def _():
            for copy in w2_copies:
                copy.wait()
            combine_down()

        @pl.when(n >= 0)
        def _():
            steps = [functools.partial(norm, j2, n + 2 < nb, xa_s, r, LB) for r in range(0, TH, LB)]
            steps += [functools.partial(attention_operands, r, LB) for r in range(0, TH, LB)]
            ffn_down(j0, side_job(steps, 35), never)

        @pl.when(n < 0)
        def _():
            norm(j2, n + 2 < nb, xa_s, 0, TH, plain=xp_s)

        @pl.when(n == -2)
        def _():
            x_copy(1).start()
            wo_copy.start()
            x_copy(2).start()
            start_in_order(DQ // UB, up_copies)
            start_in_order(nb - 3, lambda j: [x_copy(j + 3)])
            qkv_s[...] = jnp.zeros(qkv_s.shape, F32)

            n_chunks = D // PB

            @pl.loop(0, n_chunks + 1)
            def _(r):
                @pl.when(r < n_chunks)
                def _():
                    wqkv_copy(r).wait()

                @pl.when(r == 0)
                def _():
                    permute_qkv_columns(0)

                @pl.when(r > 0)
                def _():
                    project_partial(r - 1)
                    permute_qkv_columns(jnp.minimum(r, n_chunks - 1))

            for t in range(nc, 3 * nc):
                qkv_s[t, pl.ds(0, HALO), :] = first_token(t)

        @pl.when(n >= nb)
        def _():
            out_copy(j0).start()

        @pl.when(jnp.logical_and(n >= -1, n < last - 1))
        def _():
            out_project(j1, n + 1 < nb, never)
            project(j2, side_job([functools.partial(norm_for_ffn, j1, r, LB) for r in range(0, TQ, LB)], 20), never)

        @pl.when(n == last - 1)
        def _():
            @pl.loop(0, D // NC)
            def _(i):
                cols = pl.ds(pl.multiple_of(i * NC, NC), NC)
                x_s[rows(j1), cols] += _dot(o_s[...].astype(BF16), _unpack(wo_s[:, cols]))


            @pl.loop(0, TQ // LB)
            def _(g):
                norm_for_ffn(j1, pl.multiple_of(g * LB, LB), LB)

    for j in range(nb):
        out_copy(j).wait()


@jax.jit
def pallas_interleave_layers__sliding_local_dilated__glu_gated_swiglu__prompt_kernel(
    A_x: jax.Array,
    A_wqkv: jax.Array,
    A_wo: jax.Array,
    B_x: jax.Array,
    B_w1: jax.Array,
    B_w3: jax.Array,
    B_w2: jax.Array,
):
    del B_x
    B, S, D = A_x.shape
    F = B_w1.shape[1]
    assert B == 1 and D == N_HEADS * 32 == 8 * LANES and S % TM == 0 and S // TM >= 3 and F == 28 * LANES
    nb = S // TM
    nc = D // LANES
    any_spec = pl.BlockSpec(memory_space=pl.ANY)
    out = pl.pallas_call(
        _kernel,
        out_shape=jax.ShapeDtypeStruct((S, D), A_x.dtype),
        in_specs=[any_spec] * 6,
        out_specs=any_spec,
        scratch_shapes=[
            pltpu.VMEM((S, D), BF16),
            pltpu.VMEM((S, D), F32),
            pltpu.VMEM((D, 3 * D), BF16),
            pltpu.VMEM((D, D), BF16),
            pltpu.VMEM((D // 2, 3 * D), U32),
            pltpu.VMEM((D // 2, D), U32),
            pltpu.VMEM((D, F), BF16),
            pltpu.VMEM((D, F), BF16),
            pltpu.VMEM((49, D // 8, F // 2), U32),
            pltpu.VMEM((F // 8, (49 - 12) * D // 4), U32),
            pltpu.VMEM((7, D // 4, 3 * D // 2), U32),
            pltpu.VMEM((7, D // 4, D // 2), U32),
            pltpu.VMEM((3 * nc, HALO + TM, LANES), F32),
            pltpu.VMEM((TM, D), BF16),
            pltpu.VMEM((7, TM // 2, D // 2), BF16),
            pltpu.VMEM((TM, D), F32),
            pltpu.VMEM((7, TM // 2, D // 2), BF16),
            pltpu.SemaphoreType.DMA((nb,)),
            pltpu.SemaphoreType.DMA((D // PB,)),
            pltpu.SemaphoreType.DMA((5,)),
            pltpu.SemaphoreType.DMA((2 * D // UB,)),
            pltpu.SemaphoreType.DMA((nb,)),
        ],
        compiler_params=pltpu.CompilerParams(vmem_limit_bytes=127 * 1024 * 1024),
    )(A_x.reshape(S, D), A_wqkv, A_wo, B_w1, B_w3, B_w2)
    return out.reshape(B, S, D)
```

```python
import functools

import jax
import jax.numpy as jnp
import jax.experimental.pallas as pl
import jax.experimental.pallas.tpu as pltpu

N_HEADS = 32
WINDOW = 8
DILATION = 2
EPS = 1e-5
LANES = 128
HALO = 16

TM = 256
RB = 16
RC = 128
LB = 16
LF = 16
LC = 64
NS4 = 20
PB = 128
UB = 128
CB = 16
CW = 256
NC = 512
DUE_FIRST = (6, 13, 27, 41)
DUE_LATER = (13, 34)

F32 = jnp.float32
BF16 = jnp.bfloat16
U32 = jnp.uint32


def _dot(a, b):
    return jnp.dot(a, b, preferred_element_type=F32)


def _unpack(words):
    return pltpu.bitcast(words, BF16)


def _word_rows(r, n):
    return pl.ds(r // 2 if isinstance(r, int) else pl.multiple_of(r // 2, n // 2), n // 2)


def _token(*vals):
    regs = [pltpu.bitcast(v[r:r + 8, c:c + LANES], U32) for v in vals
            for r in range(0, v.shape[0], 8) for c in range(0, v.shape[1], LANES)]
    return functools.reduce(jnp.bitwise_or, regs)


def _after(x, tokens, never):
    if not tokens:
        return x
    words = pltpu.bitcast(x, U32)
    corner = jnp.where(never, functools.reduce(jnp.bitwise_or, tokens), words[:8, :LANES])
    top = jnp.concatenate([corner, words[:8, LANES:]], axis=1)
    return _unpack(jnp.concatenate([top, words[8:]], axis=0))


def _swap_bit(a, b, stride, axis):
    n = a.shape[axis]
    low = (jax.lax.broadcasted_iota(jnp.int32, a.shape, axis) & stride) == 0
    return (jnp.where(low, a, pltpu.roll(b, stride, axis)),
            jnp.where(low, pltpu.roll(a, n - stride, axis), b))


def _swap_bits(parts, strides, axis):
    parts = list(parts)
    for bit, stride in strides:
        for i in range(len(parts)):
            if not i & bit:
                parts[i], parts[i | bit] = _swap_bit(parts[i], parts[i | bit], stride, axis)
    return parts


def _left_operands(a11, a12, a21, a22):
    return (a11 + a22, a21 + a22, a11, a22, a11 + a12, a21 - a11, a12 - a22)


def _right_operands(b11, b12, b21, b22):
    return (b11 + b22, b11, b12 - b22, b21 - b11, b22, b11 + b12, b21 + b22)


_FEEDS = (((0, 1), (3, 1)), ((2, 1), (3, -1)), ((1, 1), (3, 1)), ((0, 1), (2, 1)),
          ((0, -1), (1, 1)), ((3, 1),), ((0, 1),))


def _block_product(product):
    c = [None] * 4
    for i, feeds in enumerate(_FEEDS):
        m = product(i)
        for k, sign in feeds:
            c[k] = m if c[k] is None else (c[k] + m if sign > 0 else c[k] - m)
    return c


def _twice(operands, grid):
    outer = [operands(*[grid[2 * a + u][2 * b + v] for a in range(2) for b in range(2)])
             for u in range(2) for v in range(2)]
    return [op for quarters in zip(*outer) for op in operands(*quarters)]


def _kernel(x_hbm, wqkv_hbm, wo_hbm, w1_hbm, w3_hbm, w2_hbm, out_hbm,
            io_s, x_s, wqkv_raw, wo_raw, wqkv_s, wo_s, w1_raw, w3_raw, up_s, down_s, in_s, out_s,
            qkv_s, xp_s, xa_s, o_s, oa_s, hl_s, in_sem, qkv_sem, w_sem, up_sem, out_sem):
    S, D = x_s.shape
    F = w3_raw.shape[1]
    TH, DH, FH = TM // 2, D // 2, F // 2
    TQ, DQ, FQ = TM // 4, D // 4, F // 4
    nb = S // TM
    n_items = 2 * nb
    nc = D // LANES
    scale = (D // N_HEADS) ** -0.5

    def slots(ref, n_rows, n_cols):
        return [ref.at[pl.ds(r, n_rows), pl.ds(c, n_cols)]
                for r in range(0, ref.shape[0] - n_rows + 1, n_rows)
                for c in range(0, ref.shape[1] - n_cols + 1, n_cols)]

    n_tiles = FQ // LANES
    xb_ops = slots(wo_raw, TQ, DQ)[:49]
    h_pairs = slots(wqkv_raw, TQ, 2 * LANES)
    down_ops = slots(wqkv_s, FQ // 2, DQ) + slots(down_s, FQ // 2, DQ)
    assert len(xb_ops) == len(down_ops) == 49 and len(h_pairs) >= 25 * n_tiles

    def rows(j):
        return pl.ds(j * TM if isinstance(j, int) else pl.multiple_of(j * TM, TM), TM)

    def x_copy(j):
        return pltpu.make_async_copy(x_hbm.at[rows(j)], io_s.at[rows(j)], in_sem.at[j])

    def out_copy(j):
        return pltpu.make_async_copy(io_s.at[rows(j)], out_hbm.at[rows(j)], out_sem.at[j])

    def wqkv_copy(i):
        rr = pl.ds(i * PB if isinstance(i, int) else pl.multiple_of(i * PB, PB), PB)
        return pltpu.make_async_copy(wqkv_hbm.at[rr], wqkv_raw.at[rr], qkv_sem.at[i])

    wo_copy = pltpu.make_async_copy(wo_hbm, wo_raw, w_sem.at[0])
    w2_quarters = [w.at[pl.ds(0, FQ), pl.ds(c, D)] for w in (w1_raw, w3_raw) for c in (0, D)]
    w2_copies = [pltpu.make_async_copy(w2_hbm.at[pl.ds(a * FQ, FQ)], dst, w_sem.at[1 + a])
                 for a, dst in enumerate(w2_quarters)]

    def up_copies(r):
        at = [pl.ds(pl.multiple_of(a * DQ + r * UB, UB), UB) for a in range(4)]
        return [pltpu.make_async_copy(src.at[at[a]], dst.at[at[a]], up_sem.at[8 * r + 4 * m + a])
                for m, (src, dst) in enumerate(((w1_hbm, w1_raw), (w3_hbm, w3_raw))) for a in range(4)]

    def chunk(r):
        return pl.ds(r * PB if isinstance(r, int) else pl.multiple_of(r * PB, PB), PB)

    def permute_qkv_columns(r):
        for i in range(3):
            cols = [pl.ds(i * D + c * LANES, LANES) for c in range(nc)]
            parts = [pltpu.bitcast(wqkv_raw[chunk(r), cc], U32) for cc in cols]
            for cc, part in zip(cols, _swap_bits(parts, ((4, 16), (2, 8), (1, 4)), 1)):
                wqkv_s[_word_rows(r * PB, PB), cc] = part

    def project_partial(r):
        y = _dot(xp_s[:, chunk(r)], _unpack(wqkv_s[_word_rows(r * PB, PB), :]))
        for t in range(3 * nc):
            qkv_s[t, pl.ds(HALO, TM), :] += y[:, t * LANES:(t + 1) * LANES]

    def combine(operands, blocks, store):
        halves = [operands(jax.tree.map(
            lambda w: pltpu.unpack_elementwise(w, index=k, packed_dtype=BF16, unpacked_dtype=F32), blocks))
            for k in range(2)]
        for i, pair in enumerate(zip(*halves)):
            store(i, pltpu.pack_elementwise(list(pair), packed_dtype=BF16).astype(U32))

    def combine_up(r):
        @pl.loop(0, n_tiles)
        def _(t):
            dst = up_s.at[:, _word_rows(r * UB, UB), pl.ds(pl.multiple_of(2 * t * LANES, LANES), 2 * LANES)]
            for m, w in enumerate((w1_raw, w3_raw)):
                src = w.at[pl.ds(pl.multiple_of(r * UB, UB), 3 * DQ + UB),
                           pl.ds(pl.multiple_of(t * LANES, LANES), 3 * FQ + LANES)]
                for r0 in range(0, UB, 16):
                    grid = [[pltpu.bitcast(src[pl.ds(a * DQ + r0, 16), pl.ds(b * FQ, LANES)], U32)
                             for b in range(4)] for a in range(4)]

                    def store(i, words):
                        dst[i, _word_rows(r0, 16), pl.ds(m * LANES, LANES)] = words
                    combine(functools.partial(_twice, _right_operands), grid, store)

    def combine_down():
        @pl.loop(0, FQ // CB)
        def _(g):
            for c in range(0, DQ, LANES):
                grid = [[pltpu.bitcast(w[pl.ds(pl.multiple_of(g * CB, CB), CB), pl.ds(b * DQ + c, LANES)], U32)
                         for b in range(4)] for w in w2_quarters]

                def store(i, words):
                    down_ops[i][_word_rows(g * CB, CB), pl.ds(c, LANES)] = words
                combine(functools.partial(_twice, _right_operands), grid, store)

    def combine_all(src, dst):
        half_rows, half_cols = src.shape[0], src.shape[1] // 2

        @pl.loop(0, half_rows // CB)
        def _(g):
            for c in range(0, half_cols, CW):
                blocks = [src[_word_rows(g * CB + dr, CB), pl.ds(dc + c, CW)]
                          for dr in (0, half_rows) for dc in (0, half_cols)]

                def store(i, words):
                    dst[i, _word_rows(g * CB, CB), pl.ds(c, CW)] = words
                combine(lambda b: _right_operands(*b), blocks, store)

    def permute_wo_rows():
        def body(hh, carry):
            def tile(h432, d4):
                return pl.ds(pl.multiple_of(h432 * 128 + hh * 32 + d4 * 16, 16), 16)
            src = [[pltpu.bitcast(wo_raw[tile(h, d4), :], U32) for h in range(8)] for d4 in range(2)]
            src = [_swap_bits(p, ((2, 4), (1, 2)), 0) for p in src]
            for d4 in range(2):
                for h in range(8):
                    wo_s[_word_rows(((h & 3) | (d4 << 2)) * 128 + hh * 32 + (h >> 2) * 16, 16), :] = src[d4][h]
            return carry
        jax.lax.fori_loop(0, 4, body, 0)

    def residual(rr, fresh):
        if fresh is None:
            return x_s[rr, :]
        return jnp.where(fresh, io_s[rr, :].astype(F32), x_s[rr, :])

    def normed(j, fresh, r, n):
        x = residual(pl.ds(pl.multiple_of(j * TM + r, n), n), fresh)
        xc = x - jnp.mean(x, axis=-1, keepdims=True)
        var = jnp.mean(xc * xc, axis=-1, keepdims=True)
        return xc * jax.lax.rsqrt(var + EPS)

    def store_left_operands(dst, r, top, bottom):
        ops = _left_operands(top[:, :DH], top[:, DH:], bottom[:, :DH], bottom[:, DH:])
        for i, a in enumerate(ops):
            dst[i, pl.ds(r, top.shape[0]), :] = a.astype(BF16)
        return _token(ops[0], ops[1], ops[4])

    def norm(j, fresh, dst, r, n, plain=None):
        top, bottom = normed(j, fresh, r, n), normed(j, fresh, TH + r, n)
        if plain is not None:
            plain[pl.ds(r, n), :] = top.astype(BF16)
            plain[pl.ds(TH + r, n), :] = bottom.astype(BF16)
        return store_left_operands(dst, r, top, bottom)

    def norm_for_ffn(j, r, n):
        quarters = [normed(j, None, a * TQ + r, n) for a in range(4)]
        ops = _twice(_left_operands, [[y[:, b * DQ:(b + 1) * DQ] for b in range(4)] for y in quarters])
        for i, a in enumerate(ops):
            xb_ops[i][pl.ds(r, n), :] = a.astype(BF16)
        return _token(*quarters)

    def attention_operands(r, n):
        return store_left_operands(oa_s, r, o_s[pl.ds(r, n), :], o_s[pl.ds(TH + r, n), :])

    def matmul(left, right, width, side_job, never, finish):
        tokens = []
        for p in range(right.shape[2] // width):
            def product(i):
                nonlocal tokens
                m = _dot(_after(left[i], tokens, never), _unpack(right[i, :, pl.ds(p * width, width)]))
                tokens = side_job(7 * p + i)
                return m
            finish(p, _block_product(product))

    def spread(items, i, n):
        return items[i * len(items) // n:(i + 1) * len(items) // n]

    def first_token(t):
        return jnp.broadcast_to(qkv_s[t, pl.ds(HALO, 1), :], (HALO, LANES))

    def project(j, side_job, never):
        per = DH // LANES
        tiles = [[half * 3 * nc // 2 + p * per + c for c in range(per)] for p in range(3) for half in range(2)]
        tails = {t: qkv_s[t, pl.ds(TM, HALO), :] for t in range(nc, 3 * nc)}

        def finish(p, blocks):
            for k, y in enumerate(blocks):
                for c, t in enumerate(tiles[2 * p + k % 2]):
                    yc = y[:, c * LANES:(c + 1) * LANES]
                    qkv_s[t, pl.ds(HALO + k // 2 * TH, TH), :] = yc
                    if t in tails and k < 2:
                        head = jnp.broadcast_to(yc[0:1, :], (HALO, LANES))
                        qkv_s[t, pl.ds(0, HALO), :] = jnp.where(j == 0, head, tails[t])
        matmul(xa_s, in_s, DH, side_job, never, finish)

    def out_project(j, fresh, never):
        def finish(p, blocks):
            for k, y in enumerate(blocks):
                at = (pl.ds(pl.multiple_of(j * TM + k // 2 * TH, TH), TH), pl.ds(k % 2 * DH, DH))
                x_s[at] = jnp.where(fresh, io_s[at].astype(F32), x_s[at]) + y
        matmul(oa_s, out_s, DH, lambda i: [], never, finish)

    def attention(j, r, n, masked):
        lane = jax.lax.broadcasted_iota(jnp.int32, (n, LANES), 1)
        logits = [None] * WINDOW
        for c in range(nc):
            q = qkv_s[c, pl.ds(HALO + r, n), :]
            for w in range(WINDOW):
                p = q * qkv_s[nc + c, pl.ds(HALO + r - DILATION * w, n), :]
                logits[w] = p if c == 0 else logits[w] + p
        for s in (1, 2):
            logits = [l + jnp.where((lane & s) == 0, pltpu.roll(l, LANES - s, 1), pltpu.roll(l, s, 1))
                      for l in logits]
        logits = [l * scale for l in logits]
        if masked:
            pos = j * TM + r + jax.lax.broadcasted_iota(jnp.int32, (n, LANES), 0)
            logits = [jnp.where(pos >= DILATION * w, l, -1e9) if w else l for w, l in enumerate(logits)]
        m = functools.reduce(jnp.maximum, logits)
        e = [jnp.exp(l - m) for l in logits]
        inv = 1.0 / functools.reduce(jnp.add, e)
        p = [x * inv for x in e]
        outs = []
        for c in range(nc):
            terms = [p[w] * qkv_s[2 * nc + c, pl.ds(HALO + r - DILATION * w, n), :] for w in range(WINDOW)]
            outs.append(functools.reduce(jnp.add, terms))
            o_s[pl.ds(r, n), pl.ds(c * LANES, LANES)] = outs[-1]
        return _token(*outs)

    def matmul_twice(left, right, side_job, never, tokens):
        def outer(i):
            def inner(k):
                nonlocal tokens
                m = _dot(_after(left(7 * i + k), tokens, never), _unpack(right(7 * i + k)))
                tokens = side_job(7 * i + k)
                return m
            return jnp.concatenate(_block_product(inner), axis=0)

        c = _block_product(outer)
        return [[c[a // 2 * 2 + b // 2][(a % 2 * 2 + b % 2) * TQ:][:TQ] for b in range(4)]
                for a in range(4)], tokens

    def ffn_up(side_job, never):
        tokens = []
        for t in range(n_tiles):
            grid, tokens = matmul_twice(lambda i: xb_ops[i][...],
                                        lambda i: up_s[i, :, pl.ds(2 * t * LANES, 2 * LANES)],
                                        lambda i: side_job(49 * t + i), never, tokens)

            def swiglu(gu):
                half = 0.5 * gu[:, :LANES]
                return (half + half * jnp.tanh(half)) * gu[:, LANES:]
            grid = jax.tree.map(swiglu, grid)
            if t == n_tiles - 1:
                for a in range(4):
                    hl_s[pl.ds(a * TQ, TQ), :] = jnp.concatenate(grid[a], axis=1)
                continue
            ops = _twice(_left_operands, grid)
            for i in range(0, 49, 2):
                pair = jnp.concatenate(ops[i:i + 2], axis=1)
                h_pairs[i // 2 * n_tiles + t][:, pl.ds(0, pair.shape[1])] = pair.astype(BF16)

    def ffn_down(j, side_job, never):
        last_tile = _twice(_left_operands, [[hl_s[pl.ds(a * TQ, TQ), pl.ds(b * LANES, LANES)]
                                             for b in range(4)] for a in range(4)])

        def hidden(i):
            tiles = [h_pairs[i // 2 * n_tiles + t][:, pl.ds(i % 2 * LANES, LANES)] for t in range(n_tiles - 1)]
            return jnp.concatenate(tiles + [last_tile[i].astype(BF16)], axis=1)

        grid, _ = matmul_twice(hidden, lambda i: down_ops[i][...], side_job, never, [])
        for a in range(4):
            for b in range(4):
                at = (pl.ds(pl.multiple_of(j * TM + a * TQ, TQ), TQ), pl.ds(b * DQ, DQ))
                y = x_s[at] + grid[a][b]
                x_s[at] = y
                io_s[at] = y.astype(BF16)

    def start_in_order(n, copies):
        @pl.loop(0, n)
        def _(i):
            for copy in copies(i):
                copy.start()

    x_copy(0).start()
    start_in_order(D // PB, lambda r: [wqkv_copy(r)])

    last = n_items - 1

    @pl.loop(-2, n_items)
    def _(n):
        j0 = jnp.maximum(n, 0) % nb
        j1 = jnp.maximum(n + 1, 0) % nb
        j2 = (n + 2) % nb
        never = n > n_items

        att = [functools.partial(attention, j1, r, RB, r < HALO) for r in range(0, TM, RB)]

        def side_job(steps, n_slots):
            return lambda i: [step() for step in spread(steps, i, n_slots) if i < n_slots]

        @pl.when(n + 2 < nb)
        def _():
            x_copy(j2).wait()

        @pl.when(n == 0)
        def _():
            @pl.loop(0, DQ // UB)
            def _(r):
                for copy in up_copies(r):
                    copy.wait()
                combine_up(r)

            for copy in w2_copies:
                copy.start()

        @pl.when(n >= 0)
        def _():
            due = dict(zip(list(DUE_FIRST) + [49 * t + i for t in range(1, n_tiles) for i in DUE_LATER],
                           att, strict=True))
            ffn_up(lambda i: [due[i]()] if i in due else [], never)

        @pl.when(n == -1)
        def _():
            @pl.loop(0, TM // RC)
            def _(g):
                attention(j1, pl.multiple_of(g * RC, RC), RC, True)

            wo_copy.wait()
            permute_wo_rows()
            combine_all(wo_s, out_s)
            combine_all(wqkv_s, in_s)
            attention_operands(0, TH)

        @pl.when(n == 0)
        def _():
            for copy in w2_copies:
                copy.wait()
            combine_down()

        @pl.when(n >= 0)
        def _():
            steps = [functools.partial(norm, j2, n + 2 < nb, xa_s, r, LB) for r in range(0, TH, LB)]
            steps += [functools.partial(attention_operands, r, LB) for r in range(0, TH, LB)]
            ffn_down(j0, side_job(steps, 35), never)

        @pl.when(n < 0)
        def _():
            norm(j2, n + 2 < nb, xa_s, 0, TH, plain=xp_s)

        @pl.when(n == -2)
        def _():
            x_copy(1).start()
            wo_copy.start()
            x_copy(2).start()
            start_in_order(DQ // UB, up_copies)
            start_in_order(nb - 3, lambda j: [x_copy(j + 3)])
            qkv_s[...] = jnp.zeros(qkv_s.shape, F32)

            n_chunks = D // PB

            @pl.loop(0, n_chunks + 1)
            def _(r):
                @pl.when(r < n_chunks)
                def _():
                    wqkv_copy(r).wait()

                @pl.when(r == 0)
                def _():
                    permute_qkv_columns(0)

                @pl.when(r > 0)
                def _():
                    project_partial(r - 1)
                    permute_qkv_columns(jnp.minimum(r, n_chunks - 1))

            for t in range(nc, 3 * nc):
                qkv_s[t, pl.ds(0, HALO), :] = first_token(t)

        @pl.when(n >= nb)
        def _():
            out_copy(j0).start()

        @pl.when(jnp.logical_and(n >= -1, n < last - 1))
        def _():
            out_project(j1, n + 1 < nb, never)
            project(j2, side_job([functools.partial(norm_for_ffn, j1, r, LF) for r in range(0, TQ, LF)], NS4), never)

        @pl.when(n == last - 1)
        def _():
            @pl.loop(0, D // NC)
            def _(i):
                cols = pl.ds(pl.multiple_of(i * NC, NC), NC)
                x_s[rows(j1), cols] += _dot(o_s[...].astype(BF16), _unpack(wo_s[:, cols]))


            @pl.loop(0, TQ // LC)
            def _(g):
                norm_for_ffn(j1, pl.multiple_of(g * LC, LC), LC)

    for j in range(nb):
        out_copy(j).wait()


@jax.jit
def pallas_interleave_layers__sliding_local_dilated__glu_gated_swiglu__prompt_kernel(
    A_x: jax.Array,
    A_wqkv: jax.Array,
    A_wo: jax.Array,
    B_x: jax.Array,
    B_w1: jax.Array,
    B_w3: jax.Array,
    B_w2: jax.Array,
):
    del B_x
    B, S, D = A_x.shape
    F = B_w1.shape[1]
    assert B == 1 and D == N_HEADS * 32 == 8 * LANES and S % TM == 0 and S // TM >= 3 and F == 28 * LANES
    nb = S // TM
    nc = D // LANES
    any_spec = pl.BlockSpec(memory_space=pl.ANY)
    out = pl.pallas_call(
        _kernel,
        out_shape=jax.ShapeDtypeStruct((S, D), A_x.dtype),
        in_specs=[any_spec] * 6,
        out_specs=any_spec,
        scratch_shapes=[
            pltpu.VMEM((S, D), BF16),
            pltpu.VMEM((S, D), F32),
            pltpu.VMEM((D, 3 * D), BF16),
            pltpu.VMEM((D, D), BF16),
            pltpu.VMEM((D // 2, 3 * D), U32),
            pltpu.VMEM((D // 2, D), U32),
            pltpu.VMEM((D, F), BF16),
            pltpu.VMEM((D, F), BF16),
            pltpu.VMEM((49, D // 8, F // 2), U32),
            pltpu.VMEM((F // 8, (49 - 12) * D // 4), U32),
            pltpu.VMEM((7, D // 4, 3 * D // 2), U32),
            pltpu.VMEM((7, D // 4, D // 2), U32),
            pltpu.VMEM((3 * nc, HALO + TM, LANES), F32),
            pltpu.VMEM((TM, D), BF16),
            pltpu.VMEM((7, TM // 2, D // 2), BF16),
            pltpu.VMEM((TM, D), F32),
            pltpu.VMEM((7, TM // 2, D // 2), BF16),
            pltpu.VMEM((TM, 4 * LANES), F32),
            pltpu.SemaphoreType.DMA((nb,)),
            pltpu.SemaphoreType.DMA((D // PB,)),
            pltpu.SemaphoreType.DMA((5,)),
            pltpu.SemaphoreType.DMA((2 * D // UB,)),
            pltpu.SemaphoreType.DMA((nb,)),
        ],
        compiler_params=pltpu.CompilerParams(vmem_limit_bytes=127 * 1024 * 1024),
    )(A_x.reshape(S, D), A_wqkv, A_wo, B_w1, B_w3, B_w2)
    return out.reshape(B, S, D)
```

```python
import functools

import jax
import jax.numpy as jnp
import jax.experimental.pallas as pl
import jax.experimental.pallas.tpu as pltpu

N_HEADS = 32
WINDOW = 8
DILATION = 2
EPS = 1e-5
LANES = 128
HALO = 16

TM = 256
RB = 16
RC = 128
LB = 16
LC = 64
PB = 128
UB = 128
CB = 16
CW = 256
NC = 512
DUE_ENDS = (13, 27, 41)
DUE_MIDDLE = (13, 34)

F32 = jnp.float32
BF16 = jnp.bfloat16
U32 = jnp.uint32


def _dot(a, b):
    return jnp.dot(a, b, preferred_element_type=F32)


def _unpack(words):
    return pltpu.bitcast(words, BF16)


def _word_rows(r, n):
    return pl.ds(r // 2 if isinstance(r, int) else pl.multiple_of(r // 2, n // 2), n // 2)


def _token(*vals):
    regs = [pltpu.bitcast(v[r:r + 8, c:c + LANES], U32) for v in vals
            for r in range(0, v.shape[0], 8) for c in range(0, v.shape[1], LANES)]
    return functools.reduce(jnp.bitwise_or, regs)


def _after(x, tokens, never):
    if not tokens:
        return x
    words = pltpu.bitcast(x, U32)
    corner = jnp.where(never, functools.reduce(jnp.bitwise_or, tokens), words[:8, :LANES])
    top = jnp.concatenate([corner, words[:8, LANES:]], axis=1)
    return _unpack(jnp.concatenate([top, words[8:]], axis=0))


def _swap_bit(a, b, stride, axis):
    n = a.shape[axis]
    low = (jax.lax.broadcasted_iota(jnp.int32, a.shape, axis) & stride) == 0
    return (jnp.where(low, a, pltpu.roll(b, stride, axis)),
            jnp.where(low, pltpu.roll(a, n - stride, axis), b))


def _swap_bits(parts, strides, axis):
    parts = list(parts)
    for bit, stride in strides:
        for i in range(len(parts)):
            if not i & bit:
                parts[i], parts[i | bit] = _swap_bit(parts[i], parts[i | bit], stride, axis)
    return parts


def _left_operands(a11, a12, a21, a22):
    return (a11 + a22, a21 + a22, a11, a22, a11 + a12, a21 - a11, a12 - a22)


def _right_operands(b11, b12, b21, b22):
    return (b11 + b22, b11, b12 - b22, b21 - b11, b22, b11 + b12, b21 + b22)


_FEEDS = (((0, 1), (3, 1)), ((2, 1), (3, -1)), ((1, 1), (3, 1)), ((0, 1), (2, 1)),
          ((0, -1), (1, 1)), ((3, 1),), ((0, 1),))


def _block_product(product):
    c = [None] * 4
    for i, feeds in enumerate(_FEEDS):
        m = product(i)
        for k, sign in feeds:
            c[k] = m if c[k] is None else (c[k] + m if sign > 0 else c[k] - m)
    return c


def _twice(operands, grid):
    outer = [operands(*[grid[2 * a + u][2 * b + v] for a in range(2) for b in range(2)])
             for u in range(2) for v in range(2)]
    return [op for quarters in zip(*outer) for op in operands(*quarters)]


def _kernel(x_hbm, wqkv_hbm, wo_hbm, w1_hbm, w3_hbm, w2_hbm, out_hbm,
            io_s, x_s, wqkv_raw, wo_raw, wqkv_s, wo_s, w1_raw, w3_raw, up_s, down_s, in_s, out_s,
            qkv_s, xp_s, xa_s, o_s, oa_s, hl_s, in_sem, qkv_sem, w_sem, up_sem, out_sem):
    S, D = x_s.shape
    F = w3_raw.shape[1]
    TH, DH, FH = TM // 2, D // 2, F // 2
    TQ, DQ, FQ = TM // 4, D // 4, F // 4
    nb = S // TM
    n_items = 2 * nb
    nc = D // LANES
    scale = (D // N_HEADS) ** -0.5

    def slots(ref, n_rows, n_cols):
        return [ref.at[pl.ds(r, n_rows), pl.ds(c, n_cols)]
                for r in range(0, ref.shape[0] - n_rows + 1, n_rows)
                for c in range(0, ref.shape[1] - n_cols + 1, n_cols)]

    n_tiles = FQ // LANES
    xb_ops = slots(wo_raw, TQ, DQ)[:49]
    h_pairs = slots(wqkv_raw, TQ, 2 * LANES)
    down_ops = slots(wqkv_s, FQ // 2, DQ) + slots(down_s, FQ // 2, DQ)
    assert len(xb_ops) == len(down_ops) == 49 and len(h_pairs) >= 25 * n_tiles

    def rows(j):
        return pl.ds(j * TM if isinstance(j, int) else pl.multiple_of(j * TM, TM), TM)

    def x_copy(j):
        return pltpu.make_async_copy(x_hbm.at[rows(j)], io_s.at[rows(j)], in_sem.at[j])

    def out_copy(j):
        return pltpu.make_async_copy(io_s.at[rows(j)], out_hbm.at[rows(j)], out_sem.at[j])

    def wqkv_copy(i):
        rr = pl.ds(i * PB if isinstance(i, int) else pl.multiple_of(i * PB, PB), PB)
        return pltpu.make_async_copy(wqkv_hbm.at[rr], wqkv_raw.at[rr], qkv_sem.at[i])

    wo_copy = pltpu.make_async_copy(wo_hbm, wo_raw, w_sem.at[0])
    w2_quarters = [w.at[pl.ds(0, FQ), pl.ds(c, D)] for w in (w1_raw, w3_raw) for c in (0, D)]
    w2_copies = [pltpu.make_async_copy(w2_hbm.at[pl.ds(a * FQ, FQ)], dst, w_sem.at[1 + a])
                 for a, dst in enumerate(w2_quarters)]

    def up_copies(r):
        at = [pl.ds(pl.multiple_of(a * DQ + r * UB, UB), UB) for a in range(4)]
        return [pltpu.make_async_copy(src.at[at[a]], dst.at[at[a]], up_sem.at[8 * r + 4 * m + a])
                for m, (src, dst) in enumerate(((w1_hbm, w1_raw), (w3_hbm, w3_raw))) for a in range(4)]

    def chunk(r):
        return pl.ds(r * PB if isinstance(r, int) else pl.multiple_of(r * PB, PB), PB)

    def permute_qkv_columns(r):
        for i in range(3):
            cols = [pl.ds(i * D + c * LANES, LANES) for c in range(nc)]
            parts = [pltpu.bitcast(wqkv_raw[chunk(r), cc], U32) for cc in cols]
            for cc, part in zip(cols, _swap_bits(parts, ((4, 16), (2, 8), (1, 4)), 1)):
                wqkv_s[_word_rows(r * PB, PB), cc] = part

    def project_partial(r):
        y = _dot(xp_s[:, chunk(r)], _unpack(wqkv_s[_word_rows(r * PB, PB), :]))
        for t in range(3 * nc):
            qkv_s[t, pl.ds(HALO, TM), :] += y[:, t * LANES:(t + 1) * LANES]

    def combine(operands, blocks, store):
        halves = [operands(jax.tree.map(
            lambda w: pltpu.unpack_elementwise(w, index=k, packed_dtype=BF16, unpacked_dtype=F32), blocks))
            for k in range(2)]
        for i, pair in enumerate(zip(*halves)):
            store(i, pltpu.pack_elementwise(list(pair), packed_dtype=BF16).astype(U32))

    def combine_up(r):
        @pl.loop(0, n_tiles)
        def _(t):
            dst = up_s.at[:, _word_rows(r * UB, UB), pl.ds(pl.multiple_of(2 * t * LANES, LANES), 2 * LANES)]
            for m, w in enumerate((w1_raw, w3_raw)):
                src = w.at[pl.ds(pl.multiple_of(r * UB, UB), 3 * DQ + UB),
                           pl.ds(pl.multiple_of(t * LANES, LANES), 3 * FQ + LANES)]
                for r0 in range(0, UB, 16):
                    grid = [[pltpu.bitcast(src[pl.ds(a * DQ + r0, 16), pl.ds(b * FQ, LANES)], U32)
                             for b in range(4)] for a in range(4)]

                    def store(i, words):
                        dst[i, _word_rows(r0, 16), pl.ds(m * LANES, LANES)] = words
                    combine(functools.partial(_twice, _right_operands), grid, store)

    def combine_down():
        @pl.loop(0, FQ // CB)
        def _(g):
            for c in range(0, DQ, LANES):
                grid = [[pltpu.bitcast(w[pl.ds(pl.multiple_of(g * CB, CB), CB), pl.ds(b * DQ + c, LANES)], U32)
                         for b in range(4)] for w in w2_quarters]

                def store(i, words):
                    down_ops[i][_word_rows(g * CB, CB), pl.ds(c, LANES)] = words
                combine(functools.partial(_twice, _right_operands), grid, store)

    def combine_all(src, dst):
        half_rows, half_cols = src.shape[0], src.shape[1] // 2

        @pl.loop(0, half_rows // CB)
        def _(g):
            for c in range(0, half_cols, CW):
                blocks = [src[_word_rows(g * CB + dr, CB), pl.ds(dc + c, CW)]
                          for dr in (0, half_rows) for dc in (0, half_cols)]

                def store(i, words):
                    dst[i, _word_rows(g * CB, CB), pl.ds(c, CW)] = words
                combine(lambda b: _right_operands(*b), blocks, store)

    def permute_wo_rows():
        def body(hh, carry):
            def tile(h432, d4):
                return pl.ds(pl.multiple_of(h432 * 128 + hh * 32 + d4 * 16, 16), 16)
            src = [[pltpu.bitcast(wo_raw[tile(h, d4), :], U32) for h in range(8)] for d4 in range(2)]
            src = [_swap_bits(p, ((2, 4), (1, 2)), 0) for p in src]
            for d4 in range(2):
                for h in range(8):
                    wo_s[_word_rows(((h & 3) | (d4 << 2)) * 128 + hh * 32 + (h >> 2) * 16, 16), :] = src[d4][h]
            return carry
        jax.lax.fori_loop(0, 4, body, 0)

    def residual(rr, fresh):
        if fresh is None:
            return x_s[rr, :]
        return jnp.where(fresh, io_s[rr, :].astype(F32), x_s[rr, :])

    def normed(j, fresh, r, n):
        x = residual(pl.ds(pl.multiple_of(j * TM + r, n), n), fresh)
        xc = x - jnp.mean(x, axis=-1, keepdims=True)
        var = jnp.mean(xc * xc, axis=-1, keepdims=True)
        return xc * jax.lax.rsqrt(var + EPS)

    def store_left_operands(dst, r, top, bottom):
        ops = _left_operands(top[:, :DH], top[:, DH:], bottom[:, :DH], bottom[:, DH:])
        for i, a in enumerate(ops):
            dst[i, pl.ds(r, top.shape[0]), :] = a.astype(BF16)
        return _token(ops[0], ops[1], ops[4])

    def norm(j, fresh, dst, r, n, plain=None):
        top, bottom = normed(j, fresh, r, n), normed(j, fresh, TH + r, n)
        if plain is not None:
            plain[pl.ds(r, n), :] = top.astype(BF16)
            plain[pl.ds(TH + r, n), :] = bottom.astype(BF16)
        return store_left_operands(dst, r, top, bottom)

    def norm_for_ffn(j, r, n):
        quarters = [normed(j, None, a * TQ + r, n) for a in range(4)]
        ops = _twice(_left_operands, [[y[:, b * DQ:(b + 1) * DQ] for b in range(4)] for y in quarters])
        for i, a in enumerate(ops):
            xb_ops[i][pl.ds(r, n), :] = a.astype(BF16)
        return _token(*quarters)

    def attention_operands(r, n):
        return store_left_operands(oa_s, r, o_s[pl.ds(r, n), :], o_s[pl.ds(TH + r, n), :])

    def matmul(left, right, width, side_job, never, finish):
        tokens = []
        for p in range(right.shape[2] // width):
            def product(i):
                nonlocal tokens
                m = _dot(_after(left[i], tokens, never), _unpack(right[i, :, pl.ds(p * width, width)]))
                tokens = side_job(7 * p + i)
                return m
            finish(p, _block_product(product))

    def spread(items, i, n):
        return items[i * len(items) // n:(i + 1) * len(items) // n]

    def first_token(t):
        return jnp.broadcast_to(qkv_s[t, pl.ds(HALO, 1), :], (HALO, LANES))

    def project(j, side_job, never):
        per = DH // LANES
        tiles = [[half * 3 * nc // 2 + p * per + c for c in range(per)] for p in range(3) for half in range(2)]
        tails = {t: qkv_s[t, pl.ds(TM, HALO), :] for t in range(nc, 3 * nc)}

        def finish(p, blocks):
            for k, y in enumerate(blocks):
                for c, t in enumerate(tiles[2 * p + k % 2]):
                    yc = y[:, c * LANES:(c + 1) * LANES]
                    qkv_s[t, pl.ds(HALO + k // 2 * TH, TH), :] = yc
                    if t in tails and k < 2:
                        head = jnp.broadcast_to(yc[0:1, :], (HALO, LANES))
                        qkv_s[t, pl.ds(0, HALO), :] = jnp.where(j == 0, head, tails[t])
        matmul(xa_s, in_s, DH, side_job, never, finish)

    def out_project(j, fresh, never):
        def finish(p, blocks):
            for k, y in enumerate(blocks):
                at = (pl.ds(pl.multiple_of(j * TM + k // 2 * TH, TH), TH), pl.ds(k % 2 * DH, DH))
                x_s[at] = jnp.where(fresh, io_s[at].astype(F32), x_s[at]) + y
        matmul(oa_s, out_s, DH, lambda i: [], never, finish)

    def attention(j, r, n, masked):
        lane = jax.lax.broadcasted_iota(jnp.int32, (n, LANES), 1)
        logits = [None] * WINDOW
        for c in range(nc):
            q = qkv_s[c, pl.ds(HALO + r, n), :]
            for w in range(WINDOW):
                p = q * qkv_s[nc + c, pl.ds(HALO + r - DILATION * w, n), :]
                logits[w] = p if c == 0 else logits[w] + p
        for s in (1, 2):
            logits = [l + jnp.where((lane & s) == 0, pltpu.roll(l, LANES - s, 1), pltpu.roll(l, s, 1))
                      for l in logits]
        logits = [l * scale for l in logits]
        if masked:
            pos = j * TM + r + jax.lax.broadcasted_iota(jnp.int32, (n, LANES), 0)
            logits = [jnp.where(pos >= DILATION * w, l, -1e9) if w else l for w, l in enumerate(logits)]
        m = functools.reduce(jnp.maximum, logits)
        e = [jnp.exp(l - m) for l in logits]
        inv = 1.0 / functools.reduce(jnp.add, e)
        p = [x * inv for x in e]
        outs = []
        for c in range(nc):
            terms = [p[w] * qkv_s[2 * nc + c, pl.ds(HALO + r - DILATION * w, n), :] for w in range(WINDOW)]
            outs.append(functools.reduce(jnp.add, terms))
            o_s[pl.ds(r, n), pl.ds(c * LANES, LANES)] = outs[-1]
        return _token(*outs)

    def matmul_twice(left, right, side_job, never, tokens):
        def outer(i):
            def inner(k):
                nonlocal tokens
                m = _dot(_after(left(7 * i + k), tokens, never), _unpack(right(7 * i + k)))
                tokens = side_job(7 * i + k)
                return m
            return jnp.concatenate(_block_product(inner), axis=0)

        c = _block_product(outer)
        return [[c[a // 2 * 2 + b // 2][(a % 2 * 2 + b % 2) * TQ:][:TQ] for b in range(4)]
                for a in range(4)], tokens

    def ffn_up(side_job, never):
        tokens = []
        for t in range(n_tiles):
            grid, tokens = matmul_twice(lambda i: xb_ops[i][...],
                                        lambda i: up_s[i, :, pl.ds(2 * t * LANES, 2 * LANES)],
                                        lambda i: side_job(49 * t + i), never, tokens)

            def swiglu(gu):
                half = 0.5 * gu[:, :LANES]
                return (half + half * jnp.tanh(half)) * gu[:, LANES:]
            grid = jax.tree.map(swiglu, grid)
            if t == n_tiles - 1:
                for a in range(4):
                    hl_s[pl.ds(a * TQ, TQ), :] = jnp.concatenate(grid[a], axis=1)
                continue
            ops = _twice(_left_operands, grid)
            for i in range(0, 49, 2):
                pair = jnp.concatenate(ops[i:i + 2], axis=1)
                h_pairs[i // 2 * n_tiles + t][:, pl.ds(0, pair.shape[1])] = pair.astype(BF16)

    def ffn_down(j, side_job, never):
        last_tile = _twice(_left_operands, [[hl_s[pl.ds(a * TQ, TQ), pl.ds(b * LANES, LANES)]
                                             for b in range(4)] for a in range(4)])

        def hidden(i):
            tiles = [h_pairs[i // 2 * n_tiles + t][:, pl.ds(i % 2 * LANES, LANES)] for t in range(n_tiles - 1)]
            return jnp.concatenate(tiles + [last_tile[i].astype(BF16)], axis=1)

        grid, _ = matmul_twice(hidden, lambda i: down_ops[i][...], side_job, never, [])
        for a in range(4):
            for b in range(4):
                at = (pl.ds(pl.multiple_of(j * TM + a * TQ, TQ), TQ), pl.ds(b * DQ, DQ))
                y = x_s[at] + grid[a][b]
                x_s[at] = y
                io_s[at] = y.astype(BF16)

    def start_in_order(n, copies):
        @pl.loop(0, n)
        def _(i):
            for copy in copies(i):
                copy.start()

    x_copy(0).start()
    start_in_order(D // PB, lambda r: [wqkv_copy(r)])

    last = n_items - 1

    @pl.loop(-2, n_items)
    def _(n):
        j0 = jnp.maximum(n, 0) % nb
        j1 = jnp.maximum(n + 1, 0) % nb
        j2 = (n + 2) % nb
        never = n > n_items

        att = [functools.partial(attention, j1, r, RB, r < HALO) for r in range(0, TM, RB)]

        def side_job(steps, n_slots):
            return lambda i: [step() for step in spread(steps, i, n_slots) if i < n_slots]

        @pl.when(n + 2 < nb)
        def _():
            x_copy(j2).wait()

        @pl.when(n == 0)
        def _():
            @pl.loop(0, DQ // UB)
            def _(r):
                for copy in up_copies(r):
                    copy.wait()
                combine_up(r)

            for copy in w2_copies:
                copy.start()

        @pl.when(n >= 0)
        def _():
            due = [49 * t + i for t in range(n_tiles) for i in (DUE_MIDDLE if 0 < t < n_tiles - 1 else DUE_ENDS)]
            due = dict(zip(due, att, strict=True))
            ffn_up(lambda i: [due[i]()] if i in due else [], never)

        @pl.when(n == -1)
        def _():
            @pl.loop(0, TM // RC)
            def _(g):
                attention(j1, pl.multiple_of(g * RC, RC), RC, True)

            wo_copy.wait()
            permute_wo_rows()
            combine_all(wo_s, out_s)
            combine_all(wqkv_s, in_s)
            attention_operands(0, TH)

        @pl.when(n == 0)
        def _():
            for copy in w2_copies:
                copy.wait()
            combine_down()

        @pl.when(n >= 0)
        def _():
            steps = [functools.partial(norm, j2, n + 2 < nb, xa_s, r, LB) for r in range(0, TH, LB)]
            steps += [functools.partial(attention_operands, r, LB) for r in range(0, TH, LB)]
            ffn_down(j0, side_job(steps, 35), never)

        @pl.when(n < 0)
        def _():
            norm(j2, n + 2 < nb, xa_s, 0, TH, plain=xp_s)

        @pl.when(n == -2)
        def _():
            x_copy(1).start()
            wo_copy.start()
            x_copy(2).start()
            start_in_order(DQ // UB, up_copies)
            start_in_order(nb - 3, lambda j: [x_copy(j + 3)])
            qkv_s[...] = jnp.zeros(qkv_s.shape, F32)

            n_chunks = D // PB

            @pl.loop(0, n_chunks + 1)
            def _(r):
                @pl.when(r < n_chunks)
                def _():
                    wqkv_copy(r).wait()

                @pl.when(r == 0)
                def _():
                    permute_qkv_columns(0)

                @pl.when(r > 0)
                def _():
                    project_partial(r - 1)
                    permute_qkv_columns(jnp.minimum(r, n_chunks - 1))

            for t in range(nc, 3 * nc):
                qkv_s[t, pl.ds(0, HALO), :] = first_token(t)

        @pl.when(n >= nb)
        def _():
            out_copy(j0).start()

        @pl.when(jnp.logical_and(n >= -1, n < last - 1))
        def _():
            out_project(j1, n + 1 < nb, never)
            project(j2, side_job([functools.partial(norm_for_ffn, j1, r, LB) for r in range(0, TQ, LB)], 20), never)

        @pl.when(n == last - 1)
        def _():
            @pl.loop(0, D // NC)
            def _(i):
                cols = pl.ds(pl.multiple_of(i * NC, NC), NC)
                x_s[rows(j1), cols] += _dot(o_s[...].astype(BF16), _unpack(wo_s[:, cols]))


            @pl.loop(0, TQ // LC)
            def _(g):
                norm_for_ffn(j1, pl.multiple_of(g * LC, LC), LC)

    for j in range(nb):
        out_copy(j).wait()


@jax.jit
def pallas_interleave_layers__sliding_local_dilated__glu_gated_swiglu__prompt_kernel(
    A_x: jax.Array,
    A_wqkv: jax.Array,
    A_wo: jax.Array,
    B_x: jax.Array,
    B_w1: jax.Array,
    B_w3: jax.Array,
    B_w2: jax.Array,
):
    del B_x
    B, S, D = A_x.shape
    F = B_w1.shape[1]
    assert B == 1 and D == N_HEADS * 32 == 8 * LANES and S % TM == 0 and S // TM >= 3 and F == 28 * LANES
    nb = S // TM
    nc = D // LANES
    any_spec = pl.BlockSpec(memory_space=pl.ANY)
    out = pl.pallas_call(
        _kernel,
        out_shape=jax.ShapeDtypeStruct((S, D), A_x.dtype),
        in_specs=[any_spec] * 6,
        out_specs=any_spec,
        scratch_shapes=[
            pltpu.VMEM((S, D), BF16),
            pltpu.VMEM((S, D), F32),
            pltpu.VMEM((D, 3 * D), BF16),
            pltpu.VMEM((D, D), BF16),
            pltpu.VMEM((D // 2, 3 * D), U32),
            pltpu.VMEM((D // 2, D), U32),
            pltpu.VMEM((D, F), BF16),
            pltpu.VMEM((D, F), BF16),
            pltpu.VMEM((49, D // 8, F // 2), U32),
            pltpu.VMEM((F // 8, (49 - 12) * D // 4), U32),
            pltpu.VMEM((7, D // 4, 3 * D // 2), U32),
            pltpu.VMEM((7, D // 4, D // 2), U32),
            pltpu.VMEM((3 * nc, HALO + TM, LANES), F32),
            pltpu.VMEM((TM, D), BF16),
            pltpu.VMEM((7, TM // 2, D // 2), BF16),
            pltpu.VMEM((TM, D), F32),
            pltpu.VMEM((7, TM // 2, D // 2), BF16),
            pltpu.VMEM((TM, 4 * LANES), F32),
            pltpu.SemaphoreType.DMA((nb,)),
            pltpu.SemaphoreType.DMA((D // PB,)),
            pltpu.SemaphoreType.DMA((5,)),
            pltpu.SemaphoreType.DMA((2 * D // UB,)),
            pltpu.SemaphoreType.DMA((nb,)),
        ],
        compiler_params=pltpu.CompilerParams(vmem_limit_bytes=127 * 1024 * 1024),
    )(A_x.reshape(S, D), A_wqkv, A_wo, B_w1, B_w3, B_w2)
    return out.reshape(B, S, D)
```

```python
import functools

import jax
import jax.numpy as jnp
import jax.experimental.pallas as pl
import jax.experimental.pallas.tpu as pltpu

N_HEADS = 32
WINDOW = 8
DILATION = 2
EPS = 1e-5
LANES = 128
HALO = 16

TM = 256
RB = 16
RC = 128
LB = 16
LC = 64
QW = 512
OW = 256
PB = 128
UB = 128
CB = 16
CW = 256
NC = 512
DUE_ENDS = (13, 27, 41)
DUE_MIDDLE = (13, 34)

F32 = jnp.float32
BF16 = jnp.bfloat16
U32 = jnp.uint32


def _dot(a, b):
    return jnp.dot(a, b, preferred_element_type=F32)


def _unpack(words):
    return pltpu.bitcast(words, BF16)


def _word_rows(r, n):
    return pl.ds(r // 2 if isinstance(r, int) else pl.multiple_of(r // 2, n // 2), n // 2)


def _token(*vals):
    regs = [pltpu.bitcast(v[r:r + 8, c:c + LANES], U32) for v in vals
            for r in range(0, v.shape[0], 8) for c in range(0, v.shape[1], LANES)]
    return functools.reduce(jnp.bitwise_or, regs)


def _after(x, tokens, never):
    if not tokens:
        return x
    words = pltpu.bitcast(x, U32)
    corner = jnp.where(never, functools.reduce(jnp.bitwise_or, tokens), words[:8, :LANES])
    top = jnp.concatenate([corner, words[:8, LANES:]], axis=1)
    return _unpack(jnp.concatenate([top, words[8:]], axis=0))


def _swap_bit(a, b, stride, axis):
    n = a.shape[axis]
    low = (jax.lax.broadcasted_iota(jnp.int32, a.shape, axis) & stride) == 0
    return (jnp.where(low, a, pltpu.roll(b, stride, axis)),
            jnp.where(low, pltpu.roll(a, n - stride, axis), b))


def _swap_bits(parts, strides, axis):
    parts = list(parts)
    for bit, stride in strides:
        for i in range(len(parts)):
            if not i & bit:
                parts[i], parts[i | bit] = _swap_bit(parts[i], parts[i | bit], stride, axis)
    return parts


def _left_operands(a11, a12, a21, a22):
    return (a11 + a22, a21 + a22, a11, a22, a11 + a12, a21 - a11, a12 - a22)


def _right_operands(b11, b12, b21, b22):
    return (b11 + b22, b11, b12 - b22, b21 - b11, b22, b11 + b12, b21 + b22)


_FEEDS = (((0, 1), (3, 1)), ((2, 1), (3, -1)), ((1, 1), (3, 1)), ((0, 1), (2, 1)),
          ((0, -1), (1, 1)), ((3, 1),), ((0, 1),))


def _block_product(product):
    c = [None] * 4
    for i, feeds in enumerate(_FEEDS):
        m = product(i)
        for k, sign in feeds:
            c[k] = m if c[k] is None else (c[k] + m if sign > 0 else c[k] - m)
    return c


def _twice(operands, grid):
    outer = [operands(*[grid[2 * a + u][2 * b + v] for a in range(2) for b in range(2)])
             for u in range(2) for v in range(2)]
    return [op for quarters in zip(*outer) for op in operands(*quarters)]


def _kernel(x_hbm, wqkv_hbm, wo_hbm, w1_hbm, w3_hbm, w2_hbm, out_hbm,
            io_s, x_s, wqkv_raw, wo_raw, wqkv_s, wo_s, w1_raw, w3_raw, up_s, down_s, in_s, out_s,
            qkv_s, xp_s, xa_s, o_s, oa_s, hl_s, in_sem, qkv_sem, w_sem, up_sem, out_sem):
    S, D = x_s.shape
    F = w3_raw.shape[1]
    TH, DH, FH = TM // 2, D // 2, F // 2
    TQ, DQ, FQ = TM // 4, D // 4, F // 4
    nb = S // TM
    n_items = 2 * nb
    nc = D // LANES
    scale = (D // N_HEADS) ** -0.5

    def slots(ref, n_rows, n_cols):
        return [ref.at[pl.ds(r, n_rows), pl.ds(c, n_cols)]
                for r in range(0, ref.shape[0] - n_rows + 1, n_rows)
                for c in range(0, ref.shape[1] - n_cols + 1, n_cols)]

    n_tiles = FQ // LANES
    xb_ops = slots(wo_raw, TQ, DQ)[:49]
    h_pairs = slots(wqkv_raw, TQ, 2 * LANES)
    down_ops = slots(wqkv_s, FQ // 2, DQ) + slots(down_s, FQ // 2, DQ)
    assert len(xb_ops) == len(down_ops) == 49 and len(h_pairs) >= 25 * n_tiles

    def rows(j):
        return pl.ds(j * TM if isinstance(j, int) else pl.multiple_of(j * TM, TM), TM)

    def x_copy(j):
        return pltpu.make_async_copy(x_hbm.at[rows(j)], io_s.at[rows(j)], in_sem.at[j])

    def out_copy(j):
        return pltpu.make_async_copy(io_s.at[rows(j)], out_hbm.at[rows(j)], out_sem.at[j])

    def wqkv_copy(i):
        rr = pl.ds(i * PB if isinstance(i, int) else pl.multiple_of(i * PB, PB), PB)
        return pltpu.make_async_copy(wqkv_hbm.at[rr], wqkv_raw.at[rr], qkv_sem.at[i])

    wo_copy = pltpu.make_async_copy(wo_hbm, wo_raw, w_sem.at[0])
    w2_quarters = [w.at[pl.ds(0, FQ), pl.ds(c, D)] for w in (w1_raw, w3_raw) for c in (0, D)]
    w2_copies = [pltpu.make_async_copy(w2_hbm.at[pl.ds(a * FQ, FQ)], dst, w_sem.at[1 + a])
                 for a, dst in enumerate(w2_quarters)]

    def up_copies(r):
        at = [pl.ds(pl.multiple_of(a * DQ + r * UB, UB), UB) for a in range(4)]
        return [pltpu.make_async_copy(src.at[at[a]], dst.at[at[a]], up_sem.at[8 * r + 4 * m + a])
                for m, (src, dst) in enumerate(((w1_hbm, w1_raw), (w3_hbm, w3_raw))) for a in range(4)]

    def chunk(r):
        return pl.ds(r * PB if isinstance(r, int) else pl.multiple_of(r * PB, PB), PB)

    def permute_qkv_columns(r):
        for i in range(3):
            cols = [pl.ds(i * D + c * LANES, LANES) for c in range(nc)]
            parts = [pltpu.bitcast(wqkv_raw[chunk(r), cc], U32) for cc in cols]
            for cc, part in zip(cols, _swap_bits(parts, ((4, 16), (2, 8), (1, 4)), 1)):
                wqkv_s[_word_rows(r * PB, PB), cc] = part

    def project_partial(r):
        y = _dot(xp_s[:, chunk(r)], _unpack(wqkv_s[_word_rows(r * PB, PB), :]))
        for t in range(3 * nc):
            qkv_s[t, pl.ds(HALO, TM), :] += y[:, t * LANES:(t + 1) * LANES]

    def combine(operands, blocks, store):
        halves = [operands(jax.tree.map(
            lambda w: pltpu.unpack_elementwise(w, index=k, packed_dtype=BF16, unpacked_dtype=F32), blocks))
            for k in range(2)]
        for i, pair in enumerate(zip(*halves)):
            store(i, pltpu.pack_elementwise(list(pair), packed_dtype=BF16).astype(U32))

    def combine_up(r):
        @pl.loop(0, n_tiles)
        def _(t):
            dst = up_s.at[:, _word_rows(r * UB, UB), pl.ds(pl.multiple_of(2 * t * LANES, LANES), 2 * LANES)]
            for m, w in enumerate((w1_raw, w3_raw)):
                src = w.at[pl.ds(pl.multiple_of(r * UB, UB), 3 * DQ + UB),
                           pl.ds(pl.multiple_of(t * LANES, LANES), 3 * FQ + LANES)]
                for r0 in range(0, UB, 16):
                    grid = [[pltpu.bitcast(src[pl.ds(a * DQ + r0, 16), pl.ds(b * FQ, LANES)], U32)
                             for b in range(4)] for a in range(4)]

                    def store(i, words):
                        dst[i, _word_rows(r0, 16), pl.ds(m * LANES, LANES)] = words
                    combine(functools.partial(_twice, _right_operands), grid, store)

    def combine_down():
        @pl.loop(0, FQ // CB)
        def _(g):
            for c in range(0, DQ, LANES):
                grid = [[pltpu.bitcast(w[pl.ds(pl.multiple_of(g * CB, CB), CB), pl.ds(b * DQ + c, LANES)], U32)
                         for b in range(4)] for w in w2_quarters]

                def store(i, words):
                    down_ops[i][_word_rows(g * CB, CB), pl.ds(c, LANES)] = words
                combine(functools.partial(_twice, _right_operands), grid, store)

    def combine_all(src, dst):
        half_rows, half_cols = src.shape[0], src.shape[1] // 2

        @pl.loop(0, half_rows // CB)
        def _(g):
            for c in range(0, half_cols, CW):
                blocks = [src[_word_rows(g * CB + dr, CB), pl.ds(dc + c, CW)]
                          for dr in (0, half_rows) for dc in (0, half_cols)]

                def store(i, words):
                    dst[i, _word_rows(g * CB, CB), pl.ds(c, CW)] = words
                combine(lambda b: _right_operands(*b), blocks, store)

    def permute_wo_rows():
        def body(hh, carry):
            def tile(h432, d4):
                return pl.ds(pl.multiple_of(h432 * 128 + hh * 32 + d4 * 16, 16), 16)
            src = [[pltpu.bitcast(wo_raw[tile(h, d4), :], U32) for h in range(8)] for d4 in range(2)]
            src = [_swap_bits(p, ((2, 4), (1, 2)), 0) for p in src]
            for d4 in range(2):
                for h in range(8):
                    wo_s[_word_rows(((h & 3) | (d4 << 2)) * 128 + hh * 32 + (h >> 2) * 16, 16), :] = src[d4][h]
            return carry
        jax.lax.fori_loop(0, 4, body, 0)

    def residual(rr, fresh):
        if fresh is None:
            return x_s[rr, :]
        return jnp.where(fresh, io_s[rr, :].astype(F32), x_s[rr, :])

    def normed(j, fresh, r, n):
        x = residual(pl.ds(pl.multiple_of(j * TM + r, n), n), fresh)
        xc = x - jnp.mean(x, axis=-1, keepdims=True)
        var = jnp.mean(xc * xc, axis=-1, keepdims=True)
        return xc * jax.lax.rsqrt(var + EPS)

    def store_left_operands(dst, r, top, bottom):
        ops = _left_operands(top[:, :DH], top[:, DH:], bottom[:, :DH], bottom[:, DH:])
        for i, a in enumerate(ops):
            dst[i, pl.ds(r, top.shape[0]), :] = a.astype(BF16)
        return _token(ops[0], ops[1], ops[4])

    def norm(j, fresh, dst, r, n, plain=None):
        top, bottom = normed(j, fresh, r, n), normed(j, fresh, TH + r, n)
        if plain is not None:
            plain[pl.ds(r, n), :] = top.astype(BF16)
            plain[pl.ds(TH + r, n), :] = bottom.astype(BF16)
        return store_left_operands(dst, r, top, bottom)

    def norm_for_ffn(j, r, n):
        quarters = [normed(j, None, a * TQ + r, n) for a in range(4)]
        ops = _twice(_left_operands, [[y[:, b * DQ:(b + 1) * DQ] for b in range(4)] for y in quarters])
        for i, a in enumerate(ops):
            xb_ops[i][pl.ds(r, n), :] = a.astype(BF16)
        return _token(*quarters)

    def attention_operands(r, n):
        return store_left_operands(oa_s, r, o_s[pl.ds(r, n), :], o_s[pl.ds(TH + r, n), :])

    def matmul(left, right, width, side_job, never, finish):
        tokens = []
        for p in range(right.shape[2] // width):
            def product(i):
                nonlocal tokens
                m = _dot(_after(left[i], tokens, never), _unpack(right[i, :, pl.ds(p * width, width)]))
                tokens = side_job(7 * p + i)
                return m
            finish(p, _block_product(product))

    def spread(items, i, n):
        return items[i * len(items) // n:(i + 1) * len(items) // n]

    def first_token(t):
        return jnp.broadcast_to(qkv_s[t, pl.ds(HALO, 1), :], (HALO, LANES))

    def project(j, side_job, never):
        per = QW // LANES
        tiles = [[half * 3 * nc // 2 + p * per + c for c in range(per)]
                 for p in range(3 * DH // QW) for half in range(2)]
        tails = {t: qkv_s[t, pl.ds(TM, HALO), :] for t in range(nc, 3 * nc)}

        def finish(p, blocks):
            for k, y in enumerate(blocks):
                for c, t in enumerate(tiles[2 * p + k % 2]):
                    yc = y[:, c * LANES:(c + 1) * LANES]
                    qkv_s[t, pl.ds(HALO + k // 2 * TH, TH), :] = yc
                    if t in tails and k < 2:
                        head = jnp.broadcast_to(yc[0:1, :], (HALO, LANES))
                        qkv_s[t, pl.ds(0, HALO), :] = jnp.where(j == 0, head, tails[t])
        matmul(xa_s, in_s, QW, side_job, never, finish)

    def out_project(j, fresh, never):
        def finish(p, blocks):
            for k, y in enumerate(blocks):
                at = (pl.ds(pl.multiple_of(j * TM + k // 2 * TH, TH), TH), pl.ds(k % 2 * DH + p * OW, OW))
                x_s[at] = jnp.where(fresh, io_s[at].astype(F32), x_s[at]) + y
        matmul(oa_s, out_s, OW, lambda i: [], never, finish)

    def attention(j, r, n, masked):
        lane = jax.lax.broadcasted_iota(jnp.int32, (n, LANES), 1)
        logits = [None] * WINDOW
        for c in range(nc):
            q = qkv_s[c, pl.ds(HALO + r, n), :]
            for w in range(WINDOW):
                p = q * qkv_s[nc + c, pl.ds(HALO + r - DILATION * w, n), :]
                logits[w] = p if c == 0 else logits[w] + p
        for s in (1, 2):
            logits = [l + jnp.where((lane & s) == 0, pltpu.roll(l, LANES - s, 1), pltpu.roll(l, s, 1))
                      for l in logits]
        logits = [l * scale for l in logits]
        if masked:
            pos = j * TM + r + jax.lax.broadcasted_iota(jnp.int32, (n, LANES), 0)
            logits = [jnp.where(pos >= DILATION * w, l, -1e9) if w else l for w, l in enumerate(logits)]
        m = functools.reduce(jnp.maximum, logits)
        e = [jnp.exp(l - m) for l in logits]
        inv = 1.0 / functools.reduce(jnp.add, e)
        p = [x * inv for x in e]
        outs = []
        for c in range(nc):
            terms = [p[w] * qkv_s[2 * nc + c, pl.ds(HALO + r - DILATION * w, n), :] for w in range(WINDOW)]
            outs.append(functools.reduce(jnp.add, terms))
            o_s[pl.ds(r, n), pl.ds(c * LANES, LANES)] = outs[-1]
        return _token(*outs)

    def matmul_twice(left, right, side_job, never, tokens):
        def outer(i):
            def inner(k):
                nonlocal tokens
                m = _dot(_after(left(7 * i + k), tokens, never), _unpack(right(7 * i + k)))
                tokens = side_job(7 * i + k)
                return m
            return jnp.concatenate(_block_product(inner), axis=0)

        c = _block_product(outer)
        return [[c[a // 2 * 2 + b // 2][(a % 2 * 2 + b % 2) * TQ:][:TQ] for b in range(4)]
                for a in range(4)], tokens

    def ffn_up(side_job, never):
        tokens = []
        for t in range(n_tiles):
            grid, tokens = matmul_twice(lambda i: xb_ops[i][...],
                                        lambda i: up_s[i, :, pl.ds(2 * t * LANES, 2 * LANES)],
                                        lambda i: side_job(49 * t + i), never, tokens)

            def swiglu(gu):
                half = 0.5 * gu[:, :LANES]
                return (half + half * jnp.tanh(half)) * gu[:, LANES:]
            grid = jax.tree.map(swiglu, grid)
            if t == n_tiles - 1:
                for a in range(4):
                    hl_s[pl.ds(a * TQ, TQ), :] = jnp.concatenate(grid[a], axis=1)
                continue
            ops = _twice(_left_operands, grid)
            for i in range(0, 49, 2):
                pair = jnp.concatenate(ops[i:i + 2], axis=1)
                h_pairs[i // 2 * n_tiles + t][:, pl.ds(0, pair.shape[1])] = pair.astype(BF16)

    def ffn_down(j, side_job, never):
        last_tile = _twice(_left_operands, [[hl_s[pl.ds(a * TQ, TQ), pl.ds(b * LANES, LANES)]
                                             for b in range(4)] for a in range(4)])

        def hidden(i):
            tiles = [h_pairs[i // 2 * n_tiles + t][:, pl.ds(i % 2 * LANES, LANES)] for t in range(n_tiles - 1)]
            return jnp.concatenate(tiles + [last_tile[i].astype(BF16)], axis=1)

        grid, _ = matmul_twice(hidden, lambda i: down_ops[i][...], side_job, never, [])
        for a in range(4):
            for b in range(4):
                at = (pl.ds(pl.multiple_of(j * TM + a * TQ, TQ), TQ), pl.ds(b * DQ, DQ))
                y = x_s[at] + grid[a][b]
                x_s[at] = y
                io_s[at] = y.astype(BF16)

    def start_in_order(n, copies):
        @pl.loop(0, n)
        def _(i):
            for copy in copies(i):
                copy.start()

    x_copy(0).start()
    start_in_order(D // PB, lambda r: [wqkv_copy(r)])

    last = n_items - 1

    @pl.loop(-2, n_items)
    def _(n):
        j0 = jnp.maximum(n, 0) % nb
        j1 = jnp.maximum(n + 1, 0) % nb
        j2 = (n + 2) % nb
        never = n > n_items

        att = [functools.partial(attention, j1, r, RB, r < HALO) for r in range(0, TM, RB)]

        def side_job(steps, n_slots):
            return lambda i: [step() for step in spread(steps, i, n_slots) if i < n_slots]

        @pl.when(n + 2 < nb)
        def _():
            x_copy(j2).wait()

        @pl.when(n == 0)
        def _():
            @pl.loop(0, DQ // UB)
            def _(r):
                for copy in up_copies(r):
                    copy.wait()
                combine_up(r)

            for copy in w2_copies:
                copy.start()

        @pl.when(n >= 0)
        def _():
            due = [49 * t + i for t in range(n_tiles) for i in (DUE_MIDDLE if 0 < t < n_tiles - 1 else DUE_ENDS)]
            due = dict(zip(due, att, strict=True))
            ffn_up(lambda i: [due[i]()] if i in due else [], never)

        @pl.when(n == -1)
        def _():
            @pl.loop(0, TM // RC)
            def _(g):
                attention(j1, pl.multiple_of(g * RC, RC), RC, True)

            wo_copy.wait()
            permute_wo_rows()
            combine_all(wo_s, out_s)
            combine_all(wqkv_s, in_s)
            attention_operands(0, TH)

        @pl.when(n == 0)
        def _():
            for copy in w2_copies:
                copy.wait()
            combine_down()

        @pl.when(n >= 0)
        def _():
            steps = [functools.partial(norm, j2, n + 2 < nb, xa_s, r, LB) for r in range(0, TH, LB)]
            steps += [functools.partial(attention_operands, r, LB) for r in range(0, TH, LB)]
            ffn_down(j0, side_job(steps, 35), never)

        @pl.when(n < 0)
        def _():
            norm(j2, n + 2 < nb, xa_s, 0, TH, plain=xp_s)

        @pl.when(n == -2)
        def _():
            x_copy(1).start()
            wo_copy.start()
            x_copy(2).start()
            start_in_order(DQ // UB, up_copies)
            start_in_order(nb - 3, lambda j: [x_copy(j + 3)])
            qkv_s[...] = jnp.zeros(qkv_s.shape, F32)

            n_chunks = D // PB

            @pl.loop(0, n_chunks + 1)
            def _(r):
                @pl.when(r < n_chunks)
                def _():
                    wqkv_copy(r).wait()

                @pl.when(r == 0)
                def _():
                    permute_qkv_columns(0)

                @pl.when(r > 0)
                def _():
                    project_partial(r - 1)
                    permute_qkv_columns(jnp.minimum(r, n_chunks - 1))

            for t in range(nc, 3 * nc):
                qkv_s[t, pl.ds(0, HALO), :] = first_token(t)

        @pl.when(n >= nb)
        def _():
            out_copy(j0).start()

        @pl.when(jnp.logical_and(n >= -1, n < last - 1))
        def _():
            out_project(j1, n + 1 < nb, never)
            project(j2, side_job([functools.partial(norm_for_ffn, j1, r, LB) for r in range(0, TQ, LB)],
                                 21 * DH // QW - 1), never)

        @pl.when(n == last - 1)
        def _():
            @pl.loop(0, D // NC)
            def _(i):
                cols = pl.ds(pl.multiple_of(i * NC, NC), NC)
                x_s[rows(j1), cols] += _dot(o_s[...].astype(BF16), _unpack(wo_s[:, cols]))


            @pl.loop(0, TQ // LC)
            def _(g):
                norm_for_ffn(j1, pl.multiple_of(g * LC, LC), LC)

    for j in range(nb):
        out_copy(j).wait()


@jax.jit
def pallas_interleave_layers__sliding_local_dilated__glu_gated_swiglu__prompt_kernel(
    A_x: jax.Array,
    A_wqkv: jax.Array,
    A_wo: jax.Array,
    B_x: jax.Array,
    B_w1: jax.Array,
    B_w3: jax.Array,
    B_w2: jax.Array,
):
    del B_x
    B, S, D = A_x.shape
    F = B_w1.shape[1]
    assert B == 1 and D == N_HEADS * 32 == 8 * LANES and S % TM == 0 and S // TM >= 3 and F == 28 * LANES
    nb = S // TM
    nc = D // LANES
    any_spec = pl.BlockSpec(memory_space=pl.ANY)
    out = pl.pallas_call(
        _kernel,
        out_shape=jax.ShapeDtypeStruct((S, D), A_x.dtype),
        in_specs=[any_spec] * 6,
        out_specs=any_spec,
        scratch_shapes=[
            pltpu.VMEM((S, D), BF16),
            pltpu.VMEM((S, D), F32),
            pltpu.VMEM((D, 3 * D), BF16),
            pltpu.VMEM((D, D), BF16),
            pltpu.VMEM((D // 2, 3 * D), U32),
            pltpu.VMEM((D // 2, D), U32),
            pltpu.VMEM((D, F), BF16),
            pltpu.VMEM((D, F), BF16),
            pltpu.VMEM((49, D // 8, F // 2), U32),
            pltpu.VMEM((F // 8, (49 - 12) * D // 4), U32),
            pltpu.VMEM((7, D // 4, 3 * D // 2), U32),
            pltpu.VMEM((7, D // 4, D // 2), U32),
            pltpu.VMEM((3 * nc, HALO + TM, LANES), F32),
            pltpu.VMEM((TM, D), BF16),
            pltpu.VMEM((7, TM // 2, D // 2), BF16),
            pltpu.VMEM((TM, D), F32),
            pltpu.VMEM((7, TM // 2, D // 2), BF16),
            pltpu.VMEM((TM, 4 * LANES), F32),
            pltpu.SemaphoreType.DMA((nb,)),
            pltpu.SemaphoreType.DMA((D // PB,)),
            pltpu.SemaphoreType.DMA((5,)),
            pltpu.SemaphoreType.DMA((2 * D // UB,)),
            pltpu.SemaphoreType.DMA((nb,)),
        ],
        compiler_params=pltpu.CompilerParams(vmem_limit_bytes=127 * 1024 * 1024),
    )(A_x.reshape(S, D), A_wqkv, A_wo, B_w1, B_w3, B_w2)
    return out.reshape(B, S, D)
```

```python
import functools

import jax
import jax.numpy as jnp
import jax.experimental.pallas as pl
import jax.experimental.pallas.tpu as pltpu

N_HEADS = 32
WINDOW = 8
DILATION = 2
EPS = 1e-5
LANES = 128
HALO = 16

TM = 256
RB = 16
RC = 128
LB = 16
LC = 64
QW = 512
OW = 256
PB = 128
UB = 128
CB = 16
CW = 256
NC = 512
DUE_ENDS = (13, 27, 41)
DUE_MIDDLE = (13, 34)

F32 = jnp.float32
BF16 = jnp.bfloat16
U32 = jnp.uint32


def _dot(a, b):
    return jnp.dot(a, b, preferred_element_type=F32)


def _unpack(words):
    return pltpu.bitcast(words, BF16)


def _word_rows(r, n):
    return pl.ds(r // 2 if isinstance(r, int) else pl.multiple_of(r // 2, n // 2), n // 2)


def _token(*vals):
    regs = [pltpu.bitcast(v[r:r + 8, c:c + LANES], U32) for v in vals
            for r in range(0, v.shape[0], 8) for c in range(0, v.shape[1], LANES)]
    return functools.reduce(jnp.bitwise_or, regs)


def _after(x, tokens, never):
    if not tokens:
        return x
    words = pltpu.bitcast(x, U32)
    corner = jnp.where(never, functools.reduce(jnp.bitwise_or, tokens), words[:8, :LANES])
    top = jnp.concatenate([corner, words[:8, LANES:]], axis=1)
    return _unpack(jnp.concatenate([top, words[8:]], axis=0))


def _swap_bit(a, b, stride, axis):
    n = a.shape[axis]
    low = (jax.lax.broadcasted_iota(jnp.int32, a.shape, axis) & stride) == 0
    return (jnp.where(low, a, pltpu.roll(b, stride, axis)),
            jnp.where(low, pltpu.roll(a, n - stride, axis), b))


def _swap_bits(parts, strides, axis):
    parts = list(parts)
    for bit, stride in strides:
        for i in range(len(parts)):
            if not i & bit:
                parts[i], parts[i | bit] = _swap_bit(parts[i], parts[i | bit], stride, axis)
    return parts


def _left_operands(a11, a12, a21, a22):
    return (a11 + a22, a21 + a22, a11, a22, a11 + a12, a21 - a11, a12 - a22)


def _right_operands(b11, b12, b21, b22):
    return (b11 + b22, b11, b12 - b22, b21 - b11, b22, b11 + b12, b21 + b22)


_FEEDS = (((0, 1), (3, 1)), ((2, 1), (3, -1)), ((1, 1), (3, 1)), ((0, 1), (2, 1)),
          ((0, -1), (1, 1)), ((3, 1),), ((0, 1),))


def _block_product(product):
    c = [None] * 4
    for i, feeds in enumerate(_FEEDS):
        m = product(i)
        for k, sign in feeds:
            c[k] = m if c[k] is None else (c[k] + m if sign > 0 else c[k] - m)
    return c


def _twice(operands, grid):
    outer = [operands(*[grid[2 * a + u][2 * b + v] for a in range(2) for b in range(2)])
             for u in range(2) for v in range(2)]
    return [op for quarters in zip(*outer) for op in operands(*quarters)]


def _kernel(x_hbm, wqkv_hbm, wo_hbm, w1_hbm, w3_hbm, w2_hbm, out_hbm,
            io_s, x_s, wqkv_raw, wo_raw, wqkv_s, wo_s, w1_raw, w3_raw, up_s, down_s, in_s, out_s,
            qkv_s, xp_s, xa_s, o_s, oa_s, hl_s, in_sem, qkv_sem, w_sem, up_sem, out_sem):
    S, D = x_s.shape
    F = w3_raw.shape[1]
    TH, DH, FH = TM // 2, D // 2, F // 2
    TQ, DQ, FQ = TM // 4, D // 4, F // 4
    nb = S // TM
    n_items = 2 * nb
    nc = D // LANES
    scale = (D // N_HEADS) ** -0.5

    def slots(ref, n_rows, n_cols):
        return [ref.at[pl.ds(r, n_rows), pl.ds(c, n_cols)]
                for r in range(0, ref.shape[0] - n_rows + 1, n_rows)
                for c in range(0, ref.shape[1] - n_cols + 1, n_cols)]

    n_tiles = FQ // LANES
    xb_ops = slots(wo_raw, TQ, DQ)[:49]
    h_pairs = slots(wqkv_raw, TQ, 2 * LANES)
    down_ops = slots(wqkv_s, FQ // 2, DQ) + slots(down_s, FQ // 2, DQ)
    assert len(xb_ops) == len(down_ops) == 49 and len(h_pairs) >= 25 * n_tiles

    def rows(j):
        return pl.ds(j * TM if isinstance(j, int) else pl.multiple_of(j * TM, TM), TM)

    def x_copy(j):
        return pltpu.make_async_copy(x_hbm.at[rows(j)], io_s.at[rows(j)], in_sem.at[j])

    def out_copy(j):
        return pltpu.make_async_copy(io_s.at[rows(j)], out_hbm.at[rows(j)], out_sem.at[j])

    def wqkv_copy(i):
        rr = pl.ds(i * PB if isinstance(i, int) else pl.multiple_of(i * PB, PB), PB)
        return pltpu.make_async_copy(wqkv_hbm.at[rr], wqkv_raw.at[rr], qkv_sem.at[i])

    wo_copy = pltpu.make_async_copy(wo_hbm, wo_raw, w_sem.at[0])
    w2_quarters = [w.at[pl.ds(0, FQ), pl.ds(c, D)] for w in (w1_raw, w3_raw) for c in (0, D)]
    w2_copies = [pltpu.make_async_copy(w2_hbm.at[pl.ds(a * FQ, FQ)], dst, w_sem.at[1 + a])
                 for a, dst in enumerate(w2_quarters)]

    def up_copies(r):
        at = [pl.ds(pl.multiple_of(a * DQ + r * UB, UB), UB) for a in range(4)]
        return [pltpu.make_async_copy(src.at[at[a]], dst.at[at[a]], up_sem.at[8 * r + 4 * m + a])
                for m, (src, dst) in enumerate(((w1_hbm, w1_raw), (w3_hbm, w3_raw))) for a in range(4)]

    def chunk(r):
        return pl.ds(r * PB if isinstance(r, int) else pl.multiple_of(r * PB, PB), PB)

    def permute_qkv_columns(r):
        for i in range(3):
            cols = [pl.ds(i * D + c * LANES, LANES) for c in range(nc)]
            parts = [pltpu.bitcast(wqkv_raw[chunk(r), cc], U32) for cc in cols]
            for cc, part in zip(cols, _swap_bits(parts, ((4, 16), (2, 8), (1, 4)), 1)):
                wqkv_s[_word_rows(r * PB, PB), cc] = part

    def project_partial(r):
        y = _dot(xp_s[:, chunk(r)], _unpack(wqkv_s[_word_rows(r * PB, PB), :]))
        for t in range(3 * nc):
            qkv_s[t, pl.ds(HALO, TM), :] += y[:, t * LANES:(t + 1) * LANES]

    def combine(operands, blocks, store):
        for i, b in enumerate(operands(jax.tree.map(lambda b: b.astype(F32), blocks))):
            store(i, pltpu.bitcast(b.astype(BF16), U32))

    def combine_up(r):
        @pl.loop(0, n_tiles)
        def _(t):
            dst = up_s.at[:, _word_rows(r * UB, UB), pl.ds(pl.multiple_of(2 * t * LANES, LANES), 2 * LANES)]
            srcs = [w.at[pl.ds(pl.multiple_of(r * UB, UB), 3 * DQ + UB),
                         pl.ds(pl.multiple_of(t * LANES, LANES), 3 * FQ + LANES)] for w in (w1_raw, w3_raw)]
            for r0 in range(0, UB, 16):
                grid = [[jnp.concatenate([w[pl.ds(a * DQ + r0, 16), pl.ds(b * FQ, LANES)].astype(F32)
                                          for w in srcs], axis=1) for b in range(4)] for a in range(4)]

                def store(i, words):
                    dst[i, _word_rows(r0, 16), :] = words
                combine(functools.partial(_twice, _right_operands), grid, store)

    def combine_down():
        @pl.loop(0, FQ // CB)
        def _(g):
            grid = [[w[pl.ds(pl.multiple_of(g * CB, CB), CB), pl.ds(b * DQ, DQ)] for b in range(4)]
                    for w in w2_quarters]

            def store(i, words):
                down_ops[i][_word_rows(g * CB, CB), :] = words
            combine(functools.partial(_twice, _right_operands), grid, store)

    def combine_all(src, dst):
        half_rows, half_cols = src.shape[0], src.shape[1] // 2

        @pl.loop(0, half_rows // CB)
        def _(g):
            for c in range(0, half_cols, CW):
                blocks = [_unpack(src[_word_rows(g * CB + dr, CB), pl.ds(dc + c, CW)])
                          for dr in (0, half_rows) for dc in (0, half_cols)]

                def store(i, words):
                    dst[i, _word_rows(g * CB, CB), pl.ds(c, CW)] = words
                combine(lambda b: _right_operands(*b), blocks, store)

    def permute_wo_rows():
        def body(hh, carry):
            def tile(h432, d4):
                return pl.ds(pl.multiple_of(h432 * 128 + hh * 32 + d4 * 16, 16), 16)
            src = [[pltpu.bitcast(wo_raw[tile(h, d4), :], U32) for h in range(8)] for d4 in range(2)]
            src = [_swap_bits(p, ((2, 4), (1, 2)), 0) for p in src]
            for d4 in range(2):
                for h in range(8):
                    wo_s[_word_rows(((h & 3) | (d4 << 2)) * 128 + hh * 32 + (h >> 2) * 16, 16), :] = src[d4][h]
            return carry
        jax.lax.fori_loop(0, 4, body, 0)

    def residual(rr, fresh):
        if fresh is None:
            return x_s[rr, :]
        return jnp.where(fresh, io_s[rr, :].astype(F32), x_s[rr, :])

    def normed(j, fresh, r, n):
        x = residual(pl.ds(pl.multiple_of(j * TM + r, n), n), fresh)
        xc = x - jnp.mean(x, axis=-1, keepdims=True)
        var = jnp.mean(xc * xc, axis=-1, keepdims=True)
        return xc * jax.lax.rsqrt(var + EPS)

    def store_left_operands(dst, r, top, bottom):
        ops = _left_operands(top[:, :DH], top[:, DH:], bottom[:, :DH], bottom[:, DH:])
        for i, a in enumerate(ops):
            dst[i, pl.ds(r, top.shape[0]), :] = a.astype(BF16)
        return _token(ops[0], ops[1], ops[4])

    def norm(j, fresh, dst, r, n, plain=None):
        top, bottom = normed(j, fresh, r, n), normed(j, fresh, TH + r, n)
        if plain is not None:
            plain[pl.ds(r, n), :] = top.astype(BF16)
            plain[pl.ds(TH + r, n), :] = bottom.astype(BF16)
        return store_left_operands(dst, r, top, bottom)

    def norm_for_ffn(j, r, n):
        quarters = [normed(j, None, a * TQ + r, n) for a in range(4)]
        ops = _twice(_left_operands, [[y[:, b * DQ:(b + 1) * DQ] for b in range(4)] for y in quarters])
        for i, a in enumerate(ops):
            xb_ops[i][pl.ds(r, n), :] = a.astype(BF16)
        return _token(*quarters)

    def attention_operands(r, n):
        return store_left_operands(oa_s, r, o_s[pl.ds(r, n), :], o_s[pl.ds(TH + r, n), :])

    def matmul(left, right, width, side_job, never, finish):
        tokens = []
        for p in range(right.shape[2] // width):
            def product(i):
                nonlocal tokens
                m = _dot(_after(left[i], tokens, never), _unpack(right[i, :, pl.ds(p * width, width)]))
                tokens = side_job(7 * p + i)
                return m
            finish(p, _block_product(product))

    def spread(items, i, n):
        return items[i * len(items) // n:(i + 1) * len(items) // n]

    def first_token(t):
        return jnp.broadcast_to(qkv_s[t, pl.ds(HALO, 1), :], (HALO, LANES))

    def project(j, side_job, never):
        per = QW // LANES
        tiles = [[half * 3 * nc // 2 + p * per + c for c in range(per)]
                 for p in range(3 * DH // QW) for half in range(2)]
        tails = {t: qkv_s[t, pl.ds(TM, HALO), :] for t in range(nc, 3 * nc)}

        def finish(p, blocks):
            for k, y in enumerate(blocks):
                for c, t in enumerate(tiles[2 * p + k % 2]):
                    yc = y[:, c * LANES:(c + 1) * LANES]
                    qkv_s[t, pl.ds(HALO + k // 2 * TH, TH), :] = yc
                    if t in tails and k < 2:
                        head = jnp.broadcast_to(yc[0:1, :], (HALO, LANES))
                        qkv_s[t, pl.ds(0, HALO), :] = jnp.where(j == 0, head, tails[t])
        matmul(xa_s, in_s, QW, side_job, never, finish)

    def out_project(j, fresh, never):
        def finish(p, blocks):
            for k, y in enumerate(blocks):
                at = (pl.ds(pl.multiple_of(j * TM + k // 2 * TH, TH), TH), pl.ds(k % 2 * DH + p * OW, OW))
                x_s[at] = jnp.where(fresh, io_s[at].astype(F32), x_s[at]) + y
        matmul(oa_s, out_s, OW, lambda i: [], never, finish)

    def attention(j, r, n, masked):
        lane = jax.lax.broadcasted_iota(jnp.int32, (n, LANES), 1)
        logits = [None] * WINDOW
        for c in range(nc):
            q = qkv_s[c, pl.ds(HALO + r, n), :]
            for w in range(WINDOW):
                p = q * qkv_s[nc + c, pl.ds(HALO + r - DILATION * w, n), :]
                logits[w] = p if c == 0 else logits[w] + p
        for s in (1, 2):
            logits = [l + jnp.where((lane & s) == 0, pltpu.roll(l, LANES - s, 1), pltpu.roll(l, s, 1))
                      for l in logits]
        logits = [l * scale for l in logits]
        if masked:
            pos = j * TM + r + jax.lax.broadcasted_iota(jnp.int32, (n, LANES), 0)
            logits = [jnp.where(pos >= DILATION * w, l, -1e9) if w else l for w, l in enumerate(logits)]
        m = functools.reduce(jnp.maximum, logits)
        e = [jnp.exp(l - m) for l in logits]
        inv = 1.0 / functools.reduce(jnp.add, e)
        p = [x * inv for x in e]
        outs = []
        for c in range(nc):
            terms = [p[w] * qkv_s[2 * nc + c, pl.ds(HALO + r - DILATION * w, n), :] for w in range(WINDOW)]
            outs.append(functools.reduce(jnp.add, terms))
            o_s[pl.ds(r, n), pl.ds(c * LANES, LANES)] = outs[-1]
        return _token(*outs)

    def matmul_twice(left, right, side_job, never, tokens):
        def outer(i):
            def inner(k):
                nonlocal tokens
                m = _dot(_after(left(7 * i + k), tokens, never), _unpack(right(7 * i + k)))
                tokens = side_job(7 * i + k)
                return m
            return jnp.concatenate(_block_product(inner), axis=0)

        c = _block_product(outer)
        return [[c[a // 2 * 2 + b // 2][(a % 2 * 2 + b % 2) * TQ:][:TQ] for b in range(4)]
                for a in range(4)], tokens

    def ffn_up(side_job, never):
        tokens = []
        for t in range(n_tiles):
            grid, tokens = matmul_twice(lambda i: xb_ops[i][...],
                                        lambda i: up_s[i, :, pl.ds(2 * t * LANES, 2 * LANES)],
                                        lambda i: side_job(49 * t + i), never, tokens)

            def swiglu(gu):
                half = 0.5 * gu[:, :LANES]
                return (half + half * jnp.tanh(half)) * gu[:, LANES:]
            grid = jax.tree.map(swiglu, grid)
            if t == n_tiles - 1:
                for a in range(4):
                    hl_s[pl.ds(a * TQ, TQ), :] = jnp.concatenate(grid[a], axis=1)
                continue
            ops = _twice(_left_operands, grid)
            for i in range(0, 49, 2):
                pair = jnp.concatenate(ops[i:i + 2], axis=1)
                h_pairs[i // 2 * n_tiles + t][:, pl.ds(0, pair.shape[1])] = pair.astype(BF16)

    def ffn_down(j, side_job, never):
        last_tile = _twice(_left_operands, [[hl_s[pl.ds(a * TQ, TQ), pl.ds(b * LANES, LANES)]
                                             for b in range(4)] for a in range(4)])

        def hidden(i):
            tiles = [h_pairs[i // 2 * n_tiles + t][:, pl.ds(i % 2 * LANES, LANES)] for t in range(n_tiles - 1)]
            return jnp.concatenate(tiles + [last_tile[i].astype(BF16)], axis=1)

        grid, _ = matmul_twice(hidden, lambda i: down_ops[i][...], side_job, never, [])
        for a in range(4):
            for b in range(4):
                at = (pl.ds(pl.multiple_of(j * TM + a * TQ, TQ), TQ), pl.ds(b * DQ, DQ))
                y = x_s[at] + grid[a][b]
                x_s[at] = y
                io_s[at] = y.astype(BF16)

    def start_in_order(n, copies):
        @pl.loop(0, n)
        def _(i):
            for copy in copies(i):
                copy.start()

    x_copy(0).start()
    start_in_order(D // PB, lambda r: [wqkv_copy(r)])

    last = n_items - 1

    @pl.loop(-2, n_items)
    def _(n):
        j0 = jnp.maximum(n, 0) % nb
        j1 = jnp.maximum(n + 1, 0) % nb
        j2 = (n + 2) % nb
        never = n > n_items

        att = [functools.partial(attention, j1, r, RB, r < HALO) for r in range(0, TM, RB)]

        def side_job(steps, n_slots):
            return lambda i: [step() for step in spread(steps, i, n_slots) if i < n_slots]

        @pl.when(n + 2 < nb)
        def _():
            x_copy(j2).wait()

        @pl.when(n == 0)
        def _():
            @pl.loop(0, DQ // UB)
            def _(r):
                for copy in up_copies(r):
                    copy.wait()
                combine_up(r)

            for copy in w2_copies:
                copy.start()

        @pl.when(n >= 0)
        def _():
            due = [49 * t + i for t in range(n_tiles) for i in (DUE_MIDDLE if 0 < t < n_tiles - 1 else DUE_ENDS)]
            due = dict(zip(due, att, strict=True))
            ffn_up(lambda i: [due[i]()] if i in due else [], never)

        @pl.when(n == -1)
        def _():
            @pl.loop(0, TM // RC)
            def _(g):
                attention(j1, pl.multiple_of(g * RC, RC), RC, True)

            wo_copy.wait()
            permute_wo_rows()
            combine_all(wo_s, out_s)
            combine_all(wqkv_s, in_s)
            attention_operands(0, TH)

        @pl.when(n == 0)
        def _():
            for copy in w2_copies:
                copy.wait()
            combine_down()

        @pl.when(n >= 0)
        def _():
            steps = [functools.partial(norm, j2, n + 2 < nb, xa_s, r, LB) for r in range(0, TH, LB)]
            steps += [functools.partial(attention_operands, r, LB) for r in range(0, TH, LB)]
            ffn_down(j0, side_job(steps, 35), never)

        @pl.when(n < 0)
        def _():
            norm(j2, n + 2 < nb, xa_s, 0, TH, plain=xp_s)

        @pl.when(n == -2)
        def _():
            x_copy(1).start()
            wo_copy.start()
            x_copy(2).start()
            start_in_order(DQ // UB, up_copies)
            start_in_order(nb - 3, lambda j: [x_copy(j + 3)])
            qkv_s[...] = jnp.zeros(qkv_s.shape, F32)

            n_chunks = D // PB

            @pl.loop(0, n_chunks + 1)
            def _(r):
                @pl.when(r < n_chunks)
                def _():
                    wqkv_copy(r).wait()

                @pl.when(r == 0)
                def _():
                    permute_qkv_columns(0)

                @pl.when(r > 0)
                def _():
                    project_partial(r - 1)
                    permute_qkv_columns(jnp.minimum(r, n_chunks - 1))

            for t in range(nc, 3 * nc):
                qkv_s[t, pl.ds(0, HALO), :] = first_token(t)

        @pl.when(n >= nb)
        def _():
            out_copy(j0).start()

        @pl.when(jnp.logical_and(n >= -1, n < last - 1))
        def _():
            out_project(j1, n + 1 < nb, never)
            project(j2, side_job([functools.partial(norm_for_ffn, j1, r, LB) for r in range(0, TQ, LB)],
                                 21 * DH // QW - 1), never)

        @pl.when(n == last - 1)
        def _():
            @pl.loop(0, D // NC)
            def _(i):
                cols = pl.ds(pl.multiple_of(i * NC, NC), NC)
                x_s[rows(j1), cols] += _dot(o_s[...].astype(BF16), _unpack(wo_s[:, cols]))


            @pl.loop(0, TQ // LC)
            def _(g):
                norm_for_ffn(j1, pl.multiple_of(g * LC, LC), LC)

    for j in range(nb):
        out_copy(j).wait()


@jax.jit
def pallas_interleave_layers__sliding_local_dilated__glu_gated_swiglu__prompt_kernel(
    A_x: jax.Array,
    A_wqkv: jax.Array,
    A_wo: jax.Array,
    B_x: jax.Array,
    B_w1: jax.Array,
    B_w3: jax.Array,
    B_w2: jax.Array,
):
    del B_x
    B, S, D = A_x.shape
    F = B_w1.shape[1]
    assert B == 1 and D == N_HEADS * 32 == 8 * LANES and S % TM == 0 and S // TM >= 3 and F == 28 * LANES
    nb = S // TM
    nc = D // LANES
    any_spec = pl.BlockSpec(memory_space=pl.ANY)
    out = pl.pallas_call(
        _kernel,
        out_shape=jax.ShapeDtypeStruct((S, D), A_x.dtype),
        in_specs=[any_spec] * 6,
        out_specs=any_spec,
        scratch_shapes=[
            pltpu.VMEM((S, D), BF16),
            pltpu.VMEM((S, D), F32),
            pltpu.VMEM((D, 3 * D), BF16),
            pltpu.VMEM((D, D), BF16),
            pltpu.VMEM((D // 2, 3 * D), U32),
            pltpu.VMEM((D // 2, D), U32),
            pltpu.VMEM((D, F), BF16),
            pltpu.VMEM((D, F), BF16),
            pltpu.VMEM((49, D // 8, F // 2), U32),
            pltpu.VMEM((F // 8, (49 - 12) * D // 4), U32),
            pltpu.VMEM((7, D // 4, 3 * D // 2), U32),
            pltpu.VMEM((7, D // 4, D // 2), U32),
            pltpu.VMEM((3 * nc, HALO + TM, LANES), F32),
            pltpu.VMEM((TM, D), BF16),
            pltpu.VMEM((7, TM // 2, D // 2), BF16),
            pltpu.VMEM((TM, D), F32),
            pltpu.VMEM((7, TM // 2, D // 2), BF16),
            pltpu.VMEM((TM, 4 * LANES), F32),
            pltpu.SemaphoreType.DMA((nb,)),
            pltpu.SemaphoreType.DMA((D // PB,)),
            pltpu.SemaphoreType.DMA((5,)),
            pltpu.SemaphoreType.DMA((2 * D // UB,)),
            pltpu.SemaphoreType.DMA((nb,)),
        ],
        compiler_params=pltpu.CompilerParams(vmem_limit_bytes=127 * 1024 * 1024),
    )(A_x.reshape(S, D), A_wqkv, A_wo, B_w1, B_w3, B_w2)
    return out.reshape(B, S, D)
```
